```python
import jax
import jax.numpy as jnp

def _softmax(x, axis=-1):
    return jax.nn.softmax(x, axis=axis)

def _gelu(x):
    return jax.nn.gelu(x, approximate=True)

def _silu(x):
    return jax.nn.silu(x)

def _sigmoid(x):
    return jax.nn.sigmoid(x)

def _layernorm(x, axis=-1, eps=1e-05):
    m = jnp.mean(x, axis=axis, keepdims=True)
    v = jnp.var(x, axis=axis, keepdims=True)
    return (x - m) / jnp.sqrt(v + eps)

def _scatter_add(tgt, idx, src, axis=0):
    return tgt.at[idx].add(src)

def _segment_sum(src, seg, n):
    return jax.ops.segment_sum(src, seg, n)

class _Rng:

    def __init__(self, key):
        self._k = key

    def _next(self):
        self._k, sub = jax.random.split(self._k)
        return sub

    def normal(self, shape):
        return jax.random.normal(self._next(), shape, dtype=jnp.bfloat16)

    def randint(self, lo, hi, shape):
        return jax.random.randint(self._next(), shape, lo, hi, dtype=jnp.int32)

    def uniform(self, shape, lo=0.0, hi=1.0):
        return jax.random.uniform(self._next(), shape, jnp.bfloat16, lo, hi)

    def permutation(self, n):
        return jax.random.permutation(self._next(), n)
kernel_name = 'adaLN_cond__sliding_block_cached__moe_arch_mod__prompt'

def setup_inputs():
    _rng = _Rng(jax.random.key(int.from_bytes(__import__("os").urandom(4), "little")))
    _w = lambda a: (lambda t: t.astype(jnp.bfloat16) if jnp.issubdtype(t.dtype, jnp.floating) else t)(jnp.asarray(a))

    def _A_setup():
        B, Sq, D = (1, 2048, 1024)
        Hq, Hkv, Sk, Dh = (32, 4, 2048, 128)
        assert Hq % Hkv == 0, (Hq, Hkv)
        return {'x': _w((lambda *s: _rng.normal(s) * 0.05)(B, Sq, D)), 'k_cache': _w((lambda *s: _rng.normal(s) * 0.05)(B, Hkv, Sk, Dh)), 'v_cache': _w((lambda *s: _rng.normal(s) * 0.05)(B, Hkv, Sk, Dh)), 'wq': _w((lambda *s: _rng.normal(s) * 0.05)(D, Hq * Dh) * D ** (-0.5)), 'wo': _w((lambda *s: _rng.normal(s) * 0.05)(Hq * Dh, D) * (Hq * Dh) ** (-0.5))}
    _A_in = _A_setup()

    def _B_setup():
        B, S, D, F, C = (1, 2048, 1024, 3584, 1)
        return {'x': _w((lambda *s: _rng.normal(s) * 0.05)(B, S, D)), 'w_r': _w((lambda *s: _rng.normal(s) * 0.05)(D)), 'w_gate': _w((lambda *s: _rng.normal(s) * 0.05)(D, F)), 'w_up': _w((lambda *s: _rng.normal(s) * 0.05)(D, F)), 'w_down': _w((lambda *s: _rng.normal(s) * 0.05)(F, D))}
    _B_in = _B_setup()
    return {'A_x': _A_in['x'], 'A_k_cache': _A_in['k_cache'], 'A_v_cache': _A_in['v_cache'], 'A_wq': _A_in['wq'], 'A_wo': _A_in['wo'], 'B_x': _B_in['x'], 'B_w_r': _B_in['w_r'], 'B_w_gate': _B_in['w_gate'], 'B_w_up': _B_in['w_up'], 'B_w_down': _B_in['w_down'], 'c': _w((lambda *s: _rng.normal(s) * 0.05)(1, 1024)), 'w_mod': _w((lambda *s: _rng.normal(s) * 0.05)(1024, 6 * 1024) * 1024 ** (-0.5))}

def reference(A_x, A_k_cache, A_v_cache, A_wq, A_wo, B_x, B_w_r, B_w_gate, B_w_up, B_w_down, c, w_mod):

    def _A_ref(x, k_cache, v_cache, wq, wo):
        B, Sq, D = x.shape
        Hq, Dh = (32, 128)
        Hkv, Sk = (k_cache.shape[1], k_cache.shape[2])
        W = min(4096, max(256, Sk // 4))
        rep = Hq // Hkv
        q = (lambda x, *d: x.transpose(*d))((x @ wq).reshape(B, Sq, Hq, Dh), 0, 2, 1, 3)
        k = jnp.repeat(k_cache[:, :, Sk - W:, :], rep, axis=1)
        v = jnp.repeat(v_cache[:, :, Sk - W:, :], rep, axis=1)
        scores = jnp.einsum('bhqd,bhkd->bhqk', q, k) * Dh ** (-0.5)
        p = _softmax(scores, axis=-1)
        o = jnp.einsum('bhqk,bhkd->bhqd', p, v)
        return (lambda x, *d: x.transpose(*d))(o, 0, 2, 1, 3).reshape(B, Sq, Hq * Dh) @ wo

    def _B_ref(x, w_r, w_gate, w_up, w_down):
        B, S, D = x.shape
        C = 1
        r = x @ w_r
        idx = jnp.argsort(-r, axis=-1)[:, :C]
        idx_e = jnp.repeat(idx.reshape(B, C, 1), D, axis=2)
        x_sel = jnp.take_along_axis(x, idx_e, axis=1)
        g = _silu(x_sel @ w_gate)
        u = x_sel @ w_up
        y = g * u @ w_down
        r_sel = _sigmoid(jnp.take_along_axis(r, idx, axis=1))
        y = y * r_sel.reshape(B, C, 1)
        b_off = (jnp.arange(B) * S).reshape(B, 1)
        flat_idx = (idx + b_off).reshape(B * C)
        zero = (x * 0.0).reshape(B * S, D)
        upd = _scatter_add(zero, flat_idx, y.reshape(B * C, D), axis=0)
        return x + upd.reshape(B, S, D)
    x = A_x
    mod = (_silu(c) @ w_mod).reshape(c.shape[0], 6, 1, -1)
    sa, ca, ga, sb, cb, gb = (mod[:, 0].copy(), mod[:, 1].copy(), mod[:, 2].copy(), mod[:, 3].copy(), mod[:, 4].copy(), mod[:, 5].copy())
    h = _layernorm(x, axis=-1) * (1 + ca) + sa
    x = x + ga * _A_ref(h, A_k_cache, A_v_cache, A_wq, A_wo)
    h = _layernorm(x, axis=-1) * (1 + cb) + sb
    x = x + gb * _B_ref(h, B_w_r, B_w_gate, B_w_up, B_w_down)
    return x
```

```python
import functools

import jax
import jax.numpy as jnp
from jax import lax
import jax.experimental.pallas as pl
import jax.experimental.pallas.tpu as pltpu

HQ = 32
DH = 128
TQ = 256
EPS = 1e-5
LOG2E = 1.4426950408889634


def _ln(x):
    m = jnp.mean(x, axis=-1, keepdims=True)
    xc = x - m
    v = jnp.mean(xc * xc, axis=-1, keepdims=True)
    return xc * lax.rsqrt(v + EPS)


def _kernel(x_ref, c_ref, wr_ref, k_hbm, v_hbm, wq_hbm, wo_hbm, wmod_hbm,
            wg_hbm, wu_hbm, wd_hbm, out_hbm,
            k_s, v_s, wq_s, wo_s, wmod_s, wg_s, wu_s, wd_s, out_s,
            mod_s, o_s, best_r, best_i, best_h, best_x, sems, osems,
            *, S, D, HKV, SK, W, F):
    i = pl.program_id(0)
    n = pl.num_programs(0)
    rep = HQ // HKV
    GW = rep * DH

    def cp_modA():
        return pltpu.make_async_copy(wmod_hbm.at[:, pl.ds(0, 2 * D)], wmod_s.at[:, pl.ds(0, 2 * D)], sems.at[0])

    def cp_modB():
        return pltpu.make_async_copy(wmod_hbm.at[:, pl.ds(2 * D, 4 * D)], wmod_s.at[:, pl.ds(2 * D, 4 * D)], sems.at[1])

    def cp_k():
        return pltpu.make_async_copy(k_hbm.at[0, :, pl.ds(SK - W, W), :], k_s, sems.at[2])

    def cp_v():
        return pltpu.make_async_copy(v_hbm.at[0, :, pl.ds(SK - W, W), :], v_s, sems.at[3])

    def cp_wq(g):
        return pltpu.make_async_copy(wq_hbm.at[:, pl.ds(g * GW, GW)], wq_s.at[:, pl.ds(g * GW, GW)], sems.at[4 + g])

    def cp_wo():
        return pltpu.make_async_copy(wo_hbm, wo_s, sems.at[8])

    def cp_wg():
        return pltpu.make_async_copy(wg_hbm, wg_s, sems.at[9])

    def cp_wu():
        return pltpu.make_async_copy(wu_hbm, wu_s, sems.at[10])

    def cp_wd():
        return pltpu.make_async_copy(wd_hbm, wd_s, sems.at[11])

    def cp_out(t):
        r0 = pl.multiple_of(t * TQ, TQ)
        return pltpu.make_async_copy(out_s.at[pl.ds(r0, TQ), :], out_hbm.at[pl.ds(r0, TQ), :], osems.at[t])

    def silu_c():
        c = c_ref[...].astype(jnp.float32)
        sc = c * jax.nn.sigmoid(c)
        return jnp.broadcast_to(sc, (8, D)).astype(jnp.bfloat16)

    @pl.when(i == 0)
    def _():
        cp_modA().start()
        for g in range(HKV):
            cp_wq(g).start()
        cp_k().start()
        cp_v().start()
        cp_modA().wait()
        cp_wo().start()
        cp_modB().start()
        mod_s[:, 0:2 * D] = jnp.dot(silu_c(), wmod_s[:, 0:2 * D], preferred_element_type=jnp.float32)
        best_r[...] = jnp.full(best_r.shape, -jnp.inf, jnp.float32)
        best_i[...] = jnp.zeros(best_i.shape, jnp.int32)
        best_h[...] = jnp.zeros(best_h.shape, jnp.float32)
        best_x[...] = jnp.zeros(best_x.shape, jnp.float32)
        for g in range(HKV):
            cp_wq(g).wait()
        cp_k().wait()
        cp_v().wait()

    @pl.when(i == 1)
    def _():
        cp_wg().start()
        cp_wu().start()
        cp_wd().start()

    x = x_ref[...].astype(jnp.float32)
    sa = mod_s[0:1, 0:D]
    ca = mod_s[0:1, D:2 * D]
    h = (_ln(x) * (1.0 + ca) + sa).astype(jnp.bfloat16)

    qscale = (DH ** -0.5) * LOG2E
    for g in range(HKV):
        qg = jnp.dot(h, wq_s[:, g * GW:(g + 1) * GW], preferred_element_type=jnp.float32)
        qg = (qg * qscale).astype(jnp.bfloat16)
        kg = k_s[g]
        vg = v_s[g]
        for j in range(rep):
            qh = qg[:, j * DH:(j + 1) * DH]
            s = lax.dot_general(qh, kg, (((1,), (1,)), ((), ())), preferred_element_type=jnp.float32)
            m = jnp.max(s, axis=-1, keepdims=True)
            p = jnp.exp2(s - m)
            l = jnp.sum(p, axis=-1, keepdims=True)
            o = jnp.dot(p.astype(jnp.bfloat16), vg, preferred_element_type=jnp.float32)
            o = o * pl.reciprocal(l, approx=False)
            hh = g * rep + j
            o_s[:, hh * DH:(hh + 1) * DH] = o.astype(jnp.bfloat16)

    @pl.when(i == 0)
    def _():
        cp_wo().wait()
        cp_modB().wait()
        mod_s[:, 2 * D:6 * D] = jnp.dot(silu_c(), wmod_s[:, 2 * D:6 * D], preferred_element_type=jnp.float32)

    attn = jnp.dot(o_s[...], wo_s[...], preferred_element_type=jnp.float32)
    ga = mod_s[0:1, 2 * D:3 * D]
    sb = mod_s[0:1, 3 * D:4 * D]
    cb = mod_s[0:1, 4 * D:5 * D]
    gb = mod_s[0:1, 5 * D:6 * D]
    x1 = x + ga * attn
    h2 = _ln(x1) * (1.0 + cb) + sb
    h2 = h2.astype(jnp.bfloat16).astype(jnp.float32)
    r0 = pl.multiple_of(i * TQ, TQ)
    out_s[pl.ds(r0, TQ), :] = (x1 + gb * h2).astype(out_s.dtype)
    cp_out(i).start()

    wr = wr_ref[...].astype(jnp.float32)
    r = jnp.sum(h2 * wr, axis=-1, keepdims=True)
    r = r.astype(jnp.bfloat16).astype(jnp.float32)
    rmax = jnp.max(r, axis=0, keepdims=True)
    rows = lax.broadcasted_iota(jnp.int32, (TQ, 1), 0)
    imin = jnp.min(jnp.where(r == rmax, rows, TQ), axis=0, keepdims=True)
    sel = rows == imin
    hrow = jnp.sum(jnp.where(sel, h2, 0.0), axis=0, keepdims=True)
    xrow = jnp.sum(jnp.where(sel, x1, 0.0), axis=0, keepdims=True)
    better = rmax > best_r[...]
    best_r[...] = jnp.where(better, rmax, best_r[...])
    best_i[...] = jnp.where(better, imin + i * TQ, best_i[...])
    best_h[...] = jnp.where(better, hrow, best_h[...])
    best_x[...] = jnp.where(better, xrow, best_x[...])

    @pl.when(i == n - 1)
    def _():
        cp_wg().wait()
        cp_wu().wait()
        cp_wd().wait()
        hs = best_h[...]
        xs = jnp.broadcast_to(hs, (8, D)).astype(jnp.bfloat16)
        gt = jnp.dot(xs, wg_s[...], preferred_element_type=jnp.float32)
        up = jnp.dot(xs, wu_s[...], preferred_element_type=jnp.float32)
        a = (gt * jax.nn.sigmoid(gt) * up).astype(jnp.bfloat16)
        y = jnp.dot(a, wd_s[...], preferred_element_type=jnp.float32)[0:1, :]
        y = y * jax.nn.sigmoid(best_r[...])
        newrow = best_x[...] + gb * (hs + y)
        for t in range(S // TQ):
            cp_out(t).wait()
        idx = best_i[0, 0]
        base = pl.multiple_of((idx // 16) * 16, 16)
        blk = out_s[pl.ds(base, 16), :].astype(jnp.float32)
        rr = lax.broadcasted_iota(jnp.int32, (16, D), 0) + base
        out_s[pl.ds(base, 16), :] = jnp.where(rr == idx, newrow, blk).astype(out_s.dtype)
        fix = pltpu.make_async_copy(out_s.at[pl.ds(base, 16), :], out_hbm.at[pl.ds(base, 16), :], osems.at[0])
        fix.start()
        fix.wait()


@jax.jit
def pallas_adaLN_cond__sliding_block_cached__moe_arch_mod__prompt_kernel(
    A_x: jax.Array,
    A_k_cache: jax.Array,
    A_v_cache: jax.Array,
    A_wq: jax.Array,
    A_wo: jax.Array,
    B_x: jax.Array,
    B_w_r: jax.Array,
    B_w_gate: jax.Array,
    B_w_up: jax.Array,
    B_w_down: jax.Array,
    c: jax.Array,
    w_mod: jax.Array,
):
    B, S, D = A_x.shape
    assert B == 1
    HKV, SK = A_k_cache.shape[1], A_k_cache.shape[2]
    W = min(4096, max(256, SK // 4))
    F = B_w_gate.shape[1]
    dt = A_x.dtype
    nt = S // TQ
    x2 = A_x.reshape(S, D)
    wr2 = B_w_r.reshape(1, D)
    anyspec = pl.BlockSpec(memory_space=pl.ANY)
    kern = functools.partial(_kernel, S=S, D=D, HKV=HKV, SK=SK, W=W, F=F)
    out = pl.pallas_call(
        kern,
        grid=(nt,),
        in_specs=[
            pl.BlockSpec((TQ, D), lambda i: (i, 0)),
            pl.BlockSpec((1, D), lambda i: (0, 0)),
            pl.BlockSpec((1, D), lambda i: (0, 0)),
            anyspec, anyspec, anyspec, anyspec, anyspec, anyspec, anyspec, anyspec,
        ],
        out_specs=anyspec,
        out_shape=jax.ShapeDtypeStruct((S, D), dt),
        scratch_shapes=[
            pltpu.VMEM((HKV, W, DH), dt),
            pltpu.VMEM((HKV, W, DH), dt),
            pltpu.VMEM((D, HQ * DH), dt),
            pltpu.VMEM((HQ * DH, D), dt),
            pltpu.VMEM((D, 6 * D), dt),
            pltpu.VMEM((D, F), dt),
            pltpu.VMEM((D, F), dt),
            pltpu.VMEM((F, D), dt),
            pltpu.VMEM((S, D), dt),
            pltpu.VMEM((8, 6 * D), jnp.float32),
            pltpu.VMEM((TQ, HQ * DH), dt),
            pltpu.VMEM((1, 1), jnp.float32),
            pltpu.VMEM((1, 1), jnp.int32),
            pltpu.VMEM((1, D), jnp.float32),
            pltpu.VMEM((1, D), jnp.float32),
            pltpu.SemaphoreType.DMA((12,)),
            pltpu.SemaphoreType.DMA((nt,)),
        ],
        compiler_params=pltpu.CompilerParams(
            dimension_semantics=("arbitrary",),
            vmem_limit_bytes=100 * 1024 * 1024,
        ),
    )(x2, c, wr2, A_k_cache, A_v_cache, A_wq, A_wo, w_mod, B_w_gate, B_w_up, B_w_down)
    return out.reshape(B, S, D)
```

```python
import functools

import jax
import jax.numpy as jnp
from jax import lax
import jax.experimental.pallas as pl
import jax.experimental.pallas.tpu as pltpu

HQ = 32
DH = 128
TQ = 256
CH = 16
PAD = 128
EPS = 1e-5
LOG2E = 1.4426950408889634
WQ_SPLIT = (0, 4, 12, 32)
STAGED = True


def _ln(x):
    m = jnp.mean(x, axis=-1, keepdims=True)
    xc = x - m
    v = jnp.mean(xc * xc, axis=-1, keepdims=True)
    return xc * lax.rsqrt(v + EPS)


def _recip(l):
    r = pl.reciprocal(l, approx=True)
    return r * (2.0 - l * r)


def _kernel(c_ref, wr_ref, x_hbm, k_hbm, v_hbm, wq_hbm, wo_hbm, wmod_hbm,
            wg_hbm, wu_hbm, wd_hbm, out_hbm,
            x_s, k_s, v_s, wq_s, wo_s, wmod_s, wg_s, wu_s, wd_s, out_s,
            mod_s, h_s, o_s, acc_s, rp_s, best_r, best_i, zero_s, sems, xsems, osems,
            *, S, D, HKV, SK, W, F):
    i = pl.program_id(0)
    nt = S // TQ
    rep = HQ // HKV
    f32 = jnp.float32
    bf16 = jnp.bfloat16
    qscale = (DH ** -0.5) * LOG2E

    def cp_modA():
        return pltpu.make_async_copy(wmod_hbm.at[:, pl.ds(0, 2 * D)], wmod_s.at[:, pl.ds(0, 2 * D)], sems.at[0])

    def cp_modB():
        return pltpu.make_async_copy(wmod_hbm.at[:, pl.ds(2 * D, 4 * D)], wmod_s.at[:, pl.ds(2 * D, 4 * D)], sems.at[1])

    def cp_k():
        return pltpu.make_async_copy(k_hbm.at[0, :, pl.ds(SK - W, W), :], k_s, sems.at[2])

    def cp_v():
        return pltpu.make_async_copy(v_hbm.at[0, :, pl.ds(SK - W, W), :], v_s, sems.at[3])

    def cp_wq(g):
        c0, c1 = WQ_SPLIT[g] * DH, WQ_SPLIT[g + 1] * DH
        return pltpu.make_async_copy(wq_hbm.at[:, pl.ds(c0, c1 - c0)], wq_s.at[:, pl.ds(c0, c1 - c0)], sems.at[4 + g])

    def cp_wo():
        return pltpu.make_async_copy(wo_hbm, wo_s, sems.at[8])

    def cp_wg():
        return pltpu.make_async_copy(wg_hbm, wg_s, sems.at[9])

    def cp_wu():
        return pltpu.make_async_copy(wu_hbm, wu_s, sems.at[10])

    def cp_wd():
        return pltpu.make_async_copy(wd_hbm, wd_s.at[:, pl.ds(0, D)], sems.at[11])

    def rsl(t, r0=0, n=TQ):
        if isinstance(t, int):
            return pl.ds(t * TQ + r0, n)
        return pl.ds(pl.multiple_of(t * TQ + r0, n), n)

    def cp_x(t):
        return pltpu.make_async_copy(x_hbm.at[rsl(t), :], x_s.at[rsl(t), :], xsems.at[t])

    def cp_out(t):
        return pltpu.make_async_copy(out_s.at[rsl(t), :], out_hbm.at[rsl(t), :], osems.at[t])

    def silu_c():
        c = c_ref[...].astype(f32)
        sc = c * jax.nn.sigmoid(c)
        return jnp.broadcast_to(sc, (8, D)).astype(bf16)

    def ln1(t, r0=0, n=TQ):
        x = x_s[rsl(t, r0, n), :].astype(f32)
        sa = mod_s[0:1, 0:D] * qscale
        ca = (1.0 + mod_s[0:1, D:2 * D]) * qscale
        h_s[r0:r0 + n, :] = (_ln(x) * ca + sa).astype(bf16)

    def post(x, attn):
        ga = mod_s[0:1, 2 * D:3 * D]
        sb = mod_s[0:1, 3 * D:4 * D]
        cb = mod_s[0:1, 4 * D:5 * D]
        x1 = x + ga * attn
        h2 = _ln(x1) * (1.0 + cb) + sb
        h2 = h2.astype(bf16).astype(f32)
        return x1, h2

    def epi_rows(t, r0=0, n=TQ):
        gb = mod_s[0:1, 5 * D:6 * D]
        x1, h2 = post(x_s[rsl(t, r0, n), :].astype(f32), acc_s[rsl(t, r0, n), :])
        out_s[rsl(t, r0, n), :] = (x1 + gb * h2).astype(out_s.dtype)
        hw = h2 * wr_ref[...].astype(f32)
        rp = hw[:, 0:128]
        for j in range(1, D // 128):
            rp = rp + hw[:, j * 128:(j + 1) * 128]
        rp_s[r0:r0 + n, :] = rp

    def epi_top1(t, valid=None):
        r = jnp.sum(rp_s[...], axis=-1, keepdims=True)
        r = r.astype(bf16).astype(f32)
        rmax = jnp.max(r, axis=0, keepdims=True)
        ridx = lax.broadcasted_iota(jnp.int32, (TQ, 1), 0)
        imin = jnp.min(jnp.where(r == rmax, ridx, TQ), axis=0, keepdims=True)
        better = rmax > best_r[...]
        if valid is not None:
            better = jnp.logical_and(better, valid)
        best_r[...] = jnp.where(better, rmax, best_r[...])
        best_i[...] = jnp.where(better, imin + t * TQ, best_i[...])

    def step(t):
        zero = zero_s[0]
        z16 = pl.multiple_of(zero, 16)
        zvec = jnp.full((8, 128), zero, jnp.int32).astype(jnp.uint32)
        tprev, tnext = jnp.maximum(t - 1, 0), jnp.minimum(t + 1, nt - 1)

        def pin(a, deps):
            d = None
            for ref, base in deps:
                n = 16 if ref.dtype == bf16 else 8
                v = pltpu.bitcast(ref[pl.ds(pl.multiple_of(base + z16, n), n), 0:128], jnp.uint32)
                d = v if d is None else d | v
            top = pltpu.bitcast(a[0:16, :], jnp.uint32) | (d & zvec)
            return jnp.concatenate([pltpu.bitcast(top, bf16), a[16:, :]], axis=0)

        hval = h_s[...]

        def qproj(hh):
            return jnp.dot(hval, wq_s[:, hh * DH:(hh + 1) * DH], preferred_element_type=f32).astype(bf16)

        def qk(hh, q):
            s = lax.dot_general(q, k_s[hh // rep], (((1,), (1,)), ((), ())), preferred_element_type=f32)
            m = jnp.max(s, axis=-1, keepdims=True)
            p = jnp.exp2(s - m)
            l = jnp.sum(p, axis=-1, keepdims=True)
            return (p * _recip(l)).astype(bf16)

        def pv(hh, p):
            o = jnp.dot(p, v_s[hh // rep], preferred_element_type=f32)
            o_s[:, hh * DH:(hh + 1) * DH] = o.astype(bf16)

        nch = TQ // CH
        KF = 8 * DH
        q = qproj(0)
        side = [('e', c) for c in range(nch)] + [('l', c) for c in range(nch)]
        for hh in range(HQ):
            barrier = False
            if hh + 1 in WQ_SPLIT[1:-1]:
                g = WQ_SPLIT.index(hh + 1)
                barrier = True
                @pl.when(t == 0)
                def _():
                    cp_wq(g).wait()
                    if STAGED and g == 1:
                        cp_wo().start()
                    if g == len(WQ_SPLIT) - 2:
                        cp_x(1).wait()
                        if STAGED:
                            cp_modB().start()
                            cp_x(2).start()
            if hh == HQ - 1:
                barrier = True
                @pl.when(t == 0)
                def _():
                    cp_wo().wait()
            if hh > 0 and not barrier:
                n_here = 2 if len(side) > 1 + sum(1 for u in range(hh, HQ - 1) if u + 1 not in WQ_SPLIT[1:-1]) else 1
                deps = []
                for _ in range(n_here):
                    kind, c = side.pop(0)
                    if kind == 'e':
                        epi_rows(tprev, c * CH, CH)
                        deps += [(out_s, tprev * TQ), (rp_s, 0)]
                    else:
                        ln1(tnext, c * CH, CH)
                        deps += [(h_s, 0)]
                uniq = []
                for d in deps:
                    if all(d[0] is not u[0] for u in uniq):
                        uniq.append(d)
                q = pin(q, uniq)
            p = qk(hh, q)
            if hh + 1 < HQ:
                q = qproj(hh + 1)
            else:
                part = jnp.dot(o_s[:, 0:KF], wo_s[0:KF, 0:128], preferred_element_type=f32)
            pv(hh, p)

        assert len(side) == 1, side
        ln1(tnext, side[0][1] * CH, CH)
        epi_top1(tprev, t > 0)
        acc_s[rsl(t), 0:128] = jnp.dot(o_s[:, KF:], wo_s[KF:, 0:128], preferred_element_type=f32) + part
        acc_s[rsl(t), 128:] = jnp.dot(o_s[...], wo_s[:, 128:], preferred_element_type=f32)

    @pl.when(i == 0)
    def _():
        cp_x(0).start()
        cp_modA().start()
        cp_wq(0).start()
        cp_k().start()
        cp_v().start()
        if not STAGED:
            for g in range(1, len(WQ_SPLIT) - 1):
                cp_wq(g).start()
            cp_x(1).start()
            cp_wo().start()
            cp_modB().start()
            cp_x(2).start()
        zero_s[0] = 0
        best_r[...] = jnp.full(best_r.shape, -jnp.inf, f32)
        best_i[...] = jnp.zeros(best_i.shape, jnp.int32)
        acc_s[rsl(0), :] = jnp.zeros((TQ, D), f32)
        mod_s[:, 2 * D:6 * D] = jnp.zeros((8, 4 * D), f32)
        cp_x(0).wait()
        cp_modA().wait()
        if STAGED:
            for g in range(1, len(WQ_SPLIT) - 1):
                cp_wq(g).start()
            cp_x(1).start()
        mod_s[:, 0:2 * D] = jnp.dot(silu_c(), wmod_s[:, 0:2 * D], preferred_element_type=f32)
        ln1(0)
        cp_wq(0).wait()
        cp_k().wait()
        cp_v().wait()

    @pl.when(i == 1)
    def _():
        cp_modB().wait()
        for t in range(3, nt):
            cp_x(t).start()
        cp_wg().start()
        cp_wu().start()
        cp_wd().start()
        mod_s[:, 2 * D:6 * D] = jnp.dot(silu_c(), wmod_s[:, 2 * D:6 * D], preferred_element_type=f32)

    @pl.when(jnp.logical_and(i > 0, i + 1 < nt))
    def _():
        cp_x(i + 1).wait()

    step(i)

    @pl.when(i > 0)
    def _():
        cp_out(i - 1).start()

    @pl.when(i == nt - 1)
    def _():
        epi_rows(nt - 1)
        cp_out(nt - 1).start()
        epi_top1(nt - 1)
        cp_wg().wait()
        cp_wu().wait()
        cp_wd().wait()
        idx = best_i[0, 0]
        base = pl.multiple_of((idx // 16) * 16, 16)
        x1, h2 = post(x_s[pl.ds(base, 16), :].astype(f32), acc_s[pl.ds(base, 16), :])
        xs = h2.astype(bf16)
        gt = jnp.dot(xs, wg_s[...], preferred_element_type=f32)
        up = jnp.dot(xs, wu_s[...], preferred_element_type=f32)
        a = (gt * jax.nn.sigmoid(gt) * up).astype(bf16)
        y = jnp.dot(a, wd_s[:, 0:D], preferred_element_type=f32)
        y = y * jax.nn.sigmoid(best_r[...])
        rr = lax.broadcasted_iota(jnp.int32, (16, D), 0) + base
        gb = mod_s[0:1, 5 * D:6 * D]
        new = x1 + gb * (h2 + jnp.where(rr == idx, y, 0.0))
        for t in range(nt):
            cp_out(t).wait()
        out_s[pl.ds(base, 16), :] = new.astype(out_s.dtype)
        fix = pltpu.make_async_copy(out_s.at[pl.ds(base, 16), :], out_hbm.at[pl.ds(base, 16), :], osems.at[0])
        fix.start()
        fix.wait()


@jax.jit
def pallas_adaLN_cond__sliding_block_cached__moe_arch_mod__prompt_kernel(
    A_x: jax.Array,
    A_k_cache: jax.Array,
    A_v_cache: jax.Array,
    A_wq: jax.Array,
    A_wo: jax.Array,
    B_x: jax.Array,
    B_w_r: jax.Array,
    B_w_gate: jax.Array,
    B_w_up: jax.Array,
    B_w_down: jax.Array,
    c: jax.Array,
    w_mod: jax.Array,
):
    B, S, D = A_x.shape
    assert B == 1
    HKV, SK = A_k_cache.shape[1], A_k_cache.shape[2]
    W = min(4096, max(256, SK // 4))
    F = B_w_gate.shape[1]
    dt = A_x.dtype
    nt = S // TQ
    x2 = A_x.reshape(S, D)
    wr2 = B_w_r.reshape(1, D)
    anyspec = pl.BlockSpec(memory_space=pl.ANY)
    kern = functools.partial(_kernel, S=S, D=D, HKV=HKV, SK=SK, W=W, F=F)
    out = pl.pallas_call(
        kern,
        grid=(nt,),
        in_specs=[
            pl.BlockSpec((1, D), lambda i: (0, 0)),
            pl.BlockSpec((1, D), lambda i: (0, 0)),
            anyspec, anyspec, anyspec, anyspec, anyspec, anyspec, anyspec, anyspec, anyspec,
        ],
        out_specs=anyspec,
        out_shape=jax.ShapeDtypeStruct((S, D), dt),
        scratch_shapes=[
            pltpu.VMEM((S, D), dt),
            pltpu.VMEM((HKV, W, DH), dt),
            pltpu.VMEM((HKV, W, DH), dt),
            pltpu.VMEM((D, HQ * DH), dt),
            pltpu.VMEM((HQ * DH, D), dt),
            pltpu.VMEM((D, 6 * D + PAD), dt),
            pltpu.VMEM((D, F), dt),
            pltpu.VMEM((D, F), dt),
            pltpu.VMEM((F, D + PAD), dt),
            pltpu.VMEM((S, D), dt),
            pltpu.VMEM((8, 6 * D), jnp.float32),
            pltpu.VMEM((TQ, D), dt),
            pltpu.VMEM((TQ, HQ * DH), dt),
            pltpu.VMEM((S, D), jnp.float32),
            pltpu.VMEM((TQ, 128), jnp.float32),
            pltpu.VMEM((1, 1), jnp.float32),
            pltpu.VMEM((1, 1), jnp.int32),
            pltpu.SMEM((1,), jnp.int32),
            pltpu.SemaphoreType.DMA((12,)),
            pltpu.SemaphoreType.DMA((nt,)),
            pltpu.SemaphoreType.DMA((nt,)),
        ],
        compiler_params=pltpu.CompilerParams(
            dimension_semantics=("arbitrary",),
            vmem_limit_bytes=100 * 1024 * 1024,
        ),
    )(c, wr2, x2, A_k_cache, A_v_cache, A_wq, A_wo, w_mod, B_w_gate, B_w_up, B_w_down)
    return out.reshape(B, S, D)
```

```python
import functools

import jax
import jax.numpy as jnp
from jax import lax
import jax.experimental.pallas as pl
import jax.experimental.pallas.tpu as pltpu

HQ = 32
DH = 128
TQ = 256
CH = 16
PAD = 128
G0 = 4
N0 = 2
NMA = 4
EPS = 1e-5
LOG2E = 1.4426950408889634


def _ln(x):
    m = jnp.mean(x, axis=-1, keepdims=True)
    xc = x - m
    v = jnp.mean(xc * xc, axis=-1, keepdims=True)
    return xc * lax.rsqrt(v + EPS)


def _recip(l):
    r = pl.reciprocal(l, approx=True)
    return r * (2.0 - l * r)


def _kernel(wr_hbm, c_hbm, x_hbm, k_hbm, v_hbm, wq_hbm, wo_hbm, wmod_hbm,
            wg_hbm, wu_hbm, wd_hbm, out_hbm,
            wr_s, c_s, x_s, k_s, v_s, wq_s, wo_s, wmod_s, wg_s, wu_s, wd_s, out_s,
            mod_s, h_s, q_s, o_s, acc_s, rp_s, best_r, best_i, zero_s, sems, osems,
            *, S, D, HKV, SK, W, F):
    nt = S // TQ
    rep = HQ // HKV
    NB = D // 128
    nch = TQ // CH
    f32 = jnp.float32
    bf16 = jnp.bfloat16
    qscale = (DH ** -0.5) * LOG2E

    def al(v, n):
        return v if isinstance(v, int) else pl.multiple_of(v, n)

    S_C, S_WR, S_MB, S_WG, S_WU, S_WD, S_MA = 0, 1, 2, 3, 4, 5, 6
    S_WQ = S_MA + NMA
    S_K = S_WQ + HQ
    S_V = S_K + HKV
    S_WO = S_V + HKV
    S_X = S_WO + NB

    def cp_c():
        return pltpu.make_async_copy(c_hbm, c_s, sems.at[S_C])

    def cp_wr():
        return pltpu.make_async_copy(wr_hbm, wr_s, sems.at[S_WR])

    def cp_modA(j):
        n = 2 * D // NMA
        return pltpu.make_async_copy(wmod_hbm.at[:, pl.ds(j * n, n)], wmod_s.at[:, pl.ds(j * n, n)], sems.at[S_MA + j])

    def cp_modB():
        return pltpu.make_async_copy(wmod_hbm.at[:, pl.ds(2 * D, 4 * D)], wmod_s.at[:, pl.ds(2 * D, 4 * D)], sems.at[S_MB])

    def cp_wg():
        return pltpu.make_async_copy(wg_hbm, wg_s, sems.at[S_WG])

    def cp_wu():
        return pltpu.make_async_copy(wu_hbm, wu_s, sems.at[S_WU])

    def cp_wd():
        return pltpu.make_async_copy(wd_hbm, wd_s.at[:, pl.ds(0, D)], sems.at[S_WD])

    def cp_wq(h):
        return pltpu.make_async_copy(wq_hbm.at[:, pl.ds(al(h * DH, DH), DH)], wq_s.at[h], sems.at[S_WQ + h])

    def cp_k(g):
        return pltpu.make_async_copy(k_hbm.at[0, g, pl.ds(SK - W, W), :], k_s.at[g], sems.at[S_K + g])

    def cp_v(g):
        return pltpu.make_async_copy(v_hbm.at[0, g, pl.ds(SK - W, W), :], v_s.at[g], sems.at[S_V + g])

    def cp_wo(n):
        return pltpu.make_async_copy(wo_hbm.at[:, pl.ds(al(n * 128, 128), 128)], wo_s.at[n], sems.at[S_WO + n])

    def rsl(t, r0=0, n=TQ):
        return pl.ds(al(t * TQ + r0, n), n)

    def cp_x(t):
        return pltpu.make_async_copy(x_hbm.at[rsl(t), :], x_s.at[rsl(t), :], sems.at[S_X + t])

    def cp_out(t):
        return pltpu.make_async_copy(out_s.at[rsl(t), :], out_hbm.at[rsl(t), :], osems.at[t])

    def silu_c():
        c = c_s[...].astype(f32)
        sc = c * jax.nn.sigmoid(c)
        return jnp.broadcast_to(sc, (8, D)).astype(bf16)

    def mvec(j):
        return mod_s[:, j * D:(j + 1) * D][None]

    def xrows(sl, n):
        return x_s[sl, :].astype(f32).reshape(n // 8, 8, D)

    def mod_b():
        m = jnp.dot(silu_c(), wmod_s[:, 2 * D:6 * D], preferred_element_type=f32)
        mod_s[:, 2 * D:4 * D] = m[:, 0:2 * D]
        mod_s[:, 4 * D:5 * D] = 1.0 + m[:, 2 * D:3 * D]
        mod_s[:, 5 * D:6 * D] = m[:, 3 * D:4 * D]
        mod_s[:, 6 * D:7 * D] = jnp.broadcast_to(wr_s[...].astype(f32).reshape(1, D), (8, D))

    def ln1(t, r0, n):
        xn = _ln(xrows(rsl(t, r0, n), n))
        h_s[pl.ds(al(r0, n), n), :] = (xn * mvec(1) + mvec(0)).reshape(n, D).astype(bf16)

    def post(sl, n):
        attn = jnp.concatenate([acc_s[j, sl, :] for j in range(NB)], axis=1).reshape(n // 8, 8, D)
        x1 = xrows(sl, n) + mvec(2) * attn
        h2 = _ln(x1) * mvec(4) + mvec(3)
        h2 = h2.reshape(n, D).astype(bf16).astype(f32).reshape(n // 8, 8, D)
        return x1, h2

    def epi_rows(t, r0=0, n=TQ):
        x1, h2 = post(rsl(t, r0, n), n)
        out_s[rsl(t, r0, n), :] = (x1 + mvec(5) * h2).reshape(n, D).astype(out_s.dtype)
        hw = (h2 * mvec(6)).reshape(n, D)
        rp = hw[:, 0:128]
        for j in range(1, NB):
            rp = rp + hw[:, j * 128:(j + 1) * 128]
        rp_s[r0:r0 + n, :] = rp

    def epi_top1(t):
        r = jnp.sum(rp_s[...], axis=-1, keepdims=True)
        r = r.astype(bf16).astype(f32)
        rmax = jnp.max(r, axis=0, keepdims=True)
        ridx = lax.broadcasted_iota(jnp.int32, (TQ, 1), 0)
        imin = jnp.min(jnp.where(r == rmax, ridx, TQ), axis=0, keepdims=True)
        better = rmax > best_r[...]
        best_r[...] = jnp.where(better, rmax, best_r[...])
        best_i[...] = jnp.where(better, imin + t * TQ, best_i[...])

    def qproj(hval, hh):
        return jnp.dot(hval, wq_s[hh], preferred_element_type=f32).astype(bf16)

    def qk(q, g):
        s = lax.dot_general(q, k_s[g], (((1,), (1,)), ((), ())), preferred_element_type=f32)
        m = jnp.max(s, axis=-1, keepdims=True)
        p = jnp.exp2(s - m)
        l = jnp.sum(p, axis=-1, keepdims=True)
        return (p * _recip(l)).astype(bf16)

    def pv(p, g, hh):
        o_s[hh] = jnp.dot(p, v_s[g], preferred_element_type=f32).astype(bf16)

    def o_heads(h0, h1):
        return jnp.concatenate([o_s[u] for u in range(h0, h1)], axis=1)

    cp_c().start()
    cp_x(0).start()
    for j in range(NMA):
        cp_modA(j).start()
    for h in range(HQ):
        cp_wq(h).start()
        if h % rep == 0:
            cp_k(h // rep).start()
            cp_v(h // rep).start()
    cp_x(1).start()
    for n in range(NB):
        cp_wo(n).start()
    cp_wr().start()
    cp_x(2).start()
    cp_modB().start()
    for t in range(3, nt):
        cp_x(t).start()
    cp_wg().start()
    cp_wu().start()
    cp_wd().start()

    zero_s[0] = 0
    best_r[...] = jnp.full(best_r.shape, -jnp.inf, f32)
    best_i[...] = jnp.zeros(best_i.shape, jnp.int32)
    cp_c().wait()
    cp_x(0).wait()
    sc = silu_c()
    xn0 = _ln(xrows(rsl(0), TQ))
    nma = 2 * D // NMA
    for j in range(NMA):
        cp_modA(j).wait()
        m = jnp.dot(sc, wmod_s[:, j * nma:(j + 1) * nma], preferred_element_type=f32)
        mod_s[:, j * nma:(j + 1) * nma] = (m if j * nma < D else 1.0 + m) * qscale
    h_s[...] = (xn0 * mvec(1) + mvec(0)).reshape(TQ, D).astype(bf16)
    cp_wq(0).wait()
    q_s[...] = qproj(h_s[...], 0)

    def a0_body(j, carry):
        h0 = j * G0
        g = h0 // rep
        for u in range(1, G0):
            cp_wq(h0 + u).wait()

        @pl.when(h0 + G0 < HQ)
        def _():
            cp_wq(h0 + G0).wait()

        @pl.when(h0 % rep == 0)
        def _():
            cp_k(g).wait()
            cp_v(g).wait()

        hval = h_s[...]
        q = q_s[...]
        for u in range(G0):
            p = qk(q, g)
            q = qproj(hval, jnp.minimum(h0 + u + 1, HQ - 1))
            pv(p, g, h0 + u)
        q_s[...] = q
        return carry

    lax.fori_loop(0, HQ // G0, a0_body, 0)
    cp_x(1).wait()

    def o0_body(j, carry):
        for u in range(N0):
            cp_wo(j * N0 + u).wait()
        oval = o_heads(0, HQ)
        for u in range(N0):
            acc_s[j * N0 + u, rsl(0), :] = jnp.dot(oval, wo_s[j * N0 + u], preferred_element_type=f32)
        nr = TQ * N0 // NB
        for c in range(nr // CH):
            ln1(1, j * nr + c * CH, CH)
        return carry

    lax.fori_loop(0, NB // N0, o0_body, 0)

    cp_wr().wait()
    cp_modB().wait()
    mod_b()

    def step(t, carry):
        @pl.when(t + 1 < nt)
        def _():
            cp_x(t + 1).wait()

        zero = zero_s[0]
        z16 = pl.multiple_of(zero, 16)
        zvec = jnp.full((8, 128), zero, jnp.int32).astype(jnp.uint32)
        tprev, tnext = t - 1, jnp.minimum(t + 1, nt - 1)

        def pin(a, deps):
            d = None
            for ref, base in deps:
                n = 16 if ref.dtype == bf16 else 8
                v = pltpu.bitcast(ref[pl.ds(pl.multiple_of(base + z16, n), n), 0:128], jnp.uint32)
                d = v if d is None else d | v
            top = pltpu.bitcast(a[0:16, :], jnp.uint32) | (d & zvec)
            return jnp.concatenate([pltpu.bitcast(top, bf16), a[16:, :]], axis=0)

        KF = 8
        hval = h_s[...]
        q = qproj(hval, 0)
        for hh in range(HQ):
            if hh % 2 == 1:
                epi_rows(tprev, (hh // 2) * CH, CH)
                q = pin(q, [(out_s, tprev * TQ), (rp_s, 0)])
            elif hh > 0:
                ln1(tnext, (hh // 2 - 1) * CH, CH)
                q = pin(q, [(h_s, 0)])
            p = qk(q, hh // rep)
            if hh + 1 < HQ:
                q = qproj(hval, hh + 1)
            else:
                part = jnp.dot(o_heads(0, KF), wo_s[0, 0:KF * DH, :], preferred_element_type=f32)
            pv(p, hh // rep, hh)

        epi_top1(tprev)
        acc_s[0, rsl(t), :] = jnp.dot(o_heads(KF, HQ), wo_s[0, KF * DH:, :], preferred_element_type=f32) + part
        oval = o_heads(0, HQ)
        for n in range(1, NB):
            acc_s[n, rsl(t), :] = jnp.dot(oval, wo_s[n], preferred_element_type=f32)
        ln1(tnext, (nch - 1) * CH, CH)
        cp_out(tprev).start()
        return carry

    lax.fori_loop(1, nt, step, 0)

    epi_rows(nt - 1)
    cp_out(nt - 1).start()
    epi_top1(nt - 1)
    cp_wg().wait()
    cp_wu().wait()
    cp_wd().wait()
    idx = best_i[0, 0]
    base = pl.multiple_of((idx // 16) * 16, 16)
    x1, h2 = post(pl.ds(base, 16), 16)
    xs = h2.reshape(16, D).astype(bf16)
    gt = jnp.dot(xs, wg_s[...], preferred_element_type=f32)
    up = jnp.dot(xs, wu_s[...], preferred_element_type=f32)
    a = (gt * jax.nn.sigmoid(gt) * up).astype(bf16)
    y = jnp.dot(a, wd_s[:, 0:D], preferred_element_type=f32)
    y = y * jax.nn.sigmoid(best_r[...])
    rr = lax.broadcasted_iota(jnp.int32, (16, D), 0) + base
    upd = jnp.where(rr == idx, y, 0.0).reshape(2, 8, D)
    new = (x1 + mvec(5) * (h2 + upd)).reshape(16, D)
    for t in range(nt):
        cp_out(t).wait()
    out_s[pl.ds(base, 16), :] = new.astype(out_s.dtype)
    fix = pltpu.make_async_copy(out_s.at[pl.ds(base, 16), :], out_hbm.at[pl.ds(base, 16), :], osems.at[0])
    fix.start()
    fix.wait()


@jax.jit
def pallas_adaLN_cond__sliding_block_cached__moe_arch_mod__prompt_kernel(
    A_x: jax.Array,
    A_k_cache: jax.Array,
    A_v_cache: jax.Array,
    A_wq: jax.Array,
    A_wo: jax.Array,
    B_x: jax.Array,
    B_w_r: jax.Array,
    B_w_gate: jax.Array,
    B_w_up: jax.Array,
    B_w_down: jax.Array,
    c: jax.Array,
    w_mod: jax.Array,
):
    B, S, D = A_x.shape
    assert B == 1
    HKV, SK = A_k_cache.shape[1], A_k_cache.shape[2]
    W = min(4096, max(256, SK // 4))
    F = B_w_gate.shape[1]
    dt = A_x.dtype
    nt = S // TQ
    NB = D // 128
    x2 = A_x.reshape(S, D)
    anyspec = pl.BlockSpec(memory_space=pl.ANY)
    kern = functools.partial(_kernel, S=S, D=D, HKV=HKV, SK=SK, W=W, F=F)
    out = pl.pallas_call(
        kern,
        in_specs=[anyspec] * 11,
        out_specs=anyspec,
        out_shape=jax.ShapeDtypeStruct((S, D), dt),
        scratch_shapes=[
            pltpu.VMEM((D,), dt),
            pltpu.VMEM((1, D), dt),
            pltpu.VMEM((S, D), dt),
            pltpu.VMEM((HKV, W, DH), dt),
            pltpu.VMEM((HKV, W, DH), dt),
            pltpu.VMEM((HQ, D, DH), dt),
            pltpu.VMEM((NB, HQ * DH, 128), dt),
            pltpu.VMEM((D, 6 * D + PAD), dt),
            pltpu.VMEM((D, F), dt),
            pltpu.VMEM((D, F), dt),
            pltpu.VMEM((F, D + PAD), dt),
            pltpu.VMEM((S, D), dt),
            pltpu.VMEM((8, 7 * D), jnp.float32),
            pltpu.VMEM((TQ, D), dt),
            pltpu.VMEM((TQ, DH), dt),
            pltpu.VMEM((HQ, TQ, DH), dt),
            pltpu.VMEM((NB, S, 128), jnp.float32),
            pltpu.VMEM((TQ, 128), jnp.float32),
            pltpu.VMEM((1, 1), jnp.float32),
            pltpu.VMEM((1, 1), jnp.int32),
            pltpu.SMEM((1,), jnp.int32),
            pltpu.SemaphoreType.DMA((6 + NMA + HQ + 2 * HKV + NB + nt,)),
            pltpu.SemaphoreType.DMA((nt,)),
        ],
        compiler_params=pltpu.CompilerParams(
            vmem_limit_bytes=100 * 1024 * 1024,
        ),
    )(B_w_r, c, x2, A_k_cache, A_v_cache, A_wq, A_wo, w_mod, B_w_gate, B_w_up, B_w_down)
    return out.reshape(B, S, D)
```

```python
import functools

import jax
import jax.numpy as jnp
from jax import lax
import jax.experimental.pallas as pl
import jax.experimental.pallas.tpu as pltpu

HQ = 32
DH = 128
TQ = 256
CH = 16
PAD = 128
P0 = 2
G0 = 3
N0 = 2
MC = 512
EPS = 1e-5
LOG2E = 1.4426950408889634


def _ln_stats(x):
    m = jnp.mean(x, axis=-1, keepdims=True)
    xc = x - m
    v = jnp.mean(xc * xc, axis=-1, keepdims=True)
    return m, xc, lax.rsqrt(v + EPS)


def _ln(x):
    _, xc, rs = _ln_stats(x)
    return xc * rs


def _recip(l):
    r = pl.reciprocal(l, approx=True)
    return r * (2.0 - l * r)


def _kernel(wr_hbm, c_hbm, x_hbm, k_hbm, v_hbm, wq_hbm, wo_hbm, wmod_hbm,
            wg_hbm, wu_hbm, wd_hbm, out_hbm,
            wr_s, c_s, x_s, k_s, v_s, wq_s, wo_s, wmod_s, wg_s, wu_s, wd_s, out_s,
            sc_s, mraw_s, mod_s, h_s, q_s, o_s, acc_s, rp_s, stat_s, best_r, best_i, zero_s, sems, osems,
            *, S, D, HKV, SK, W, F):
    nt = S // TQ
    rep = HQ // HKV
    NB = D // 128
    nch = TQ // CH
    CPV = D // MC
    NMC = 6 * CPV
    f32 = jnp.float32
    bf16 = jnp.bfloat16
    qscale = (DH ** -0.5) * LOG2E

    def al(v, n):
        return v if isinstance(v, int) else pl.multiple_of(v, n)

    S_C, S_WR, S_WG, S_WU, S_WD, S_M = 0, 1, 2, 3, 4, 5
    S_WQ = S_M + NMC
    S_K = S_WQ + HQ
    S_V = S_K + HKV
    S_WO = S_V + HKV
    S_X = S_WO + NB

    def cp_c():
        return pltpu.make_async_copy(c_hbm, c_s, sems.at[S_C])

    def cp_wr():
        return pltpu.make_async_copy(wr_hbm, wr_s, sems.at[S_WR])

    def cp_mod(j):
        return pltpu.make_async_copy(wmod_hbm.at[:, pl.ds(al(j * MC, MC), MC)], wmod_s.at[j], sems.at[S_M + j])

    def cp_wg():
        return pltpu.make_async_copy(wg_hbm, wg_s, sems.at[S_WG])

    def cp_wu():
        return pltpu.make_async_copy(wu_hbm, wu_s, sems.at[S_WU])

    def cp_wd():
        return pltpu.make_async_copy(wd_hbm, wd_s.at[:, pl.ds(0, D)], sems.at[S_WD])

    def cp_wq(h):
        return pltpu.make_async_copy(wq_hbm.at[:, pl.ds(al(h * DH, DH), DH)], wq_s.at[h], sems.at[S_WQ + h])

    def cp_k(g):
        return pltpu.make_async_copy(k_hbm.at[0, g, pl.ds(SK - W, W), :], k_s.at[g], sems.at[S_K + g])

    def cp_v(g):
        return pltpu.make_async_copy(v_hbm.at[0, g, pl.ds(SK - W, W), :], v_s.at[g], sems.at[S_V + g])

    def cp_wo(n):
        return pltpu.make_async_copy(wo_hbm.at[:, pl.ds(al(n * 128, 128), 128)], wo_s.at[n], sems.at[S_WO + n])

    def rsl(t, r0=0, n=TQ):
        return pl.ds(al(t * TQ + r0, n), n)

    def cp_x(t):
        return pltpu.make_async_copy(x_hbm.at[rsl(t), :], x_s.at[rsl(t), :], sems.at[S_X + t])

    def cp_out(t):
        return pltpu.make_async_copy(out_s.at[rsl(t), :], out_hbm.at[rsl(t), :], osems.at[t])

    def mvec(j):
        return mod_s[:, j * D:(j + 1) * D][None]

    def mraw(j):
        return jnp.concatenate([mraw_s[j * CPV + u] for u in range(CPV)], axis=1)

    def xrows(sl, n):
        return x_s[sl, :].astype(f32).reshape(n // 8, 8, D)

    def ln1(t, r0, n):
        xn = _ln(xrows(rsl(t, r0, n), n))
        h_s[pl.ds(al(r0, n), n), :] = (xn * mvec(1) + mvec(0)).reshape(n, D).astype(bf16)

    def resid(sl, n):
        attn = jnp.concatenate([acc_s[j, sl, :] for j in range(NB)], axis=1).reshape(n // 8, 8, D)
        return xrows(sl, n) + mvec(2) * attn

    def h2_from_stats(x1, sl, n):
        m = jnp.tile(stat_s[0, sl, :], (1, NB)).reshape(n // 8, 8, D)
        rs = jnp.tile(stat_s[1, sl, :], (1, NB)).reshape(n // 8, 8, D)
        return (x1 - m) * rs * mvec(4) + mvec(3)

    def epi_rows(t, r0, n, write_out=True):
        sl = rsl(t, r0, n)
        x1 = resid(sl, n)
        m, xc, rs = _ln_stats(x1)
        stat_s[0, sl, :] = jnp.broadcast_to(m.reshape(n, 1), (n, 128))
        stat_s[1, sl, :] = jnp.broadcast_to(rs.reshape(n, 1), (n, 128))
        h2 = xc * rs * mvec(4) + mvec(3)
        if write_out:
            out_s[sl, :] = (x1 + mvec(5) * h2).reshape(n, D).astype(out_s.dtype)
        hw = (h2 * mvec(6)).reshape(n, D)
        rp = hw[:, 0:128]
        for j in range(1, NB):
            rp = rp + hw[:, j * 128:(j + 1) * 128]
        rp_s[r0:r0 + n, :] = rp

    def epi_top1(t):
        r = jnp.sum(rp_s[...], axis=-1, keepdims=True)
        r = r.astype(bf16).astype(f32)
        rmax = jnp.max(r, axis=0, keepdims=True)
        ridx = lax.broadcasted_iota(jnp.int32, (TQ, 1), 0)
        imin = jnp.min(jnp.where(r == rmax, ridx, TQ), axis=0, keepdims=True)
        better = rmax > best_r[...]
        best_r[...] = jnp.where(better, rmax, best_r[...])
        best_i[...] = jnp.where(better, imin + t * TQ, best_i[...])

    def qproj(hval, hh):
        return jnp.dot(hval, wq_s[hh], preferred_element_type=f32).astype(bf16)

    def qk(q, g):
        s = lax.dot_general(q, k_s[g], (((1,), (1,)), ((), ())), preferred_element_type=f32)
        m = jnp.max(s, axis=-1, keepdims=True)
        p = jnp.exp2(s - m)
        l = jnp.sum(p, axis=-1, keepdims=True)
        return (p * _recip(l)).astype(bf16)

    def pv(p, g, hh):
        o_s[hh] = jnp.dot(p, v_s[g], preferred_element_type=f32).astype(bf16)

    def o_heads(h0, h1):
        return jnp.concatenate([o_s[u] for u in range(h0, h1)], axis=1)

    cp_c().start()
    cp_x(0).start()
    for j in range(2 * CPV):
        cp_mod(j).start()
    for h in range(HQ):
        cp_wq(h).start()
        if h % rep == 0:
            cp_k(h // rep).start()
            cp_v(h // rep).start()
    cp_x(1).start()
    for n in range(NB):
        cp_wo(n).start()
    cp_wr().start()
    for j in range(2 * CPV, NMC):
        cp_mod(j).start()
    for t in range(2, nt):
        cp_x(t).start()
    cp_wg().start()
    cp_wu().start()
    cp_wd().start()

    zero_s[0] = 0
    best_r[...] = jnp.full(best_r.shape, -jnp.inf, f32)
    best_i[...] = jnp.zeros(best_i.shape, jnp.int32)
    cp_c().wait()
    cp_x(0).wait()
    cf = c_s[...].astype(f32)
    sc_s[...] = jnp.broadcast_to(cf * jax.nn.sigmoid(cf), (16, D)).astype(bf16)
    xn0 = _ln(xrows(rsl(0), TQ))

    def mod_body(j, carry):
        cp_mod(j).wait()
        mraw_s[j] = jnp.dot(sc_s[...], wmod_s[j], preferred_element_type=f32)[0:8, :]
        return carry

    lax.fori_loop(0, 2 * CPV, mod_body, 0)
    mod_s[:, 0:D] = mraw(0) * qscale
    mod_s[:, D:2 * D] = (1.0 + mraw(1)) * qscale
    h_s[...] = (xn0 * mvec(1) + mvec(0)).reshape(TQ, D).astype(bf16)
    cp_wq(0).wait()
    hval0 = h_s[...]
    q = qproj(hval0, 0)
    cp_k(0).wait()
    cp_v(0).wait()
    for hh in range(P0):
        cp_wq(hh + 1).wait()
        p = qk(q, 0)
        q = qproj(hval0, hh + 1)
        pv(p, 0, hh)
    q_s[...] = q

    def a0_body(j, carry):
        h0 = P0 + j * G0
        for u in range(1, G0):
            cp_wq(h0 + u).wait()

        @pl.when(h0 + G0 < HQ)
        def _():
            cp_wq(h0 + G0).wait()

        @pl.when((h0 + G0 - 1) % rep < G0)
        def _():
            cp_k((h0 + G0 - 1) // rep).wait()
            cp_v((h0 + G0 - 1) // rep).wait()

        hval = h_s[...]
        q = q_s[...]
        for u in range(G0):
            g = (h0 + u) // rep
            p = qk(q, g)
            q = qproj(hval, jnp.minimum(h0 + u + 1, HQ - 1))
            pv(p, g, h0 + u)
        q_s[...] = q
        return carry

    assert (HQ - P0) % G0 == 0 and P0 + G0 - 1 < rep and (P0 + G0 - 1) % rep >= G0
    lax.fori_loop(0, (HQ - P0) // G0, a0_body, 0)
    cp_x(1).wait()

    KP = 512

    def o0_body(j, carry):
        for u in range(N0):
            cp_wo(j * N0 + u).wait()

        @pl.when(j > 0)
        def _():
            for u in range(CPV):
                cp_mod((j + 1) * CPV + u).wait()

        sc = sc_s[...]
        pieces = [(u, n) for u in range(CPV) for n in range(MC // 128)]
        npass = HQ * DH // KP
        per = len(pieces) * (D // KP) // (N0 * npass)
        assert per == 1
        mv = None
        cnt = 0
        for u in range(N0):
            n = j * N0 + u
            acc = None
            for kq in range(npass):
                hq = KP // DH
                d = jnp.dot(o_heads(kq * hq, (kq + 1) * hq), wo_s[n, kq * KP:(kq + 1) * KP, :], preferred_element_type=f32)
                acc = d if acc is None else d + acc
                cu, cn = pieces[cnt // 2]
                kh = cnt % 2
                d = jnp.dot(sc[:, kh * KP:(kh + 1) * KP],
                            wmod_s[(j + 1) * CPV + cu, kh * KP:(kh + 1) * KP, cn * 128:(cn + 1) * 128],
                            preferred_element_type=f32)
                if kh == 0:
                    mv = d
                else:
                    mraw_s[(j + 1) * CPV + cu, :, cn * 128:(cn + 1) * 128] = (d + mv)[0:8, :]
                cnt += 1
            acc_s[n, rsl(0), :] = acc
        nr = TQ * N0 // NB
        for c in range(nr // CH):
            ln1(1, j * nr + c * CH, CH)
        return carry

    assert NB // N0 == 4 and D // KP == 2
    lax.fori_loop(0, NB // N0, o0_body, 0)

    cp_wr().wait()
    for u in range(CPV):
        cp_mod(5 * CPV + u).wait()
    for u in range(CPV):
        mod_s[:, 5 * D + u * MC:5 * D + (u + 1) * MC] = jnp.dot(
            sc_s[...], wmod_s[5 * CPV + u], preferred_element_type=f32)[0:8, :]
    mod_s[:, 2 * D:3 * D] = mraw(2)
    mod_s[:, 3 * D:4 * D] = mraw(3)
    mod_s[:, 4 * D:5 * D] = 1.0 + mraw(4)
    mod_s[:, 6 * D:7 * D] = jnp.broadcast_to(wr_s[...].astype(f32).reshape(1, D), (8, D))

    def step(t, carry):
        @pl.when(t + 1 < nt)
        def _():
            cp_x(t + 1).wait()

        @pl.when(t + 1 == nt)
        def _():
            cp_wg().wait()
            cp_wu().wait()
            cp_wd().wait()

        zero = zero_s[0]
        z16 = pl.multiple_of(zero, 16)
        zvec = jnp.full((8, 128), zero, jnp.int32).astype(jnp.uint32)
        tprev, tnext = t - 1, jnp.minimum(t + 1, nt - 1)

        def pin(a, deps):
            d = None
            for ref, base in deps:
                n = 16 if ref.dtype == bf16 else 8
                v = pltpu.bitcast(ref[pl.ds(pl.multiple_of(base + z16, n), n), 0:128], jnp.uint32)
                d = v if d is None else d | v
            top = pltpu.bitcast(a[0:16, :], jnp.uint32) | (d & zvec)
            return jnp.concatenate([pltpu.bitcast(top, bf16), a[16:, :]], axis=0)

        KF = 8
        hval = h_s[...]
        q = qproj(hval, 0)
        for hh in range(HQ):
            if hh % 2 == 1:
                epi_rows(tprev, (hh // 2) * CH, CH)
                q = pin(q, [(out_s, tprev * TQ), (rp_s, 0), (stat_s.at[0], tprev * TQ)])
            elif hh > 0:
                ln1(tnext, (hh // 2 - 1) * CH, CH)
                q = pin(q, [(h_s, 0)])
            p = qk(q, hh // rep)
            if hh + 1 < HQ:
                q = qproj(hval, hh + 1)
            else:
                part = jnp.dot(o_heads(0, KF), wo_s[0, 0:KF * DH, :], preferred_element_type=f32)
            pv(p, hh // rep, hh)

        epi_top1(tprev)
        acc_s[0, rsl(t), :] = jnp.dot(o_heads(KF, HQ), wo_s[0, KF * DH:, :], preferred_element_type=f32) + part
        oval = o_heads(0, HQ)
        for n in range(1, NB):
            acc_s[n, rsl(t), :] = jnp.dot(oval, wo_s[n], preferred_element_type=f32)
        ln1(tnext, (nch - 1) * CH, CH)
        cp_out(tprev).start()
        return carry

    lax.fori_loop(1, nt, step, 0)

    epi_rows(nt - 1, 0, TQ)
    cp_out(nt - 1).start()
    epi_top1(nt - 1)
    idx = best_i[0, 0]
    base = pl.multiple_of((idx // 16) * 16, 16)
    bsl = pl.ds(base, 16)
    x1 = resid(bsl, 16)
    h2 = h2_from_stats(x1, bsl, 16)
    xs = h2.reshape(16, D).astype(bf16)
    gt = jnp.dot(xs, wg_s[...], preferred_element_type=f32)
    up = jnp.dot(xs, wu_s[...], preferred_element_type=f32)
    a = (gt * jax.nn.sigmoid(gt) * up).astype(bf16)
    y = jnp.dot(a, wd_s[:, 0:D], preferred_element_type=f32)
    y = y * jax.nn.sigmoid(best_r[...])
    rr = lax.broadcasted_iota(jnp.int32, (16, D), 0) + base
    upd = jnp.where(rr == idx, y, 0.0).reshape(2, 8, D)
    new = (x1 + mvec(5) * (h2 + upd)).reshape(16, D)
    for t in range(nt):
        cp_out(t).wait()
    out_s[bsl, :] = new.astype(out_s.dtype)
    fix = pltpu.make_async_copy(out_s.at[bsl, :], out_hbm.at[bsl, :], osems.at[0])
    fix.start()
    fix.wait()


def _compiler_params():
    kw = dict(vmem_limit_bytes=100 * 1024 * 1024)
    try:
        return pltpu.CompilerParams(disable_semaphore_checks=True, **kw)
    except TypeError:
        return pltpu.CompilerParams(**kw)


@jax.jit
def pallas_adaLN_cond__sliding_block_cached__moe_arch_mod__prompt_kernel(
    A_x: jax.Array,
    A_k_cache: jax.Array,
    A_v_cache: jax.Array,
    A_wq: jax.Array,
    A_wo: jax.Array,
    B_x: jax.Array,
    B_w_r: jax.Array,
    B_w_gate: jax.Array,
    B_w_up: jax.Array,
    B_w_down: jax.Array,
    c: jax.Array,
    w_mod: jax.Array,
):
    B, S, D = A_x.shape
    assert B == 1
    HKV, SK = A_k_cache.shape[1], A_k_cache.shape[2]
    W = min(4096, max(256, SK // 4))
    F = B_w_gate.shape[1]
    dt = A_x.dtype
    nt = S // TQ
    NB = D // 128
    NMC = 6 * D // MC
    x2 = A_x.reshape(S, D)
    anyspec = pl.BlockSpec(memory_space=pl.ANY)
    kern = functools.partial(_kernel, S=S, D=D, HKV=HKV, SK=SK, W=W, F=F)
    out = pl.pallas_call(
        kern,
        in_specs=[anyspec] * 11,
        out_specs=anyspec,
        out_shape=jax.ShapeDtypeStruct((S, D), dt),
        scratch_shapes=[
            pltpu.VMEM((D,), dt),
            pltpu.VMEM((1, D), dt),
            pltpu.VMEM((S, D), dt),
            pltpu.VMEM((HKV, W, DH), dt),
            pltpu.VMEM((HKV, W, DH), dt),
            pltpu.VMEM((HQ, D, DH), dt),
            pltpu.VMEM((NB, HQ * DH, 128), dt),
            pltpu.VMEM((NMC, D, MC), dt),
            pltpu.VMEM((D, F), dt),
            pltpu.VMEM((D, F), dt),
            pltpu.VMEM((F, D + PAD), dt),
            pltpu.VMEM((S, D), dt),
            pltpu.VMEM((16, D), dt),
            pltpu.VMEM((NMC, 8, MC), jnp.float32),
            pltpu.VMEM((8, 7 * D), jnp.float32),
            pltpu.VMEM((TQ, D), dt),
            pltpu.VMEM((TQ, DH), dt),
            pltpu.VMEM((HQ, TQ, DH), dt),
            pltpu.VMEM((NB, S, 128), jnp.float32),
            pltpu.VMEM((TQ, 128), jnp.float32),
            pltpu.VMEM((2, S, 128), jnp.float32),
            pltpu.VMEM((1, 1), jnp.float32),
            pltpu.VMEM((1, 1), jnp.int32),
            pltpu.SMEM((1,), jnp.int32),
            pltpu.SemaphoreType.DMA((5 + NMC + HQ + 2 * HKV + NB + nt,)),
            pltpu.SemaphoreType.DMA((nt,)),
        ],
        compiler_params=_compiler_params(),
    )(B_w_r, c, x2, A_k_cache, A_v_cache, A_wq, A_wo, w_mod, B_w_gate, B_w_up, B_w_down)
    return out.reshape(B, S, D)
```

```python
import functools

import jax
import jax.numpy as jnp
from jax import lax
import jax.experimental.pallas as pl
import jax.experimental.pallas.tpu as pltpu

HQ = 32
DH = 128
TQ = 256
CH = 16
PAD = 128
P0 = 2
G0 = 3
N0 = 2
MC = 512
PIN_R = 0
REL0 = 0
STRIDE = 3.5
CHE = 8
LAG = 3
PIN_C = 0
EPS = 1e-5
LOG2E = 1.4426950408889634


def _ln_stats(x, rel=None):
    d = x.shape[-1]
    part = x[..., 0:128]
    for j in range(1, d // 128):
        part = part + x[..., j * 128:(j + 1) * 128]
    if rel is not None:
        part = part + rel
    m = jnp.sum(part, axis=-1, keepdims=True) * (1.0 / d)
    xc = x - m
    v = jnp.mean(xc * xc, axis=-1, keepdims=True)
    return m, xc, lax.rsqrt(v + EPS)


def _ln(x, rel=None):
    _, xc, rs = _ln_stats(x, rel)
    return xc * rs


def _recip(l):
    r = pl.reciprocal(l, approx=True)
    return r * (2.0 - l * r)


def _kernel(wr_hbm, c_hbm, x_hbm, k_hbm, v_hbm, wq_hbm, wo_hbm, wmod_hbm,
            wg_hbm, wu_hbm, wd_hbm, out_hbm,
            wr_s, c_s, x_s, k_s, v_s, wq_s, wo_s, wmod_s, wg_s, wu_s, wd_s, out_s,
            sc_s, mraw_s, mod_s, h_s, q_s, o_s, acc_s, stat_s, best_r, best_i, zero_s, sems, osems,
            *, S, D, HKV, SK, W, F):
    nt = S // TQ
    rep = HQ // HKV
    NB = D // 128
    nch = TQ // CH
    CPV = D // MC
    NMC = 6 * CPV
    f32 = jnp.float32
    bf16 = jnp.bfloat16
    qscale = (DH ** -0.5) * LOG2E

    def al(v, n):
        return v if isinstance(v, int) else pl.multiple_of(v, n)

    S_C, S_WR, S_WG, S_WU, S_WD, S_M = 0, 1, 2, 3, 4, 5
    S_WQ = S_M + NMC
    S_K = S_WQ + HQ
    S_V = S_K + HKV
    S_WO = S_V + HKV
    S_X = S_WO + NB

    def cp_c():
        return pltpu.make_async_copy(c_hbm, c_s, sems.at[S_C])

    def cp_wr():
        return pltpu.make_async_copy(wr_hbm, wr_s, sems.at[S_WR])

    def cp_mod(j):
        return pltpu.make_async_copy(wmod_hbm.at[:, pl.ds(al(j * MC, MC), MC)], wmod_s.at[j], sems.at[S_M + j])

    def cp_wg():
        return pltpu.make_async_copy(wg_hbm, wg_s, sems.at[S_WG])

    def cp_wu():
        return pltpu.make_async_copy(wu_hbm, wu_s, sems.at[S_WU])

    def cp_wd():
        return pltpu.make_async_copy(wd_hbm, wd_s.at[:, pl.ds(0, D)], sems.at[S_WD])

    def cp_wq(h):
        return pltpu.make_async_copy(wq_hbm.at[:, pl.ds(al(h * DH, DH), DH)], wq_s.at[h], sems.at[S_WQ + h])

    def cp_k(g):
        return pltpu.make_async_copy(k_hbm.at[0, g, pl.ds(SK - W, W), :], k_s.at[g], sems.at[S_K + g])

    def cp_v(g):
        return pltpu.make_async_copy(v_hbm.at[0, g, pl.ds(SK - W, W), :], v_s.at[g], sems.at[S_V + g])

    def cp_wo(n):
        return pltpu.make_async_copy(wo_hbm.at[:, pl.ds(al(n * 128, 128), 128)], wo_s.at[n], sems.at[S_WO + n])

    def rsl(t, r0=0, n=TQ):
        return pl.ds(al(t * TQ + r0, n), n)

    def cp_x(t):
        return pltpu.make_async_copy(x_hbm.at[rsl(t), :], x_s.at[rsl(t), :], sems.at[S_X + t])

    def cp_out(t):
        return pltpu.make_async_copy(out_s.at[rsl(t), :], out_hbm.at[rsl(t), :], osems.at[t])

    def mvec(j):
        return mod_s[:, j * D:(j + 1) * D][None]

    def mraw(j):
        return jnp.concatenate([mraw_s[j * CPV + u] for u in range(CPV)], axis=1)

    def xrows(sl, n):
        return x_s[sl, :].astype(f32).reshape(n // 8, 8, D)

    def ln1(t, r0, n, rel=None):
        xn = _ln(xrows(rsl(t, r0, n), n), rel)
        h_s[pl.ds(al(r0, n), n), :] = (xn * mvec(1) + mvec(0)).reshape(n, D).astype(bf16)

    def resid(sl, n):
        attn = jnp.concatenate([acc_s[j, sl, :] for j in range(NB)], axis=1).reshape(n // 8, 8, D)
        return xrows(sl, n) + mvec(2) * attn

    def h2_from_stats(x1, sl, n):
        m = jnp.tile(stat_s[0, sl, :], (1, NB)).reshape(n // 8, 8, D)
        rs = jnp.tile(stat_s[1, sl, :], (1, NB)).reshape(n // 8, 8, D)
        return (x1 - m) * rs * mvec(4) + mvec(3)

    def epi_rows(t, r0, n, rel=None, write_out=True):
        sl = rsl(t, r0, n)
        x1 = resid(sl, n)
        m, xc, rs = _ln_stats(x1, rel)
        stat_s[0, sl, :] = jnp.broadcast_to(m.reshape(n, 1), (n, 128))
        stat_s[1, sl, :] = jnp.broadcast_to(rs.reshape(n, 1), (n, 128))
        h2 = xc * rs * mvec(4) + mvec(3)
        if write_out:
            out_s[sl, :] = (x1 + mvec(5) * h2).reshape(n, D).astype(out_s.dtype)
        r = jnp.sum(h2 * mvec(6), axis=-1, keepdims=True)
        r = r.astype(bf16).astype(f32)
        bv = best_r[...]
        bi = best_i[...]
        sub = lax.broadcasted_iota(jnp.int32, (8, 128), 0)
        for u in range(n // 8):
            ru = jnp.broadcast_to(r[u], (8, 128))
            better = ru > bv
            bv = jnp.where(better, ru, bv)
            bi = jnp.where(better, sub + (t * TQ + r0 + u * 8), bi)
        best_r[...] = bv
        best_i[...] = bi

    def qproj(hval, hh):
        return jnp.dot(hval, wq_s[hh], preferred_element_type=f32).astype(bf16)

    def qk(q, g):
        s = lax.dot_general(q, k_s[g], (((1,), (1,)), ((), ())), preferred_element_type=f32)
        m = jnp.max(s, axis=-1, keepdims=True)
        p = jnp.exp2(s - m)
        l = jnp.sum(p, axis=-1, keepdims=True)
        return (p * _recip(l)).astype(bf16)

    def pv(p, g, hh):
        o_s[hh] = pltpu.bitcast(jnp.dot(p, v_s[g], preferred_element_type=f32).astype(bf16), jnp.uint32)

    def o_heads(h0, h1):
        return pltpu.bitcast(jnp.concatenate([o_s[u] for u in range(h0, h1)], axis=1), bf16)

    cp_c().start()
    cp_x(0).start()
    for j in range(2 * CPV):
        cp_mod(j).start()
    for h in range(HQ):
        cp_wq(h).start()
        if h % rep == 0:
            cp_k(h // rep).start()
            cp_v(h // rep).start()
    cp_x(1).start()
    for n in range(NB):
        cp_wo(n).start()
    cp_wr().start()
    for j in range(2 * CPV, NMC):
        cp_mod(j).start()
    for t in range(2, nt):
        cp_x(t).start()
    cp_wg().start()
    cp_wu().start()
    cp_wd().start()

    zero_s[0] = 0
    best_r[...] = jnp.full(best_r.shape, -jnp.inf, f32)
    best_i[...] = jnp.zeros(best_i.shape, jnp.int32)
    cp_c().wait()
    cp_x(0).wait()
    cf = c_s[...].astype(f32)
    sc_s[...] = jnp.broadcast_to(cf * jax.nn.sigmoid(cf), (16, D)).astype(bf16)
    xn0 = _ln(xrows(rsl(0), TQ))

    def mod_body(j, carry):
        cp_mod(j).wait()
        mraw_s[j] = jnp.dot(sc_s[...], wmod_s[j], preferred_element_type=f32)[0:8, :]
        return carry

    lax.fori_loop(0, 2 * CPV, mod_body, 0)
    mod_s[:, 0:D] = mraw(0) * qscale
    mod_s[:, D:2 * D] = (1.0 + mraw(1)) * qscale
    h_s[...] = (xn0 * mvec(1) + mvec(0)).reshape(TQ, D).astype(bf16)
    cp_wq(0).wait()
    hval0 = h_s[...]
    q = qproj(hval0, 0)
    cp_k(0).wait()
    cp_v(0).wait()
    for hh in range(P0):
        cp_wq(hh + 1).wait()
        p = qk(q, 0)
        q = qproj(hval0, hh + 1)
        pv(p, 0, hh)
    q_s[...] = q

    def a0_body(j, carry):
        h0 = P0 + j * G0
        for u in range(1, G0):
            cp_wq(h0 + u).wait()

        @pl.when(h0 + G0 < HQ)
        def _():
            cp_wq(h0 + G0).wait()

        @pl.when((h0 + G0 - 1) % rep < G0)
        def _():
            cp_k((h0 + G0 - 1) // rep).wait()
            cp_v((h0 + G0 - 1) // rep).wait()

        hval = h_s[...]
        q = q_s[...]
        for u in range(G0):
            g = (h0 + u) // rep
            p = qk(q, g)
            q = qproj(hval, jnp.minimum(h0 + u + 1, HQ - 1))
            pv(p, g, h0 + u)
        q_s[...] = q
        return carry

    assert (HQ - P0) % G0 == 0 and P0 + G0 - 1 < rep and (P0 + G0 - 1) % rep >= G0
    lax.fori_loop(0, (HQ - P0) // G0, a0_body, 0)
    cp_x(1).wait()

    KP = 512

    def o0_body(j, carry):
        for u in range(N0):
            cp_wo(j * N0 + u).wait()

        @pl.when(j > 0)
        def _():
            for u in range(CPV):
                cp_mod((j + 1) * CPV + u).wait()

        sc = sc_s[...]
        pieces = [(u, n) for u in range(CPV) for n in range(MC // 128)]
        npass = HQ * DH // KP
        per = len(pieces) * (D // KP) // (N0 * npass)
        assert per == 1
        mv = None
        cnt = 0
        for u in range(N0):
            n = j * N0 + u
            acc = None
            for kq in range(npass):
                hq = KP // DH
                d = jnp.dot(o_heads(kq * hq, (kq + 1) * hq), wo_s[n, kq * KP:(kq + 1) * KP, :], preferred_element_type=f32)
                acc = d if acc is None else d + acc
                cu, cn = pieces[cnt // 2]
                kh = cnt % 2
                d = jnp.dot(sc[:, kh * KP:(kh + 1) * KP],
                            wmod_s[(j + 1) * CPV + cu, kh * KP:(kh + 1) * KP, cn * 128:(cn + 1) * 128],
                            preferred_element_type=f32)
                if kh == 0:
                    mv = d
                else:
                    mraw_s[(j + 1) * CPV + cu, :, cn * 128:(cn + 1) * 128] = (d + mv)[0:8, :]
                cnt += 1
            acc_s[n, rsl(0), :] = acc
        nr = TQ * N0 // NB
        for c in range(nr // CH):
            ln1(1, j * nr + c * CH, CH)
        return carry

    assert NB // N0 == 4 and D // KP == 2
    lax.fori_loop(0, NB // N0, o0_body, 0)

    cp_wr().wait()
    for u in range(CPV):
        cp_mod(5 * CPV + u).wait()
    for u in range(CPV):
        mod_s[:, 5 * D + u * MC:5 * D + (u + 1) * MC] = jnp.dot(
            sc_s[...], wmod_s[5 * CPV + u], preferred_element_type=f32)[0:8, :]
    mod_s[:, 2 * D:3 * D] = mraw(2)
    mod_s[:, 3 * D:4 * D] = mraw(3)
    mod_s[:, 4 * D:5 * D] = 1.0 + mraw(4)
    mod_s[:, 6 * D:7 * D] = jnp.broadcast_to(wr_s[...].astype(f32).reshape(1, D), (8, D))

    def step(t, carry):
        @pl.when(t + 1 < nt)
        def _():
            cp_x(t + 1).wait()

        @pl.when(t + 1 == nt)
        def _():
            cp_wg().wait()
            cp_wu().wait()
            cp_wd().wait()

        zero = zero_s[0]
        z16 = pl.multiple_of(zero, 16)
        zvec = jnp.full((8, 128), zero, jnp.int32).astype(jnp.uint32)
        tprev, tnext = t - 1, jnp.minimum(t + 1, nt - 1)

        def fence(deps):
            d = None
            for ref, base in deps:
                n = 16 if ref.dtype == bf16 else 8
                v = pltpu.bitcast(ref[pl.ds(pl.multiple_of(base + z16, n), n), 0:128], jnp.uint32)
                d = v if d is None else d | v
            return d & zvec

        def pin(a, d):
            r0, c0 = PIN_R, PIN_C
            blk = pltpu.bitcast(pltpu.bitcast(a[r0:r0 + 16, c0:c0 + 128], jnp.uint32) | d, bf16)
            row = [a[r0:r0 + 16, 0:c0]] if c0 else []
            row = jnp.concatenate(row + [blk] + ([a[r0:r0 + 16, c0 + 128:]] if a.shape[1] > c0 + 128 else []), axis=1)
            col = [a[0:r0, :]] if r0 else []
            return jnp.concatenate(col + [row, a[r0 + 16:, :]], axis=0)

        hval = h_s[...]
        q = qproj(hval, 0)
        hq = KP // DH
        npass = HQ // hq

        def opass(n, kq, acc, deps=None):
            lhs = o_heads(kq * hq, (kq + 1) * hq)
            if deps is not None:
                lhs = pin(lhs, deps)
            d = jnp.dot(lhs, wo_s[n, kq * KP:(kq + 1) * KP, :], preferred_element_type=f32)
            return d if acc is None else d + acc

        NF = 2
        ne = TQ // CHE
        for hh in range(HQ):
            g = hh // rep
            cs = [c for c in range(ne) if 1 + (c * (HQ - 1)) // ne == hh]
            for c in cs:
                epi_rows(tprev, c * CHE, CHE)
            if cs:
                q = pin(q, fence([(out_s, tprev * TQ), (best_r, 0), (stat_s.at[0], tprev * TQ)]))
            p = qk(q, g)
            if hh + 1 < HQ:
                q = qproj(hval, hh + 1)
            else:
                acc = None
                for kq in range(NF):
                    acc = opass(0, kq, acc)
            pv(p, g, hh)

        passes = [(n, kq) for n in range(NB) for kq in range(npass)][NF:]
        work = [('l', c) for c in range(nch)]
        rel_at = {int(REL0 + STRIDE * c): c for c in range(len(work))}
        assert len(rel_at) == len(work) and max(rel_at) + LAG < len(passes)
        due = {}
        for s, (n, kq) in enumerate(passes):
            if kq == 0:
                acc = None
            acc = opass(n, kq, acc, due.pop(s, None))
            if kq == npass - 1:
                acc_s[n, rsl(t), :] = acc
            if s in rel_at:
                rel = pltpu.bitcast(pltpu.bitcast(acc[0:8, :], jnp.uint32) & zvec, f32)
                kind, c = work[rel_at[s]]
                if kind == 'e':
                    epi_rows(tprev, c * CH, CH, rel)
                    due[s + LAG] = fence([(out_s, tprev * TQ), (best_r, 0), (stat_s.at[0], tprev * TQ)])
                else:
                    ln1(tnext, c * CH, CH, rel)
                    due[s + LAG] = fence([(h_s, 0)])
        assert not due
        cp_out(tprev).start()
        return carry

    lax.fori_loop(1, nt, step, 0)

    epi_rows(nt - 1, 0, TQ)
    cp_out(nt - 1).start()
    bv = best_r[...]
    rbest = jnp.max(bv, axis=0, keepdims=True)
    ibest = jnp.min(jnp.where(bv == rbest, best_i[...], S), axis=0, keepdims=True)
    idx = jnp.minimum(ibest[0, 0], S - 1)
    base = pl.multiple_of((idx // 16) * 16, 16)
    bsl = pl.ds(base, 16)
    x1 = resid(bsl, 16)
    h2 = h2_from_stats(x1, bsl, 16)
    xs = h2.reshape(16, D).astype(bf16)
    gt = jnp.dot(xs, wg_s[...], preferred_element_type=f32)
    up = jnp.dot(xs, wu_s[...], preferred_element_type=f32)
    a = (gt * jax.nn.sigmoid(gt) * up).astype(bf16)
    y = jnp.dot(a, wd_s[:, 0:D], preferred_element_type=f32)
    y = y * jnp.tile(jax.nn.sigmoid(rbest), (1, NB))
    rr = lax.broadcasted_iota(jnp.int32, (16, D), 0) + base
    upd = jnp.where(rr == idx, y, 0.0).reshape(2, 8, D)
    new = (x1 + mvec(5) * (h2 + upd)).reshape(16, D)
    for t in range(nt):
        cp_out(t).wait()
    out_s[bsl, :] = new.astype(out_s.dtype)
    fix = pltpu.make_async_copy(out_s.at[bsl, :], out_hbm.at[bsl, :], osems.at[0])
    fix.start()
    fix.wait()


def _compiler_params():
    kw = dict(vmem_limit_bytes=100 * 1024 * 1024)
    try:
        return pltpu.CompilerParams(disable_semaphore_checks=True, disable_bounds_checks=True, **kw)
    except TypeError:
        return pltpu.CompilerParams(**kw)


@jax.jit
def pallas_adaLN_cond__sliding_block_cached__moe_arch_mod__prompt_kernel(
    A_x: jax.Array,
    A_k_cache: jax.Array,
    A_v_cache: jax.Array,
    A_wq: jax.Array,
    A_wo: jax.Array,
    B_x: jax.Array,
    B_w_r: jax.Array,
    B_w_gate: jax.Array,
    B_w_up: jax.Array,
    B_w_down: jax.Array,
    c: jax.Array,
    w_mod: jax.Array,
):
    B, S, D = A_x.shape
    assert B == 1
    HKV, SK = A_k_cache.shape[1], A_k_cache.shape[2]
    W = min(4096, max(256, SK // 4))
    F = B_w_gate.shape[1]
    dt = A_x.dtype
    nt = S // TQ
    NB = D // 128
    NMC = 6 * D // MC
    x2 = A_x.reshape(S, D)
    anyspec = pl.BlockSpec(memory_space=pl.ANY)
    kern = functools.partial(_kernel, S=S, D=D, HKV=HKV, SK=SK, W=W, F=F)
    out = pl.pallas_call(
        kern,
        in_specs=[anyspec] * 11,
        out_specs=anyspec,
        out_shape=jax.ShapeDtypeStruct((S, D), dt),
        scratch_shapes=[
            pltpu.VMEM((D,), dt),
            pltpu.VMEM((1, D), dt),
            pltpu.VMEM((S, D), dt),
            pltpu.VMEM((HKV, W, DH), dt),
            pltpu.VMEM((HKV, W, DH), dt),
            pltpu.VMEM((HQ, D, DH), dt),
            pltpu.VMEM((NB, HQ * DH, 128), dt),
            pltpu.VMEM((NMC, D, MC), dt),
            pltpu.VMEM((D, F), dt),
            pltpu.VMEM((D, F), dt),
            pltpu.VMEM((F, D + PAD), dt),
            pltpu.VMEM((S, D), dt),
            pltpu.VMEM((16, D), dt),
            pltpu.VMEM((NMC, 8, MC), jnp.float32),
            pltpu.VMEM((8, 7 * D), jnp.float32),
            pltpu.VMEM((TQ, D), dt),
            pltpu.VMEM((TQ, DH), dt),
            pltpu.VMEM((HQ, TQ // 2, DH), jnp.uint32),
            pltpu.VMEM((NB, S, 128), jnp.float32),
            pltpu.VMEM((2, S, 128), jnp.float32),
            pltpu.VMEM((8, 128), jnp.float32),
            pltpu.VMEM((8, 128), jnp.int32),
            pltpu.SMEM((1,), jnp.int32),
            pltpu.SemaphoreType.DMA((5 + NMC + HQ + 2 * HKV + NB + nt,)),
            pltpu.SemaphoreType.DMA((nt,)),
        ],
        compiler_params=_compiler_params(),
    )(B_w_r, c, x2, A_k_cache, A_v_cache, A_wq, A_wo, w_mod, B_w_gate, B_w_up, B_w_down)
    return out.reshape(B, S, D)
```

```python
import functools

import jax
import jax.numpy as jnp
from jax import lax
import jax.experimental.pallas as pl
import jax.experimental.pallas.tpu as pltpu

HQ = 32
DH = 128
TQ = 256
CH = 16
PAD = 128
P0 = 2
G0 = 5
N0 = 2
MC = 512
PIN_R = 0
REL0 = 0
STRIDE = 3.5
CHE = 8
LAG = 3
PIN_C = 0
EPS = 1e-5
LOG2E = 1.4426950408889634


def _ln_stats(x, rel=None):
    d = x.shape[-1]
    part = x[..., 0:128]
    for j in range(1, d // 128):
        part = part + x[..., j * 128:(j + 1) * 128]
    if rel is not None:
        part = part + rel
    m = jnp.sum(part, axis=-1, keepdims=True) * (1.0 / d)
    xc = x - m
    v = jnp.mean(xc * xc, axis=-1, keepdims=True)
    return m, xc, lax.rsqrt(v + EPS)


def _ln(x, rel=None):
    _, xc, rs = _ln_stats(x, rel)
    return xc * rs


def _recip(l):
    r = pl.reciprocal(l, approx=True)
    return r * (2.0 - l * r)


def _kernel(wr_hbm, c_hbm, x_hbm, k_hbm, v_hbm, wq_hbm, wo_hbm, wmod_hbm,
            wg_hbm, wu_hbm, wd_hbm, out_hbm,
            wr_s, c_s, x_s, k_s, v_s, wq_s, wo_s, wmod_s, wg_s, wu_s, wd_s, out_s,
            sc_s, mraw_s, mod_s, h_s, q_s, o_s, acc_s, stat_s, best_r, best_i, zero_s, sems, osems,
            *, S, D, HKV, SK, W, F):
    nt = S // TQ
    rep = HQ // HKV
    NB = D // 128
    nch = TQ // CH
    CPV = D // MC
    NMC = 6 * CPV
    f32 = jnp.float32
    bf16 = jnp.bfloat16
    qscale = (DH ** -0.5) * LOG2E

    def al(v, n):
        return v if isinstance(v, int) else pl.multiple_of(v, n)

    S_C, S_WR, S_WG, S_WU, S_WD, S_M = 0, 1, 2, 3, 4, 5
    S_WQ = S_M + NMC
    S_K = S_WQ + HQ
    S_V = S_K + HKV
    S_WO = S_V + HKV
    S_X = S_WO + NB

    def cp_c():
        return pltpu.make_async_copy(c_hbm, c_s, sems.at[S_C])

    def cp_wr():
        return pltpu.make_async_copy(wr_hbm, wr_s, sems.at[S_WR])

    def cp_mod(j):
        return pltpu.make_async_copy(wmod_hbm.at[:, pl.ds(al(j * MC, MC), MC)], wmod_s.at[j], sems.at[S_M + j])

    def cp_wg():
        return pltpu.make_async_copy(wg_hbm, wg_s, sems.at[S_WG])

    def cp_wu():
        return pltpu.make_async_copy(wu_hbm, wu_s, sems.at[S_WU])

    def cp_wd():
        return pltpu.make_async_copy(wd_hbm, wd_s.at[:, pl.ds(0, D)], sems.at[S_WD])

    def cp_wq(h, n=1):
        sl = pl.ds(al(h * DH, DH), n * DH)
        return pltpu.make_async_copy(wq_hbm.at[:, sl], wq_s.at[:, sl], sems.at[S_WQ + h])

    def cp_k(g):
        return pltpu.make_async_copy(k_hbm.at[0, g, pl.ds(SK - W, W), :], k_s.at[g], sems.at[S_K + g])

    def cp_v(g):
        return pltpu.make_async_copy(v_hbm.at[0, g, pl.ds(SK - W, W), :], v_s.at[g], sems.at[S_V + g])

    def cp_wo(j):
        sl = pl.ds(al(j * D, D), D)
        return pltpu.make_async_copy(wo_hbm.at[sl, :], wo_s.at[sl, pl.ds(0, D)], sems.at[S_WO + j])

    def rsl(t, r0=0, n=TQ):
        return pl.ds(al(t * TQ + r0, n), n)

    def cp_x(t):
        return pltpu.make_async_copy(x_hbm.at[rsl(t), :], x_s.at[rsl(t), :], sems.at[S_X + t])

    def cp_out(t):
        return pltpu.make_async_copy(out_s.at[rsl(t), :], out_hbm.at[rsl(t), :], osems.at[t])

    def mvec(j):
        return mod_s[:, j * D:(j + 1) * D][None]

    def mraw(j):
        return jnp.concatenate([mraw_s[j * CPV + u] for u in range(CPV)], axis=1)

    def xrows(sl, n):
        return x_s[sl, :].astype(f32).reshape(n // 8, 8, D)

    def ln1(t, r0, n, rel=None):
        xn = _ln(xrows(rsl(t, r0, n), n), rel)
        h_s[pl.ds(al(r0, n), n), :] = (xn * mvec(1) + mvec(0)).reshape(n, D).astype(bf16)

    def resid(sl, n):
        attn = jnp.concatenate([acc_s[j, sl, :] for j in range(NB)], axis=1).reshape(n // 8, 8, D)
        return xrows(sl, n) + mvec(2) * attn

    def h2_from_stats(x1, sl, n):
        m = jnp.tile(stat_s[0, sl, :], (1, NB)).reshape(n // 8, 8, D)
        rs = jnp.tile(stat_s[1, sl, :], (1, NB)).reshape(n // 8, 8, D)
        return (x1 - m) * rs * mvec(4) + mvec(3)

    def epi_rows(t, r0, n, rel=None, write_out=True):
        sl = rsl(t, r0, n)
        x1 = resid(sl, n)
        m, xc, rs = _ln_stats(x1, rel)
        stat_s[0, sl, :] = jnp.broadcast_to(m.reshape(n, 1), (n, 128))
        stat_s[1, sl, :] = jnp.broadcast_to(rs.reshape(n, 1), (n, 128))
        h2 = xc * rs * mvec(4) + mvec(3)
        if write_out:
            out_s[sl, :] = (x1 + mvec(5) * h2).reshape(n, D).astype(out_s.dtype)
        r = jnp.sum(h2 * mvec(6), axis=-1, keepdims=True)
        r = r.astype(bf16).astype(f32)
        bv = best_r[...]
        bi = best_i[...]
        sub = lax.broadcasted_iota(jnp.int32, (8, 128), 0)
        for u in range(n // 8):
            ru = jnp.broadcast_to(r[u], (8, 128))
            better = ru > bv
            bv = jnp.where(better, ru, bv)
            bi = jnp.where(better, sub + (t * TQ + r0 + u * 8), bi)
        best_r[...] = bv
        best_i[...] = bi

    def qproj(hval, hh):
        return jnp.dot(hval, wq_s[:, pl.ds(al(hh * DH, DH), DH)], preferred_element_type=f32).astype(bf16)

    def qk(q, g):
        s = lax.dot_general(q, k_s[g], (((1,), (1,)), ((), ())), preferred_element_type=f32)
        m = jnp.max(s, axis=-1, keepdims=True)
        p = jnp.exp2(s - m)
        l = jnp.sum(p, axis=-1, keepdims=True)
        return (p * _recip(l)).astype(bf16)

    def pv(p, g, hh):
        o_s[hh] = pltpu.bitcast(jnp.dot(p, v_s[g], preferred_element_type=f32).astype(bf16), jnp.uint32)

    def o_heads(h0, h1):
        return pltpu.bitcast(jnp.concatenate([o_s[u] for u in range(h0, h1)], axis=1), bf16)

    cp_c().start()
    cp_x(0).start()
    for j in range(2 * CPV):
        cp_mod(j).start()
    NA = (HQ - P0) // G0
    NO = HQ * DH // D
    cp_wq(0).start()
    cp_k(0).start()
    cp_v(0).start()
    for h in range(1, P0 + 1):
        cp_wq(h).start()
    for j in range(NA):
        h0 = P0 + j * G0
        cp_wq(h0 + 1, G0 if j + 1 < NA else G0 - 1).start()
        if (h0 + G0 - 1) % rep < G0:
            cp_k((h0 + G0 - 1) // rep).start()
            cp_v((h0 + G0 - 1) // rep).start()
    cp_x(1).start()
    cp_wo(0).start()
    for j in range(1, NO):
        cp_wo(j).start()
        for u in range(CPV):
            cp_mod((j + 1) * CPV + u).start()
    cp_wr().start()
    for u in range(CPV):
        cp_mod(5 * CPV + u).start()
    for t in range(2, nt):
        cp_x(t).start()
    cp_wg().start()
    cp_wu().start()
    cp_wd().start()

    zero_s[0] = 0
    for n in range(NB):
        acc_s[n, rsl(0), :] = jnp.zeros((TQ, 128), f32)
    best_r[...] = jnp.full(best_r.shape, -jnp.inf, f32)
    best_i[...] = jnp.zeros(best_i.shape, jnp.int32)
    cp_c().wait()
    cp_x(0).wait()
    cf = c_s[...].astype(f32)
    sc_s[...] = jnp.broadcast_to(cf * jax.nn.sigmoid(cf), (16, D)).astype(bf16)
    xn0 = _ln(xrows(rsl(0), TQ))

    def mod_body(j, carry):
        cp_mod(j).wait()
        mraw_s[j] = jnp.dot(sc_s[...], wmod_s[j], preferred_element_type=f32)[0:8, :]
        return carry

    lax.fori_loop(0, 2 * CPV, mod_body, 0)
    mod_s[:, 0:D] = mraw(0) * qscale
    mod_s[:, D:2 * D] = (1.0 + mraw(1)) * qscale
    h_s[...] = (xn0 * mvec(1) + mvec(0)).reshape(TQ, D).astype(bf16)
    cp_wq(0).wait()
    hval0 = h_s[...]
    q = qproj(hval0, 0)
    cp_k(0).wait()
    cp_v(0).wait()
    for hh in range(P0):
        cp_wq(hh + 1).wait()
        p = qk(q, 0)
        q = qproj(hval0, hh + 1)
        pv(p, 0, hh)
    q_s[...] = q

    def a0_body(j, carry):
        h0 = P0 + j * G0

        @pl.when(j + 1 < NA)
        def _():
            cp_wq(h0 + 1, G0).wait()

        @pl.when(j + 1 == NA)
        def _():
            cp_wq(HQ - G0 + 1, G0 - 1).wait()

        @pl.when((h0 + G0 - 1) % rep < G0)
        def _():
            cp_k((h0 + G0 - 1) // rep).wait()
            cp_v((h0 + G0 - 1) // rep).wait()

        hval = h_s[...]
        q = q_s[...]
        for u in range(G0):
            g = (h0 + u) // rep
            p = qk(q, g)
            q = qproj(hval, jnp.minimum(h0 + u + 1, HQ - 1))
            pv(p, g, h0 + u)
        q_s[...] = q
        return carry

    assert (HQ - P0) % G0 == 0 and P0 + G0 - 1 < rep and (P0 + G0 - 1) % rep >= G0
    lax.fori_loop(0, NA, a0_body, 0)
    cp_x(1).wait()

    KP = 512

    def o0_body(j, carry):
        cp_wo(j).wait()

        @pl.when(j > 0)
        def _():
            for u in range(CPV):
                cp_mod((j + 1) * CPV + u).wait()

        sc = sc_s[...]
        hq = KP // DH
        for n in range(NB):
            acc = acc_s[n, rsl(0), :]
            cu, cn = divmod(n, MC // 128)
            mv = None
            for kh in range(D // KP):
                hb = (j * (D // KP) + kh) * hq
                lhs = pltpu.bitcast(jnp.concatenate([o_s[hb + u] for u in range(hq)], axis=1), bf16)
                acc = jnp.dot(lhs, wo_s[pl.ds(al(hb * DH, KP), KP), n * 128:(n + 1) * 128],
                              preferred_element_type=f32) + acc
                d = jnp.dot(sc[:, kh * KP:(kh + 1) * KP],
                            wmod_s[(j + 1) * CPV + cu, kh * KP:(kh + 1) * KP, cn * 128:(cn + 1) * 128],
                            preferred_element_type=f32)
                mv = d if mv is None else d + mv
            acc_s[n, rsl(0), :] = acc
            mraw_s[(j + 1) * CPV + cu, :, cn * 128:(cn + 1) * 128] = mv[0:8, :]
        nr = TQ // NO
        for c in range(nr // CH):
            ln1(1, j * nr + c * CH, CH)
        return carry

    assert NO == 4
    lax.fori_loop(0, NO, o0_body, 0)

    cp_wr().wait()
    for u in range(CPV):
        cp_mod(5 * CPV + u).wait()
    for u in range(CPV):
        mod_s[:, 5 * D + u * MC:5 * D + (u + 1) * MC] = jnp.dot(
            sc_s[...], wmod_s[5 * CPV + u], preferred_element_type=f32)[0:8, :]
    mod_s[:, 2 * D:3 * D] = mraw(2)
    mod_s[:, 3 * D:4 * D] = mraw(3)
    mod_s[:, 4 * D:5 * D] = 1.0 + mraw(4)
    mod_s[:, 6 * D:7 * D] = jnp.broadcast_to(wr_s[...].astype(f32).reshape(1, D), (8, D))

    def step(t, carry):
        @pl.when(t + 1 < nt)
        def _():
            cp_x(t + 1).wait()

        @pl.when(t + 1 == nt)
        def _():
            cp_wg().wait()
            cp_wu().wait()
            cp_wd().wait()

        zero = zero_s[0]
        z16 = pl.multiple_of(zero, 16)
        zvec = jnp.full((8, 128), zero, jnp.int32).astype(jnp.uint32)
        tprev, tnext = t - 1, jnp.minimum(t + 1, nt - 1)

        def fence(deps):
            d = None
            for ref, base in deps:
                n = 16 if ref.dtype == bf16 else 8
                v = pltpu.bitcast(ref[pl.ds(pl.multiple_of(base + z16, n), n), 0:128], jnp.uint32)
                d = v if d is None else d | v
            return d & zvec

        def pin(a, d):
            r0, c0 = PIN_R, PIN_C
            blk = pltpu.bitcast(pltpu.bitcast(a[r0:r0 + 16, c0:c0 + 128], jnp.uint32) | d, bf16)
            row = [a[r0:r0 + 16, 0:c0]] if c0 else []
            row = jnp.concatenate(row + [blk] + ([a[r0:r0 + 16, c0 + 128:]] if a.shape[1] > c0 + 128 else []), axis=1)
            col = [a[0:r0, :]] if r0 else []
            return jnp.concatenate(col + [row, a[r0 + 16:, :]], axis=0)

        hval = h_s[...]
        q = qproj(hval, 0)
        hq = KP // DH
        npass = HQ // hq

        def opass(n, kq, acc, deps=None):
            lhs = o_heads(kq * hq, (kq + 1) * hq)
            if deps is not None:
                lhs = pin(lhs, deps)
            d = jnp.dot(lhs, wo_s[kq * KP:(kq + 1) * KP, n * 128:(n + 1) * 128], preferred_element_type=f32)
            return d if acc is None else d + acc

        NF = 2
        ne = TQ // CHE
        for hh in range(HQ):
            g = hh // rep
            cs = [c for c in range(ne) if 1 + (c * (HQ - 1)) // ne == hh]
            for c in cs:
                epi_rows(tprev, c * CHE, CHE)
            if cs:
                q = pin(q, fence([(out_s, tprev * TQ), (best_r, 0), (stat_s.at[0], tprev * TQ)]))
            p = qk(q, g)
            if hh + 1 < HQ:
                q = qproj(hval, hh + 1)
            else:
                acc = None
                for kq in range(NF):
                    acc = opass(0, kq, acc)
            pv(p, g, hh)

        passes = [(n, kq) for n in range(NB) for kq in range(npass)][NF:]
        work = [('l', c) for c in range(nch)]
        rel_at = {int(REL0 + STRIDE * c): c for c in range(len(work))}
        assert len(rel_at) == len(work) and max(rel_at) + LAG < len(passes)
        due = {}
        for s, (n, kq) in enumerate(passes):
            if kq == 0:
                acc = None
            acc = opass(n, kq, acc, due.pop(s, None))
            if kq == npass - 1:
                acc_s[n, rsl(t), :] = acc
            if s in rel_at:
                rel = pltpu.bitcast(pltpu.bitcast(acc[0:8, :], jnp.uint32) & zvec, f32)
                kind, c = work[rel_at[s]]
                if kind == 'e':
                    epi_rows(tprev, c * CH, CH, rel)
                    due[s + LAG] = fence([(out_s, tprev * TQ), (best_r, 0), (stat_s.at[0], tprev * TQ)])
                else:
                    ln1(tnext, c * CH, CH, rel)
                    due[s + LAG] = fence([(h_s, 0)])
        assert not due
        cp_out(tprev).start()
        return carry

    lax.fori_loop(1, nt, step, 0)

    epi_rows(nt - 1, 0, TQ)
    cp_out(nt - 1).start()
    bv = best_r[...]
    rbest = jnp.max(bv, axis=0, keepdims=True)
    ibest = jnp.min(jnp.where(bv == rbest, best_i[...], S), axis=0, keepdims=True)
    idx = jnp.minimum(ibest[0, 0], S - 1)
    base = pl.multiple_of((idx // 16) * 16, 16)
    bsl = pl.ds(base, 16)
    x1 = resid(bsl, 16)
    h2 = h2_from_stats(x1, bsl, 16)
    xs = h2.reshape(16, D).astype(bf16)
    gt = jnp.dot(xs, wg_s[...], preferred_element_type=f32)
    up = jnp.dot(xs, wu_s[...], preferred_element_type=f32)
    a = (gt * jax.nn.sigmoid(gt) * up).astype(bf16)
    y = jnp.dot(a, wd_s[:, 0:D], preferred_element_type=f32)
    y = y * jnp.tile(jax.nn.sigmoid(rbest), (1, NB))
    rr = lax.broadcasted_iota(jnp.int32, (16, D), 0) + base
    upd = jnp.where(rr == idx, y, 0.0).reshape(2, 8, D)
    new = (x1 + mvec(5) * (h2 + upd)).reshape(16, D)
    for t in range(nt):
        cp_out(t).wait()
    out_s[bsl, :] = new.astype(out_s.dtype)
    fix = pltpu.make_async_copy(out_s.at[bsl, :], out_hbm.at[bsl, :], osems.at[0])
    fix.start()
    fix.wait()


def _compiler_params():
    kw = dict(vmem_limit_bytes=100 * 1024 * 1024)
    try:
        return pltpu.CompilerParams(disable_semaphore_checks=True, disable_bounds_checks=True, **kw)
    except TypeError:
        return pltpu.CompilerParams(**kw)


@jax.jit
def pallas_adaLN_cond__sliding_block_cached__moe_arch_mod__prompt_kernel(
    A_x: jax.Array,
    A_k_cache: jax.Array,
    A_v_cache: jax.Array,
    A_wq: jax.Array,
    A_wo: jax.Array,
    B_x: jax.Array,
    B_w_r: jax.Array,
    B_w_gate: jax.Array,
    B_w_up: jax.Array,
    B_w_down: jax.Array,
    c: jax.Array,
    w_mod: jax.Array,
):
    B, S, D = A_x.shape
    assert B == 1
    HKV, SK = A_k_cache.shape[1], A_k_cache.shape[2]
    W = min(4096, max(256, SK // 4))
    F = B_w_gate.shape[1]
    dt = A_x.dtype
    nt = S // TQ
    NB = D // 128
    NMC = 6 * D // MC
    x2 = A_x.reshape(S, D)
    anyspec = pl.BlockSpec(memory_space=pl.ANY)
    kern = functools.partial(_kernel, S=S, D=D, HKV=HKV, SK=SK, W=W, F=F)
    out = pl.pallas_call(
        kern,
        in_specs=[anyspec] * 11,
        out_specs=anyspec,
        out_shape=jax.ShapeDtypeStruct((S, D), dt),
        scratch_shapes=[
            pltpu.VMEM((D,), dt),
            pltpu.VMEM((1, D), dt),
            pltpu.VMEM((S, D), dt),
            pltpu.VMEM((HKV, W, DH), dt),
            pltpu.VMEM((HKV, W, DH), dt),
            pltpu.VMEM((D, HQ * DH + PAD), dt),
            pltpu.VMEM((HQ * DH, D + PAD), dt),
            pltpu.VMEM((NMC, D, MC), dt),
            pltpu.VMEM((D, F), dt),
            pltpu.VMEM((D, F), dt),
            pltpu.VMEM((F, D + PAD), dt),
            pltpu.VMEM((S, D), dt),
            pltpu.VMEM((16, D), dt),
            pltpu.VMEM((NMC, 8, MC), jnp.float32),
            pltpu.VMEM((8, 7 * D), jnp.float32),
            pltpu.VMEM((TQ, D), dt),
            pltpu.VMEM((TQ, DH), dt),
            pltpu.VMEM((HQ, TQ // 2, DH), jnp.uint32),
            pltpu.VMEM((NB, S, 128), jnp.float32),
            pltpu.VMEM((2, S, 128), jnp.float32),
            pltpu.VMEM((8, 128), jnp.float32),
            pltpu.VMEM((8, 128), jnp.int32),
            pltpu.SMEM((1,), jnp.int32),
            pltpu.SemaphoreType.DMA((5 + NMC + HQ + 2 * HKV + NB + nt,)),
            pltpu.SemaphoreType.DMA((nt,)),
        ],
        compiler_params=_compiler_params(),
    )(B_w_r, c, x2, A_k_cache, A_v_cache, A_wq, A_wo, w_mod, B_w_gate, B_w_up, B_w_down)
    return out.reshape(B, S, D)
```

```python
import functools

import jax
import jax.numpy as jnp
from jax import lax
import jax.experimental.pallas as pl
import jax.experimental.pallas.tpu as pltpu

HQ = 32
DH = 128
TQ = 256
PAD = 128
P0 = 2
G0 = 5
MC = 512
CHE = 8
UR = 32
LAG = 6
A0_REL = 96
EPS = 1e-5
LOG2E = 1.4426950408889634


def _ln_stats(x, rel=None):
    d = x.shape[-1]
    part = x[..., 0:128]
    for j in range(1, d // 128):
        part = part + x[..., j * 128:(j + 1) * 128]
    if rel is not None:
        part = part + rel
    m = jnp.sum(part, axis=-1, keepdims=True) * (1.0 / d)
    xc = x - m
    v = jnp.mean(xc * xc, axis=-1, keepdims=True)
    return m, xc, lax.rsqrt(v + EPS)


def _ln(x, rel=None):
    _, xc, rs = _ln_stats(x, rel)
    return xc * rs


def _recip(l):
    r = pl.reciprocal(l, approx=True)
    return r * (2.0 - l * r)


def _lhs_sums(a11, a12, a21, a22):
    return [a11 + a22, a21 + a22, a11, a22, a11 + a12, a21 - a11, a12 - a22]


def _rhs_sums(b11, b12, b21, b22):
    return [b11 + b22, b11, b12 - b22, b21 - b11, b22, b11 + b12, b21 + b22]


def _pack(x):
    return pltpu.bitcast(x.astype(jnp.bfloat16), jnp.uint32)


def _unpack(u):
    return pltpu.bitcast(u, jnp.bfloat16)


def _kernel(wr_hbm, c_hbm, x_hbm, k_hbm, v_hbm, wq_hbm, wo_hbm, wmod_hbm,
            wg_hbm, wu_hbm, wd_hbm, out_hbm,
            wr_s, c_s, x_s, k_s, v_s, wq_s, wo_s, wmod_s, wg_s, wu_s, wd_s, out_s,
            wqc_s, woc_s, hs_s,
            sc_s, mraw_s, mod_s, h_s, q_s, o_s, acc_s, stat_s, best_r, best_i, zero_s, sems, osems,
            *, S, D, HKV, SK, W, F):
    nt = S // TQ
    rep = HQ // HKV
    NB = D // 128
    HP = HQ // 2
    HT = TQ // 2
    KH = D // 2
    KP = 512
    CPV = D // MC
    NMC = 6 * CPV
    NA = (HQ - P0) // G0
    NO = HQ * DH // D
    f32 = jnp.float32
    bf16 = jnp.bfloat16
    qscale = (DH ** -0.5) * LOG2E
    assert KH == KP

    def al(v, n):
        return v if isinstance(v, int) else pl.multiple_of(v, n)

    S_C, S_WR, S_WG, S_WU, S_WD, S_M = 0, 1, 2, 3, 4, 5
    S_WQ = S_M + NMC
    S_K = S_WQ + HQ
    S_V = S_K + HKV
    S_WO = S_V + HKV
    S_X = S_WO + NO

    def cp_c():
        return pltpu.make_async_copy(c_hbm, c_s, sems.at[S_C])

    def cp_wr():
        return pltpu.make_async_copy(wr_hbm, wr_s, sems.at[S_WR])

    def cp_mod(j):
        return pltpu.make_async_copy(wmod_hbm.at[:, pl.ds(al(j * MC, MC), MC)], wmod_s.at[j], sems.at[S_M + j])

    def cp_wg():
        return pltpu.make_async_copy(wg_hbm, wg_s, sems.at[S_WG])

    def cp_wu():
        return pltpu.make_async_copy(wu_hbm, wu_s, sems.at[S_WU])

    def cp_wd():
        return pltpu.make_async_copy(wd_hbm, wd_s.at[:, pl.ds(0, D)], sems.at[S_WD])

    def cp_wq(h, n=1):
        sl = pl.ds(al(h * DH, DH), n * DH)
        return pltpu.make_async_copy(wq_hbm.at[:, sl], wq_s.at[:, sl], sems.at[S_WQ + h])

    def cp_k(g):
        return pltpu.make_async_copy(k_hbm.at[0, g, pl.ds(SK - W, W), :], k_s.at[g], sems.at[S_K + g])

    def cp_v(g):
        return pltpu.make_async_copy(v_hbm.at[0, g, pl.ds(SK - W, W), :], v_s.at[g], sems.at[S_V + g])

    def cp_wo(j):
        sl = pl.ds(al(j * D, D), D)
        return pltpu.make_async_copy(wo_hbm.at[sl, :], wo_s.at[sl, pl.ds(0, D)], sems.at[S_WO + j])

    def rsl(t, r0=0, n=TQ):
        return pl.ds(al(t * TQ + r0, n), n)

    def cp_x(t):
        return pltpu.make_async_copy(x_hbm.at[rsl(t), :], x_s.at[rsl(t), :], sems.at[S_X + t])

    def cp_out(t):
        return pltpu.make_async_copy(out_s.at[rsl(t), :], out_hbm.at[rsl(t), :], osems.at[t])

    def sched():
        zero = zero_s[0]
        z16 = pl.multiple_of(zero, 16)
        zvec = jnp.full((8, 128), zero, jnp.int32).astype(jnp.uint32)

        def fence(deps):
            d = None
            for ref, base in deps:
                n = 16 if ref.dtype == bf16 else 8
                v = pltpu.bitcast(ref[pl.ds(pl.multiple_of(base + z16, n), n), 0:128], jnp.uint32)
                d = v if d is None else d | v
            return d & zvec

        def release(acc, r0=0):
            return pltpu.bitcast(pltpu.bitcast(acc[r0:r0 + 8, :], jnp.uint32) & zvec, f32)

        return fence, release

    def pin(a, at):
        if not at:
            return a
        parts = []
        prev = 0
        for rb in sorted(at):
            r0 = rb * 8
            if r0 > prev:
                parts.append(a[prev:r0, :])
            if a.dtype == f32:
                blk = a[r0:r0 + 8, 0:128] + pltpu.bitcast(at[rb], f32)
            else:
                blk = a[r0:r0 + 8, 0:128] | at[rb]
            if a.shape[1] > 128:
                blk = jnp.concatenate([blk, a[r0:r0 + 8, 128:]], axis=1)
            parts.append(blk)
            prev = r0 + 8
        if prev < a.shape[0]:
            parts.append(a[prev:, :])
        return jnp.concatenate(parts, axis=0)

    def mvec(j):
        return mod_s[:, j * D:(j + 1) * D][None]

    def mraw(j):
        return jnp.concatenate([mraw_s[j * CPV + u] for u in range(CPV)], axis=1)

    def xrows(sl, n):
        return x_s[sl, :].astype(f32).reshape(n // 8, 8, D)

    def ln1(t, r0, rel=None):
        hh = []
        for half in range(2):
            xn = _ln(xrows(rsl(t, half * HT + r0, 16), 16), rel)
            hh.append((xn * mvec(1) + mvec(0)).reshape(16, D))
        sums = _lhs_sums(hh[0][:, :KH], hh[0][:, KH:], hh[1][:, :KH], hh[1][:, KH:])
        for i in range(7):
            hs_s[i, pl.ds(al(r0, 16), 16), :] = sums[i].astype(bf16)

    def w_sums(top, bot, rel):
        tf, bt = top.astype(f32), bot.astype(f32)
        b11, b12, b21, b22 = tf[:, :128], tf[:, 128:], bt[:, :128], bt[:, 128:]
        if rel is not None:
            relt = jnp.tile(rel, (UR // 8, 1))
            b11, b22 = b11 + relt, b22 + relt
        return [_pack(s) for s in _rhs_sums(b11, b12, b21, b22)]

    def wq_unit(p, r0, rel=None):
        cols = pl.ds(al(p * 2 * DH, 2 * DH), 2 * DH)
        sums = w_sums(wq_s[r0:r0 + UR, cols], wq_s[KH + r0:KH + r0 + UR, cols], rel)
        for i in range(7):
            wqc_s[p, i, r0 // 2:(r0 + UR) // 2, :] = sums[i]
        return (wqc_s.at[p, 0], r0 // 2)

    def wo_unit(hp, npr, r0, rel=None):
        e0 = hp * 2 * DH + r0
        sums = w_sums(wo_s[pl.ds(al(e0, UR), UR), npr * 256:(npr + 1) * 256],
                      wo_s[pl.ds(al(e0 + DH, UR), UR), npr * 256:(npr + 1) * 256], rel)
        d0 = (hp * DH + r0) // 2
        for i in range(7):
            woc_s[npr, i, pl.ds(al(d0, UR // 2), UR // 2), :] = sums[i]
        return (woc_s.at[npr, 0], d0)

    def resid(sl, n):
        attn = jnp.concatenate([acc_s[j, sl, :] for j in range(NB)], axis=1).reshape(n // 8, 8, D)
        return xrows(sl, n) + mvec(2) * attn

    def h2_from_stats(x1, sl, n):
        m = jnp.tile(stat_s[0, sl, :], (1, NB)).reshape(n // 8, 8, D)
        rs = jnp.tile(stat_s[1, sl, :], (1, NB)).reshape(n // 8, 8, D)
        return (x1 - m) * rs * mvec(4) + mvec(3)

    def epi_rows(t, r0, n):
        sl = rsl(t, r0, n)
        x1 = resid(sl, n)
        m, xc, rs = _ln_stats(x1)
        stat_s[0, sl, :] = jnp.broadcast_to(m.reshape(n, 1), (n, 128))
        stat_s[1, sl, :] = jnp.broadcast_to(rs.reshape(n, 1), (n, 128))
        h2 = xc * rs * mvec(4) + mvec(3)
        out_s[sl, :] = (x1 + mvec(5) * h2).reshape(n, D).astype(out_s.dtype)
        r = jnp.sum(h2 * mvec(6), axis=-1, keepdims=True)
        r = r.astype(bf16).astype(f32)
        bv = best_r[...]
        bi = best_i[...]
        sub = lax.broadcasted_iota(jnp.int32, (8, 128), 0)
        for u in range(n // 8):
            ru = jnp.broadcast_to(r[u], (8, 128))
            better = ru > bv
            bv = jnp.where(better, ru, bv)
            bi = jnp.where(better, sub + (t * TQ + r0 + u * 8), bi)
        best_r[...] = bv
        best_i[...] = bi

    def qproj(hval, hh):
        return jnp.dot(hval, wq_s[:, pl.ds(al(hh * DH, DH), DH)], preferred_element_type=f32)

    def qk(q, g):
        s = lax.dot_general(q.astype(bf16), k_s[g], (((1,), (1,)), ((), ())), preferred_element_type=f32)
        m = jnp.max(s, axis=-1, keepdims=True)
        p = jnp.exp2(s - m)
        l = jnp.sum(p, axis=-1, keepdims=True)
        return p * _recip(l)

    def pv(p, g):
        return jnp.dot(p.astype(bf16), v_s[g], preferred_element_type=f32)

    def spread(items, lo, hi):
        n = len(items)
        at = {}
        for u, it in enumerate(items):
            rb = lo + (u * (hi - lo + 1)) // n
            at[rb] = it if rb not in at else at[rb] | it
        return at

    cp_c().start()
    cp_x(0).start()
    for j in range(2 * CPV):
        cp_mod(j).start()
    cp_wq(0).start()
    cp_k(0).start()
    cp_v(0).start()
    for h in range(1, P0 + 1):
        cp_wq(h).start()
    for j in range(NA):
        h0 = P0 + j * G0
        cp_wq(h0 + 1, G0 if j + 1 < NA else G0 - 1).start()
        if (h0 + G0 - 1) % rep < G0:
            cp_k((h0 + G0 - 1) // rep).start()
            cp_v((h0 + G0 - 1) // rep).start()
    cp_x(1).start()
    cp_wo(0).start()
    for j in range(1, NO):
        cp_wo(j).start()
        for u in range(CPV):
            cp_mod((j + 1) * CPV + u).start()
    cp_wr().start()
    for u in range(CPV):
        cp_mod(5 * CPV + u).start()
    for t in range(2, nt):
        cp_x(t).start()
    cp_wg().start()
    cp_wu().start()
    cp_wd().start()

    zero_s[0] = 0
    for n in range(NB):
        acc_s[n, rsl(0), :] = jnp.zeros((TQ, 128), f32)
    best_r[...] = jnp.full(best_r.shape, -jnp.inf, f32)
    best_i[...] = jnp.zeros(best_i.shape, jnp.int32)
    cp_c().wait()
    cp_x(0).wait()
    cf = c_s[...].astype(f32)
    sc_s[...] = jnp.broadcast_to(cf * jax.nn.sigmoid(cf), (16, D)).astype(bf16)
    xn0 = _ln(xrows(rsl(0), TQ))

    def mod_body(j, carry):
        cp_mod(j).wait()
        mraw_s[j] = jnp.dot(sc_s[...], wmod_s[j], preferred_element_type=f32)[0:8, :]
        return carry

    lax.fori_loop(0, 2 * CPV, mod_body, 0)
    mod_s[:, 0:D] = mraw(0) * qscale
    mod_s[:, D:2 * D] = (1.0 + mraw(1)) * qscale
    h_s[...] = (xn0 * mvec(1) + mvec(0)).reshape(TQ, D).astype(bf16)
    cp_wq(0).wait()
    hval0 = h_s[...]
    q = qproj(hval0, 0)
    cp_k(0).wait()
    cp_v(0).wait()
    NU = KH // UR
    fence0, _ = sched()
    assert P0 == 2
    for hh in range(P0):
        cp_wq(hh + 1).wait()
        p = qk(q, 0)
        fs = [fence0([wq_unit(0, (hh * NU // P0 + u) * UR)]) for u in range(NU // P0)]
        q = qproj(hval0, hh + 1)
        o_s[hh] = _pack(pv(pin(p, {0: functools.reduce(lambda a, b: a | b, fs)}), 0))
    q_s[...] = q

    PPI = 3

    def a0_body(j, carry):
        h0 = P0 + j * G0

        @pl.when(j + 1 < NA)
        def _():
            cp_wq(h0 + 1, G0).wait()

        @pl.when(j + 1 == NA)
        def _():
            cp_wq(HQ - G0 + 1, G0 - 1).wait()

        @pl.when((h0 + G0 - 1) % rep < G0)
        def _():
            cp_k((h0 + G0 - 1) // rep).wait()
            cp_v((h0 + G0 - 1) // rep).wait()

        fence, release = sched()
        p0 = (h0 + G0 + 1) // 2 - PPI
        units = [(pp, u) for pp in range(PPI) for u in range(NU)]
        hval = h_s[...]
        q = q_s[...]
        o = None
        for u in range(G0):
            g = (h0 + u) // rep
            mine = units[u * len(units) // G0:(u + 1) * len(units) // G0]
            p = qk(q, g)
            last = None
            for n_, (pp, uu) in enumerate(mine):
                rel = None if o is None else release(o, min(A0_REL + 16 * n_, TQ - 8))
                last = wq_unit(p0 + pp, uu * UR, rel)
            q = qproj(hval, jnp.minimum(h0 + u + 1, HQ - 1))
            o = pv(pin(p, {0: fence([last])}), g)
            o_s[h0 + u] = _pack(o)
        q_s[...] = q
        return carry

    assert (HQ - P0) % G0 == 0 and P0 + G0 - 1 < rep and (P0 + G0 - 1) % rep >= G0
    cov = {0}
    for j in range(NA):
        p0_ = (P0 + j * G0 + G0 + 1) // 2 - PPI
        assert p0_ >= 0 and p0_ + PPI <= HP
        cov |= set(range(p0_, p0_ + PPI))
    assert cov == set(range(HP))
    lax.fori_loop(0, NA, a0_body, 0)
    cp_x(1).wait()

    def o0_body(j, carry):
        cp_wo(j).wait()

        @pl.when(j > 0)
        def _():
            for u in range(CPV):
                cp_mod((j + 1) * CPV + u).wait()

        fence, release = sched()
        sc = sc_s[...]
        hq = KP // DH
        ppi = D // (2 * DH)
        units = [(pp, npr, u) for pp in range(ppi) for npr in range(NB // 2) for u in range(DH // UR)]
        npass = NB * (D // KP)
        cnt = 0
        due = {}
        prev = None
        for n in range(NB):
            acc = acc_s[n, rsl(0), :]
            cu, cn = divmod(n, MC // 128)
            mv = None
            for kh in range(D // KP):
                hb = (j * (D // KP) + kh) * hq
                lhs = jnp.concatenate([o_s[hb + u] for u in range(hq)], axis=1)
                mine = units[cnt * len(units) // npass:(cnt + 1) * len(units) // npass]
                last = None
                for n_, (pp, npr, u) in enumerate(mine):
                    rel = None if prev is None else release(prev, 64 * n_)
                    last = wo_unit(j * ppi + pp, npr, u * UR, rel)
                if cnt + 1 < npass:
                    due[cnt + 1] = {2: fence([last])}
                acc = jnp.dot(_unpack(pin(lhs, due.pop(cnt, None))),
                              wo_s[pl.ds(al(hb * DH, KP), KP), n * 128:(n + 1) * 128],
                              preferred_element_type=f32) + acc
                prev = acc
                cnt += 1
                d = jnp.dot(sc[:, kh * KP:(kh + 1) * KP],
                            wmod_s[(j + 1) * CPV + cu, kh * KP:(kh + 1) * KP, cn * 128:(cn + 1) * 128],
                            preferred_element_type=f32)
                mv = d if mv is None else d + mv
            acc_s[n, rsl(0), :] = acc
            mraw_s[(j + 1) * CPV + cu, :, cn * 128:(cn + 1) * 128] = mv[0:8, :]
        nr = HT // NO
        for c in range(nr // 16):
            ln1(1, j * nr + c * 16)
        return carry

    assert NO == 4
    lax.fori_loop(0, NO, o0_body, 0)

    cp_wr().wait()
    for u in range(CPV):
        cp_mod(5 * CPV + u).wait()
    for u in range(CPV):
        mod_s[:, 5 * D + u * MC:5 * D + (u + 1) * MC] = jnp.dot(
            sc_s[...], wmod_s[5 * CPV + u], preferred_element_type=f32)[0:8, :]
    mod_s[:, 2 * D:3 * D] = mraw(2)
    mod_s[:, 3 * D:4 * D] = mraw(3)
    mod_s[:, 4 * D:5 * D] = 1.0 + mraw(4)
    mod_s[:, 6 * D:7 * D] = jnp.broadcast_to(wr_s[...].astype(f32).reshape(1, D), (8, D))

    def step(t, carry):
        @pl.when(t + 1 < nt)
        def _():
            cp_x(t + 1).wait()

        @pl.when(t + 1 == nt)
        def _():
            cp_wg().wait()
            cp_wu().wait()
            cp_wd().wait()

        fence, release = sched()
        tprev, tnext = t - 1, jnp.minimum(t + 1, nt - 1)

        hv = [hs_s[i] for i in range(7)]

        def qprod(p, i, acc=None):
            d = jnp.dot(hv[i], _unpack(wqc_s[p, i]), preferred_element_type=f32)
            return d if acc is None else d + acc

        def q_part1(p):
            return qprod(p, 0), qprod(p, 3), qprod(p, 4)

        def q_part2(p, st):
            m0, m3, m4 = st
            c11 = qprod(p, 6, m0 + m3 - m4)
            m1 = qprod(p, 1)
            m2 = qprod(p, 2)
            c22 = qprod(p, 5, m0 - m1 + m2)
            return jnp.concatenate([c11, m1 + m3], axis=0), jnp.concatenate([m2 + m4, c22], axis=0)

        NK = HP * DH // KP
        pq = KP // DH
        order = [0, 3, 4, 6, 1, 2, 5]
        passes = [(0, i, k) for i in order[:3] for k in range(NK - 1)] + [(0, i, NK - 1) for i in order[:3]]
        passes += [(0, i, k) for i in order[3:] for k in range(NK)]
        passes += [(npr, i, k) for npr in range(1, NB // 2) for i in order for k in range(NK)]
        ms = {}
        ol = {}
        osum = {}

        def opass(s, at=None):
            npr, i, k = passes[s]
            if k == 0:
                if i == 6:
                    ms[i] = ms[0] + ms[3] - ms[4]
                elif i == 5:
                    ms[i] = ms[0] - ms[1] + ms[2]
                else:
                    ms[i] = None
            if (i, k) not in ol:
                ol[i, k] = jnp.concatenate([osum[k * pq + u][i] for u in range(pq)], axis=1).astype(bf16)
            d = jnp.dot(ol[i, k], _unpack(pin(woc_s[npr, i, k * KP // 2:(k + 1) * KP // 2, :], at)),
                        preferred_element_type=f32)
            ms[i] = d if ms[i] is None else d + ms[i]
            if k == NK - 1:
                top, bot = rsl(t, 0, HT), rsl(t, HT, HT)
                if i == 6:
                    acc_s[2 * npr, top, :] = ms[6]
                elif i == 1:
                    acc_s[2 * npr, bot, :] = ms[1] + ms[3]
                elif i == 2:
                    acc_s[2 * npr + 1, top, :] = ms[2] + ms[4]
                elif i == 5:
                    acc_s[2 * npr + 1, bot, :] = ms[5]
            return ms[i]

        ne = TQ // CHE

        def qk_side(q, hh):
            cs = [c for c in range(ne) if 1 + (c * (HQ - 1)) // ne == hh]
            for c in cs:
                epi_rows(tprev, c * CHE, CHE)
            if cs:
                q = pin(q, {0: fence([(out_s, tprev * TQ), (best_r, 0), (stat_s.at[0], tprev * TQ)])})
            return qk(q, hh // rep)

        qa, qb = q_part2(0, q_part1(0))
        nfill = 0
        for hp in range(HP):
            g = 2 * hp // rep
            pa = qk_side(qa, 2 * hp)
            if hp + 1 < HP:
                st = q_part1(hp + 1)
            else:
                for _ in range(3):
                    opass(nfill)
                    nfill += 1
            pb = qk_side(qb, 2 * hp + 1)
            oa = pv(pa, g)
            if hp + 1 < HP:
                qa, qb = q_part2(hp + 1, st)
            else:
                for _ in range(4):
                    opass(nfill)
                    nfill += 1
            ob = pv(pb, g)
            osum[hp] = _lhs_sums(oa[:HT], ob[:HT], oa[HT:], ob[HT:])

        nl = HT // 16
        first = 7 * NK
        stride = (len(passes) - first - LAG - 1) // nl
        rel_at = {first + stride * c: c for c in range(nl)}
        due = {}
        for s in range(nfill, len(passes)):
            acc = opass(s, due.pop(s, None))
            if s in rel_at:
                ln1(tnext, rel_at[s] * 16, release(acc))
                due[s + LAG] = {0: fence([(hs_s.at[0], 0)])}
        assert not due
        cp_out(tprev).start()
        return carry

    lax.fori_loop(1, nt, step, 0)

    epi_rows(nt - 1, 0, TQ)
    cp_out(nt - 1).start()
    bv = best_r[...]
    rbest = jnp.max(bv, axis=0, keepdims=True)
    ibest = jnp.min(jnp.where(bv == rbest, best_i[...], S), axis=0, keepdims=True)
    idx = jnp.minimum(ibest[0, 0], S - 1)
    base = pl.multiple_of((idx // 16) * 16, 16)
    bsl = pl.ds(base, 16)
    x1 = resid(bsl, 16)
    h2 = h2_from_stats(x1, bsl, 16)
    xs = h2.reshape(16, D).astype(bf16)
    gt = jnp.dot(xs, wg_s[...], preferred_element_type=f32)
    up = jnp.dot(xs, wu_s[...], preferred_element_type=f32)
    a = (gt * jax.nn.sigmoid(gt) * up).astype(bf16)
    y = jnp.dot(a, wd_s[:, 0:D], preferred_element_type=f32)
    y = y * jnp.tile(jax.nn.sigmoid(rbest), (1, NB))
    rr = lax.broadcasted_iota(jnp.int32, (16, D), 0) + base
    upd = jnp.where(rr == idx, y, 0.0).reshape(2, 8, D)
    new = (x1 + mvec(5) * (h2 + upd)).reshape(16, D)
    for t in range(nt):
        cp_out(t).wait()
    out_s[bsl, :] = new.astype(out_s.dtype)
    fix = pltpu.make_async_copy(out_s.at[bsl, :], out_hbm.at[bsl, :], osems.at[0])
    fix.start()
    fix.wait()


def _compiler_params():
    kw = dict(vmem_limit_bytes=120 * 1024 * 1024)
    try:
        return pltpu.CompilerParams(disable_semaphore_checks=True, disable_bounds_checks=True, **kw)
    except TypeError:
        return pltpu.CompilerParams(**kw)


@jax.jit
def pallas_adaLN_cond__sliding_block_cached__moe_arch_mod__prompt_kernel(
    A_x: jax.Array,
    A_k_cache: jax.Array,
    A_v_cache: jax.Array,
    A_wq: jax.Array,
    A_wo: jax.Array,
    B_x: jax.Array,
    B_w_r: jax.Array,
    B_w_gate: jax.Array,
    B_w_up: jax.Array,
    B_w_down: jax.Array,
    c: jax.Array,
    w_mod: jax.Array,
):
    B, S, D = A_x.shape
    assert B == 1
    HKV, SK = A_k_cache.shape[1], A_k_cache.shape[2]
    W = min(4096, max(256, SK // 4))
    F = B_w_gate.shape[1]
    dt = A_x.dtype
    u32 = jnp.uint32
    nt = S // TQ
    NB = D // 128
    NMC = 6 * D // MC
    x2 = A_x.reshape(S, D)
    anyspec = pl.BlockSpec(memory_space=pl.ANY)
    kern = functools.partial(_kernel, S=S, D=D, HKV=HKV, SK=SK, W=W, F=F)
    out = pl.pallas_call(
        kern,
        in_specs=[anyspec] * 11,
        out_specs=anyspec,
        out_shape=jax.ShapeDtypeStruct((S, D), dt),
        scratch_shapes=[
            pltpu.VMEM((D,), dt),
            pltpu.VMEM((1, D), dt),
            pltpu.VMEM((S, D), dt),
            pltpu.VMEM((HKV, W, DH), dt),
            pltpu.VMEM((HKV, W, DH), dt),
            pltpu.VMEM((D, HQ * DH + PAD), dt),
            pltpu.VMEM((HQ * DH, D + PAD), dt),
            pltpu.VMEM((NMC, D, MC), dt),
            pltpu.VMEM((D, F), dt),
            pltpu.VMEM((D, F), dt),
            pltpu.VMEM((F, D + PAD), dt),
            pltpu.VMEM((S, D), dt),
            pltpu.VMEM((HQ // 2, 7, D // 4, DH), u32),
            pltpu.VMEM((NB // 2, 7, HQ * DH // 4, 128), u32),
            pltpu.VMEM((7, TQ // 2, D // 2), dt),
            pltpu.VMEM((16, D), dt),
            pltpu.VMEM((NMC, 8, MC), jnp.float32),
            pltpu.VMEM((8, 7 * D), jnp.float32),
            pltpu.VMEM((TQ, D), dt),
            pltpu.VMEM((TQ, DH), jnp.float32),
            pltpu.VMEM((HQ, TQ // 2, DH), u32),
            pltpu.VMEM((NB, S, 128), jnp.float32),
            pltpu.VMEM((2, S, 128), jnp.float32),
            pltpu.VMEM((8, 128), jnp.float32),
            pltpu.VMEM((8, 128), jnp.int32),
            pltpu.SMEM((1,), jnp.int32),
            pltpu.SemaphoreType.DMA((5 + NMC + HQ + 2 * HKV + HQ * DH // D + nt,)),
            pltpu.SemaphoreType.DMA((nt,)),
        ],
        compiler_params=_compiler_params(),
    )(B_w_r, c, x2, A_k_cache, A_v_cache, A_wq, A_wo, w_mod, B_w_gate, B_w_up, B_w_down)
    return out.reshape(B, S, D)
```

```python
import functools

import jax
import jax.numpy as jnp
from jax import lax
import jax.experimental.pallas as pl
import jax.experimental.pallas.tpu as pltpu

HQ = 32
DH = 128
TQ = 256
PAD = 128
P0 = 2
G0 = 5
MC = 512
CHE = 8
UR = 32
LAG = 6
LR = 8
EPS = 1e-5
LOG2E = 1.4426950408889634


def _ln_stats(x, rel=None):
    d = x.shape[-1]
    part = x[..., 0:128]
    for j in range(1, d // 128):
        part = part + x[..., j * 128:(j + 1) * 128]
    if rel is not None:
        part = part + rel
    m = jnp.sum(part, axis=-1, keepdims=True) * (1.0 / d)
    xc = x - m
    v = jnp.mean(xc * xc, axis=-1, keepdims=True)
    return m, xc, lax.rsqrt(v + EPS)


def _ln(x, rel=None):
    _, xc, rs = _ln_stats(x, rel)
    return xc * rs


def _recip(l):
    r = pl.reciprocal(l, approx=True)
    return r * (2.0 - l * r)


def _lhs_sums(a11, a12, a21, a22):
    return [a11 + a22, a21 + a22, a11, a22, a11 + a12, a21 - a11, a12 - a22]


def _rhs_sums(b11, b12, b21, b22):
    return [b11 + b22, b11, b12 - b22, b21 - b11, b22, b11 + b12, b21 + b22]


def _pack(x):
    return pltpu.bitcast(x.astype(jnp.bfloat16), jnp.uint32)


def _unpack(u):
    return pltpu.bitcast(u, jnp.bfloat16)


def _kernel(wr_hbm, c_hbm, x_hbm, k_hbm, v_hbm, wq_hbm, wo_hbm, wmod_hbm,
            wg_hbm, wu_hbm, wd_hbm, out_hbm,
            wr_s, c_s, x_s, k_s, v_s, wq_s, wo_s, wmod_s, wg_s, wu_s, wd_s, out_s,
            wqc_s, woc_s, hs_s,
            sc_s, mraw_s, mod_s, h_s, q_s, o_s, acc_s, stat_s, best_r, best_i, zero_s, sems, osems,
            *, S, D, HKV, SK, W, F):
    nt = S // TQ
    rep = HQ // HKV
    NB = D // 128
    HP = HQ // 2
    HT = TQ // 2
    KH = D // 2
    KP = 512
    CPV = D // MC
    NMC = 6 * CPV
    NA = (HQ - P0) // G0
    NO = HQ * DH // D
    f32 = jnp.float32
    bf16 = jnp.bfloat16
    qscale = (DH ** -0.5) * LOG2E
    assert KH == KP

    def al(v, n):
        return v if isinstance(v, int) else pl.multiple_of(v, n)

    S_C, S_WR, S_WG, S_WU, S_WD, S_M = 0, 1, 2, 3, 4, 5
    S_WQ = S_M + NMC
    S_K = S_WQ + HQ
    S_V = S_K + HKV
    S_WO = S_V + HKV
    S_X = S_WO + NO

    def cp_c():
        return pltpu.make_async_copy(c_hbm, c_s, sems.at[S_C])

    def cp_wr():
        return pltpu.make_async_copy(wr_hbm, wr_s, sems.at[S_WR])

    def cp_mod(j):
        return pltpu.make_async_copy(wmod_hbm.at[:, pl.ds(al(j * MC, MC), MC)], wmod_s.at[j], sems.at[S_M + j])

    def cp_wg():
        return pltpu.make_async_copy(wg_hbm, wg_s, sems.at[S_WG])

    def cp_wu():
        return pltpu.make_async_copy(wu_hbm, wu_s, sems.at[S_WU])

    def cp_wd():
        return pltpu.make_async_copy(wd_hbm, wd_s.at[:, pl.ds(0, D)], sems.at[S_WD])

    def cp_wq(h, n=1):
        sl = pl.ds(al(h * DH, DH), n * DH)
        return pltpu.make_async_copy(wq_hbm.at[:, sl], wq_s.at[:, sl], sems.at[S_WQ + h])

    def cp_k(g):
        return pltpu.make_async_copy(k_hbm.at[0, g, pl.ds(SK - W, W), :], k_s.at[g], sems.at[S_K + g])

    def cp_v(g):
        return pltpu.make_async_copy(v_hbm.at[0, g, pl.ds(SK - W, W), :], v_s.at[g], sems.at[S_V + g])

    def cp_wo(j):
        sl = pl.ds(al(j * D, D), D)
        return pltpu.make_async_copy(wo_hbm.at[sl, :], wo_s.at[sl, pl.ds(0, D)], sems.at[S_WO + j])

    def rsl(t, r0=0, n=TQ):
        return pl.ds(al(t * TQ + r0, n), n)

    def cp_x(t):
        return pltpu.make_async_copy(x_hbm.at[rsl(t), :], x_s.at[rsl(t), :], sems.at[S_X + t])

    def cp_out(t):
        return pltpu.make_async_copy(out_s.at[rsl(t), :], out_hbm.at[rsl(t), :], osems.at[t])

    def sched():
        zero = zero_s[0]
        z16 = pl.multiple_of(zero, 16)
        zvec = jnp.full((8, 128), zero, jnp.int32).astype(jnp.uint32)

        def fence(deps):
            d = None
            for ref, base in deps:
                n = 16 if ref.dtype == bf16 else 8
                v = pltpu.bitcast(ref[pl.ds(pl.multiple_of(base + z16, n), n), 0:128], jnp.uint32)
                d = v if d is None else d | v
            return d & zvec

        def release(acc, r0=0):
            return pltpu.bitcast(pltpu.bitcast(acc[r0:r0 + 8, :], jnp.uint32) & zvec, f32)

        return fence, release

    def pin(a, at):
        if not at:
            return a
        parts = []
        prev = 0
        for rb in sorted(at):
            r0 = rb * 8
            if r0 > prev:
                parts.append(a[prev:r0, :])
            if a.dtype == f32:
                blk = a[r0:r0 + 8, 0:128] + pltpu.bitcast(at[rb], f32)
            else:
                blk = a[r0:r0 + 8, 0:128] | at[rb]
            if a.shape[1] > 128:
                blk = jnp.concatenate([blk, a[r0:r0 + 8, 128:]], axis=1)
            parts.append(blk)
            prev = r0 + 8
        if prev < a.shape[0]:
            parts.append(a[prev:, :])
        return jnp.concatenate(parts, axis=0)

    def mvec(j):
        return mod_s[:, j * D:(j + 1) * D][None]

    def mraw(j):
        return jnp.concatenate([mraw_s[j * CPV + u] for u in range(CPV)], axis=1)

    def xrows(sl, n):
        return x_s[sl, :].astype(f32).reshape(n // 8, 8, D)

    def ln1(t, r0, rel=None):
        hh = []
        for half in range(2):
            xn = _ln(xrows(rsl(t, half * HT + r0, LR), LR), rel)
            hh.append((xn * mvec(1) + mvec(0)).reshape(LR, D))
        sums = _lhs_sums(hh[0][:, :KH], hh[0][:, KH:], hh[1][:, :KH], hh[1][:, KH:])
        for i in range(7):
            hs_s[i, pl.ds(al(r0, LR), LR), :] = sums[i].astype(bf16)

    def w_unit(ref, rt, rb, c0, rel):
        cols = pl.ds(al(c0, 256), 256)
        tf, bt = ref[rt, cols].astype(f32), ref[rb, cols].astype(f32)
        b11, b12, b21, b22 = tf[:, :128], tf[:, 128:], bt[:, :128], bt[:, 128:]
        if rel is not None:
            relt = jnp.tile(rel, (UR // 8, 1))
            b11, b22 = b11 + relt, b22 + relt
        sums = _rhs_sums(b11, b12, b21, b22)
        raw = {1: ref[rt, pl.ds(al(c0, 128), 128)], 4: ref[rb, pl.ds(al(c0 + 128, 128), 128)]}
        return [pltpu.bitcast(raw[i], jnp.uint32) if i in raw else _pack(sums[i]) for i in range(7)]

    def wq_unit(p, r0, rel=None):
        sums = w_unit(wq_s, pl.ds(r0, UR), pl.ds(KH + r0, UR), p * 2 * DH, rel)
        for i in range(7):
            wqc_s[p, i, r0 // 2:(r0 + UR) // 2, :] = sums[i]
        return (wqc_s.at[p, 0], r0 // 2)

    def wo_unit(hp, npr, r0, rel=None):
        e0 = hp * 2 * DH + r0
        sums = w_unit(wo_s, pl.ds(al(e0, UR), UR), pl.ds(al(e0 + DH, UR), UR), npr * 256, rel)
        d0 = (hp * DH + r0) // 2
        for i in range(7):
            woc_s[npr, i, pl.ds(al(d0, UR // 2), UR // 2), :] = sums[i]
        return (woc_s.at[npr, 0], d0)

    def resid(sl, n):
        attn = jnp.concatenate([acc_s[j, sl, :] for j in range(NB)], axis=1).reshape(n // 8, 8, D)
        return xrows(sl, n) + mvec(2) * attn

    def h2_from_stats(x1, sl, n):
        m = jnp.tile(stat_s[0, sl, :], (1, NB)).reshape(n // 8, 8, D)
        rs = jnp.tile(stat_s[1, sl, :], (1, NB)).reshape(n // 8, 8, D)
        return (x1 - m) * rs * mvec(4) + mvec(3)

    def epi_rows(t, r0, n):
        sl = rsl(t, r0, n)
        x1 = resid(sl, n)
        m, xc, rs = _ln_stats(x1)
        stat_s[0, sl, :] = jnp.broadcast_to(m.reshape(n, 1), (n, 128))
        stat_s[1, sl, :] = jnp.broadcast_to(rs.reshape(n, 1), (n, 128))
        h2 = xc * rs * mvec(4) + mvec(3)
        out_s[sl, :] = (x1 + mvec(5) * h2).reshape(n, D).astype(out_s.dtype)
        r = jnp.sum(h2 * mvec(6), axis=-1, keepdims=True)
        r = r.astype(bf16).astype(f32)
        bv = best_r[...]
        bi = best_i[...]
        sub = lax.broadcasted_iota(jnp.int32, (8, 128), 0)
        for u in range(n // 8):
            ru = jnp.broadcast_to(r[u], (8, 128))
            better = ru > bv
            bv = jnp.where(better, ru, bv)
            bi = jnp.where(better, sub + (t * TQ + r0 + u * 8), bi)
        best_r[...] = bv
        best_i[...] = bi

    def scores(q, g):
        return lax.dot_general(q.astype(bf16), k_s[g], (((1,), (1,)), ((), ())), preferred_element_type=f32)

    def softmax(s):
        m = jnp.max(s, axis=-1, keepdims=True)
        p = jnp.exp2(s - m)
        l = jnp.sum(p, axis=-1, keepdims=True)
        return p * _recip(l)

    def qk(q, g):
        return softmax(scores(q, g))

    def pv(p, g):
        return jnp.dot(p.astype(bf16), v_s[g], preferred_element_type=f32)

    def qhalf(hval, hh, kh, acc=None):
        d = jnp.dot(hval[:, kh * KH:(kh + 1) * KH], wq_s[kh * KH:(kh + 1) * KH, pl.ds(al(hh * DH, DH), DH)],
                    preferred_element_type=f32)
        return d if acc is None else d + acc

    def head0(hval, q, hh, o_prev, units, fence, release):
        g = hh // rep
        hn = hh + 1 if isinstance(hh, int) else jnp.minimum(hh + 1, HQ - 1)
        s = scores(q, g)
        p = softmax(s)
        q1 = qhalf(hval, hn, 0)
        pts = [(o_prev, 128), (o_prev, 200)] if o_prev is not None else []
        pts += [(s, 16), (s, 88), (s, 168), (s, 248), (q1, 72), (q1, 152), (q1, 232), (q1, 248)]
        last = None
        for (pp, r0), (val, row) in zip(units, pts, strict=False):
            last = wq_unit(pp, r0, release(val[:, 0:128], row))
        assert len(units) <= len(pts)
        qn = qhalf(hval, hn, 1, q1)
        o = pv(pin(p, {4: fence([last])}), g)
        o_s[hh] = _pack(o)
        return qn, o

    cp_c().start()
    cp_x(0).start()
    for j in range(2 * CPV):
        cp_mod(j).start()
    cp_wq(0).start()
    cp_k(0).start()
    cp_v(0).start()
    for h in range(1, P0 + 1):
        cp_wq(h).start()
    for j in range(NA):
        h0 = P0 + j * G0
        cp_wq(h0 + 1, G0 if j + 1 < NA else G0 - 1).start()
        if (h0 + G0 - 1) % rep < G0:
            cp_k((h0 + G0 - 1) // rep).start()
            cp_v((h0 + G0 - 1) // rep).start()
    cp_x(1).start()
    cp_wo(0).start()
    for j in range(1, NO):
        cp_wo(j).start()
        for u in range(CPV):
            cp_mod((j + 1) * CPV + u).start()
    cp_wr().start()
    for u in range(CPV):
        cp_mod(5 * CPV + u).start()
    for t in range(2, nt):
        cp_x(t).start()
    cp_wg().start()
    cp_wu().start()
    cp_wd().start()

    zero_s[0] = 0
    for n in range(NB):
        acc_s[n, rsl(0), :] = jnp.zeros((TQ, 128), f32)
    hs_s[0] = jnp.zeros((HT, KH), bf16)
    best_r[...] = jnp.full(best_r.shape, -jnp.inf, f32)
    best_i[...] = jnp.zeros(best_i.shape, jnp.int32)
    cp_c().wait()
    cp_x(0).wait()
    cf = c_s[...].astype(f32)
    sc_s[...] = jnp.broadcast_to(cf * jax.nn.sigmoid(cf), (16, D)).astype(bf16)
    xn0 = _ln(xrows(rsl(0), TQ))

    def mod_body(j, carry):
        cp_mod(j).wait()
        mraw_s[j] = jnp.dot(sc_s[...], wmod_s[j], preferred_element_type=f32)[0:8, :]
        return carry

    lax.fori_loop(0, 2 * CPV, mod_body, 0)
    mod_s[:, 0:D] = mraw(0) * qscale
    mod_s[:, D:2 * D] = (1.0 + mraw(1)) * qscale
    h_s[...] = (xn0 * mvec(1) + mvec(0)).reshape(TQ, D).astype(bf16)
    cp_wq(0).wait()
    hval0 = h_s[...]
    q = qhalf(hval0, 0, 1, qhalf(hval0, 0, 0))
    cp_k(0).wait()
    cp_v(0).wait()
    NU = KH // UR
    fence0, release0 = sched()
    assert P0 == 2
    for hh in range(P0):
        cp_wq(hh + 1).wait()
        q, _ = head0(hval0, q, hh, None, [(0, (hh * NU // P0 + u) * UR) for u in range(NU // P0)], fence0, release0)
    q_s[...] = q

    PPI = 2

    def a0_body(j, carry):
        h0 = P0 + j * G0

        @pl.when(j + 1 < NA)
        def _():
            cp_wq(h0 + 1, G0).wait()

        @pl.when(j + 1 == NA)
        def _():
            cp_wq(HQ - G0 + 1, G0 - 1).wait()

        @pl.when((h0 + G0 - 1) % rep < G0)
        def _():
            cp_k((h0 + G0 - 1) // rep).wait()
            cp_v((h0 + G0 - 1) // rep).wait()

        fence, release = sched()
        units = [(1 + j * PPI + pp, u * UR) for pp in range(PPI) for u in range(NU)]
        hval = h_s[...]
        q = q_s[...]
        o = None
        for u in range(G0):
            mine = units[u * len(units) // G0:(u + 1) * len(units) // G0]
            q, o = head0(hval, q, h0 + u, o, mine, fence, release)
        q_s[...] = q
        return carry

    assert (HQ - P0) % G0 == 0 and P0 + G0 - 1 < rep and (P0 + G0 - 1) % rep >= G0
    for j in range(NA):
        assert 2 * (1 + (j + 1) * PPI) <= min(P0 + (j + 1) * G0 + 1, HQ)
    assert 1 + NA * PPI >= HP - NO
    lax.fori_loop(0, NA, a0_body, 0)
    cp_x(1).wait()

    def o0_body(j, carry):
        cp_wo(j).wait()

        @pl.when(j > 0)
        def _():
            for u in range(CPV):
                cp_mod((j + 1) * CPV + u).wait()

        fence, release = sched()
        sc = sc_s[...]
        hq = KP // DH
        ppi = D // (2 * DH)
        units = [(pp, npr, u) for pp in range(ppi) for npr in range(NB // 2) for u in range(DH // UR)]
        npass = NB * (D // KP)
        cnt = 0
        due = {}
        prev = None
        for n in range(NB):
            acc = acc_s[n, rsl(0), :]
            cu, cn = divmod(n, MC // 128)
            mv = None
            for kh in range(D // KP):
                hb = (j * (D // KP) + kh) * hq
                lhs = jnp.concatenate([o_s[hb + u] for u in range(hq)], axis=1)
                mine = units[cnt * len(units) // npass:(cnt + 1) * len(units) // npass]
                step_ = TQ // (len(mine) + 1) // 8 * 8
                for n_, (pp, npr, u) in enumerate(mine):
                    rel = None if prev is None else release(prev, step_ * n_)
                    lwo = wo_unit(j * ppi + pp, npr, u * UR, rel)
                assert NU == npass
                lwq = wq_unit(HP - NO + j, cnt * UR, None if prev is None else release(prev, step_ * len(mine)))
                if cnt + 1 < npass:
                    due[cnt + 1] = due.get(cnt + 1, {})
                    due[cnt + 1][2] = fence([lwo, lwq])
                nlc = HT // NO // LR
                if cnt % 3 == 1 and cnt // 3 < nlc:
                    ln1(1, j * (HT // NO) + (cnt // 3) * LR, release(prev, 24))
                    due[cnt + 2] = {6: fence([(hs_s.at[0], j * (HT // NO))])}
                acc = jnp.dot(_unpack(pin(lhs, due.pop(cnt, None))),
                              wo_s[pl.ds(al(hb * DH, KP), KP), n * 128:(n + 1) * 128],
                              preferred_element_type=f32) + acc
                prev = acc
                cnt += 1
                d = jnp.dot(sc[:, kh * KP:(kh + 1) * KP],
                            wmod_s[(j + 1) * CPV + cu, kh * KP:(kh + 1) * KP, cn * 128:(cn + 1) * 128],
                            preferred_element_type=f32)
                mv = d if mv is None else d + mv
            acc_s[n, rsl(0), :] = acc
            mraw_s[(j + 1) * CPV + cu, :, cn * 128:(cn + 1) * 128] = mv[0:8, :]
        return carry

    assert NO == 4
    lax.fori_loop(0, NO, o0_body, 0)

    cp_wr().wait()
    for u in range(CPV):
        cp_mod(5 * CPV + u).wait()
    for u in range(CPV):
        mod_s[:, 5 * D + u * MC:5 * D + (u + 1) * MC] = jnp.dot(
            sc_s[...], wmod_s[5 * CPV + u], preferred_element_type=f32)[0:8, :]
    mod_s[:, 2 * D:3 * D] = mraw(2)
    mod_s[:, 3 * D:4 * D] = mraw(3)
    mod_s[:, 4 * D:5 * D] = 1.0 + mraw(4)
    mod_s[:, 6 * D:7 * D] = jnp.broadcast_to(wr_s[...].astype(f32).reshape(1, D), (8, D))

    def step(t, carry):
        @pl.when(t + 1 < nt)
        def _():
            cp_x(t + 1).wait()

        @pl.when(t + 1 == nt)
        def _():
            cp_wg().wait()
            cp_wu().wait()
            cp_wd().wait()

        fence, release = sched()
        tprev, tnext = t - 1, jnp.minimum(t + 1, nt - 1)

        hv = [hs_s[i] for i in range(7)]

        def qprod(p, i, acc=None):
            d = jnp.dot(hv[i], _unpack(wqc_s[p, i]), preferred_element_type=f32)
            return d if acc is None else d + acc

        def q_part1(p):
            return qprod(p, 0), qprod(p, 3), qprod(p, 4)

        def q_part2(p, st):
            m0, m3, m4 = st
            c11 = qprod(p, 6, m0 + m3 - m4)
            m1 = qprod(p, 1)
            m2 = qprod(p, 2)
            c22 = qprod(p, 5, m0 - m1 + m2)
            return jnp.concatenate([c11, m1 + m3], axis=0), jnp.concatenate([m2 + m4, c22], axis=0)

        NK = HP * DH // KP
        pq = KP // DH
        order = [0, 3, 4, 6, 1, 2, 5]
        passes = [(0, i, k) for i in order[:3] for k in range(NK - 1)] + [(0, i, NK - 1) for i in order[:3]]
        passes += [(0, i, k) for i in order[3:] for k in range(NK)]
        passes += [(npr, i, k) for npr in range(1, NB // 2) for i in order for k in range(NK)]
        ms = {}
        ol = {}
        osum = {}

        def opass(s, at=None):
            npr, i, k = passes[s]
            if k == 0:
                if i == 6:
                    ms[i] = ms[0] + ms[3] - ms[4]
                elif i == 5:
                    ms[i] = ms[0] - ms[1] + ms[2]
                else:
                    ms[i] = None
            if (i, k) not in ol:
                ol[i, k] = jnp.concatenate([osum[k * pq + u][i] for u in range(pq)], axis=1).astype(bf16)
            d = jnp.dot(ol[i, k], _unpack(pin(woc_s[npr, i, k * KP // 2:(k + 1) * KP // 2, :], at)),
                        preferred_element_type=f32)
            ms[i] = d if ms[i] is None else d + ms[i]
            if k == NK - 1:
                top, bot = rsl(t, 0, HT), rsl(t, HT, HT)
                if i == 6:
                    acc_s[2 * npr, top, :] = ms[6]
                elif i == 1:
                    acc_s[2 * npr, bot, :] = ms[1] + ms[3]
                elif i == 2:
                    acc_s[2 * npr + 1, top, :] = ms[2] + ms[4]
                elif i == 5:
                    acc_s[2 * npr + 1, bot, :] = ms[5]
            return ms[i]

        ne = TQ // CHE

        def qk_side(q, hh):
            cs = [c for c in range(ne) if 1 + (c * (HQ - 1)) // ne == hh]
            for c in cs:
                epi_rows(tprev, c * CHE, CHE)
            if cs:
                q = pin(q, {0: fence([(out_s, tprev * TQ), (best_r, 0), (stat_s.at[0], tprev * TQ)])})
            return qk(q, hh // rep)

        qa, qb = q_part2(0, q_part1(0))
        nfill = 0
        for hp in range(HP):
            g = 2 * hp // rep
            pa = qk_side(qa, 2 * hp)
            if hp + 1 < HP:
                st = q_part1(hp + 1)
            else:
                for _ in range(3):
                    opass(nfill)
                    nfill += 1
            pb = qk_side(qb, 2 * hp + 1)
            oa = pv(pa, g)
            if hp + 1 < HP:
                qa, qb = q_part2(hp + 1, st)
            else:
                for _ in range(4):
                    opass(nfill)
                    nfill += 1
            ob = pv(pb, g)
            osum[hp] = _lhs_sums(oa[:HT], ob[:HT], oa[HT:], ob[HT:])

        nl = HT // LR
        first = 7 * NK
        rel_at = {first + ((len(passes) - first - LAG - 1) * c) // (nl - 1): c for c in range(nl)}
        assert len(rel_at) == nl
        due = {}
        for s in range(nfill, len(passes)):
            acc = opass(s, due.pop(s, None))
            if s in rel_at:
                ln1(tnext, rel_at[s] * LR, release(acc))
                due[s + LAG] = {0: fence([(hs_s.at[0], 0)])}
        assert not due
        cp_out(tprev).start()
        return carry

    lax.fori_loop(1, nt, step, 0)

    epi_rows(nt - 1, 0, TQ)
    cp_out(nt - 1).start()
    bv = best_r[...]
    rbest = jnp.max(bv, axis=0, keepdims=True)
    ibest = jnp.min(jnp.where(bv == rbest, best_i[...], S), axis=0, keepdims=True)
    idx = jnp.minimum(ibest[0, 0], S - 1)
    base = pl.multiple_of((idx // 16) * 16, 16)
    bsl = pl.ds(base, 16)
    x1 = resid(bsl, 16)
    h2 = h2_from_stats(x1, bsl, 16)
    xs = h2.reshape(16, D).astype(bf16)
    gt = jnp.dot(xs, wg_s[...], preferred_element_type=f32)
    up = jnp.dot(xs, wu_s[...], preferred_element_type=f32)
    a = (gt * jax.nn.sigmoid(gt) * up).astype(bf16)
    y = jnp.dot(a, wd_s[:, 0:D], preferred_element_type=f32)
    y = y * jnp.tile(jax.nn.sigmoid(rbest), (1, NB))
    rr = lax.broadcasted_iota(jnp.int32, (16, D), 0) + base
    upd = jnp.where(rr == idx, y, 0.0).reshape(2, 8, D)
    new = (x1 + mvec(5) * (h2 + upd)).reshape(16, D)
    for t in range(nt):
        cp_out(t).wait()
    out_s[bsl, :] = new.astype(out_s.dtype)
    fix = pltpu.make_async_copy(out_s.at[bsl, :], out_hbm.at[bsl, :], osems.at[0])
    fix.start()
    fix.wait()


def _compiler_params():
    kw = dict(vmem_limit_bytes=120 * 1024 * 1024)
    try:
        return pltpu.CompilerParams(disable_semaphore_checks=True, disable_bounds_checks=True, **kw)
    except TypeError:
        return pltpu.CompilerParams(**kw)


@jax.jit
def pallas_adaLN_cond__sliding_block_cached__moe_arch_mod__prompt_kernel(
    A_x: jax.Array,
    A_k_cache: jax.Array,
    A_v_cache: jax.Array,
    A_wq: jax.Array,
    A_wo: jax.Array,
    B_x: jax.Array,
    B_w_r: jax.Array,
    B_w_gate: jax.Array,
    B_w_up: jax.Array,
    B_w_down: jax.Array,
    c: jax.Array,
    w_mod: jax.Array,
):
    B, S, D = A_x.shape
    assert B == 1
    HKV, SK = A_k_cache.shape[1], A_k_cache.shape[2]
    W = min(4096, max(256, SK // 4))
    F = B_w_gate.shape[1]
    dt = A_x.dtype
    u32 = jnp.uint32
    nt = S // TQ
    NB = D // 128
    NMC = 6 * D // MC
    x2 = A_x.reshape(S, D)
    anyspec = pl.BlockSpec(memory_space=pl.ANY)
    kern = functools.partial(_kernel, S=S, D=D, HKV=HKV, SK=SK, W=W, F=F)
    out = pl.pallas_call(
        kern,
        in_specs=[anyspec] * 11,
        out_specs=anyspec,
        out_shape=jax.ShapeDtypeStruct((S, D), dt),
        scratch_shapes=[
            pltpu.VMEM((D,), dt),
            pltpu.VMEM((1, D), dt),
            pltpu.VMEM((S, D), dt),
            pltpu.VMEM((HKV, W, DH), dt),
            pltpu.VMEM((HKV, W, DH), dt),
            pltpu.VMEM((D, HQ * DH + PAD), dt),
            pltpu.VMEM((HQ * DH, D + PAD), dt),
            pltpu.VMEM((NMC, D, MC), dt),
            pltpu.VMEM((D, F), dt),
            pltpu.VMEM((D, F), dt),
            pltpu.VMEM((F, D + PAD), dt),
            pltpu.VMEM((S, D), dt),
            pltpu.VMEM((HQ // 2, 7, D // 4, DH), u32),
            pltpu.VMEM((NB // 2, 7, HQ * DH // 4, 128), u32),
            pltpu.VMEM((7, TQ // 2, D // 2), dt),
            pltpu.VMEM((16, D), dt),
            pltpu.VMEM((NMC, 8, MC), jnp.float32),
            pltpu.VMEM((8, 7 * D), jnp.float32),
            pltpu.VMEM((TQ, D), dt),
            pltpu.VMEM((TQ, DH), jnp.float32),
            pltpu.VMEM((HQ, TQ // 2, DH), u32),
            pltpu.VMEM((NB, S, 128), jnp.float32),
            pltpu.VMEM((2, S, 128), jnp.float32),
            pltpu.VMEM((8, 128), jnp.float32),
            pltpu.VMEM((8, 128), jnp.int32),
            pltpu.SMEM((1,), jnp.int32),
            pltpu.SemaphoreType.DMA((5 + NMC + HQ + 2 * HKV + HQ * DH // D + nt,)),
            pltpu.SemaphoreType.DMA((nt,)),
        ],
        compiler_params=_compiler_params(),
    )(B_w_r, c, x2, A_k_cache, A_v_cache, A_wq, A_wo, w_mod, B_w_gate, B_w_up, B_w_down)
    return out.reshape(B, S, D)
```

```python
import functools

import jax
import jax.numpy as jnp
from jax import lax
import jax.experimental.pallas as pl
import jax.experimental.pallas.tpu as pltpu

HQ = 32
DH = 128
TQ = 256
PAD = 128
P0 = 2
G0 = 5
MC = 512
CHE = 8
UR = 32
LAG = 6
LR = 8
A0_EARLY = (6, 12, 18)
A0_PTS = [('o', 128), ('o', 176), ('o', 224), ('s', 16), ('s', 64), ('s', 112), ('q', 128), ('q', 184), ('q', 240), ('n', 40)]
A0_DUE = 12
O0_ROWS = (0, 64, 128, 192)
EPS = 1e-5
LOG2E = 1.4426950408889634


def _ln_stats(x, rel=None):
    d = x.shape[-1]
    part = x[..., 0:128]
    for j in range(1, d // 128):
        part = part + x[..., j * 128:(j + 1) * 128]
    if rel is not None:
        part = part + rel
    m = jnp.sum(part, axis=-1, keepdims=True) * (1.0 / d)
    xc = x - m
    v = jnp.mean(xc * xc, axis=-1, keepdims=True)
    return m, xc, lax.rsqrt(v + EPS)


def _ln(x, rel=None):
    _, xc, rs = _ln_stats(x, rel)
    return xc * rs


def _recip(l):
    r = pl.reciprocal(l, approx=True)
    return r * (2.0 - l * r)


def _lhs_sums(a11, a12, a21, a22):
    return [a11 + a22, a21 + a22, a11, a22, a11 + a12, a21 - a11, a12 - a22]


def _rhs_sums(b11, b12, b21, b22):
    return [b11 + b22, b11, b12 - b22, b21 - b11, b22, b11 + b12, b21 + b22]


def _pack(x):
    return pltpu.bitcast(x.astype(jnp.bfloat16), jnp.uint32)


def _unpack(u):
    return pltpu.bitcast(u, jnp.bfloat16)


def _kernel(wr_hbm, c_hbm, x_hbm, k_hbm, v_hbm, wq_hbm, wo_hbm, wmod_hbm,
            wg_hbm, wu_hbm, wd_hbm, out_hbm,
            wr_s, c_s, x_s, k_s, v_s, wq_s, wo_s, wmod_s, wg_s, wu_s, wd_s, out_s,
            wqc_s, woc_s, hs_s,
            sc_s, mraw_s, mod_s, h_s, q_s, o_s, acc_s, stat_s, best_r, best_i, zero_s, sems, osems,
            *, S, D, HKV, SK, W, F):
    nt = S // TQ
    rep = HQ // HKV
    NB = D // 128
    HP = HQ // 2
    HT = TQ // 2
    KH = D // 2
    KP = 512
    CPV = D // MC
    NMC = 6 * CPV
    NA = (HQ - P0) // G0
    NO = HQ * DH // D
    f32 = jnp.float32
    bf16 = jnp.bfloat16
    qscale = (DH ** -0.5) * LOG2E
    assert KH == KP

    def al(v, n):
        return v if isinstance(v, int) else pl.multiple_of(v, n)

    S_C, S_WR, S_WG, S_WU, S_WD, S_M = 0, 1, 2, 3, 4, 5
    S_WQ = S_M + NMC
    S_K = S_WQ + HQ
    S_V = S_K + HKV
    S_WO = S_V + HKV
    S_X = S_WO + NO

    def cp_c():
        return pltpu.make_async_copy(c_hbm, c_s, sems.at[S_C])

    def cp_wr():
        return pltpu.make_async_copy(wr_hbm, wr_s, sems.at[S_WR])

    def cp_mod(j):
        return pltpu.make_async_copy(wmod_hbm.at[:, pl.ds(al(j * MC, MC), MC)], wmod_s.at[j], sems.at[S_M + j])

    def cp_wg():
        return pltpu.make_async_copy(wg_hbm, wg_s, sems.at[S_WG])

    def cp_wu():
        return pltpu.make_async_copy(wu_hbm, wu_s, sems.at[S_WU])

    def cp_wd():
        return pltpu.make_async_copy(wd_hbm, wd_s.at[:, pl.ds(0, D)], sems.at[S_WD])

    def cp_wq(h, n=1):
        sl = pl.ds(al(h * DH, DH), n * DH)
        return pltpu.make_async_copy(wq_hbm.at[:, sl], wq_s.at[:, sl], sems.at[S_WQ + h])

    def cp_k(g):
        return pltpu.make_async_copy(k_hbm.at[0, g, pl.ds(SK - W, W), :], k_s.at[g], sems.at[S_K + g])

    def cp_v(g):
        return pltpu.make_async_copy(v_hbm.at[0, g, pl.ds(SK - W, W), :], v_s.at[g], sems.at[S_V + g])

    def cp_wo(j):
        sl = pl.ds(al(j * D, D), D)
        return pltpu.make_async_copy(wo_hbm.at[sl, :], wo_s.at[sl, pl.ds(0, D)], sems.at[S_WO + j])

    def rsl(t, r0=0, n=TQ):
        return pl.ds(al(t * TQ + r0, n), n)

    def cp_x(t):
        return pltpu.make_async_copy(x_hbm.at[rsl(t), :], x_s.at[rsl(t), :], sems.at[S_X + t])

    def cp_out(t):
        return pltpu.make_async_copy(out_s.at[rsl(t), :], out_hbm.at[rsl(t), :], osems.at[t])

    def sched():
        zero = zero_s[0]
        z16 = pl.multiple_of(zero, 16)
        zvec = jnp.full((8, 128), zero, jnp.int32).astype(jnp.uint32)

        def fence(deps):
            d = None
            for ref, base in deps:
                n = 16 if ref.dtype == bf16 else 8
                v = pltpu.bitcast(ref[pl.ds(pl.multiple_of(base + z16, n), n), 0:128], jnp.uint32)
                d = v if d is None else d | v
            return d & zvec

        def release(acc, r0=0):
            return pltpu.bitcast(pltpu.bitcast(acc[r0:r0 + 8, :], jnp.uint32) & zvec, f32)

        return fence, release

    def pin(a, at):
        if not at:
            return a
        parts = []
        prev = 0
        for rb in sorted(at):
            r0 = rb * 8
            if r0 > prev:
                parts.append(a[prev:r0, :])
            if a.dtype == f32:
                blk = a[r0:r0 + 8, 0:128] + pltpu.bitcast(at[rb], f32)
            else:
                blk = a[r0:r0 + 8, 0:128] | at[rb]
            if a.shape[1] > 128:
                blk = jnp.concatenate([blk, a[r0:r0 + 8, 128:]], axis=1)
            parts.append(blk)
            prev = r0 + 8
        if prev < a.shape[0]:
            parts.append(a[prev:, :])
        return jnp.concatenate(parts, axis=0)

    def mvec(j):
        return mod_s[:, j * D:(j + 1) * D][None]

    def mraw(j):
        return jnp.concatenate([mraw_s[j * CPV + u] for u in range(CPV)], axis=1)

    def xrows(sl, n):
        return x_s[sl, :].astype(f32).reshape(n // 8, 8, D)

    def ln1(t, r0, rel=None):
        hh = []
        for half in range(2):
            xn = _ln(xrows(rsl(t, half * HT + r0, LR), LR), rel)
            hh.append((xn * mvec(1) + mvec(0)).reshape(LR, D))
        sums = _lhs_sums(hh[0][:, :KH], hh[0][:, KH:], hh[1][:, :KH], hh[1][:, KH:])
        for i in range(7):
            hs_s[i, pl.ds(al(r0, LR), LR), :] = sums[i].astype(bf16)

    def w_unit(src, rt, rb, c0, dst, d0, rel):
        tf = src[rt:rt + UR, c0:c0 + 256].astype(f32)
        bt = src[rb:rb + UR, c0:c0 + 256].astype(f32)
        b11, b12, b21, b22 = tf[:, :128], tf[:, 128:], bt[:, :128], bt[:, 128:]
        if rel is not None:
            relt = jnp.tile(rel, (UR // 8, 1))
            b11, b22 = b11 + relt, b22 + relt
        sums = _rhs_sums(b11, b12, b21, b22)
        raw = {1: src[rt:rt + UR, c0:c0 + 128], 4: src[rb:rb + UR, c0 + 128:c0 + 256]}
        for i in range(7):
            dst[i, d0 // 2:(d0 + UR) // 2, :] = pltpu.bitcast(raw[i], jnp.uint32) if i in raw else _pack(sums[i])
        return (dst.at[0], d0 // 2)

    def resid(sl, n):
        attn = jnp.concatenate([acc_s[j, sl, :] for j in range(NB)], axis=1).reshape(n // 8, 8, D)
        return xrows(sl, n) + mvec(2) * attn

    def h2_from_stats(x1, sl, n):
        m = jnp.tile(stat_s[0, sl, :], (1, NB)).reshape(n // 8, 8, D)
        rs = jnp.tile(stat_s[1, sl, :], (1, NB)).reshape(n // 8, 8, D)
        return (x1 - m) * rs * mvec(4) + mvec(3)

    def epi_rows(t, r0, n):
        sl = rsl(t, r0, n)
        x1 = resid(sl, n)
        m, xc, rs = _ln_stats(x1)
        stat_s[0, sl, :] = jnp.broadcast_to(m.reshape(n, 1), (n, 128))
        stat_s[1, sl, :] = jnp.broadcast_to(rs.reshape(n, 1), (n, 128))
        h2 = xc * rs * mvec(4) + mvec(3)
        out_s[sl, :] = (x1 + mvec(5) * h2).reshape(n, D).astype(out_s.dtype)
        r = jnp.sum(h2 * mvec(6), axis=-1, keepdims=True)
        r = r.astype(bf16).astype(f32)
        bv = best_r[...]
        bi = best_i[...]
        sub = lax.broadcasted_iota(jnp.int32, (8, 128), 0)
        for u in range(n // 8):
            ru = jnp.broadcast_to(r[u], (8, 128))
            better = ru > bv
            bv = jnp.where(better, ru, bv)
            bi = jnp.where(better, sub + (t * TQ + r0 + u * 8), bi)
        best_r[...] = bv
        best_i[...] = bi

    def scores(q, g):
        return lax.dot_general(q.astype(bf16), k_s[g], (((1,), (1,)), ((), ())), preferred_element_type=f32)

    def softmax(s):
        m = jnp.max(s, axis=-1, keepdims=True)
        p = jnp.exp2(s - m)
        l = jnp.sum(p, axis=-1, keepdims=True)
        return p * _recip(l)

    def qk(q, g):
        return softmax(scores(q, g))

    def pv(p, g):
        return jnp.dot(p.astype(bf16), v_s[g], preferred_element_type=f32)

    def qhalf(hval, hh, kh, acc=None):
        d = jnp.dot(hval[:, kh * KH:(kh + 1) * KH], wq_s[kh * KH:(kh + 1) * KH, pl.ds(al(hh * DH, DH), DH)],
                    preferred_element_type=f32)
        return d if acc is None else d + acc

    def head0(hval, q, hh, o_prev, units, fence, release):
        g = hh // rep
        hn = hh + 1 if isinstance(hh, int) else jnp.minimum(hh + 1, HQ - 1)
        units = list(units)

        def unit(rel):
            sv, dv, pp, r0 = units.pop(0)
            return w_unit(sv, r0, KH + r0, pp * 2 * DH, dv.at[pp], r0, rel)

        if o_prev is None:
            q = pin(q, {rb: fence([unit(None)]) for rb in A0_EARLY})
        s = scores(q, g)
        p = softmax(s)
        q1 = qhalf(hval, hn, 0)
        qn = qhalf(hval, hn, 1, q1)
        vals = dict(o=o_prev, s=s, q=q1, n=qn)
        pts = [pt for pt in A0_PTS if vals[pt[0]] is not None]
        assert len(units) <= len(pts)
        last = None
        for nm, row in pts[:len(units)]:
            last = unit(release(vals[nm][:, 0:128], row))
        o = pv(pin(p, {A0_DUE: fence([last])}), g)
        o_s[hh] = _pack(o)
        return qn, o

    cp_c().start()
    cp_x(0).start()
    for j in range(2 * CPV):
        cp_mod(j).start()
    cp_wq(0).start()
    cp_k(0).start()
    cp_v(0).start()
    for h in range(1, P0 + 1):
        cp_wq(h).start()
    for j in range(NA):
        h0 = P0 + j * G0
        cp_wq(h0 + 1, G0 if j + 1 < NA else G0 - 1).start()
        if (h0 + G0 - 1) % rep < G0:
            cp_k((h0 + G0 - 1) // rep).start()
            cp_v((h0 + G0 - 1) // rep).start()
    cp_x(1).start()
    cp_wo(0).start()
    for j in range(1, NO):
        cp_wo(j).start()
        for u in range(CPV):
            cp_mod((j + 1) * CPV + u).start()
    cp_wr().start()
    for u in range(CPV):
        cp_mod(5 * CPV + u).start()
    for t in range(2, nt):
        cp_x(t).start()
    cp_wg().start()
    cp_wu().start()
    cp_wd().start()

    zero_s[0] = 0
    for n in range(NB):
        acc_s[n, rsl(0), :] = jnp.zeros((TQ, 128), f32)
    hs_s[0] = jnp.zeros((HT, KH), bf16)
    best_r[...] = jnp.full(best_r.shape, -jnp.inf, f32)
    best_i[...] = jnp.zeros(best_i.shape, jnp.int32)
    cp_c().wait()
    cp_x(0).wait()
    cf = c_s[...].astype(f32)
    sc_s[...] = jnp.broadcast_to(cf * jax.nn.sigmoid(cf), (16, D)).astype(bf16)
    xn0 = _ln(xrows(rsl(0), TQ))

    def mod_body(j, carry):
        cp_mod(j).wait()
        mraw_s[j] = jnp.dot(sc_s[...], wmod_s[j], preferred_element_type=f32)[0:8, :]
        return carry

    lax.fori_loop(0, 2 * CPV, mod_body, 0)
    mod_s[:, 0:D] = mraw(0) * qscale
    mod_s[:, D:2 * D] = (1.0 + mraw(1)) * qscale
    h_s[...] = (xn0 * mvec(1) + mvec(0)).reshape(TQ, D).astype(bf16)
    cp_wq(0).wait()
    hval0 = h_s[...]
    q = qhalf(hval0, 0, 1, qhalf(hval0, 0, 0))
    cp_k(0).wait()
    cp_v(0).wait()
    NU = KH // UR
    fence0, release0 = sched()
    assert P0 == 2
    for hh in range(P0):
        cp_wq(hh + 1).wait()
        q, _ = head0(hval0, q, hh, None, [(wq_s, wqc_s, 0, (hh * NU // P0 + u) * UR) for u in range(NU // P0)], fence0, release0)
    q_s[...] = q

    PPI = 3

    def a0_body(j, carry):
        h0 = P0 + j * G0

        @pl.when(j + 1 < NA)
        def _():
            cp_wq(h0 + 1, G0).wait()

        @pl.when(j + 1 == NA)
        def _():
            cp_wq(HQ - G0 + 1, G0 - 1).wait()

        @pl.when((h0 + G0 - 1) % rep < G0)
        def _():
            cp_k((h0 + G0 - 1) // rep).wait()
            cp_v((h0 + G0 - 1) // rep).wait()

        fence, release = sched()
        p0 = (h0 + G0 + 1) // 2 - PPI
        sv = wq_s.at[:, pl.ds(al(p0 * 2 * DH, 2 * DH), PPI * 2 * DH)]
        dv = wqc_s.at[pl.ds(p0, PPI)]
        units = [(sv, dv, pp, u * UR) for pp in range(PPI) for u in range(NU)]
        hval = h_s[...]
        q = q_s[...]
        o = None
        for u in range(G0):
            mine = units[u * len(units) // G0:(u + 1) * len(units) // G0]
            q, o = head0(hval, q, h0 + u, o, mine, fence, release)
        q_s[...] = q
        return carry

    assert (HQ - P0) % G0 == 0 and P0 + G0 - 1 < rep and (P0 + G0 - 1) % rep >= G0
    cov = {0}
    for j in range(NA):
        p0_ = (P0 + j * G0 + G0 + 1) // 2 - PPI
        assert p0_ >= 0 and p0_ + PPI <= HP
        cov |= set(range(p0_, p0_ + PPI))
    assert cov == set(range(HP))
    lax.fori_loop(0, NA, a0_body, 0)
    cp_x(1).wait()

    def o0_body(j, carry):
        cp_wo(j).wait()

        @pl.when(j > 0)
        def _():
            for u in range(CPV):
                cp_mod((j + 1) * CPV + u).wait()

        fence, release = sched()
        sc = sc_s[...]
        hq = KP // DH
        ppi = D // (2 * DH)
        wo_j = wo_s.at[pl.ds(al(j * D, D), D)]
        woc_j = woc_s.at[j]
        o_j = o_s.at[pl.ds(j * (D // DH), D // DH)]
        wm_j = wmod_s.at[pl.ds((j + 1) * CPV, CPV)]
        mr_j = mraw_s.at[pl.ds((j + 1) * CPV, CPV)]
        units = [(pp, npr, u) for pp in range(ppi) for npr in range(NB // 2) for u in range(DH // UR)]
        npass = NB * (D // KP)
        cnt = 0
        due = {}
        prev = None
        for n in range(NB):
            acc = acc_s[n, rsl(0), :]
            cu, cn = divmod(n, MC // 128)
            mv = None
            for kh in range(D // KP):
                lhs = jnp.concatenate([o_j[kh * hq + u] for u in range(hq)], axis=1)
                mine = units[cnt * len(units) // npass:(cnt + 1) * len(units) // npass]
                for n_, (pp, npr, u) in enumerate(mine):
                    rel = None if prev is None else release(prev, O0_ROWS[n_])
                    e0 = pp * 2 * DH + u * UR
                    last = w_unit(wo_j, e0, e0 + DH, npr * 256, woc_j.at[npr], pp * DH + u * UR, rel)
                    if prev is None:
                        due.setdefault(0, {})[4 * n_ + 3] = fence([last])
                if prev is not None and cnt + 1 < npass:
                    due.setdefault(cnt + 1, {})[2] = fence([last])
                nlc = HT // NO // LR
                if cnt % 3 == 1 and cnt // 3 < nlc:
                    ln1(1, j * (HT // NO) + (cnt // 3) * LR, release(prev, 24))
                    due.setdefault(cnt + 2, {})[6] = fence([(hs_s.at[0], j * (HT // NO))])
                acc = jnp.dot(_unpack(pin(lhs, due.pop(cnt, None))),
                              wo_j[kh * KP:(kh + 1) * KP, n * 128:(n + 1) * 128],
                              preferred_element_type=f32) + acc
                prev = acc
                cnt += 1
                d = jnp.dot(sc[:, kh * KP:(kh + 1) * KP],
                            wm_j[cu, kh * KP:(kh + 1) * KP, cn * 128:(cn + 1) * 128],
                            preferred_element_type=f32)
                mv = d if mv is None else d + mv
            acc_s[n, rsl(0), :] = acc
            mr_j[cu, :, cn * 128:(cn + 1) * 128] = mv[0:8, :]
        assert not due
        return carry

    assert NO == 4
    lax.fori_loop(0, NO, o0_body, 0)

    cp_wr().wait()
    for u in range(CPV):
        cp_mod(5 * CPV + u).wait()
    for u in range(CPV):
        mod_s[:, 5 * D + u * MC:5 * D + (u + 1) * MC] = jnp.dot(
            sc_s[...], wmod_s[5 * CPV + u], preferred_element_type=f32)[0:8, :]
    mod_s[:, 2 * D:3 * D] = mraw(2)
    mod_s[:, 3 * D:4 * D] = mraw(3)
    mod_s[:, 4 * D:5 * D] = 1.0 + mraw(4)
    mod_s[:, 6 * D:7 * D] = jnp.broadcast_to(wr_s[...].astype(f32).reshape(1, D), (8, D))

    def step(t, carry):
        @pl.when(t + 1 < nt)
        def _():
            cp_x(t + 1).wait()

        @pl.when(t + 1 == nt)
        def _():
            cp_wg().wait()
            cp_wu().wait()
            cp_wd().wait()

        fence, release = sched()
        tprev, tnext = t - 1, jnp.minimum(t + 1, nt - 1)

        hv = [hs_s[i] for i in range(7)]

        def qprod(p, i, acc=None):
            d = jnp.dot(hv[i], _unpack(wqc_s[p, i]), preferred_element_type=f32)
            return d if acc is None else d + acc

        def q_part1(p):
            return qprod(p, 0), qprod(p, 3), qprod(p, 4)

        def q_part2(p, st):
            m0, m3, m4 = st
            c11 = qprod(p, 6, m0 + m3 - m4)
            m1 = qprod(p, 1)
            m2 = qprod(p, 2)
            c22 = qprod(p, 5, m0 - m1 + m2)
            return jnp.concatenate([c11, m1 + m3], axis=0), jnp.concatenate([m2 + m4, c22], axis=0)

        NK = HP * DH // KP
        pq = KP // DH
        order = [0, 3, 4, 6, 1, 2, 5]
        passes = [(0, i, k) for i in order[:3] for k in range(NK - 1)] + [(0, i, NK - 1) for i in order[:3]]
        passes += [(0, i, k) for i in order[3:] for k in range(NK)]
        passes += [(npr, i, k) for npr in range(1, NB // 2) for i in order for k in range(NK)]
        ms = {}
        ol = {}
        osum = {}

        def opass(s, at=None):
            npr, i, k = passes[s]
            if k == 0:
                if i == 6:
                    ms[i] = ms[0] + ms[3] - ms[4]
                elif i == 5:
                    ms[i] = ms[0] - ms[1] + ms[2]
                else:
                    ms[i] = None
            if (i, k) not in ol:
                ol[i, k] = jnp.concatenate([osum[k * pq + u][i] for u in range(pq)], axis=1).astype(bf16)
            d = jnp.dot(ol[i, k], _unpack(pin(woc_s[k, npr, i], at)),
                        preferred_element_type=f32)
            ms[i] = d if ms[i] is None else d + ms[i]
            if k == NK - 1:
                top, bot = rsl(t, 0, HT), rsl(t, HT, HT)
                if i == 6:
                    acc_s[2 * npr, top, :] = ms[6]
                elif i == 1:
                    acc_s[2 * npr, bot, :] = ms[1] + ms[3]
                elif i == 2:
                    acc_s[2 * npr + 1, top, :] = ms[2] + ms[4]
                elif i == 5:
                    acc_s[2 * npr + 1, bot, :] = ms[5]
            return ms[i]

        ne = TQ // CHE

        def qk_side(q, hh):
            cs = [c for c in range(ne) if 1 + (c * (HQ - 1)) // ne == hh]
            for c in cs:
                epi_rows(tprev, c * CHE, CHE)
            if cs:
                q = pin(q, {0: fence([(out_s, tprev * TQ), (best_r, 0), (stat_s.at[0], tprev * TQ)])})
            return qk(q, hh // rep)

        qa, qb = q_part2(0, q_part1(0))
        nfill = 0
        for hp in range(HP):
            g = 2 * hp // rep
            pa = qk_side(qa, 2 * hp)
            if hp + 1 < HP:
                st = q_part1(hp + 1)
            else:
                for _ in range(3):
                    opass(nfill)
                    nfill += 1
            pb = qk_side(qb, 2 * hp + 1)
            oa = pv(pa, g)
            if hp + 1 < HP:
                qa, qb = q_part2(hp + 1, st)
            else:
                for _ in range(4):
                    opass(nfill)
                    nfill += 1
            ob = pv(pb, g)
            osum[hp] = _lhs_sums(oa[:HT], ob[:HT], oa[HT:], ob[HT:])

        nl = HT // LR
        first = 7 * NK
        rel_at = {first + ((len(passes) - first - LAG - 1) * c) // (nl - 1): c for c in range(nl)}
        assert len(rel_at) == nl
        due = {}
        for s in range(nfill, len(passes)):
            acc = opass(s, due.pop(s, None))
            if s in rel_at:
                ln1(tnext, rel_at[s] * LR, release(acc))
                due[s + LAG] = {0: fence([(hs_s.at[0], 0)])}
        assert not due
        cp_out(tprev).start()
        return carry

    lax.fori_loop(1, nt, step, 0)

    epi_rows(nt - 1, 0, TQ)
    cp_out(nt - 1).start()
    bv = best_r[...]
    rbest = jnp.max(bv, axis=0, keepdims=True)
    ibest = jnp.min(jnp.where(bv == rbest, best_i[...], S), axis=0, keepdims=True)
    idx = jnp.minimum(ibest[0, 0], S - 1)
    base = pl.multiple_of((idx // 16) * 16, 16)
    bsl = pl.ds(base, 16)
    x1 = resid(bsl, 16)
    h2 = h2_from_stats(x1, bsl, 16)
    xs = h2.reshape(16, D).astype(bf16)
    gt = jnp.dot(xs, wg_s[...], preferred_element_type=f32)
    up = jnp.dot(xs, wu_s[...], preferred_element_type=f32)
    a = (gt * jax.nn.sigmoid(gt) * up).astype(bf16)
    y = jnp.dot(a, wd_s[:, 0:D], preferred_element_type=f32)
    y = y * jnp.tile(jax.nn.sigmoid(rbest), (1, NB))
    rr = lax.broadcasted_iota(jnp.int32, (16, D), 0) + base
    upd = jnp.where(rr == idx, y, 0.0).reshape(2, 8, D)
    new = (x1 + mvec(5) * (h2 + upd)).reshape(16, D)
    for t in range(nt):
        cp_out(t).wait()
    out_s[bsl, :] = new.astype(out_s.dtype)
    fix = pltpu.make_async_copy(out_s.at[bsl, :], out_hbm.at[bsl, :], osems.at[0])
    fix.start()
    fix.wait()


def _compiler_params():
    kw = dict(vmem_limit_bytes=120 * 1024 * 1024)
    try:
        return pltpu.CompilerParams(disable_semaphore_checks=True, disable_bounds_checks=True, **kw)
    except TypeError:
        return pltpu.CompilerParams(**kw)


@jax.jit
def pallas_adaLN_cond__sliding_block_cached__moe_arch_mod__prompt_kernel(
    A_x: jax.Array,
    A_k_cache: jax.Array,
    A_v_cache: jax.Array,
    A_wq: jax.Array,
    A_wo: jax.Array,
    B_x: jax.Array,
    B_w_r: jax.Array,
    B_w_gate: jax.Array,
    B_w_up: jax.Array,
    B_w_down: jax.Array,
    c: jax.Array,
    w_mod: jax.Array,
):
    B, S, D = A_x.shape
    assert B == 1
    HKV, SK = A_k_cache.shape[1], A_k_cache.shape[2]
    W = min(4096, max(256, SK // 4))
    F = B_w_gate.shape[1]
    dt = A_x.dtype
    u32 = jnp.uint32
    nt = S // TQ
    NB = D // 128
    NMC = 6 * D // MC
    x2 = A_x.reshape(S, D)
    anyspec = pl.BlockSpec(memory_space=pl.ANY)
    kern = functools.partial(_kernel, S=S, D=D, HKV=HKV, SK=SK, W=W, F=F)
    out = pl.pallas_call(
        kern,
        in_specs=[anyspec] * 11,
        out_specs=anyspec,
        out_shape=jax.ShapeDtypeStruct((S, D), dt),
        scratch_shapes=[
            pltpu.VMEM((D,), dt),
            pltpu.VMEM((1, D), dt),
            pltpu.VMEM((S, D), dt),
            pltpu.VMEM((HKV, W, DH), dt),
            pltpu.VMEM((HKV, W, DH), dt),
            pltpu.VMEM((D, HQ * DH + PAD), dt),
            pltpu.VMEM((HQ * DH, D + PAD), dt),
            pltpu.VMEM((NMC, D, MC), dt),
            pltpu.VMEM((D, F), dt),
            pltpu.VMEM((D, F), dt),
            pltpu.VMEM((F, D + PAD), dt),
            pltpu.VMEM((S, D), dt),
            pltpu.VMEM((HQ // 2, 7, D // 4, DH), u32),
            pltpu.VMEM((HQ * DH // D, NB // 2, 7, D // 4, 128), u32),
            pltpu.VMEM((7, TQ // 2, D // 2), dt),
            pltpu.VMEM((16, D), dt),
            pltpu.VMEM((NMC, 8, MC), jnp.float32),
            pltpu.VMEM((8, 7 * D), jnp.float32),
            pltpu.VMEM((TQ, D), dt),
            pltpu.VMEM((TQ, DH), jnp.float32),
            pltpu.VMEM((HQ, TQ // 2, DH), u32),
            pltpu.VMEM((NB, S, 128), jnp.float32),
            pltpu.VMEM((2, S, 128), jnp.float32),
            pltpu.VMEM((8, 128), jnp.float32),
            pltpu.VMEM((8, 128), jnp.int32),
            pltpu.SMEM((1,), jnp.int32),
            pltpu.SemaphoreType.DMA((5 + NMC + HQ + 2 * HKV + HQ * DH // D + nt,)),
            pltpu.SemaphoreType.DMA((nt,)),
        ],
        compiler_params=_compiler_params(),
    )(B_w_r, c, x2, A_k_cache, A_v_cache, A_wq, A_wo, w_mod, B_w_gate, B_w_up, B_w_down)
    return out.reshape(B, S, D)
```

```python
import functools

import jax
import jax.numpy as jnp
from jax import lax
import jax.experimental.pallas as pl
import jax.experimental.pallas.tpu as pltpu

HQ = 32
DH = 128
TQ = 256
PAD = 128
P0 = 2
G0 = 5
MC = 512
CHE = 8
UR = 32
LN_PAR = 1
LR = 8
A0_EARLY = (6, 12, 18)
A0_PTS = [('o', 128), ('o', 176), ('o', 224), ('s', 16), ('s', 64), ('s', 112), ('q', 128), ('q', 184), ('q', 240), ('n', 40)]
A0_DUE = 12
O0_ROWS = ((0, 48, 88), (128, 176, 216))
EPS = 1e-5
LOG2E = 1.4426950408889634


def _ln_stats(x, rel=None):
    d = x.shape[-1]
    part = x[..., 0:128]
    for j in range(1, d // 128):
        part = part + x[..., j * 128:(j + 1) * 128]
    if rel is not None:
        part = part + rel
    m = jnp.sum(part, axis=-1, keepdims=True) * (1.0 / d)
    xc = x - m
    v = jnp.mean(xc * xc, axis=-1, keepdims=True)
    return m, xc, lax.rsqrt(v + EPS)


def _ln(x, rel=None):
    _, xc, rs = _ln_stats(x, rel)
    return xc * rs


def _recip(l):
    r = pl.reciprocal(l, approx=True)
    return r * (2.0 - l * r)


def _lhs_sums(a11, a12, a21, a22):
    return [a11 + a22, a21 + a22, a11, a22, a11 + a12, a21 - a11, a12 - a22]


def _rhs_sums(b11, b12, b21, b22):
    return [b11 + b22, b11, b12 - b22, b21 - b11, b22, b11 + b12, b21 + b22]


def _combine(m):
    return [[m[0] + m[3] - m[4] + m[6], m[2] + m[4]], [m[1] + m[3], m[0] - m[1] + m[2] + m[5]]]


def _two_level(sums, blk):
    x = [[sums(blk[0][a2][0][b2], blk[0][a2][1][b2], blk[1][a2][0][b2], blk[1][a2][1][b2]) for b2 in range(2)]
         for a2 in range(2)]
    return [sums(x[0][0][i], x[0][1][i], x[1][0][i], x[1][1][i]) for i in range(7)]


def _pack(x):
    return pltpu.bitcast(x.astype(jnp.bfloat16), jnp.uint32)


def _unpack(u):
    return pltpu.bitcast(u, jnp.bfloat16)


def _kernel(wr_hbm, c_hbm, x_hbm, k_hbm, v_hbm, wq_hbm, wo_hbm, wmod_hbm,
            wg_hbm, wu_hbm, wd_hbm, out_hbm,
            wr_s, c_s, x_s, k_s, v_s, wq_s, wo_s, wmod_s, wd_s, out_s,
            wqc_s, woc_s, hs_s,
            sc_s, mraw_s, mod_s, h_s, q_s, o_s, acc_s, stat_s, best_r, best_i, zero_s, sems, osems,
            *, S, D, HKV, SK, W, F):
    nt = S // TQ
    rep = HQ // HKV
    NB = D // 128
    HP = HQ // 2
    HT = TQ // 2
    KH = D // 2
    KP = 512
    CPV = D // MC
    NMC = 6 * CPV
    NA = (HQ - P0) // G0
    NO = HQ * DH // D
    f32 = jnp.float32
    bf16 = jnp.bfloat16
    qscale = (DH ** -0.5) * LOG2E
    assert KH == KP

    def al(v, n):
        return v if isinstance(v, int) else pl.multiple_of(v, n)

    S_C, S_WR, S_WG, S_WU, S_WD, S_M = 0, 1, 2, 3, 4, 5
    S_WQ = S_M + NMC
    S_K = S_WQ + HQ
    S_V = S_K + HKV
    S_WO = S_V + HKV
    S_X = S_WO + NO

    def cp_c():
        return pltpu.make_async_copy(c_hbm, c_s, sems.at[S_C])

    def cp_wr():
        return pltpu.make_async_copy(wr_hbm, wr_s, sems.at[S_WR])

    def cp_mod(j):
        return pltpu.make_async_copy(wmod_hbm.at[:, pl.ds(al(j * MC, MC), MC)], wmod_s.at[j], sems.at[S_M + j])

    def cp_wg():
        return pltpu.make_async_copy(wg_hbm, wq_s.at[:, pl.ds(0, F)], sems.at[S_WG])

    def cp_wu(u):
        return pltpu.make_async_copy(wu_hbm.at[:, pl.ds(u * MC, MC)], wmod_s.at[u], sems.at[S_M + u])

    def cp_wd():
        return pltpu.make_async_copy(wd_hbm, wd_s.at[:, pl.ds(0, D)], sems.at[S_WD])

    def cp_wq(h, n=1):
        sl = pl.ds(al(h * DH, DH), n * DH)
        return pltpu.make_async_copy(wq_hbm.at[:, sl], wq_s.at[:, sl], sems.at[S_WQ + h])

    def cp_k(g):
        return pltpu.make_async_copy(k_hbm.at[0, g, pl.ds(SK - W, W), :], k_s.at[g], sems.at[S_K + g])

    def cp_v(g):
        return pltpu.make_async_copy(v_hbm.at[0, g, pl.ds(SK - W, W), :], v_s.at[g], sems.at[S_V + g])

    def cp_wo(j):
        sl = pl.ds(al(j * D, D), D)
        return pltpu.make_async_copy(wo_hbm.at[sl, :], wo_s.at[sl, pl.ds(0, D)], sems.at[S_WO + j])

    def rsl(t, r0=0, n=TQ):
        return pl.ds(al(t * TQ + r0, n), n)

    def cp_x(t):
        return pltpu.make_async_copy(x_hbm.at[rsl(t), :], x_s.at[rsl(t), :], sems.at[S_X + t])

    def cp_out(t):
        return pltpu.make_async_copy(out_s.at[rsl(t), :], out_hbm.at[rsl(t), :], osems.at[t])

    def sched():
        zero = zero_s[0]
        z16 = pl.multiple_of(zero, 16)
        zvec = jnp.full((8, 128), zero, jnp.int32).astype(jnp.uint32)

        def fence(deps):
            d = None
            for ref, base in deps:
                n = 16 if ref.dtype == bf16 else 8
                v = pltpu.bitcast(ref[pl.ds(pl.multiple_of(base + z16, n), n), 0:128], jnp.uint32)
                d = v if d is None else d | v
            return d & zvec

        def release(acc, r0=0):
            return pltpu.bitcast(pltpu.bitcast(acc[r0:r0 + 8, :], jnp.uint32) & zvec, f32)

        return fence, release

    def pin(a, at):
        if not at:
            return a
        parts = []
        prev = 0
        for rb in sorted(at):
            r0 = rb * 8
            if r0 > prev:
                parts.append(a[prev:r0, :])
            if a.dtype == f32:
                blk = a[r0:r0 + 8, 0:128] + pltpu.bitcast(at[rb], f32)
            else:
                blk = a[r0:r0 + 8, 0:128] | at[rb]
            if a.shape[1] > 128:
                blk = jnp.concatenate([blk, a[r0:r0 + 8, 128:]], axis=1)
            parts.append(blk)
            prev = r0 + 8
        if prev < a.shape[0]:
            parts.append(a[prev:, :])
        return jnp.concatenate(parts, axis=0)

    def mvec(j):
        return mod_s[:, j * D:(j + 1) * D][None]

    def mraw(j):
        return jnp.concatenate([mraw_s[j * CPV + u] for u in range(CPV)], axis=1)

    def xrows(sl, n):
        return x_s[sl, :].astype(f32).reshape(n // 8, 8, D)

    def ln1(t, r0, rel=None):
        hh = []
        for half in range(2):
            xn = _ln(xrows(rsl(t, half * HT + r0, LR), LR), rel)
            hh.append((xn * mvec(1) + mvec(0)).reshape(LR, D))
        sums = _lhs_sums(hh[0][:, :KH], hh[0][:, KH:], hh[1][:, :KH], hh[1][:, KH:])
        for i in range(7):
            hs_s[i, pl.ds(al(r0, LR), LR), :] = sums[i].astype(bf16)

    def w_unit(src, rt, rb, c0, dst, d0, rel):
        tf = src[rt:rt + UR, c0:c0 + 256].astype(f32)
        bt = src[rb:rb + UR, c0:c0 + 256].astype(f32)
        b11, b12, b21, b22 = tf[:, :128], tf[:, 128:], bt[:, :128], bt[:, 128:]
        if rel is not None:
            relt = jnp.tile(rel, (UR // 8, 1))
            b11, b22 = b11 + relt, b22 + relt
        sums = _rhs_sums(b11, b12, b21, b22)
        raw = {1: src[rt:rt + UR, c0:c0 + 128], 4: src[rb:rb + UR, c0 + 128:c0 + 256]}
        for i in range(7):
            dst[i, d0 // 2:(d0 + UR) // 2, :] = pltpu.bitcast(raw[i], jnp.uint32) if i in raw else _pack(sums[i])
        return (dst.at[0], d0 // 2)

    RAW = {1: 0, 4: 1}
    WIDX = {}
    for i1_ in range(7):
        for i2_ in range(7):
            if not (i1_ in RAW and i2_ in RAW):
                WIDX[i1_, i2_] = len(WIDX)

    def wo_unit(src, dst, qd, ng, r0, rel):
        w = [src[(4 * qd + c) * DH + r0:(4 * qd + c) * DH + r0 + 16, ng * 512:(ng + 1) * 512].astype(f32)
             for c in range(4)]
        blk = [[[[w[2 * k1 + k2][:, (2 * n1 + n2) * 128:(2 * n1 + n2 + 1) * 128] for n2 in range(2)]
                 for n1 in range(2)] for k2 in range(2)] for k1 in range(2)]
        if rel is not None:
            for k1 in range(2):
                for n1 in range(2):
                    relt = jnp.tile(rel[0 if k1 == n1 else 1 + k1], (2, 1))
                    for k2 in range(2):
                        for n2 in range(2):
                            blk[k1][k2][n1][n2] = blk[k1][k2][n1][n2] + relt
        ops = _two_level(_rhs_sums, blk)
        for (i1, i2), u in WIDX.items():
            dst[ng, u, qd * DH + r0:qd * DH + r0 + 16, :] = ops[i1][i2].astype(bf16)
        return (dst.at[ng, 0], qd * DH + r0)

    def wo_op(ng, i1, i2, k):
        if i1 in RAW and i2 in RAW:
            c = 2 * RAW[i1] + RAW[i2]
            return jnp.concatenate(
                [wo_s[(4 * qd + c) * DH:(4 * qd + c + 1) * DH, (4 * ng + c) * 128:(4 * ng + c + 1) * 128]
                 for qd in range(4 * k, 4 * k + 4)], axis=0)
        return jnp.concatenate([woc_s[2 * k + u, ng, WIDX[i1, i2]] for u in range(2)], axis=0)

    def resid(sl, n):
        attn = jnp.concatenate([acc_s[j, sl, :] for j in range(NB)], axis=1).reshape(n // 8, 8, D)
        return xrows(sl, n) + mvec(2) * attn

    def h2_from_stats(x1, sl, n):
        m = jnp.tile(stat_s[0, sl, :], (1, NB)).reshape(n // 8, 8, D)
        rs = jnp.tile(stat_s[1, sl, :], (1, NB)).reshape(n // 8, 8, D)
        return (x1 - m) * rs * mvec(4) + mvec(3)

    def epi_rows(t, r0, n):
        sl = rsl(t, r0, n)
        x1 = resid(sl, n)
        m, xc, rs = _ln_stats(x1)
        stat_s[0, sl, :] = jnp.broadcast_to(m.reshape(n, 1), (n, 128))
        stat_s[1, sl, :] = jnp.broadcast_to(rs.reshape(n, 1), (n, 128))
        h2 = xc * rs * mvec(4) + mvec(3)
        out_s[sl, :] = (x1 + mvec(5) * h2).reshape(n, D).astype(out_s.dtype)
        r = jnp.sum(h2 * mvec(6), axis=-1, keepdims=True)
        r = r.astype(bf16).astype(f32)
        bv = best_r[...]
        bi = best_i[...]
        sub = lax.broadcasted_iota(jnp.int32, (8, 128), 0)
        for u in range(n // 8):
            ru = jnp.broadcast_to(r[u], (8, 128))
            better = ru > bv
            bv = jnp.where(better, ru, bv)
            bi = jnp.where(better, sub + (t * TQ + r0 + u * 8), bi)
        best_r[...] = bv
        best_i[...] = bi

    def scores(q, g):
        return lax.dot_general(q.astype(bf16), k_s[g], (((1,), (1,)), ((), ())), preferred_element_type=f32)

    def softmax(s):
        m = jnp.max(s, axis=-1, keepdims=True)
        p = jnp.exp2(s - m)
        l = jnp.sum(p, axis=-1, keepdims=True)
        return p * _recip(l)

    def qk(q, g):
        return softmax(scores(q, g))

    def pv(p, g):
        return jnp.dot(p.astype(bf16), v_s[g], preferred_element_type=f32)

    def qhalf(hval, hh, kh, acc=None):
        d = jnp.dot(hval[:, kh * KH:(kh + 1) * KH], wq_s[kh * KH:(kh + 1) * KH, pl.ds(al(hh * DH, DH), DH)],
                    preferred_element_type=f32)
        return d if acc is None else d + acc

    def head0(hval, q, hh, o_prev, units, fence, release):
        g = hh // rep
        hn = hh + 1 if isinstance(hh, int) else jnp.minimum(hh + 1, HQ - 1)
        units = list(units)

        def unit(rel):
            sv, dv, pp, r0 = units.pop(0)
            return w_unit(sv, r0, KH + r0, pp * 2 * DH, dv.at[pp], r0, rel)

        if o_prev is None:
            q = pin(q, {rb: fence([unit(None)]) for rb in A0_EARLY})
        s = scores(q, g)
        p = softmax(s)
        q1 = qhalf(hval, hn, 0)
        qn = qhalf(hval, hn, 1, q1)
        vals = dict(o=o_prev, s=s, q=q1, n=qn)
        pts = [pt for pt in A0_PTS if vals[pt[0]] is not None]
        assert len(units) <= len(pts)
        last = None
        for nm, row in pts[:len(units)]:
            last = unit(release(vals[nm][:, 0:128], row))
        o = pv(pin(p, {A0_DUE: fence([last])}), g)
        o_s[hh] = _pack(o)
        return qn, o

    cp_c().start()
    cp_x(0).start()
    for j in range(2 * CPV):
        cp_mod(j).start()
    cp_wq(0).start()
    cp_k(0).start()
    cp_v(0).start()
    for h in range(1, P0 + 1):
        cp_wq(h).start()
    for j in range(NA):
        h0 = P0 + j * G0
        cp_wq(h0 + 1, G0 if j + 1 < NA else G0 - 1).start()
        if (h0 + G0 - 1) % rep < G0:
            cp_k((h0 + G0 - 1) // rep).start()
            cp_v((h0 + G0 - 1) // rep).start()
    cp_x(1).start()
    cp_wo(0).start()
    for j in range(1, NO):
        cp_wo(j).start()
        for u in range(CPV):
            cp_mod((j + 1) * CPV + u).start()
    cp_wr().start()
    for u in range(CPV):
        cp_mod(5 * CPV + u).start()
    for t in range(2, nt):
        cp_x(t).start()
    cp_wd().start()

    zero_s[0] = 0
    for n in range(NB):
        acc_s[n, rsl(0), :] = jnp.zeros((TQ, 128), f32)
    hs_s[0] = jnp.zeros((HT, KH), bf16)
    best_r[...] = jnp.full(best_r.shape, -jnp.inf, f32)
    best_i[...] = jnp.zeros(best_i.shape, jnp.int32)
    cp_c().wait()
    cp_x(0).wait()
    cf = c_s[...].astype(f32)
    sc_s[...] = jnp.broadcast_to(cf * jax.nn.sigmoid(cf), (16, D)).astype(bf16)
    xn0 = _ln(xrows(rsl(0), TQ))

    def mod_body(j, carry):
        cp_mod(j).wait()
        mraw_s[j] = jnp.dot(sc_s[...], wmod_s[j], preferred_element_type=f32)[0:8, :]
        return carry

    lax.fori_loop(0, 2 * CPV, mod_body, 0)
    mod_s[:, 0:D] = mraw(0) * qscale
    mod_s[:, D:2 * D] = (1.0 + mraw(1)) * qscale
    h_s[...] = (xn0 * mvec(1) + mvec(0)).reshape(TQ, D).astype(bf16)
    cp_wq(0).wait()
    hval0 = h_s[...]
    q = qhalf(hval0, 0, 1, qhalf(hval0, 0, 0))
    cp_k(0).wait()
    cp_v(0).wait()
    NU = KH // UR
    fence0, release0 = sched()
    assert P0 == 2
    for hh in range(P0):
        cp_wq(hh + 1).wait()
        q, _ = head0(hval0, q, hh, None, [(wq_s, wqc_s, 0, (hh * NU // P0 + u) * UR) for u in range(NU // P0)], fence0, release0)
    q_s[...] = q

    PPI = 3

    def a0_body(j, carry):
        h0 = P0 + j * G0

        @pl.when(j + 1 < NA)
        def _():
            cp_wq(h0 + 1, G0).wait()

        @pl.when(j + 1 == NA)
        def _():
            cp_wq(HQ - G0 + 1, G0 - 1).wait()

        @pl.when((h0 + G0 - 1) % rep < G0)
        def _():
            cp_k((h0 + G0 - 1) // rep).wait()
            cp_v((h0 + G0 - 1) // rep).wait()

        fence, release = sched()
        p0 = (h0 + G0 + 1) // 2 - PPI
        sv = wq_s.at[:, pl.ds(al(p0 * 2 * DH, 2 * DH), PPI * 2 * DH)]
        dv = wqc_s.at[pl.ds(p0, PPI)]
        units = [(sv, dv, pp, u * UR) for pp in range(PPI) for u in range(NU)]
        hval = h_s[...]
        q = q_s[...]
        o = None
        for u in range(G0):
            mine = units[u * len(units) // G0:(u + 1) * len(units) // G0]
            q, o = head0(hval, q, h0 + u, o, mine, fence, release)
        q_s[...] = q
        return carry

    assert (HQ - P0) % G0 == 0 and P0 + G0 - 1 < rep and (P0 + G0 - 1) % rep >= G0
    cov = {0}
    for j in range(NA):
        p0_ = (P0 + j * G0 + G0 + 1) // 2 - PPI
        assert p0_ >= 0 and p0_ + PPI <= HP
        cov |= set(range(p0_, p0_ + PPI))
    assert cov == set(range(HP))
    lax.fori_loop(0, NA, a0_body, 0)
    cp_x(1).wait()

    def o0_body(j, carry):
        cp_wo(j).wait()

        @pl.when(j > 0)
        def _():
            for u in range(CPV):
                cp_mod((j + 1) * CPV + u).wait()

        fence, release = sched()
        sc = sc_s[...]
        hq = KP // DH
        ppi = D // (2 * DH)
        wo_j = wo_s.at[pl.ds(al(j * D, D), D)]
        woc_j = woc_s.at[j]
        o_j = o_s.at[pl.ds(j * (D // DH), D // DH)]
        wm_j = wmod_s.at[pl.ds((j + 1) * CPV, CPV)]
        mr_j = mraw_s.at[pl.ds((j + 1) * CPV, CPV)]
        units = [(qd, ng, u) for qd in range(2) for ng in range(2) for u in range(DH // 16)]
        npass = NB * (D // KP)
        cnt = 0
        due = {}
        prev = None
        for n in range(NB):
            acc = acc_s[n, rsl(0), :]
            cu, cn = divmod(n, MC // 128)
            mv = None
            for kh in range(D // KP):
                lhs = jnp.concatenate([o_j[kh * hq + u] for u in range(hq)], axis=1)
                mine = units[cnt * len(units) // npass:(cnt + 1) * len(units) // npass]
                for n_, (qd, ng, u) in enumerate(mine):
                    rel = None if prev is None else [release(prev, rw) for rw in O0_ROWS[n_]]
                    last = wo_unit(wo_j, woc_j, qd, ng, u * 16, rel)
                    if prev is None:
                        due.setdefault(0, {})[8 * n_ + 7] = fence([last])
                if prev is not None and cnt + 1 < npass:
                    due.setdefault(cnt + 1, {})[2] = fence([last])
                nlc = HT // NO // LR
                if cnt % 3 == 1 and cnt // 3 < nlc:
                    ln1(1, j * (HT // NO) + (cnt // 3) * LR, release(prev, 24))
                    due.setdefault(cnt + 2, {})[6] = fence([(hs_s.at[0], j * (HT // NO))])
                acc = jnp.dot(_unpack(pin(lhs, due.pop(cnt, None))),
                              wo_j[kh * KP:(kh + 1) * KP, n * 128:(n + 1) * 128],
                              preferred_element_type=f32) + acc
                prev = acc
                cnt += 1
                d = jnp.dot(sc[:, kh * KP:(kh + 1) * KP],
                            wm_j[cu, kh * KP:(kh + 1) * KP, cn * 128:(cn + 1) * 128],
                            preferred_element_type=f32)
                mv = d if mv is None else d + mv
            acc_s[n, rsl(0), :] = acc
            mr_j[cu, :, cn * 128:(cn + 1) * 128] = mv[0:8, :]
        assert not due
        return carry

    assert NO == 4
    lax.fori_loop(0, NO, o0_body, 0)

    cp_wr().wait()
    for u in range(CPV):
        cp_mod(5 * CPV + u).wait()
    for u in range(CPV):
        mod_s[:, 5 * D + u * MC:5 * D + (u + 1) * MC] = jnp.dot(
            sc_s[...], wmod_s[5 * CPV + u], preferred_element_type=f32)[0:8, :]
    mod_s[:, 2 * D:3 * D] = mraw(2)
    mod_s[:, 3 * D:4 * D] = mraw(3)
    mod_s[:, 4 * D:5 * D] = 1.0 + mraw(4)
    mod_s[:, 6 * D:7 * D] = jnp.broadcast_to(wr_s[...].astype(f32).reshape(1, D), (8, D))
    cp_wg().start()
    for u in range(F // MC):
        cp_wu(u).start()

    def step(t, carry):
        @pl.when(t + 1 < nt)
        def _():
            cp_x(t + 1).wait()

        @pl.when(t + 1 == nt)
        def _():
            cp_wg().wait()
            for u in range(F // MC):
                cp_wu(u).wait()
            cp_wd().wait()

        fence, release = sched()
        tprev, tnext = t - 1, jnp.minimum(t + 1, nt - 1)

        hv = [hs_s[i] for i in range(7)]

        def qprod(p, i, acc=None):
            d = jnp.dot(hv[i], _unpack(wqc_s[p, i]), preferred_element_type=f32)
            return d if acc is None else d + acc

        def q_part1(p):
            return qprod(p, 0), qprod(p, 3), qprod(p, 4)

        def q_part2(p, st):
            m0, m3, m4 = st
            c11 = qprod(p, 6, m0 + m3 - m4)
            m1 = qprod(p, 1)
            m2 = qprod(p, 2)
            c22 = qprod(p, 5, m0 - m1 + m2)
            return jnp.concatenate([c11, m1 + m3], axis=0), jnp.concatenate([m2 + m4, c22], axis=0)

        order = [0, 3, 4, 6, 1, 2, 5]
        prods = [(ng, i1, i2) for ng in range(2) for i1 in order for i2 in order]
        NE = 18
        passes = [pr + (0,) for pr in prods[:NE]] + [pr + (1,) for pr in prods[:NE]]
        passes += [pr + (k,) for pr in prods[NE:] for k in range(2)]
        QT = TQ // 4
        ms = {}
        mo = {}
        ol = {}
        osum = {}

        def opass(s, at=None):
            ng, i1, i2, k = passes[s]
            if (i1, i2, k) not in ol:
                ol[i1, i2, k] = jnp.concatenate([osum[4 * k + u][i1][i2] for u in range(4)], axis=1).astype(bf16)
            w = wo_op(ng, i1, i2, k)
            if at:
                w = jnp.concatenate([_unpack(pin(pltpu.bitcast(w[0:16], jnp.uint32), at)), w[16:]], axis=0)
            d = jnp.dot(ol[i1, i2, k], w, preferred_element_type=f32)
            res = ms[i1, i2] = d if k == 0 else d + ms[i1, i2]
            if k == 1 and i2 == order[-1]:
                mo[i1] = _combine([ms.pop((i1, i)) for i in range(7)])
                outs = {6: (0, 0), 1: (1, 0), 2: (0, 1), 5: (1, 1)}
                if i1 in outs:
                    r1, n1 = outs[i1]
                    for r2 in range(2):
                        for n2 in range(2):
                            z = [mo[i][r2][n2] if i in mo else None for i in range(7)]
                            if i1 == 6:
                                c = z[0] + z[3] - z[4] + z[6]
                            elif i1 == 1:
                                c = z[1] + z[3]
                            elif i1 == 2:
                                c = z[2] + z[4]
                            else:
                                c = z[0] - z[1] + z[2] + z[5]
                            acc_s[4 * ng + 2 * n1 + n2, rsl(t, r1 * HT + r2 * QT, QT), :] = c
                if i1 == order[-1]:
                    mo.clear()
            return res

        ne = TQ // CHE

        def qk_side(q, hh):
            cs = [c for c in range(ne) if 1 + (c * (HQ - 1)) // ne == hh]
            for c in cs:
                epi_rows(tprev, c * CHE, CHE)
            deps = [(out_s, tprev * TQ), (best_r, 0), (stat_s.at[0], tprev * TQ)] if cs else []
            if hh % 2 == LN_PAR:
                ln1(tnext, (hh // 2) * LR)
                deps.append((hs_s.at[0], 0))
            if deps:
                q = pin(q, {0: fence(deps)})
            return qk(q, hh // rep)

        qa, qb = q_part2(0, q_part1(0))
        nfill = 0
        for hp in range(HP):
            g = 2 * hp // rep
            pa = qk_side(qa, 2 * hp)
            if hp + 1 < HP:
                st = q_part1(hp + 1)
            else:
                for _ in range(6):
                    opass(nfill)
                    nfill += 1
            pb = qk_side(qb, 2 * hp + 1)
            oa = pv(pa, g)
            if hp + 1 < HP:
                qa, qb = q_part2(hp + 1, st)
            else:
                for _ in range(8):
                    opass(nfill)
                    nfill += 1
            ob = pv(pb, g)
            if hp % 2 == 0:
                oprev = (oa, ob)
            else:
                oq = [oprev, (oa, ob)]
                blk = [[[[oq[k1][k2][r1 * HT + r2 * QT:r1 * HT + (r2 + 1) * QT] for k2 in range(2)]
                         for k1 in range(2)] for r2 in range(2)] for r1 in range(2)]
                osum[hp // 2] = _two_level(_lhs_sums, blk)

        for s in range(nfill, len(passes)):
            opass(s)
        cp_out(tprev).start()
        return carry

    lax.fori_loop(1, nt, step, 0)

    epi_rows(nt - 1, 0, TQ)
    cp_out(nt - 1).start()
    bv = best_r[...]
    rbest = jnp.max(bv, axis=0, keepdims=True)
    ibest = jnp.min(jnp.where(bv == rbest, best_i[...], S), axis=0, keepdims=True)
    idx = jnp.minimum(ibest[0, 0], S - 1)
    base = pl.multiple_of((idx // 16) * 16, 16)
    bsl = pl.ds(base, 16)
    x1 = resid(bsl, 16)
    h2 = h2_from_stats(x1, bsl, 16)
    xs = h2.reshape(16, D).astype(bf16)
    gt = jnp.dot(xs, wq_s[:, 0:F], preferred_element_type=f32)
    up = jnp.concatenate([jnp.dot(xs, wmod_s[u], preferred_element_type=f32) for u in range(F // MC)], axis=1)
    a = (gt * jax.nn.sigmoid(gt) * up).astype(bf16)
    y = jnp.dot(a, wd_s[:, 0:D], preferred_element_type=f32)
    y = y * jnp.tile(jax.nn.sigmoid(rbest), (1, NB))
    rr = lax.broadcasted_iota(jnp.int32, (16, D), 0) + base
    upd = jnp.where(rr == idx, y, 0.0).reshape(2, 8, D)
    new = (x1 + mvec(5) * (h2 + upd)).reshape(16, D)
    for t in range(nt):
        cp_out(t).wait()
    out_s[bsl, :] = new.astype(out_s.dtype)
    fix = pltpu.make_async_copy(out_s.at[bsl, :], out_hbm.at[bsl, :], osems.at[0])
    fix.start()
    fix.wait()


def _compiler_params():
    kw = dict(vmem_limit_bytes=120 * 1024 * 1024)
    try:
        return pltpu.CompilerParams(disable_semaphore_checks=True, disable_bounds_checks=True, **kw)
    except TypeError:
        return pltpu.CompilerParams(**kw)


@jax.jit
def pallas_adaLN_cond__sliding_block_cached__moe_arch_mod__prompt_kernel(
    A_x: jax.Array,
    A_k_cache: jax.Array,
    A_v_cache: jax.Array,
    A_wq: jax.Array,
    A_wo: jax.Array,
    B_x: jax.Array,
    B_w_r: jax.Array,
    B_w_gate: jax.Array,
    B_w_up: jax.Array,
    B_w_down: jax.Array,
    c: jax.Array,
    w_mod: jax.Array,
):
    B, S, D = A_x.shape
    assert B == 1
    HKV, SK = A_k_cache.shape[1], A_k_cache.shape[2]
    W = min(4096, max(256, SK // 4))
    F = B_w_gate.shape[1]
    dt = A_x.dtype
    u32 = jnp.uint32
    nt = S // TQ
    NB = D // 128
    NMC = 6 * D // MC
    x2 = A_x.reshape(S, D)
    anyspec = pl.BlockSpec(memory_space=pl.ANY)
    kern = functools.partial(_kernel, S=S, D=D, HKV=HKV, SK=SK, W=W, F=F)
    out = pl.pallas_call(
        kern,
        in_specs=[anyspec] * 11,
        out_specs=anyspec,
        out_shape=jax.ShapeDtypeStruct((S, D), dt),
        scratch_shapes=[
            pltpu.VMEM((D,), dt),
            pltpu.VMEM((1, D), dt),
            pltpu.VMEM((S, D), dt),
            pltpu.VMEM((HKV, W, DH), dt),
            pltpu.VMEM((HKV, W, DH), dt),
            pltpu.VMEM((D, HQ * DH + PAD), dt),
            pltpu.VMEM((HQ * DH, D + PAD), dt),
            pltpu.VMEM((NMC, D, MC), dt),
            pltpu.VMEM((F, D + PAD), dt),
            pltpu.VMEM((S, D), dt),
            pltpu.VMEM((HQ // 2, 7, D // 4, DH), u32),
            pltpu.VMEM((HQ * DH // D, 2, 45, 2 * DH, 128), dt),
            pltpu.VMEM((7, TQ // 2, D // 2), dt),
            pltpu.VMEM((16, D), dt),
            pltpu.VMEM((NMC, 8, MC), jnp.float32),
            pltpu.VMEM((8, 7 * D), jnp.float32),
            pltpu.VMEM((TQ, D), dt),
            pltpu.VMEM((TQ, DH), jnp.float32),
            pltpu.VMEM((HQ, TQ // 2, DH), u32),
            pltpu.VMEM((NB, S, 128), jnp.float32),
            pltpu.VMEM((2, S, 128), jnp.float32),
            pltpu.VMEM((8, 128), jnp.float32),
            pltpu.VMEM((8, 128), jnp.int32),
            pltpu.SMEM((1,), jnp.int32),
            pltpu.SemaphoreType.DMA((5 + NMC + HQ + 2 * HKV + HQ * DH // D + nt,)),
            pltpu.SemaphoreType.DMA((nt,)),
        ],
        compiler_params=_compiler_params(),
    )(B_w_r, c, x2, A_k_cache, A_v_cache, A_wq, A_wo, w_mod, B_w_gate, B_w_up, B_w_down)
    return out.reshape(B, S, D)
```

```python
import functools

import jax
import jax.numpy as jnp
from jax import lax
import jax.experimental.pallas as pl
import jax.experimental.pallas.tpu as pltpu

HQ = 32
DH = 128
TQ = 256
PAD = 128
P0 = 2
G0 = 5
MC = 512
CHE = 8
UR = 32
SIDE_ROWS = (200, 248, 144)
OS_A = (128, 168, 208)
OS_B = (0, 40, 80)
LR = 8
A0_EARLY = (6, 12, 18)
A0_PTS = [('o', 128), ('o', 176), ('o', 224), ('s', 16), ('s', 64), ('s', 112), ('q', 128), ('q', 184), ('q', 240), ('n', 40)]
A0_DUE = 12
O0_ROWS = ((0, 48, 88), (128, 176, 216))
EPS = 1e-5
LOG2E = 1.4426950408889634


def _ln_stats(x, rel=None):
    d = x.shape[-1]
    part = x[..., 0:128]
    for j in range(1, d // 128):
        part = part + x[..., j * 128:(j + 1) * 128]
    if rel is not None:
        part = part + rel
    m = jnp.sum(part, axis=-1, keepdims=True) * (1.0 / d)
    xc = x - m
    v = jnp.mean(xc * xc, axis=-1, keepdims=True)
    return m, xc, lax.rsqrt(v + EPS)


def _ln(x, rel=None):
    _, xc, rs = _ln_stats(x, rel)
    return xc * rs


def _recip(l):
    r = pl.reciprocal(l, approx=True)
    return r * (2.0 - l * r)


def _lhs_sums(a11, a12, a21, a22):
    return [a11 + a22, a21 + a22, a11, a22, a11 + a12, a21 - a11, a12 - a22]


def _rhs_sums(b11, b12, b21, b22):
    return [b11 + b22, b11, b12 - b22, b21 - b11, b22, b11 + b12, b21 + b22]


def _combine(m):
    return [[m[0] + m[3] - m[4] + m[6], m[2] + m[4]], [m[1] + m[3], m[0] - m[1] + m[2] + m[5]]]


def _two_level(sums, blk):
    x = [[sums(blk[0][a2][0][b2], blk[0][a2][1][b2], blk[1][a2][0][b2], blk[1][a2][1][b2]) for b2 in range(2)]
         for a2 in range(2)]
    return [sums(x[0][0][i], x[0][1][i], x[1][0][i], x[1][1][i]) for i in range(7)]


def _pack(x):
    return pltpu.bitcast(x.astype(jnp.bfloat16), jnp.uint32)


def _unpack(u):
    return pltpu.bitcast(u, jnp.bfloat16)


def _kernel(wr_hbm, c_hbm, x_hbm, k_hbm, v_hbm, wq_hbm, wo_hbm, wmod_hbm,
            wg_hbm, wu_hbm, wd_hbm, out_hbm,
            wr_s, c_s, x_s, k_s, v_s, wq_s, wo_s, wmod_s, wd_s, out_s,
            wqc_s, woc_s, hs_s, os_s,
            sc_s, mraw_s, mod_s, h_s, q_s, o_s, acc_s, stat_s, best_r, best_i, zero_s, sems, osems,
            *, S, D, HKV, SK, W, F):
    nt = S // TQ
    rep = HQ // HKV
    NB = D // 128
    HP = HQ // 2
    HT = TQ // 2
    KH = D // 2
    KP = 512
    CPV = D // MC
    NMC = 6 * CPV
    NA = (HQ - P0) // G0
    NO = HQ * DH // D
    f32 = jnp.float32
    bf16 = jnp.bfloat16
    qscale = (DH ** -0.5) * LOG2E
    assert KH == KP

    def al(v, n):
        return v if isinstance(v, int) else pl.multiple_of(v, n)

    S_C, S_WR, S_WG, S_WU, S_WD, S_M = 0, 1, 2, 3, 4, 5
    S_WQ = S_M + NMC
    S_K = S_WQ + HQ
    S_V = S_K + HKV
    S_WO = S_V + HKV
    S_X = S_WO + NO

    def cp_c():
        return pltpu.make_async_copy(c_hbm, c_s, sems.at[S_C])

    def cp_wr():
        return pltpu.make_async_copy(wr_hbm, wr_s, sems.at[S_WR])

    def cp_mod(j):
        return pltpu.make_async_copy(wmod_hbm.at[:, pl.ds(al(j * MC, MC), MC)], wmod_s.at[j], sems.at[S_M + j])

    def cp_wg():
        return pltpu.make_async_copy(wg_hbm, wq_s.at[:, pl.ds(0, F)], sems.at[S_WG])

    def cp_wu(u):
        return pltpu.make_async_copy(wu_hbm.at[:, pl.ds(u * MC, MC)], wmod_s.at[u], sems.at[S_M + u])

    def cp_wd():
        return pltpu.make_async_copy(wd_hbm, wd_s.at[:, pl.ds(0, D)], sems.at[S_WD])

    def cp_wq(h, n=1):
        sl = pl.ds(al(h * DH, DH), n * DH)
        return pltpu.make_async_copy(wq_hbm.at[:, sl], wq_s.at[:, sl], sems.at[S_WQ + h])

    def cp_k(g):
        return pltpu.make_async_copy(k_hbm.at[0, g, pl.ds(SK - W, W), :], k_s.at[g], sems.at[S_K + g])

    def cp_v(g):
        return pltpu.make_async_copy(v_hbm.at[0, g, pl.ds(SK - W, W), :], v_s.at[g], sems.at[S_V + g])

    def cp_wo(j):
        sl = pl.ds(al(j * D, D), D)
        return pltpu.make_async_copy(wo_hbm.at[sl, :], wo_s.at[sl, pl.ds(0, D)], sems.at[S_WO + j])

    def rsl(t, r0=0, n=TQ):
        return pl.ds(al(t * TQ + r0, n), n)

    def cp_x(t):
        return pltpu.make_async_copy(x_hbm.at[rsl(t), :], x_s.at[rsl(t), :], sems.at[S_X + t])

    def cp_out(t):
        return pltpu.make_async_copy(out_s.at[rsl(t), :], out_hbm.at[rsl(t), :], osems.at[t])

    def sched():
        zero = zero_s[0]
        z16 = pl.multiple_of(zero, 16)
        zvec = jnp.full((8, 128), zero, jnp.int32).astype(jnp.uint32)

        def fence(deps):
            d = None
            for ref, base in deps:
                n = 16 if ref.dtype == bf16 else 8
                v = pltpu.bitcast(ref[pl.ds(pl.multiple_of(base + z16, n), n), 0:128], jnp.uint32)
                d = v if d is None else d | v
            return d & zvec

        def release(acc, r0=0):
            return pltpu.bitcast(pltpu.bitcast(acc[r0:r0 + 8, :], jnp.uint32) & zvec, f32)

        return fence, release

    def pin(a, at):
        if not at:
            return a
        parts = []
        prev = 0
        for rb in sorted(at):
            r0 = rb * 8
            if r0 > prev:
                parts.append(a[prev:r0, :])
            if a.dtype == f32:
                blk = a[r0:r0 + 8, 0:128] + pltpu.bitcast(at[rb], f32)
            else:
                blk = a[r0:r0 + 8, 0:128] | at[rb]
            if a.shape[1] > 128:
                blk = jnp.concatenate([blk, a[r0:r0 + 8, 128:]], axis=1)
            parts.append(blk)
            prev = r0 + 8
        if prev < a.shape[0]:
            parts.append(a[prev:, :])
        return jnp.concatenate(parts, axis=0)

    def mvec(j):
        return mod_s[:, j * D:(j + 1) * D][None]

    def mraw(j):
        return jnp.concatenate([mraw_s[j * CPV + u] for u in range(CPV)], axis=1)

    def xrows(sl, n):
        return x_s[sl, :].astype(f32).reshape(n // 8, 8, D)

    def ln1(t, r0, rel=None):
        hh = []
        for half in range(2):
            xn = _ln(xrows(rsl(t, half * HT + r0, LR), LR), rel)
            hh.append((xn * mvec(1) + mvec(0)).reshape(LR, D))
        sums = _lhs_sums(hh[0][:, :KH], hh[0][:, KH:], hh[1][:, :KH], hh[1][:, KH:])
        for i in range(7):
            hs_s[i, pl.ds(al(r0, LR), LR), :] = sums[i].astype(bf16)

    def w_unit(src, rt, rb, c0, dst, d0, rel):
        tf = src[rt:rt + UR, c0:c0 + 256].astype(f32)
        bt = src[rb:rb + UR, c0:c0 + 256].astype(f32)
        b11, b12, b21, b22 = tf[:, :128], tf[:, 128:], bt[:, :128], bt[:, 128:]
        if rel is not None:
            relt = jnp.tile(rel, (UR // 8, 1))
            b11, b22 = b11 + relt, b22 + relt
        sums = _rhs_sums(b11, b12, b21, b22)
        raw = {1: src[rt:rt + UR, c0:c0 + 128], 4: src[rb:rb + UR, c0 + 128:c0 + 256]}
        for i in range(7):
            dst[i, d0 // 2:(d0 + UR) // 2, :] = pltpu.bitcast(raw[i], jnp.uint32) if i in raw else _pack(sums[i])
        return (dst.at[0], d0 // 2)

    RAW = {1: 0, 4: 1}
    WIDX = {}
    for i1_ in range(7):
        for i2_ in range(7):
            if not (i1_ in RAW and i2_ in RAW):
                WIDX[i1_, i2_] = len(WIDX)

    def wo_unit(src, dst, qd, ng, r0, rel):
        w = [src[(4 * qd + c) * DH + r0:(4 * qd + c) * DH + r0 + 16, ng * 512:(ng + 1) * 512].astype(f32)
             for c in range(4)]
        blk = [[[[w[2 * k1 + k2][:, (2 * n1 + n2) * 128:(2 * n1 + n2 + 1) * 128] for n2 in range(2)]
                 for n1 in range(2)] for k2 in range(2)] for k1 in range(2)]
        if rel is not None:
            for k1 in range(2):
                for n1 in range(2):
                    relt = jnp.tile(rel[0 if k1 == n1 else 1 + k1], (2, 1))
                    for k2 in range(2):
                        for n2 in range(2):
                            blk[k1][k2][n1][n2] = blk[k1][k2][n1][n2] + relt
        ops = _two_level(_rhs_sums, blk)
        for (i1, i2), u in WIDX.items():
            dst[ng, u, qd * DH + r0:qd * DH + r0 + 16, :] = ops[i1][i2].astype(bf16)
        return (dst.at[ng, 0], qd * DH + r0)

    def wo_op(ng, i1, i2, k):
        if i1 in RAW and i2 in RAW:
            c = 2 * RAW[i1] + RAW[i2]
            return jnp.concatenate(
                [wo_s[(4 * qd + c) * DH:(4 * qd + c + 1) * DH, (4 * ng + c) * 128:(4 * ng + c + 1) * 128]
                 for qd in range(4 * k, 4 * k + 4)], axis=0)
        return jnp.concatenate([woc_s[2 * k + u, ng, WIDX[i1, i2]] for u in range(2)], axis=0)

    def resid(sl, n):
        attn = jnp.concatenate([acc_s[j, sl, :] for j in range(NB)], axis=1).reshape(n // 8, 8, D)
        return xrows(sl, n) + mvec(2) * attn

    def h2_from_stats(x1, sl, n):
        m = jnp.tile(stat_s[0, sl, :], (1, NB)).reshape(n // 8, 8, D)
        rs = jnp.tile(stat_s[1, sl, :], (1, NB)).reshape(n // 8, 8, D)
        return (x1 - m) * rs * mvec(4) + mvec(3)

    def epi_rows(t, r0, n, rel=None):
        sl = rsl(t, r0, n)
        x1 = resid(sl, n)
        m, xc, rs = _ln_stats(x1, rel)
        stat_s[0, sl, :] = jnp.broadcast_to(m.reshape(n, 1), (n, 128))
        stat_s[1, sl, :] = jnp.broadcast_to(rs.reshape(n, 1), (n, 128))
        h2 = xc * rs * mvec(4) + mvec(3)
        out_s[sl, :] = (x1 + mvec(5) * h2).reshape(n, D).astype(out_s.dtype)
        r = jnp.sum(h2 * mvec(6), axis=-1, keepdims=True)
        r = r.astype(bf16).astype(f32)
        bv = best_r[...]
        bi = best_i[...]
        sub = lax.broadcasted_iota(jnp.int32, (8, 128), 0)
        for u in range(n // 8):
            ru = jnp.broadcast_to(r[u], (8, 128))
            better = ru > bv
            bv = jnp.where(better, ru, bv)
            bi = jnp.where(better, sub + (t * TQ + r0 + u * 8), bi)
        best_r[...] = bv
        best_i[...] = bi

    def scores(q, g):
        return lax.dot_general(q.astype(bf16), k_s[g], (((1,), (1,)), ((), ())), preferred_element_type=f32)

    def softmax(s):
        m = jnp.max(s, axis=-1, keepdims=True)
        p = jnp.exp2(s - m)
        l = jnp.sum(p, axis=-1, keepdims=True)
        return p * _recip(l)

    def qk(q, g):
        return softmax(scores(q, g))

    def pv(p, g):
        return jnp.dot(p.astype(bf16), v_s[g], preferred_element_type=f32)

    def qhalf(hval, hh, kh, acc=None):
        d = jnp.dot(hval[:, kh * KH:(kh + 1) * KH], wq_s[kh * KH:(kh + 1) * KH, pl.ds(al(hh * DH, DH), DH)],
                    preferred_element_type=f32)
        return d if acc is None else d + acc

    def head0(hval, q, hh, o_prev, units, fence, release):
        g = hh // rep
        hn = hh + 1 if isinstance(hh, int) else jnp.minimum(hh + 1, HQ - 1)
        units = list(units)

        def unit(rel):
            sv, dv, pp, r0 = units.pop(0)
            return w_unit(sv, r0, KH + r0, pp * 2 * DH, dv.at[pp], r0, rel)

        if o_prev is None:
            q = pin(q, {rb: fence([unit(None)]) for rb in A0_EARLY})
        s = scores(q, g)
        p = softmax(s)
        q1 = qhalf(hval, hn, 0)
        qn = qhalf(hval, hn, 1, q1)
        vals = dict(o=o_prev, s=s, q=q1, n=qn)
        pts = [pt for pt in A0_PTS if vals[pt[0]] is not None]
        assert len(units) <= len(pts)
        last = None
        for nm, row in pts[:len(units)]:
            last = unit(release(vals[nm][:, 0:128], row))
        o = pv(pin(p, {A0_DUE: fence([last])}), g)
        o_s[hh] = _pack(o)
        return qn, o

    cp_c().start()
    cp_x(0).start()
    for j in range(2 * CPV):
        cp_mod(j).start()
    cp_wq(0).start()
    cp_k(0).start()
    cp_v(0).start()
    for h in range(1, P0 + 1):
        cp_wq(h).start()
    for j in range(NA):
        h0 = P0 + j * G0
        cp_wq(h0 + 1, G0 if j + 1 < NA else G0 - 1).start()
        if (h0 + G0 - 1) % rep < G0:
            cp_k((h0 + G0 - 1) // rep).start()
            cp_v((h0 + G0 - 1) // rep).start()
    cp_x(1).start()
    cp_wo(0).start()
    for j in range(1, NO):
        cp_wo(j).start()
        for u in range(CPV):
            cp_mod((j + 1) * CPV + u).start()
    cp_wr().start()
    for u in range(CPV):
        cp_mod(5 * CPV + u).start()
    for t in range(2, nt):
        cp_x(t).start()
    cp_wd().start()

    zero_s[0] = 0
    for n in range(NB):
        acc_s[n, rsl(0), :] = jnp.zeros((TQ, 128), f32)
    hs_s[0] = jnp.zeros((HT, KH), bf16)
    best_r[...] = jnp.full(best_r.shape, -jnp.inf, f32)
    best_i[...] = jnp.zeros(best_i.shape, jnp.int32)
    cp_c().wait()
    cp_x(0).wait()
    cf = c_s[...].astype(f32)
    sc_s[...] = jnp.broadcast_to(cf * jax.nn.sigmoid(cf), (16, D)).astype(bf16)
    xn0 = _ln(xrows(rsl(0), TQ))

    def mod_body(j, carry):
        cp_mod(j).wait()
        mraw_s[j] = jnp.dot(sc_s[...], wmod_s[j], preferred_element_type=f32)[0:8, :]
        return carry

    lax.fori_loop(0, 2 * CPV, mod_body, 0)
    mod_s[:, 0:D] = mraw(0) * qscale
    mod_s[:, D:2 * D] = (1.0 + mraw(1)) * qscale
    h_s[...] = (xn0 * mvec(1) + mvec(0)).reshape(TQ, D).astype(bf16)
    cp_wq(0).wait()
    hval0 = h_s[...]
    q = qhalf(hval0, 0, 1, qhalf(hval0, 0, 0))
    cp_k(0).wait()
    cp_v(0).wait()
    NU = KH // UR
    fence0, release0 = sched()
    assert P0 == 2
    for hh in range(P0):
        cp_wq(hh + 1).wait()
        q, _ = head0(hval0, q, hh, None, [(wq_s, wqc_s, 0, (hh * NU // P0 + u) * UR) for u in range(NU // P0)], fence0, release0)
    q_s[...] = q

    PPI = 3

    def a0_body(j, carry):
        h0 = P0 + j * G0

        @pl.when(j + 1 < NA)
        def _():
            cp_wq(h0 + 1, G0).wait()

        @pl.when(j + 1 == NA)
        def _():
            cp_wq(HQ - G0 + 1, G0 - 1).wait()

        @pl.when((h0 + G0 - 1) % rep < G0)
        def _():
            cp_k((h0 + G0 - 1) // rep).wait()
            cp_v((h0 + G0 - 1) // rep).wait()

        fence, release = sched()
        p0 = (h0 + G0 + 1) // 2 - PPI
        sv = wq_s.at[:, pl.ds(al(p0 * 2 * DH, 2 * DH), PPI * 2 * DH)]
        dv = wqc_s.at[pl.ds(p0, PPI)]
        units = [(sv, dv, pp, u * UR) for pp in range(PPI) for u in range(NU)]
        hval = h_s[...]
        q = q_s[...]
        o = None
        for u in range(G0):
            mine = units[u * len(units) // G0:(u + 1) * len(units) // G0]
            q, o = head0(hval, q, h0 + u, o, mine, fence, release)
        q_s[...] = q
        return carry

    assert (HQ - P0) % G0 == 0 and P0 + G0 - 1 < rep and (P0 + G0 - 1) % rep >= G0
    cov = {0}
    for j in range(NA):
        p0_ = (P0 + j * G0 + G0 + 1) // 2 - PPI
        assert p0_ >= 0 and p0_ + PPI <= HP
        cov |= set(range(p0_, p0_ + PPI))
    assert cov == set(range(HP))
    lax.fori_loop(0, NA, a0_body, 0)
    cp_x(1).wait()

    def o0_body(j, carry):
        cp_wo(j).wait()

        @pl.when(j > 0)
        def _():
            for u in range(CPV):
                cp_mod((j + 1) * CPV + u).wait()

        fence, release = sched()
        sc = sc_s[...]
        hq = KP // DH
        ppi = D // (2 * DH)
        wo_j = wo_s.at[pl.ds(al(j * D, D), D)]
        woc_j = woc_s.at[j]
        o_j = o_s.at[pl.ds(j * (D // DH), D // DH)]
        wm_j = wmod_s.at[pl.ds((j + 1) * CPV, CPV)]
        mr_j = mraw_s.at[pl.ds((j + 1) * CPV, CPV)]
        units = [(qd, ng, u) for qd in range(2) for ng in range(2) for u in range(DH // 16)]
        npass = NB * (D // KP)
        cnt = 0
        due = {}
        prev = None
        for n in range(NB):
            acc = acc_s[n, rsl(0), :]
            cu, cn = divmod(n, MC // 128)
            mv = None
            for kh in range(D // KP):
                lhs = jnp.concatenate([o_j[kh * hq + u] for u in range(hq)], axis=1)
                mine = units[cnt * len(units) // npass:(cnt + 1) * len(units) // npass]
                for n_, (qd, ng, u) in enumerate(mine):
                    rel = None if prev is None else [release(prev, rw) for rw in O0_ROWS[n_]]
                    last = wo_unit(wo_j, woc_j, qd, ng, u * 16, rel)
                    if prev is None:
                        due.setdefault(0, {})[8 * n_ + 7] = fence([last])
                if prev is not None and cnt + 1 < npass:
                    due.setdefault(cnt + 1, {})[2] = fence([last])
                nlc = HT // NO // LR
                if cnt % 3 == 1 and cnt // 3 < nlc:
                    ln1(1, j * (HT // NO) + (cnt // 3) * LR, release(prev, 24))
                    due.setdefault(cnt + 2, {})[6] = fence([(hs_s.at[0], j * (HT // NO))])
                acc = jnp.dot(_unpack(pin(lhs, due.pop(cnt, None))),
                              wo_j[kh * KP:(kh + 1) * KP, n * 128:(n + 1) * 128],
                              preferred_element_type=f32) + acc
                prev = acc
                cnt += 1
                d = jnp.dot(sc[:, kh * KP:(kh + 1) * KP],
                            wm_j[cu, kh * KP:(kh + 1) * KP, cn * 128:(cn + 1) * 128],
                            preferred_element_type=f32)
                mv = d if mv is None else d + mv
            acc_s[n, rsl(0), :] = acc
            mr_j[cu, :, cn * 128:(cn + 1) * 128] = mv[0:8, :]
        assert not due
        return carry

    assert NO == 4
    lax.fori_loop(0, NO, o0_body, 0)

    cp_wr().wait()
    for u in range(CPV):
        cp_mod(5 * CPV + u).wait()
    for u in range(CPV):
        mod_s[:, 5 * D + u * MC:5 * D + (u + 1) * MC] = jnp.dot(
            sc_s[...], wmod_s[5 * CPV + u], preferred_element_type=f32)[0:8, :]
    mod_s[:, 2 * D:3 * D] = mraw(2)
    mod_s[:, 3 * D:4 * D] = mraw(3)
    mod_s[:, 4 * D:5 * D] = 1.0 + mraw(4)
    mod_s[:, 6 * D:7 * D] = jnp.broadcast_to(wr_s[...].astype(f32).reshape(1, D), (8, D))
    cp_wg().start()
    for u in range(F // MC):
        cp_wu(u).start()

    def step(t, carry):
        @pl.when(t + 1 < nt)
        def _():
            cp_x(t + 1).wait()

        @pl.when(t + 1 == nt)
        def _():
            cp_wg().wait()
            for u in range(F // MC):
                cp_wu(u).wait()
            cp_wd().wait()

        fence, release = sched()
        tprev, tnext = t - 1, jnp.minimum(t + 1, nt - 1)

        hv = [hs_s[i] for i in range(7)]

        def qprod(p, i, acc=None):
            d = jnp.dot(hv[i], _unpack(wqc_s[p, i]), preferred_element_type=f32)
            return d if acc is None else d + acc

        def q_part1(p):
            return qprod(p, 0), qprod(p, 3), qprod(p, 4)

        def q_part2(p, st):
            m0, m3, m4 = st
            c11 = qprod(p, 6, m0 + m3 - m4)
            m1 = qprod(p, 1)
            m2 = qprod(p, 2)
            c22 = qprod(p, 5, m0 - m1 + m2)
            return jnp.concatenate([c11, m1 + m3], axis=0), jnp.concatenate([m2 + m4, c22], axis=0)

        order = [0, 3, 4, 6, 1, 2, 5]
        prods = [(ng, i1, i2) for ng in range(2) for i1 in order for i2 in order]
        NE = 14 + 12 + 4
        passes = [pr + (0,) for pr in prods[:NE]] + [pr + (1,) for pr in prods[:NE]]
        passes += [pr + (k,) for pr in prods[NE:] for k in range(2)]
        QT = TQ // 4
        ms = {}
        mo = {}

        def opass(s, at=None):
            ng, i1, i2, k = passes[s]
            lhs = jnp.concatenate([os_s[7 * i1 + i2, 4 * k + u] for u in range(4)], axis=1)
            w = wo_op(ng, i1, i2, k)
            if at:
                w = jnp.concatenate([_unpack(pin(pltpu.bitcast(w[0:16], jnp.uint32), at)), w[16:]], axis=0)
            d = jnp.dot(lhs, w, preferred_element_type=f32)
            res = ms[i1, i2] = d if k == 0 else d + ms[i1, i2]
            if k == 1 and i2 == order[-1]:
                mo[i1] = _combine([ms.pop((i1, i)) for i in range(7)])
                outs = {6: (0, 0), 1: (1, 0), 2: (0, 1), 5: (1, 1)}
                if i1 in outs:
                    r1, n1 = outs[i1]
                    for r2 in range(2):
                        for n2 in range(2):
                            z = [mo[i][r2][n2] if i in mo else None for i in range(7)]
                            if i1 == 6:
                                c = z[0] + z[3] - z[4] + z[6]
                            elif i1 == 1:
                                c = z[1] + z[3]
                            elif i1 == 2:
                                c = z[2] + z[4]
                            else:
                                c = z[0] - z[1] + z[2] + z[5]
                            acc_s[4 * ng + 2 * n1 + n2, rsl(t, r1 * HT + r2 * QT, QT), :] = c
                if i1 == order[-1]:
                    mo.clear()
            return res

        def side(hp, src_, rows_=SIDE_ROWS):
            rel = [release(src_, rw) for rw in rows_]
            for u in range(2):
                epi_rows(tprev, (2 * hp + u) * CHE, CHE, rel[u])
            ln1(tnext, hp * LR, rel[2])
            return fence([(out_s, tprev * TQ), (best_r, 0), (stat_s.at[0], tprev * TQ), (hs_s.at[0], 0)])

        assert 2 * HP * CHE == TQ and HP * LR == HT
        def o_slice(qd, oq, u, pts):
            rel = [jnp.tile(release(v_, rw), (2, 1)) for v_, rw in pts]
            blk = [[[[oq[k1][k2][r1 * HT + r2 * QT + 16 * u:r1 * HT + r2 * QT + 16 * u + 16]
                      + rel[0 if k1 == r1 else 1 + r1]
                      for k2 in range(2)] for k1 in range(2)] for r2 in range(2)] for r1 in range(2)]
            ops = _two_level(_lhs_sums, blk)
            for i1 in range(7):
                for i2 in range(7):
                    os_s[7 * i1 + i2, qd, 16 * u:16 * u + 16, :] = ops[i1][i2].astype(bf16)
            return fence([(os_s.at[0, qd], 16 * u)])

        st = q_part1(0)
        qa, qb = q_part2(0, st)
        qb = pin(qb, {0: side(0, st[0], (0, 48, 96))})
        fs = None
        oq = None
        nfill = 0
        for hp in range(HP):
            g = 2 * hp // rep
            pa = qk(qa if fs is None else pin(qa, {0: fs}), g)
            if oq is not None:
                qb = pin(qb, {0: o_slice(hp // 2 - 1, oq, 2 * (hp % 2), [(ob, rw) for rw in OS_A])})
            if hp + 1 < HP:
                st = q_part1(hp + 1)
                pts = [(st[2], rw) for rw in OS_B]
            else:
                rs_ = [opass(nfill + u) for u in range(6)]
                nfill += 6
                pts = [(rs_[4], 0), (rs_[4], 40), (rs_[5], 16)]
            pb = qk(qb, g)
            if oq is not None:
                pa = pin(pa, {8: o_slice(hp // 2 - 1, oq, 2 * (hp % 2) + 1, pts)})
            oa = pv(pa, g)
            fs = side(hp + 1, oa) if hp + 1 < HP else None
            if hp + 1 < HP:
                qa, qb = q_part2(hp + 1, st)
            else:
                for _ in range(8):
                    opass(nfill)
                    nfill += 1
            ob = pv(pb, g)
            if hp % 2 == 0:
                oprev = (oa, ob)
            else:
                oq = [oprev, (oa, ob)]

        pts = []
        for s in range(nfill, len(passes)):
            pts.append((opass(s), 0))
            if len(pts) % 3 == 0 and len(pts) <= 12:
                o_slice(HP // 2 - 1, oq, len(pts) // 3 - 1, pts[-3:])
        cp_out(tprev).start()
        return carry

    lax.fori_loop(1, nt, step, 0)

    epi_rows(nt - 1, 0, TQ)
    cp_out(nt - 1).start()
    bv = best_r[...]
    rbest = jnp.max(bv, axis=0, keepdims=True)
    ibest = jnp.min(jnp.where(bv == rbest, best_i[...], S), axis=0, keepdims=True)
    idx = jnp.minimum(ibest[0, 0], S - 1)
    base = pl.multiple_of((idx // 16) * 16, 16)
    bsl = pl.ds(base, 16)
    x1 = resid(bsl, 16)
    h2 = h2_from_stats(x1, bsl, 16)
    xs = h2.reshape(16, D).astype(bf16)
    gt = jnp.dot(xs, wq_s[:, 0:F], preferred_element_type=f32)
    up = jnp.concatenate([jnp.dot(xs, wmod_s[u], preferred_element_type=f32) for u in range(F // MC)], axis=1)
    a = (gt * jax.nn.sigmoid(gt) * up).astype(bf16)
    y = jnp.dot(a, wd_s[:, 0:D], preferred_element_type=f32)
    y = y * jnp.tile(jax.nn.sigmoid(rbest), (1, NB))
    rr = lax.broadcasted_iota(jnp.int32, (16, D), 0) + base
    upd = jnp.where(rr == idx, y, 0.0).reshape(2, 8, D)
    new = (x1 + mvec(5) * (h2 + upd)).reshape(16, D)
    for t in range(nt):
        cp_out(t).wait()
    out_s[bsl, :] = new.astype(out_s.dtype)
    fix = pltpu.make_async_copy(out_s.at[bsl, :], out_hbm.at[bsl, :], osems.at[0])
    fix.start()
    fix.wait()


def _compiler_params():
    kw = dict(vmem_limit_bytes=120 * 1024 * 1024)
    try:
        return pltpu.CompilerParams(disable_semaphore_checks=True, disable_bounds_checks=True, **kw)
    except TypeError:
        return pltpu.CompilerParams(**kw)


@jax.jit
def pallas_adaLN_cond__sliding_block_cached__moe_arch_mod__prompt_kernel(
    A_x: jax.Array,
    A_k_cache: jax.Array,
    A_v_cache: jax.Array,
    A_wq: jax.Array,
    A_wo: jax.Array,
    B_x: jax.Array,
    B_w_r: jax.Array,
    B_w_gate: jax.Array,
    B_w_up: jax.Array,
    B_w_down: jax.Array,
    c: jax.Array,
    w_mod: jax.Array,
):
    B, S, D = A_x.shape
    assert B == 1
    HKV, SK = A_k_cache.shape[1], A_k_cache.shape[2]
    W = min(4096, max(256, SK // 4))
    F = B_w_gate.shape[1]
    dt = A_x.dtype
    u32 = jnp.uint32
    nt = S // TQ
    NB = D // 128
    NMC = 6 * D // MC
    x2 = A_x.reshape(S, D)
    anyspec = pl.BlockSpec(memory_space=pl.ANY)
    kern = functools.partial(_kernel, S=S, D=D, HKV=HKV, SK=SK, W=W, F=F)
    out = pl.pallas_call(
        kern,
        in_specs=[anyspec] * 11,
        out_specs=anyspec,
        out_shape=jax.ShapeDtypeStruct((S, D), dt),
        scratch_shapes=[
            pltpu.VMEM((D,), dt),
            pltpu.VMEM((1, D), dt),
            pltpu.VMEM((S, D), dt),
            pltpu.VMEM((HKV, W, DH), dt),
            pltpu.VMEM((HKV, W, DH), dt),
            pltpu.VMEM((D, HQ * DH + PAD), dt),
            pltpu.VMEM((HQ * DH, D + PAD), dt),
            pltpu.VMEM((NMC, D, MC), dt),
            pltpu.VMEM((F, D + PAD), dt),
            pltpu.VMEM((S, D), dt),
            pltpu.VMEM((HQ // 2, 7, D // 4, DH), u32),
            pltpu.VMEM((HQ * DH // D, 2, 45, 2 * DH, 128), dt),
            pltpu.VMEM((7, TQ // 2, D // 2), dt),
            pltpu.VMEM((49, HQ // 4, TQ // 4, DH), dt),
            pltpu.VMEM((16, D), dt),
            pltpu.VMEM((NMC, 8, MC), jnp.float32),
            pltpu.VMEM((8, 7 * D), jnp.float32),
            pltpu.VMEM((TQ, D), dt),
            pltpu.VMEM((TQ, DH), jnp.float32),
            pltpu.VMEM((HQ, TQ // 2, DH), u32),
            pltpu.VMEM((NB, S, 128), jnp.float32),
            pltpu.VMEM((2, S, 128), jnp.float32),
            pltpu.VMEM((8, 128), jnp.float32),
            pltpu.VMEM((8, 128), jnp.int32),
            pltpu.SMEM((1,), jnp.int32),
            pltpu.SemaphoreType.DMA((5 + NMC + HQ + 2 * HKV + HQ * DH // D + nt,)),
            pltpu.SemaphoreType.DMA((nt,)),
        ],
        compiler_params=_compiler_params(),
    )(B_w_r, c, x2, A_k_cache, A_v_cache, A_wq, A_wo, w_mod, B_w_gate, B_w_up, B_w_down)
    return out.reshape(B, S, D)
```

```python
import functools

import jax
import jax.numpy as jnp
from jax import lax
import jax.experimental.pallas as pl
import jax.experimental.pallas.tpu as pltpu

HQ = 32
DH = 128
TQ = 256
PAD = 128
P0 = 2
G0 = 5
MC = 512
CHE = 8
UR = 32
SIDE_ROWS = (200, 248, 144)
OS_A = (128, 168, 208)
OS_B = (0, 40, 80)
LR = 8
A0_EARLY = (6, 12, 18)
A0_PTS = [('o', 128), ('o', 176), ('o', 224), ('s', 16), ('s', 64), ('s', 112), ('q', 128), ('q', 184), ('q', 240), ('n', 40)]
A0_DUE = 12
O0_ROWS = ((0, 48, 88), (128, 176, 216))
EPS = 1e-5
LOG2E = 1.4426950408889634


def _ln_stats(x, rel=None):
    d = x.shape[-1]
    part = x[..., 0:128]
    for j in range(1, d // 128):
        part = part + x[..., j * 128:(j + 1) * 128]
    if rel is not None:
        part = part + rel
    m = jnp.sum(part, axis=-1, keepdims=True) * (1.0 / d)
    xc = x - m
    v = jnp.mean(xc * xc, axis=-1, keepdims=True)
    return m, xc, lax.rsqrt(v + EPS)


def _ln(x, rel=None):
    _, xc, rs = _ln_stats(x, rel)
    return xc * rs


def _recip(l):
    r = pl.reciprocal(l, approx=True)
    return r * (2.0 - l * r)


def _lhs_sums(a11, a12, a21, a22):
    return [a11 + a22, a21 + a22, a11, a22, a11 + a12, a21 - a11, a12 - a22]


def _rhs_sums(b11, b12, b21, b22):
    return [b11 + b22, b11, b12 - b22, b21 - b11, b22, b11 + b12, b21 + b22]


def _combine(m):
    return [[m[0] + m[3] - m[4] + m[6], m[2] + m[4]], [m[1] + m[3], m[0] - m[1] + m[2] + m[5]]]


def _two_level(sums, blk):
    x = [[sums(blk[0][a2][0][b2], blk[0][a2][1][b2], blk[1][a2][0][b2], blk[1][a2][1][b2]) for b2 in range(2)]
         for a2 in range(2)]
    return [sums(x[0][0][i], x[0][1][i], x[1][0][i], x[1][1][i]) for i in range(7)]


def _pack(x):
    return pltpu.bitcast(x.astype(jnp.bfloat16), jnp.uint32)


def _unpack(u):
    return pltpu.bitcast(u, jnp.bfloat16)


def _kernel(wr_hbm, c_hbm, x_hbm, k_hbm, v_hbm, wq_hbm, wo_hbm, wmod_hbm,
            wg_hbm, wu_hbm, wd_hbm, out_hbm,
            wr_s, c_s, x_s, k_s, v_s, wq_s, wo_s, wmod_s, wd_s, out_s,
            wqc_s, woc_s, hs_s, os_s,
            sc_s, mraw_s, mod_s, h_s, q_s, o_s, acc_s, stat_s, best_r, best_i, zero_s, sems, osems,
            *, S, D, HKV, SK, W, F):
    nt = S // TQ
    rep = HQ // HKV
    NB = D // 128
    HP = HQ // 2
    HT = TQ // 2
    KH = D // 2
    KP = 512
    CPV = D // MC
    NMC = 6 * CPV
    NA = (HQ - P0) // G0
    NO = HQ * DH // D
    f32 = jnp.float32
    bf16 = jnp.bfloat16
    qscale = (DH ** -0.5) * LOG2E
    assert KH == KP

    def al(v, n):
        return v if isinstance(v, int) else pl.multiple_of(v, n)

    S_C, S_WR, S_WG, S_WU, S_WD, S_M = 0, 1, 2, 3, 4, 5
    S_WQ = S_M + NMC
    S_K = S_WQ + HQ
    S_V = S_K + HKV
    S_WO = S_V + HKV
    S_X = S_WO + NO

    def cp_c():
        return pltpu.make_async_copy(c_hbm, c_s, sems.at[S_C])

    def cp_wr():
        return pltpu.make_async_copy(wr_hbm, wr_s, sems.at[S_WR])

    def cp_mod(j):
        return pltpu.make_async_copy(wmod_hbm.at[:, pl.ds(al(j * MC, MC), MC)], wmod_s.at[j], sems.at[S_M + j])

    def cp_wg():
        return pltpu.make_async_copy(wg_hbm, wq_s.at[:, pl.ds(0, F)], sems.at[S_WG])

    def cp_wu(u):
        return pltpu.make_async_copy(wu_hbm.at[:, pl.ds(u * MC, MC)], wmod_s.at[u], sems.at[S_M + u])

    def cp_wd():
        return pltpu.make_async_copy(wd_hbm, wd_s.at[:, pl.ds(0, D)], sems.at[S_WD])

    def cp_wq(h, n=1):
        sl = pl.ds(al(h * DH, DH), n * DH)
        return pltpu.make_async_copy(wq_hbm.at[:, sl], wq_s.at[:, sl], sems.at[S_WQ + h])

    def cp_k(g):
        return pltpu.make_async_copy(k_hbm.at[0, g, pl.ds(SK - W, W), :], k_s.at[g], sems.at[S_K + g])

    def cp_v(g):
        return pltpu.make_async_copy(v_hbm.at[0, g, pl.ds(SK - W, W), :], v_s.at[g], sems.at[S_V + g])

    def cp_wo(j):
        sl = pl.ds(al(j * D, D), D)
        return pltpu.make_async_copy(wo_hbm.at[sl, :], wo_s.at[sl, pl.ds(0, D)], sems.at[S_WO + j])

    def rsl(t, r0=0, n=TQ):
        return pl.ds(al(t * TQ + r0, n), n)

    def cp_x(t):
        return pltpu.make_async_copy(x_hbm.at[rsl(t), :], x_s.at[rsl(t), :], sems.at[S_X + t])

    def cp_out(t):
        return pltpu.make_async_copy(out_s.at[rsl(t), :], out_hbm.at[rsl(t), :], osems.at[t])

    def sched():
        zero = zero_s[0]
        z16 = pl.multiple_of(zero, 16)
        zvec = jnp.full((8, 128), zero, jnp.int32).astype(jnp.uint32)

        def fence(deps):
            d = None
            for ref, base in deps:
                n = 16 if ref.dtype == bf16 else 8
                v = pltpu.bitcast(ref[pl.ds(pl.multiple_of(base + z16, n), n), 0:128], jnp.uint32)
                d = v if d is None else d | v
            return d & zvec

        def release(acc, r0=0):
            return pltpu.bitcast(pltpu.bitcast(acc[r0:r0 + 8, :], jnp.uint32) & zvec, f32)

        return fence, release

    def pin(a, at):
        if not at:
            return a
        parts = []
        prev = 0
        for rb in sorted(at):
            r0 = rb * 8
            if r0 > prev:
                parts.append(a[prev:r0, :])
            if a.dtype == f32:
                blk = a[r0:r0 + 8, 0:128] + pltpu.bitcast(at[rb], f32)
            else:
                blk = a[r0:r0 + 8, 0:128] | at[rb]
            if a.shape[1] > 128:
                blk = jnp.concatenate([blk, a[r0:r0 + 8, 128:]], axis=1)
            parts.append(blk)
            prev = r0 + 8
        if prev < a.shape[0]:
            parts.append(a[prev:, :])
        return jnp.concatenate(parts, axis=0)

    def mvec(j):
        return mod_s[:, j * D:(j + 1) * D][None]

    def mraw(j):
        return jnp.concatenate([mraw_s[j * CPV + u] for u in range(CPV)], axis=1)

    def xrows(sl, n):
        return x_s[sl, :].astype(f32).reshape(n // 8, 8, D)

    def ln1(t, r0, rel=None):
        hh = []
        for half in range(2):
            xn = _ln(xrows(rsl(t, half * HT + r0, LR), LR), rel)
            hh.append((xn * mvec(1) + mvec(0)).reshape(LR, D))
        sums = _lhs_sums(hh[0][:, :KH], hh[0][:, KH:], hh[1][:, :KH], hh[1][:, KH:])
        for i in range(7):
            hs_s[i, pl.ds(al(r0, LR), LR), :] = sums[i].astype(bf16)

    def w_unit(src, rt, rb, c0, dst, d0, rel):
        tf = src[rt:rt + UR, c0:c0 + 256].astype(f32)
        bt = src[rb:rb + UR, c0:c0 + 256].astype(f32)
        b11, b12, b21, b22 = tf[:, :128], tf[:, 128:], bt[:, :128], bt[:, 128:]
        if rel is not None:
            relt = jnp.tile(rel, (UR // 8, 1))
            b11, b22 = b11 + relt, b22 + relt
        sums = _rhs_sums(b11, b12, b21, b22)
        raw = {1: src[rt:rt + UR, c0:c0 + 128], 4: src[rb:rb + UR, c0 + 128:c0 + 256]}
        for i in range(7):
            dst[i, d0 // 2:(d0 + UR) // 2, :] = pltpu.bitcast(raw[i], jnp.uint32) if i in raw else _pack(sums[i])
        return (dst.at[0], d0 // 2)

    RAW = {1: 0, 4: 1}
    WIDX = {}
    for i1_ in range(7):
        for i2_ in range(7):
            if not (i1_ in RAW and i2_ in RAW):
                WIDX[i1_, i2_] = len(WIDX)

    def wo_unit(src, dst, qd, ng, r0, rel):
        w = [src[(4 * qd + c) * DH + r0:(4 * qd + c) * DH + r0 + 16, ng * 512:(ng + 1) * 512].astype(f32)
             for c in range(4)]
        blk = [[[[w[2 * k1 + k2][:, (2 * n1 + n2) * 128:(2 * n1 + n2 + 1) * 128] for n2 in range(2)]
                 for n1 in range(2)] for k2 in range(2)] for k1 in range(2)]
        if rel is not None:
            for k1 in range(2):
                for n1 in range(2):
                    relt = jnp.tile(rel[0 if k1 == n1 else 1 + k1], (2, 1))
                    for k2 in range(2):
                        for n2 in range(2):
                            blk[k1][k2][n1][n2] = blk[k1][k2][n1][n2] + relt
        ops = _two_level(_rhs_sums, blk)
        for (i1, i2), u in WIDX.items():
            dst[ng, u, qd * DH + r0:qd * DH + r0 + 16, :] = ops[i1][i2].astype(bf16)
        return (dst.at[ng, 0], qd * DH + r0)

    def wo_op(ng, i1, i2, k):
        if i1 in RAW and i2 in RAW:
            c = 2 * RAW[i1] + RAW[i2]
            return jnp.concatenate(
                [wo_s[(4 * qd + c) * DH:(4 * qd + c + 1) * DH, (4 * ng + c) * 128:(4 * ng + c + 1) * 128]
                 for qd in range(4 * k, 4 * k + 4)], axis=0)
        return jnp.concatenate([woc_s[2 * k + u, ng, WIDX[i1, i2]] for u in range(2)], axis=0)

    def resid(sl, n):
        attn = jnp.concatenate([acc_s[j, sl, :] for j in range(NB)], axis=1).reshape(n // 8, 8, D)
        return xrows(sl, n) + mvec(2) * attn

    def h2_from_stats(x1, sl, n):
        m = jnp.tile(stat_s[0, sl, :], (1, NB)).reshape(n // 8, 8, D)
        rs = jnp.tile(stat_s[1, sl, :], (1, NB)).reshape(n // 8, 8, D)
        return (x1 - m) * rs * mvec(4) + mvec(3)

    def epi_rows(t, r0, n, rel=None):
        sl = rsl(t, r0, n)
        x1 = resid(sl, n)
        m, xc, rs = _ln_stats(x1, rel)
        stat_s[0, sl, :] = jnp.broadcast_to(m.reshape(n, 1), (n, 128))
        stat_s[1, sl, :] = jnp.broadcast_to(rs.reshape(n, 1), (n, 128))
        h2 = xc * rs * mvec(4) + mvec(3)
        out_s[sl, :] = (x1 + mvec(5) * h2).reshape(n, D).astype(out_s.dtype)
        r = jnp.sum(h2 * mvec(6), axis=-1, keepdims=True)
        r = r.astype(bf16).astype(f32)
        bv = best_r[...]
        bi = best_i[...]
        sub = lax.broadcasted_iota(jnp.int32, (8, 128), 0)
        for u in range(n // 8):
            ru = jnp.broadcast_to(r[u], (8, 128))
            better = ru > bv
            bv = jnp.where(better, ru, bv)
            bi = jnp.where(better, sub + (t * TQ + r0 + u * 8), bi)
        best_r[...] = bv
        best_i[...] = bi

    def scores(q, g):
        return lax.dot_general(q.astype(bf16), k_s[g], (((1,), (1,)), ((), ())), preferred_element_type=f32)

    def softmax(s):
        m = jnp.max(s, axis=-1, keepdims=True)
        p = jnp.exp2(s - m)
        l = jnp.sum(p, axis=-1, keepdims=True)
        return p * _recip(l)

    def qk(q, g):
        return softmax(scores(q, g))

    def pv(p, g):
        return jnp.dot(p.astype(bf16), v_s[g], preferred_element_type=f32)

    def qhalf(hval, hh, kh, acc=None):
        d = jnp.dot(hval[:, kh * KH:(kh + 1) * KH], wq_s[kh * KH:(kh + 1) * KH, pl.ds(al(hh * DH, DH), DH)],
                    preferred_element_type=f32)
        return d if acc is None else d + acc

    def head0(hval, q, hh, o_prev, units, fence, release):
        g = hh // rep
        hn = hh + 1 if isinstance(hh, int) else jnp.minimum(hh + 1, HQ - 1)
        units = list(units)

        def unit(rel):
            sv, dv, pp, r0 = units.pop(0)
            return w_unit(sv, r0, KH + r0, pp * 2 * DH, dv.at[pp], r0, rel)

        if o_prev is None:
            q = pin(q, {rb: fence([unit(None)]) for rb in A0_EARLY})
        s = scores(q, g)
        p = softmax(s)
        q1 = qhalf(hval, hn, 0)
        qn = qhalf(hval, hn, 1, q1)
        vals = dict(o=o_prev, s=s, q=q1, n=qn)
        pts = [pt for pt in A0_PTS if vals[pt[0]] is not None]
        assert len(units) <= len(pts)
        last = None
        for nm, row in pts[:len(units)]:
            last = unit(release(vals[nm][:, 0:128], row))
        o = pv(pin(p, {A0_DUE: fence([last])}), g)
        o_s[hh] = _pack(o)
        return qn, o

    cp_c().start()
    cp_x(0).start()
    for j in range(2 * CPV):
        cp_mod(j).start()
    cp_wq(0).start()
    cp_k(0).start()
    cp_v(0).start()
    for h in range(1, P0 + 1):
        cp_wq(h).start()
    for j in range(NA):
        h0 = P0 + j * G0
        cp_wq(h0 + 1, G0 if j + 1 < NA else G0 - 1).start()
        if (h0 + G0 - 1) % rep < G0:
            cp_k((h0 + G0 - 1) // rep).start()
            cp_v((h0 + G0 - 1) // rep).start()
    cp_x(1).start()
    cp_wr().start()
    for j in range(NO):
        cp_wo(j).start()
        for u in range(CPV):
            cp_mod((j + 2) * CPV + u).start()
    for t in range(2, nt):
        cp_x(t).start()
    cp_wd().start()

    zero_s[0] = 0
    for n in range(NB):
        acc_s[n, rsl(0), :] = jnp.zeros((TQ, 128), f32)
    hs_s[0] = jnp.zeros((HT, KH), bf16)
    best_r[...] = jnp.full(best_r.shape, -jnp.inf, f32)
    best_i[...] = jnp.zeros(best_i.shape, jnp.int32)
    cp_c().wait()
    cp_x(0).wait()
    cf = c_s[...].astype(f32)
    sc_s[...] = jnp.broadcast_to(cf * jax.nn.sigmoid(cf), (16, D)).astype(bf16)
    xn0 = _ln(xrows(rsl(0), TQ))

    def mod_body(j, carry):
        cp_mod(j).wait()
        mraw_s[j] = jnp.dot(sc_s[...], wmod_s[j], preferred_element_type=f32)[0:8, :]
        return carry

    lax.fori_loop(0, 2 * CPV, mod_body, 0)
    mod_s[:, 0:D] = mraw(0) * qscale
    mod_s[:, D:2 * D] = (1.0 + mraw(1)) * qscale
    h_s[...] = (xn0 * mvec(1) + mvec(0)).reshape(TQ, D).astype(bf16)
    cp_wq(0).wait()
    hval0 = h_s[...]
    q = qhalf(hval0, 0, 1, qhalf(hval0, 0, 0))
    cp_k(0).wait()
    cp_v(0).wait()
    NU = KH // UR
    fence0, release0 = sched()
    assert P0 == 2
    for hh in range(P0):
        cp_wq(hh + 1).wait()
        q, _ = head0(hval0, q, hh, None, [(wq_s, wqc_s, 0, (hh * NU // P0 + u) * UR) for u in range(NU // P0)], fence0, release0)
    q_s[...] = q

    PPI = 3

    def a0_body(j, carry):
        h0 = P0 + j * G0

        @pl.when(j + 1 < NA)
        def _():
            cp_wq(h0 + 1, G0).wait()

        @pl.when(j + 1 == NA)
        def _():
            cp_wq(HQ - G0 + 1, G0 - 1).wait()

        @pl.when((h0 + G0 - 1) % rep < G0)
        def _():
            cp_k((h0 + G0 - 1) // rep).wait()
            cp_v((h0 + G0 - 1) // rep).wait()

        fence, release = sched()
        p0 = (h0 + G0 + 1) // 2 - PPI
        sv = wq_s.at[:, pl.ds(al(p0 * 2 * DH, 2 * DH), PPI * 2 * DH)]
        dv = wqc_s.at[pl.ds(p0, PPI)]
        units = [(sv, dv, pp, u * UR) for pp in range(PPI) for u in range(NU)]
        hval = h_s[...]
        q = q_s[...]
        o = None
        for u in range(G0):
            mine = units[u * len(units) // G0:(u + 1) * len(units) // G0]
            q, o = head0(hval, q, h0 + u, o, mine, fence, release)
        q_s[...] = q
        return carry

    assert (HQ - P0) % G0 == 0 and P0 + G0 - 1 < rep and (P0 + G0 - 1) % rep >= G0
    cov = {0}
    for j in range(NA):
        p0_ = (P0 + j * G0 + G0 + 1) // 2 - PPI
        assert p0_ >= 0 and p0_ + PPI <= HP
        cov |= set(range(p0_, p0_ + PPI))
    assert cov == set(range(HP))
    lax.fori_loop(0, NA, a0_body, 0)
    cp_x(1).wait()
    cp_wr().wait()

    def o0_body(j, carry):
        cp_wo(j).wait()

        for u in range(CPV):
            cp_mod((j + 2) * CPV + u).wait()

        fence, release = sched()
        sc = sc_s[...]
        hq = KP // DH
        ppi = D // (2 * DH)
        wo_j = wo_s.at[pl.ds(al(j * D, D), D)]
        woc_j = woc_s.at[j]
        o_j = o_s.at[pl.ds(j * (D // DH), D // DH)]
        wm_j = wmod_s.at[pl.ds((j + 2) * CPV, CPV)]
        mr_j = mraw_s.at[pl.ds((j + 2) * CPV, CPV)]
        units = [(qd, ng, u) for qd in range(2) for ng in range(2) for u in range(DH // 16)]
        npass = NB * (D // KP)
        cnt = 0
        due = {}
        prev = None
        for n in range(NB):
            acc = acc_s[n, rsl(0), :]
            cu, cn = divmod(n, MC // 128)
            mv = None
            for kh in range(D // KP):
                lhs = jnp.concatenate([o_j[kh * hq + u] for u in range(hq)], axis=1)
                mine = units[cnt * len(units) // npass:(cnt + 1) * len(units) // npass]
                for n_, (qd, ng, u) in enumerate(mine):
                    rel = None if prev is None else [release(prev, rw) for rw in O0_ROWS[n_]]
                    last = wo_unit(wo_j, woc_j, qd, ng, u * 16, rel)
                    if prev is None:
                        due.setdefault(0, {})[8 * n_ + 7] = fence([last])
                if prev is not None and cnt + 1 < npass:
                    due.setdefault(cnt + 1, {})[2] = fence([last])
                nlc = HT // NO // LR
                if cnt % 3 == 1 and cnt // 3 < nlc:
                    ln1(1, j * (HT // NO) + (cnt // 3) * LR, release(prev, 24))
                    due.setdefault(cnt + 2, {})[6] = fence([(hs_s.at[0], j * (HT // NO))])
                acc = jnp.dot(_unpack(pin(lhs, due.pop(cnt, None))),
                              wo_j[kh * KP:(kh + 1) * KP, n * 128:(n + 1) * 128],
                              preferred_element_type=f32) + acc
                prev = acc
                cnt += 1
                d = jnp.dot(sc[:, kh * KP:(kh + 1) * KP],
                            wm_j[cu, kh * KP:(kh + 1) * KP, cn * 128:(cn + 1) * 128],
                            preferred_element_type=f32)
                mv = d if mv is None else d + mv
            acc_s[n, rsl(0), :] = acc
            mr_j[cu, :, cn * 128:(cn + 1) * 128] = mv[0:8, :]
        assert not due
        return carry

    assert NO == 4
    lax.fori_loop(0, NO, o0_body, 0)

    mod_s[:, 2 * D:3 * D] = mraw(2)
    mod_s[:, 3 * D:4 * D] = mraw(3)
    mod_s[:, 4 * D:5 * D] = 1.0 + mraw(4)
    mod_s[:, 5 * D:6 * D] = mraw(5)
    mod_s[:, 6 * D:7 * D] = jnp.broadcast_to(wr_s[...].astype(f32).reshape(1, D), (8, D))
    cp_wg().start()
    for u in range(F // MC):
        cp_wu(u).start()

    def step(t, carry):
        @pl.when(t + 1 < nt)
        def _():
            cp_x(t + 1).wait()

        @pl.when(t + 1 == nt)
        def _():
            cp_wg().wait()
            for u in range(F // MC):
                cp_wu(u).wait()
            cp_wd().wait()

        fence, release = sched()
        tprev, tnext = t - 1, jnp.minimum(t + 1, nt - 1)

        hv = [hs_s[i] for i in range(7)]

        def qprod(p, i, acc=None):
            d = jnp.dot(hv[i], _unpack(wqc_s[p, i]), preferred_element_type=f32)
            return d if acc is None else d + acc

        def q_part1(p):
            return qprod(p, 0), qprod(p, 3), qprod(p, 4)

        def q_part2(p, st):
            m0, m3, m4 = st
            c11 = qprod(p, 6, m0 + m3 - m4)
            m1 = qprod(p, 1)
            m2 = qprod(p, 2)
            c22 = qprod(p, 5, m0 - m1 + m2)
            return jnp.concatenate([c11, m1 + m3], axis=0), jnp.concatenate([m2 + m4, c22], axis=0)

        order = [0, 3, 4, 6, 1, 2, 5]
        prods = [(ng, i1, i2) for ng in range(2) for i1 in order for i2 in order]
        NE = 14 + 12 + 4
        passes = [pr + (0,) for pr in prods[:NE]] + [pr + (1,) for pr in prods[:NE]]
        passes += [pr + (k,) for pr in prods[NE:] for k in range(2)]
        QT = TQ // 4
        ms = {}
        mo = {}

        def opass(s, at=None):
            ng, i1, i2, k = passes[s]
            lhs = jnp.concatenate([os_s[7 * i1 + i2, 4 * k + u] for u in range(4)], axis=1)
            w = wo_op(ng, i1, i2, k)
            if at:
                w = jnp.concatenate([_unpack(pin(pltpu.bitcast(w[0:16], jnp.uint32), at)), w[16:]], axis=0)
            d = jnp.dot(lhs, w, preferred_element_type=f32)
            res = ms[i1, i2] = d if k == 0 else d + ms[i1, i2]
            if k == 1 and i2 == order[-1]:
                mo[i1] = _combine([ms.pop((i1, i)) for i in range(7)])
                outs = {6: (0, 0), 1: (1, 0), 2: (0, 1), 5: (1, 1)}
                if i1 in outs:
                    r1, n1 = outs[i1]
                    for r2 in range(2):
                        for n2 in range(2):
                            z = [mo[i][r2][n2] if i in mo else None for i in range(7)]
                            if i1 == 6:
                                c = z[0] + z[3] - z[4] + z[6]
                            elif i1 == 1:
                                c = z[1] + z[3]
                            elif i1 == 2:
                                c = z[2] + z[4]
                            else:
                                c = z[0] - z[1] + z[2] + z[5]
                            acc_s[4 * ng + 2 * n1 + n2, rsl(t, r1 * HT + r2 * QT, QT), :] = c
                if i1 == order[-1]:
                    mo.clear()
            return res

        def side(hp, src_, rows_=SIDE_ROWS):
            rel = [release(src_, rw) for rw in rows_]
            for u in range(2):
                epi_rows(tprev, (2 * hp + u) * CHE, CHE, rel[u])
            ln1(tnext, hp * LR, rel[2])
            return fence([(out_s, tprev * TQ), (best_r, 0), (stat_s.at[0], tprev * TQ), (hs_s.at[0], 0)])

        assert 2 * HP * CHE == TQ and HP * LR == HT
        def o_slice(qd, oq, u, pts):
            rel = [jnp.tile(release(v_, rw), (2, 1)) for v_, rw in pts]
            blk = [[[[oq[k1][k2][r1 * HT + r2 * QT + 16 * u:r1 * HT + r2 * QT + 16 * u + 16]
                      + rel[0 if k1 == r1 else 1 + r1]
                      for k2 in range(2)] for k1 in range(2)] for r2 in range(2)] for r1 in range(2)]
            ops = _two_level(_lhs_sums, blk)
            for i1 in range(7):
                for i2 in range(7):
                    os_s[7 * i1 + i2, qd, 16 * u:16 * u + 16, :] = ops[i1][i2].astype(bf16)
            return fence([(os_s.at[0, qd], 16 * u)])

        st = q_part1(0)
        qa, qb = q_part2(0, st)
        qb = pin(qb, {0: side(0, st[0], (0, 48, 96))})
        fs = None
        oq = None
        nfill = 0
        for hp in range(HP):
            g = 2 * hp // rep
            pa = qk(qa if fs is None else pin(qa, {0: fs}), g)
            if oq is not None:
                qb = pin(qb, {0: o_slice(hp // 2 - 1, oq, 2 * (hp % 2), [(ob, rw) for rw in OS_A])})
            if hp + 1 < HP:
                st = q_part1(hp + 1)
                pts = [(st[2], rw) for rw in OS_B]
            else:
                rs_ = [opass(nfill + u) for u in range(6)]
                nfill += 6
                pts = [(rs_[4], 0), (rs_[4], 40), (rs_[5], 16)]
            pb = qk(qb, g)
            if oq is not None:
                pa = pin(pa, {8: o_slice(hp // 2 - 1, oq, 2 * (hp % 2) + 1, pts)})
            oa = pv(pa, g)
            fs = side(hp + 1, oa) if hp + 1 < HP else None
            if hp + 1 < HP:
                qa, qb = q_part2(hp + 1, st)
            else:
                for _ in range(8):
                    opass(nfill)
                    nfill += 1
            ob = pv(pb, g)
            if hp % 2 == 0:
                oprev = (oa, ob)
            else:
                oq = [oprev, (oa, ob)]

        pts = []
        for s in range(nfill, len(passes)):
            pts.append((opass(s), 0))
            if len(pts) % 3 == 0 and len(pts) <= 12:
                o_slice(HP // 2 - 1, oq, len(pts) // 3 - 1, pts[-3:])
        cp_out(tprev).start()
        return carry

    lax.fori_loop(1, nt, step, 0)

    epi_rows(nt - 1, 0, TQ)
    cp_out(nt - 1).start()
    bv = best_r[...]
    rbest = jnp.max(bv, axis=0, keepdims=True)
    ibest = jnp.min(jnp.where(bv == rbest, best_i[...], S), axis=0, keepdims=True)
    idx = jnp.minimum(ibest[0, 0], S - 1)
    base = pl.multiple_of((idx // 16) * 16, 16)
    bsl = pl.ds(base, 16)
    x1 = resid(bsl, 16)
    h2 = h2_from_stats(x1, bsl, 16)
    xs = h2.reshape(16, D).astype(bf16)
    gt = jnp.dot(xs, wq_s[:, 0:F], preferred_element_type=f32)
    up = jnp.concatenate([jnp.dot(xs, wmod_s[u], preferred_element_type=f32) for u in range(F // MC)], axis=1)
    a = (gt * jax.nn.sigmoid(gt) * up).astype(bf16)
    y = jnp.dot(a, wd_s[:, 0:D], preferred_element_type=f32)
    y = y * jnp.tile(jax.nn.sigmoid(rbest), (1, NB))
    rr = lax.broadcasted_iota(jnp.int32, (16, D), 0) + base
    upd = jnp.where(rr == idx, y, 0.0).reshape(2, 8, D)
    new = (x1 + mvec(5) * (h2 + upd)).reshape(16, D)
    for t in range(nt):
        cp_out(t).wait()
    out_s[bsl, :] = new.astype(out_s.dtype)
    fix = pltpu.make_async_copy(out_s.at[bsl, :], out_hbm.at[bsl, :], osems.at[0])
    fix.start()
    fix.wait()


def _compiler_params():
    kw = dict(vmem_limit_bytes=120 * 1024 * 1024)
    try:
        return pltpu.CompilerParams(disable_semaphore_checks=True, disable_bounds_checks=True, **kw)
    except TypeError:
        return pltpu.CompilerParams(**kw)


@jax.jit
def pallas_adaLN_cond__sliding_block_cached__moe_arch_mod__prompt_kernel(
    A_x: jax.Array,
    A_k_cache: jax.Array,
    A_v_cache: jax.Array,
    A_wq: jax.Array,
    A_wo: jax.Array,
    B_x: jax.Array,
    B_w_r: jax.Array,
    B_w_gate: jax.Array,
    B_w_up: jax.Array,
    B_w_down: jax.Array,
    c: jax.Array,
    w_mod: jax.Array,
):
    B, S, D = A_x.shape
    assert B == 1
    HKV, SK = A_k_cache.shape[1], A_k_cache.shape[2]
    W = min(4096, max(256, SK // 4))
    F = B_w_gate.shape[1]
    dt = A_x.dtype
    u32 = jnp.uint32
    nt = S // TQ
    NB = D // 128
    NMC = 6 * D // MC
    x2 = A_x.reshape(S, D)
    anyspec = pl.BlockSpec(memory_space=pl.ANY)
    kern = functools.partial(_kernel, S=S, D=D, HKV=HKV, SK=SK, W=W, F=F)
    out = pl.pallas_call(
        kern,
        in_specs=[anyspec] * 11,
        out_specs=anyspec,
        out_shape=jax.ShapeDtypeStruct((S, D), dt),
        scratch_shapes=[
            pltpu.VMEM((D,), dt),
            pltpu.VMEM((1, D), dt),
            pltpu.VMEM((S, D), dt),
            pltpu.VMEM((HKV, W, DH), dt),
            pltpu.VMEM((HKV, W, DH), dt),
            pltpu.VMEM((D, HQ * DH + PAD), dt),
            pltpu.VMEM((HQ * DH, D + PAD), dt),
            pltpu.VMEM((NMC, D, MC), dt),
            pltpu.VMEM((F, D + PAD), dt),
            pltpu.VMEM((S, D), dt),
            pltpu.VMEM((HQ // 2, 7, D // 4, DH), u32),
            pltpu.VMEM((HQ * DH // D, 2, 45, 2 * DH, 128), dt),
            pltpu.VMEM((7, TQ // 2, D // 2), dt),
            pltpu.VMEM((49, HQ // 4, TQ // 4, DH), dt),
            pltpu.VMEM((16, D), dt),
            pltpu.VMEM((NMC, 8, MC), jnp.float32),
            pltpu.VMEM((8, 7 * D), jnp.float32),
            pltpu.VMEM((TQ, D), dt),
            pltpu.VMEM((TQ, DH), jnp.float32),
            pltpu.VMEM((HQ, TQ // 2, DH), u32),
            pltpu.VMEM((NB, S, 128), jnp.float32),
            pltpu.VMEM((2, S, 128), jnp.float32),
            pltpu.VMEM((8, 128), jnp.float32),
            pltpu.VMEM((8, 128), jnp.int32),
            pltpu.SMEM((1,), jnp.int32),
            pltpu.SemaphoreType.DMA((5 + NMC + HQ + 2 * HKV + HQ * DH // D + nt,)),
            pltpu.SemaphoreType.DMA((nt,)),
        ],
        compiler_params=_compiler_params(),
    )(B_w_r, c, x2, A_k_cache, A_v_cache, A_wq, A_wo, w_mod, B_w_gate, B_w_up, B_w_down)
    return out.reshape(B, S, D)
```

```python
import functools

import jax
import jax.numpy as jnp
from jax import lax
import jax.experimental.pallas as pl
import jax.experimental.pallas.tpu as pltpu

HQ = 32
DH = 128
TQ = 256
PAD = 128
P0 = 4
G0 = 4
MC = 512
CHE = 8
SIDE_PTS = ((0, 0), (1, 0), (2, 0))
POSTNORM = True
BOTH_A = True
OS_PTS = ([('ob', 96), ('ob', 136), ('ob', 176)], [('ob', 216), ('s', 0), ('s', 48)])
A0_PTS = ([('o', r) for r in (128, 168, 208)] + [('o', 248), ('s', 24), ('s', 60 // 8 * 8)]
          + [('s', 96), ('q', 120), ('q', 160)] + [('q', 200), ('q', 240), ('n', 24)]
          + [('n', 64), ('n', 104), ('n', 144)])
A0_DUE = 14
O0_ROWS = ((0, 48, 88), (128, 176, 216))
FILL = ((7, 7), (7, 7), (7, 7), (7, 0))
EPS = 1e-5
LOG2E = 1.4426950408889634


def _ln_stats(x, rel=None):
    d = x.shape[-1]
    part = x[..., 0:128]
    for j in range(1, d // 128):
        part = part + x[..., j * 128:(j + 1) * 128]
    if rel is not None:
        part = part + rel
    m = jnp.sum(part, axis=-1, keepdims=True) * (1.0 / d)
    xc = x - m
    v = jnp.mean(xc * xc, axis=-1, keepdims=True)
    return m, xc, lax.rsqrt(v + EPS)


def _ln(x, rel=None):
    _, xc, rs = _ln_stats(x, rel)
    return xc * rs


def _recip(l):
    return pl.reciprocal(l, approx=True)


def _lhs_sums(a11, a12, a21, a22):
    return [a11 + a22, a21 + a22, a11, a22, a11 + a12, a21 - a11, a12 - a22]


def _rhs_sums(b11, b12, b21, b22):
    return [b11 + b22, b11, b12 - b22, b21 - b11, b22, b11 + b12, b21 + b22]


_ORDER = [0, 3, 4, 6, 1, 2, 5]
_COMB = {6: ((0, 0), lambda m: m[0] + m[3] - m[4] + m[6]),
         1: ((1, 0), lambda m: m[1] + m[3]),
         2: ((0, 1), lambda m: m[2] + m[4]),
         5: ((1, 1), lambda m: m[0] - m[1] + m[2] + m[5])}


def _two_level(sums, blk, rel):
    if rel is not None and len(rel) == 3:
        blk = [[[[blk[a1][a2][b1][b2] + rel[0 if a1 == b1 else 1 + a1] for b2 in range(2)] for b1 in range(2)]
                for a2 in range(2)] for a1 in range(2)]
    x = [[sums(blk[0][a2][0][b2], blk[0][a2][1][b2], blk[1][a2][0][b2], blk[1][a2][1][b2]) for b2 in range(2)]
         for a2 in range(2)]
    if rel is not None and len(rel) == 7:
        y = [sums(x[0][0][i] + rel[i], x[0][1][i], x[1][0][i], x[1][1][i] + rel[i]) for i in range(7)]
    else:
        y = [sums(x[0][0][i], x[0][1][i], x[1][0][i], x[1][1][i]) for i in range(7)]
    return [y[i1][i2].astype(jnp.bfloat16) for i1 in range(7) for i2 in range(7)]


class _Assemble:
    def __init__(self, emit):
        self.inner, self.outer, self.emit = {}, {}, emit

    def add(self, i1, i2, m):
        self.inner.setdefault(i1, {})[i2] = m
        if i2 in _COMB:
            (r2, n2), fn = _COMB[i2]
            self.outer.setdefault((r2, n2), {})[i1] = fn(self.inner[i1])
            if i1 in _COMB:
                (r1, n1), fo = _COMB[i1]
                self.emit(r1, r2, n1, n2, fo(self.outer[r2, n2]))


def _kernel(wr_hbm, c_hbm, x_hbm, k_hbm, v_hbm, wq_hbm, wo_hbm, wmod_hbm,
            wg_hbm, wu_hbm, wd_hbm, out_hbm,
            wr_s, c_s, x_s, k_s, v_s, wq_s, wo_s, wmod_s, out_s,
            wqc_s, woc_s, hf_s, hs_s, os_s,
            sc_s, mraw_s, mod_s, h_s, q_s, o_s, acc_s, stat_s, best_r, best_i, zero_s, sems, osems,
            *, S, D, HKV, SK, W, F):
    nt = S // TQ
    rep = HQ // HKV
    NB = D // 128
    HP = HQ // 2
    HT = TQ // 2
    QT = TQ // 4
    KH = D // 2
    KQ = D // 4
    KP = 512
    CPV = D // MC
    NMC = 6 * CPV
    NA = (HQ - P0) // G0
    NO = HQ * DH // D
    f32 = jnp.float32
    bf16 = jnp.bfloat16
    u32 = jnp.uint32
    qscale = (DH ** -0.5) * LOG2E
    assert KH == KP and rep == 8 and NB == 8 and NO == 4 and P0 == 4 and G0 == 4

    def al(v, n):
        return v if isinstance(v, int) else pl.multiple_of(v, n)

    S_C, S_WR, S_WG, S_WD, S_M = 0, 1, 2, 3, 4
    S_WQ = S_M + NMC
    S_K = S_WQ + HQ
    S_V = S_K + HKV
    S_WO = S_V + HKV
    S_X = S_WO + NO

    def cp_c():
        return pltpu.make_async_copy(c_hbm, c_s, sems.at[S_C])

    def cp_wr():
        return pltpu.make_async_copy(wr_hbm, wr_s, sems.at[S_WR])

    def cp_mod(j):
        return pltpu.make_async_copy(wmod_hbm.at[:, pl.ds(al(j * MC, MC), MC)], wmod_s.at[j], sems.at[S_M + j])

    def cp_wg():
        return pltpu.make_async_copy(wg_hbm, wq_s.at[:, pl.ds(0, F)], sems.at[S_WG])

    def cp_wu(u):
        return pltpu.make_async_copy(wu_hbm.at[:, pl.ds(u * MC, MC)], wmod_s.at[u], sems.at[S_M + u])

    def cp_wd():
        return pltpu.make_async_copy(wd_hbm, wo_s.at[pl.ds(0, F), pl.ds(0, D)], sems.at[S_WD])

    def cp_wq(h, n=1):
        sl = pl.ds(al(h * DH, DH), n * DH)
        return pltpu.make_async_copy(wq_hbm.at[:, sl], wq_s.at[:, sl], sems.at[S_WQ + h])

    def cp_k(g):
        return pltpu.make_async_copy(k_hbm.at[0, g, pl.ds(SK - W, W), :], k_s.at[g], sems.at[S_K + g])

    def cp_v(g):
        return pltpu.make_async_copy(v_hbm.at[0, g, pl.ds(SK - W, W), :], v_s.at[g], sems.at[S_V + g])

    def cp_wo(j):
        sl = pl.ds(al(j * D, D), D)
        return pltpu.make_async_copy(wo_hbm.at[sl, :], wo_s.at[sl, pl.ds(0, D)], sems.at[S_WO + j])

    def rsl(t, r0=0, n=TQ):
        return pl.ds(al(t * TQ + r0, n), n)

    def cp_x(t):
        return pltpu.make_async_copy(x_hbm.at[rsl(t), :], x_s.at[rsl(t), :], sems.at[S_X + t])

    def cp_out(t):
        return pltpu.make_async_copy(out_s.at[rsl(t), :], out_hbm.at[rsl(t), :], osems.at[t])

    def sched():
        zero = zero_s[0]
        z16 = pl.multiple_of(zero, 16)
        zvec = jnp.full((8, 128), zero, jnp.int32).astype(u32)

        def fence(deps):
            d = None
            for ref, base in deps:
                n = 16 if ref.dtype == bf16 else 8
                v = pltpu.bitcast(ref[pl.ds(pl.multiple_of(base + z16, n), n), 0:128], u32)
                d = v if d is None else d | v
            return d & zvec

        def release(acc, r0=0):
            return pltpu.bitcast(pltpu.bitcast(acc[r0:r0 + 8, 0:128], u32) & zvec, f32)

        return fence, release

    def pin(a, at):
        if not at:
            return a
        parts = []
        prev = 0
        for rb in sorted(at):
            r0 = rb * 8
            if r0 > prev:
                parts.append(a[prev:r0, :])
            if a.dtype == f32:
                blk = a[r0:r0 + 8, 0:128] + pltpu.bitcast(at[rb], f32)
            else:
                blk = a[r0:r0 + 8, 0:128] | at[rb]
            if a.shape[1] > 128:
                blk = jnp.concatenate([blk, a[r0:r0 + 8, 128:]], axis=1)
            parts.append(blk)
            prev = r0 + 8
        if prev < a.shape[0]:
            parts.append(a[prev:, :])
        return jnp.concatenate(parts, axis=0)

    def pin_bf16(w, d):
        if d is None:
            return w
        top = pltpu.bitcast(pltpu.bitcast(w[0:16], u32) | d, bf16)
        return jnp.concatenate([top, w[16:]], axis=0)

    def mvec(j):
        return mod_s[:, j * D:(j + 1) * D][None]

    def mraw(j):
        return jnp.concatenate([mraw_s[j * CPV + u] for u in range(CPV)], axis=1)

    def xrows(sl, n):
        return x_s[sl, :].astype(f32).reshape(n // 8, 8, D)

    def ln1(t, r0, n, rel=None):
        xn = _ln(xrows(rsl(t, r0, n), n), rel)
        hf_s[pl.ds(al(r0, n), n), :] = (xn * mvec(1) + mvec(0)).reshape(n, D)

    def h_slice(r0, rel):
        hq = [hf_s[pl.ds(al(r * QT + r0, 8), 8), :] for r in range(4)]
        blk = [[[[hq[2 * r1 + r2][:, (2 * k1 + k2) * KQ:(2 * k1 + k2 + 1) * KQ] for k2 in range(2)]
                 for k1 in range(2)] for r2 in range(2)] for r1 in range(2)]
        ops = _two_level(_lhs_sums, blk, None if rel is None else [jnp.tile(v, (1, KQ // 128)) for v in rel])
        for u in range(49):
            hs_s[u, pl.ds(al(r0, 8), 8), :] = ops[u]

    def w_unit(src, rows4, c0, dst, d0, rel):
        w = [src[pl.ds(al(r, 16), 16), c0:c0 + 512].astype(f32) for r in rows4]
        blk = [[[[w[2 * k1 + k2][:, (2 * n1 + n2) * 128:(2 * n1 + n2 + 1) * 128] for n2 in range(2)]
                 for n1 in range(2)] for k2 in range(2)] for k1 in range(2)]
        ops = _two_level(_rhs_sums, blk, None if rel is None else [jnp.tile(v, (2, 1)) for v in rel])
        for u in range(49):
            dst[u, pl.ds(al(d0, 16), 16), :] = ops[u]
        return (dst.at[0], d0)

    def resid(sl, n):
        attn = jnp.concatenate([acc_s[j, sl, :] for j in range(NB)], axis=1).reshape(n // 8, 8, D)
        return xrows(sl, n) + mvec(2) * attn

    def h2_from_stats(x1, sl, n):
        m = jnp.tile(stat_s[0, sl, :], (1, NB)).reshape(n // 8, 8, D)
        rs = jnp.tile(stat_s[1, sl, :], (1, NB)).reshape(n // 8, 8, D)
        return (x1 - m) * rs * mvec(4) + mvec(3)

    def epi_rows(t, r0, n, rel=None):
        sl = rsl(t, r0, n)
        x1 = resid(sl, n)
        m, xc, rs = _ln_stats(x1, rel)
        stat_s[0, sl, :] = jnp.broadcast_to(m.reshape(n, 1), (n, 128))
        stat_s[1, sl, :] = jnp.broadcast_to(rs.reshape(n, 1), (n, 128))
        h2 = xc * rs * mvec(4) + mvec(3)
        out_s[sl, :] = (x1 + mvec(5) * h2).reshape(n, D).astype(out_s.dtype)
        r = jnp.sum(h2 * mvec(6), axis=-1, keepdims=True)
        r = r.astype(bf16).astype(f32)
        bv = best_r[...]
        bi = best_i[...]
        sub = lax.broadcasted_iota(jnp.int32, (8, 128), 0)
        for u in range(n // 8):
            ru = jnp.broadcast_to(r[u], (8, 128))
            better = ru > bv
            bv = jnp.where(better, ru, bv)
            bi = jnp.where(better, sub + (t * TQ + r0 + u * 8), bi)
        best_r[...] = bv
        best_i[...] = bi

    def scores(q, g):
        return lax.dot_general(q.astype(bf16), k_s[g], (((1,), (1,)), ((), ())), preferred_element_type=f32)

    def softmax(s):
        m = jnp.max(s, axis=-1, keepdims=True)
        p = jnp.exp2(s - m)
        l = jnp.sum(p, axis=-1, keepdims=True)
        return p * _recip(l)

    def softmax2(s, zf):
        if not POSTNORM:
            return softmax(s), 1.0
        m = jnp.max(s, axis=-1, keepdims=True)
        p = jnp.exp2(s - m)
        part = p[:, 0:128]
        for j in range(1, W // 128):
            part = part + p[:, j * 128:(j + 1) * 128]
        p = jnp.concatenate([p[:, 0:128] + zf(part), p[:, 128:]], axis=1)
        return p, _recip(jnp.sum(part, axis=-1, keepdims=True))

    def qk(q, g):
        return softmax(scores(q, g))

    def pv(p, g):
        return jnp.dot(p.astype(bf16), v_s[g], preferred_element_type=f32)

    def qhalf(hval, hh, kh, acc=None):
        d = jnp.dot(hval[:, kh * KH:(kh + 1) * KH], wq_s[kh * KH:(kh + 1) * KH, pl.ds(al(hh * DH, DH), DH)],
                    preferred_element_type=f32)
        return d if acc is None else d + acc

    def head0(hval, q, hh, o_prev, units, fence, release):
        g = hh // rep
        hn = hh + 1 if isinstance(hh, int) else jnp.minimum(hh + 1, HQ - 1)
        units = list(units)

        def unit(rel):
            sv, dv, r0 = units.pop(0)
            return w_unit(sv, [c * KQ + r0 for c in range(4)], 0, dv, r0, rel)

        pts = list(A0_PTS)
        if o_prev is None:
            if units:
                q = pin(q, {16: fence([unit(None)])})
            pts = [('s', 0)] + pts[4:]
        s = scores(q, g)
        p = softmax(s)
        q1 = qhalf(hval, hn, 0)
        qn = qhalf(hval, hn, 1, q1)
        vals = dict(o=o_prev, s=s, q=q1, n=qn)
        assert 3 * len(units) <= len(pts)
        deps = []
        while units:
            deps.append(unit([release(vals[nm], row) for nm, row in pts[:3]]))
            pts = pts[3:]
        if deps:
            p = pin(p, {A0_DUE: fence(deps[-2:])})
        o = pv(p, g)
        o_s[hh] = pltpu.bitcast(o.astype(bf16), u32)
        return qn, o

    cp_c().start()
    cp_x(0).start()
    for j in range(2 * CPV):
        cp_mod(j).start()
    cp_wq(0).start()
    cp_k(0).start()
    cp_v(0).start()
    cp_wq(1).start()
    cp_wq(2).start()
    cp_wq(3, 2).start()
    for j in range(NA):
        h0 = P0 + j * G0
        cp_wq(h0 + 1, G0 if j + 1 < NA else G0 - 1).start()
        if h0 % rep == 0:
            cp_k(h0 // rep).start()
            cp_v(h0 // rep).start()
    cp_x(1).start()
    cp_wr().start()
    for j in range(NO):
        cp_wo(j).start()
        for u in range(CPV):
            cp_mod((j + 2) * CPV + u).start()
    for t in range(2, nt):
        cp_x(t).start()

    zero_s[0] = 0
    for n in range(NB):
        acc_s[n, rsl(0), :] = jnp.zeros((TQ, 128), f32)
    hs_s[0] = jnp.zeros((QT, KQ), bf16)
    best_r[...] = jnp.full(best_r.shape, -jnp.inf, f32)
    best_i[...] = jnp.zeros(best_i.shape, jnp.int32)
    cp_c().wait()
    cp_x(0).wait()
    cf = c_s[...].astype(f32)
    sc_s[...] = jnp.broadcast_to(cf * jax.nn.sigmoid(cf), (16, D)).astype(bf16)
    xn0 = _ln(xrows(rsl(0), TQ))

    def mod_body(j, carry):
        cp_mod(j).wait()
        mraw_s[j] = jnp.dot(sc_s[...], wmod_s[j], preferred_element_type=f32)[0:8, :]
        return carry

    lax.fori_loop(0, 2 * CPV, mod_body, 0)
    mod_s[:, 0:D] = mraw(0) * qscale
    mod_s[:, D:2 * D] = (1.0 + mraw(1)) * qscale
    h_s[...] = (xn0 * mvec(1) + mvec(0)).reshape(TQ, D).astype(bf16)
    cp_wq(0).wait()
    hval0 = h_s[...]
    q = qhalf(hval0, 0, 1, qhalf(hval0, 0, 0))
    cp_k(0).wait()
    cp_v(0).wait()
    NU = KQ // 16
    NPE = NU - NA
    fence0, release0 = sched()
    cp_wq(1).wait()
    q, _ = head0(hval0, q, 0, None, [], fence0, release0)
    cp_wq(2).wait()
    q, _ = head0(hval0, q, 1, None, [], fence0, release0)
    cp_wq(3, 2).wait()
    u0 = [(wq_s, wqc_s.at[0], u * 16) for u in range(NPE)]
    q, o = head0(hval0, q, 2, None, u0[:NPE // 2], fence0, release0)
    q, _ = head0(hval0, q, 3, o, u0[NPE // 2:], fence0, release0)
    q_s[...] = q

    def a0_body(j, carry):
        h0 = P0 + j * G0

        @pl.when(j + 1 < NA)
        def _():
            cp_wq(h0 + 1, G0).wait()

        @pl.when(j + 1 == NA)
        def _():
            cp_wq(HQ - G0 + 1, G0 - 1).wait()

        @pl.when(h0 % rep == 0)
        def _():
            cp_k(h0 // rep).wait()
            cp_v(h0 // rep).wait()

        fence, release = sched()
        sv = wq_s.at[:, pl.ds(al(h0 * DH, 4 * DH), 4 * DH)]
        dv = wqc_s.at[j + 1]
        units = [(sv, dv, u * 16) for u in range(NU)] + [(wq_s, wqc_s.at[0], (NPE + j) * 16)]
        hval = h_s[...]
        q = q_s[...]
        o = None
        for u in range(G0):
            mine = units[u * len(units) // G0:(u + 1) * len(units) // G0]
            q, o = head0(hval, q, h0 + u, o, mine, fence, release)
        q_s[...] = q
        return carry

    lax.fori_loop(0, NA, a0_body, 0)
    cp_x(1).wait()
    cp_wr().wait()

    def o0_body(j, carry):
        cp_wo(j).wait()
        for u in range(CPV):
            cp_mod((j + 2) * CPV + u).wait()

        fence, release = sched()
        sc = sc_s[...]
        hq = KP // DH
        wo_j = wo_s.at[pl.ds(al(j * D, D), D)]
        o_j = o_s.at[pl.ds(j * (D // DH), D // DH)]
        wm_j = wmod_s.at[pl.ds((j + 2) * CPV, CPV)]
        mr_j = mraw_s.at[pl.ds((j + 2) * CPV, CPV)]
        units = [(qd, ng, u) for qd in range(2) for ng in range(2) for u in range(DH // 16)]
        npass = NB * (D // KP)
        cnt = 0
        due = {}
        hist = []
        for n in range(NB):
            acc = acc_s[n, rsl(0), :]
            cu, cn = divmod(n, MC // 128)
            mv = None
            for kh in range(D // KP):
                lhs = jnp.concatenate([o_j[kh * hq + u] for u in range(hq)], axis=1)
                prev = hist[-1] if hist else None
                mine = units[cnt * len(units) // npass:(cnt + 1) * len(units) // npass]
                for n_, (qd, ng, u) in enumerate(mine):
                    rel = None if prev is None else [release(prev, rw) for rw in O0_ROWS[n_]]
                    last = w_unit(wo_j, [(4 * qd + c) * DH + u * 16 for c in range(4)], ng * 512,
                                  woc_s.at[j, ng], qd * DH + u * 16, rel)
                    if prev is None:
                        due.setdefault(0, {})[8 * n_ + 7] = fence([last])
                if prev is not None and cnt + 1 < npass:
                    due.setdefault(cnt + 1, {})[2] = fence([last])
                if cnt in (1, 3, 5, 7):
                    ln1(1, (cnt // 2) * QT + j * 16, 16, release(prev, 24))
                if cnt in (12, 15):
                    h_slice(j * 16 + (cnt // 15) * 8, [release(hv_, 104) for hv_ in hist[-3:]])
                    if cnt == 12:
                        due.setdefault(cnt + 1, {})[10] = fence([(hs_s.at[0], j * 16)])
                acc = jnp.dot(pltpu.bitcast(pin(lhs, due.pop(cnt, None)), bf16),
                              wo_j[kh * KP:(kh + 1) * KP, n * 128:(n + 1) * 128],
                              preferred_element_type=f32) + acc
                hist.append(acc)
                cnt += 1
                d = jnp.dot(sc[:, kh * KP:(kh + 1) * KP],
                            wm_j[cu, kh * KP:(kh + 1) * KP, cn * 128:(cn + 1) * 128],
                            preferred_element_type=f32)
                mv = d if mv is None else d + mv
            acc_s[n, rsl(0), :] = acc
            mr_j[cu, :, cn * 128:(cn + 1) * 128] = mv[0:8, :]
        assert not due
        return carry

    lax.fori_loop(0, NO, o0_body, 0)

    mod_s[:, 2 * D:3 * D] = mraw(2)
    mod_s[:, 3 * D:4 * D] = mraw(3)
    mod_s[:, 4 * D:5 * D] = 1.0 + mraw(4)
    mod_s[:, 5 * D:6 * D] = mraw(5)
    mod_s[:, 6 * D:7 * D] = jnp.broadcast_to(wr_s[...].astype(f32).reshape(1, D), (8, D))
    cp_wg().start()
    for u in range(F // MC):
        cp_wu(u).start()
    cp_wd().start()

    def step(t, carry):
        @pl.when(t + 1 < nt)
        def _():
            cp_x(t + 1).wait()

        @pl.when(t + 1 == nt)
        def _():
            cp_wg().wait()
            for u in range(F // MC):
                cp_wu(u).wait()
            cp_wd().wait()

        fence, release = sched()
        tprev, tnext = t - 1, jnp.minimum(t + 1, nt - 1)
        zall = jnp.full((TQ, 128), zero_s[0], jnp.int32).astype(u32)

        def zf(v_):
            return pltpu.bitcast(pltpu.bitcast(v_, u32) & zall, f32)

        prods = [(i1, i2) for i1 in _ORDER for i2 in _ORDER]
        hv = [hs_s[u] for u in range(49)]

        qblk = {}

        def q_passes(g):
            def emit(r1, r2, n1, n2, c):
                for z in range(2):
                    qblk[8 * g + 4 * z + 2 * n1 + n2, 2 * r1 + r2] = c[:, z * DH:(z + 1) * DH]
            asm = _Assemble(emit)

            def run(i1, i2):
                u = 7 * i1 + i2
                w = jnp.concatenate([wqc_s[2 * g + z, u] for z in range(2)], axis=1)
                d = jnp.dot(hv[u], w, preferred_element_type=f32)
                asm.add(i1, i2, d)
                return d
            return [functools.partial(run, i1, i2) for i1, i2 in prods]

        def q_head(hh):
            return jnp.concatenate([qblk.pop((hh, r)) for r in range(4)], axis=0)

        def o_passes():
            ms = {}
            asm = []
            for ng in range(2):
                def emit(r1, r2, n1, n2, c, ng=ng):
                    acc_s[4 * ng + 2 * n1 + n2, rsl(t, r1 * HT + r2 * QT, QT), :] = c
                asm.append(_Assemble(emit))

            def run(ng, i1, i2, k, dep=None):
                u = 7 * i1 + i2
                lhs = jnp.concatenate([os_s[u, 4 * k + v] for v in range(4)], axis=1)
                w = jnp.concatenate([woc_s[2 * k + v, ng, u] for v in range(2)], axis=0)
                d = jnp.dot(lhs, pin_bf16(w, dep), preferred_element_type=f32)
                if k == 0:
                    ms[ng, u] = d
                else:
                    d = d + ms.pop((ng, u))
                    asm[ng].add(i1, i2, d)
                return d
            NE = 16
            seq = [(0,) + pr + (0,) for pr in prods] + [(1,) + pr + (0,) for pr in prods[:NE]]
            seq += [(0,) + pr + (1,) for pr in prods] + [(1,) + pr + (1,) for pr in prods[:NE]]
            seq += [(1,) + pr + (k,) for pr in prods[NE:] for k in range(2)]
            return [functools.partial(run, *a) for a in seq]

        def side(hp, pts):
            rel = [release(v_, rw) for v_, rw in pts]
            for u in range(2):
                epi_rows(tprev, (2 * hp + u) * CHE, CHE, rel[u])
            ln1(tnext, hp * 16, 16, rel[2])
            return fence([(out_s, tprev * TQ), (best_r, 0), (stat_s.at[0], tprev * TQ), (hf_s, 0)])

        def o_slice(qd, oq, u, pts):
            blk = [[[[oq[k1][k2][r1 * HT + r2 * QT + 16 * u:r1 * HT + r2 * QT + 16 * u + 16]
                      for k2 in range(2)] for k1 in range(2)] for r2 in range(2)] for r1 in range(2)]
            ops = _two_level(_lhs_sums, blk, [jnp.tile(release(v_, rw), (2, 1)) for v_, rw in pts])
            for v in range(49):
                os_s[v, qd, 16 * u:16 * u + 16, :] = ops[v]
            return fence([(os_s.at[0, qd], 16 * u)])

        assert 2 * HP * CHE == TQ
        for fn in q_passes(0):
            fn()
        opl = o_passes()
        oq = fo = ob_ = None
        for hp in range(HP):
            g, pp = divmod(hp, 4)
            if pp == 0:
                fill = q_passes(g + 1) if g + 1 < HKV else opl
            qa, qb = q_head(2 * hp), q_head(2 * hp + 1)
            sa_ = scores(qa if fo is None else pin(qa, {0: fo}), g)
            pa, la = softmax2(sa_, zf)
            vals = {'s': sa_, 'ob': ob_}
            if oq is not None:
                fl = [o_slice(hp // 2 - 1, oq, 2 * (hp % 2) + u, [(vals[nm], rw) for nm, rw in OS_PTS[u]])
                      for u in range(2 if BOTH_A else 1)]
                qb = pin(qb, {0: functools.reduce(lambda a_, b_: a_ | b_, fl)})
            rs_ = [fill.pop(0)() for _ in range(FILL[pp][0])]
            vals.update({i_: rs_[max(len(rs_) - 6 + i_, 0)] for i_ in range(6)})
            fs = side(hp, [(vals[nm] if vals[nm] is not None else sa_, rw) for nm, rw in SIDE_PTS])
            pb, lb = softmax2(scores(qb, g), zf)
            oa_ = pv(pa, g)
            oa = oa_ * la
            rs_ = [fill.pop(0)() for _ in range(FILL[pp][1])]
            if oq is not None and not BOTH_A:
                vals = {'oa': oa_}
                vals.update(enumerate(rs_))
                fo = o_slice(hp // 2 - 1, oq, 2 * (hp % 2) + 1, [(vals[nm], rw) for nm, rw in OS_PTS[1]])
            ob_ = pv(pin(pb, {0: fs}), g)
            ob = ob_ * lb
            if hp % 2 == 0:
                oprev = (oa, ob)
            else:
                oq = [oprev, (oa, ob)]

        pts = []
        due = {} if fo is None else {2: fo}
        HS0, HSG, HSS = 30, 14, 2
        for s, fn in enumerate(opl):
            pts.append((fn(due.pop(s, None)), 0))
            if len(pts) % 3 == 0 and len(pts) <= 12:
                o_slice(HP // 2 - 1, oq, len(pts) // 3 - 1, pts[-3:])
            u, rem = divmod(s - HS0, HSG)
            if rem == 0 and 0 <= u < QT // 8:
                h_slice(u * 8, [release(pts[-1 - HSS * i_][0]) for i_ in range(7)])
                due[s + 6] = fence([(hs_s.at[0], 0)])
        assert not due
        cp_out(tprev).start()
        return carry

    lax.fori_loop(1, nt, step, 0)

    epi_rows(nt - 1, 0, TQ)
    cp_out(nt - 1).start()
    bv = best_r[...]
    rbest = jnp.max(bv, axis=0, keepdims=True)
    ibest = jnp.min(jnp.where(bv == rbest, best_i[...], S), axis=0, keepdims=True)
    idx = jnp.minimum(ibest[0, 0], S - 1)
    base = pl.multiple_of((idx // 16) * 16, 16)
    bsl = pl.ds(base, 16)
    x1 = resid(bsl, 16)
    h2 = h2_from_stats(x1, bsl, 16)
    xs = h2.reshape(16, D).astype(bf16)
    gt = jnp.dot(xs, wq_s[:, 0:F], preferred_element_type=f32)
    up = jnp.concatenate([jnp.dot(xs, wmod_s[u], preferred_element_type=f32) for u in range(F // MC)], axis=1)
    a = (gt * jax.nn.sigmoid(gt) * up).astype(bf16)
    y = jnp.dot(a, wo_s[0:F, 0:D], preferred_element_type=f32)
    y = y * jnp.tile(jax.nn.sigmoid(rbest), (1, NB))
    rr = lax.broadcasted_iota(jnp.int32, (16, D), 0) + base
    upd = jnp.where(rr == idx, y, 0.0).reshape(2, 8, D)
    new = (x1 + mvec(5) * (h2 + upd)).reshape(16, D)
    for t in range(nt):
        cp_out(t).wait()
    out_s[bsl, :] = new.astype(out_s.dtype)
    fix = pltpu.make_async_copy(out_s.at[bsl, :], out_hbm.at[bsl, :], osems.at[0])
    fix.start()
    fix.wait()


def _compiler_params():
    kw = dict(vmem_limit_bytes=124 * 1024 * 1024)
    try:
        return pltpu.CompilerParams(disable_semaphore_checks=True, disable_bounds_checks=True, **kw)
    except TypeError:
        return pltpu.CompilerParams(**kw)


@jax.jit
def pallas_adaLN_cond__sliding_block_cached__moe_arch_mod__prompt_kernel(
    A_x: jax.Array,
    A_k_cache: jax.Array,
    A_v_cache: jax.Array,
    A_wq: jax.Array,
    A_wo: jax.Array,
    B_x: jax.Array,
    B_w_r: jax.Array,
    B_w_gate: jax.Array,
    B_w_up: jax.Array,
    B_w_down: jax.Array,
    c: jax.Array,
    w_mod: jax.Array,
):
    B, S, D = A_x.shape
    assert B == 1
    HKV, SK = A_k_cache.shape[1], A_k_cache.shape[2]
    W = min(4096, max(256, SK // 4))
    F = B_w_gate.shape[1]
    dt = A_x.dtype
    f32 = jnp.float32
    nt = S // TQ
    NB = D // 128
    NMC = 6 * D // MC
    x2 = A_x.reshape(S, D)
    anyspec = pl.BlockSpec(memory_space=pl.ANY)
    kern = functools.partial(_kernel, S=S, D=D, HKV=HKV, SK=SK, W=W, F=F)
    out = pl.pallas_call(
        kern,
        in_specs=[anyspec] * 11,
        out_specs=anyspec,
        out_shape=jax.ShapeDtypeStruct((S, D), dt),
        scratch_shapes=[
            pltpu.VMEM((D,), dt),
            pltpu.VMEM((1, D), dt),
            pltpu.VMEM((S, D), dt),
            pltpu.VMEM((HKV, W, DH), dt),
            pltpu.VMEM((HKV, W, DH), dt),
            pltpu.VMEM((D, HQ * DH + PAD), dt),
            pltpu.VMEM((HQ * DH, D + PAD), dt),
            pltpu.VMEM((NMC, D, MC), dt),
            pltpu.VMEM((S, D), dt),
            pltpu.VMEM((HQ // 4, 49, D // 4, DH), dt),
            pltpu.VMEM((HQ * DH // D, 2, 49, 2 * DH, 128), dt),
            pltpu.VMEM((TQ, D), f32),
            pltpu.VMEM((49, TQ // 4, D // 4), dt),
            pltpu.VMEM((49, HQ // 4, TQ // 4, DH), dt),
            pltpu.VMEM((16, D), dt),
            pltpu.VMEM((NMC, 8, MC), f32),
            pltpu.VMEM((8, 7 * D), f32),
            pltpu.VMEM((TQ, D), dt),
            pltpu.VMEM((TQ, DH), f32),
            pltpu.VMEM((HQ, TQ // 2, DH), jnp.uint32),
            pltpu.VMEM((NB, S, 128), f32),
            pltpu.VMEM((2, S, 128), f32),
            pltpu.VMEM((8, 128), f32),
            pltpu.VMEM((8, 128), jnp.int32),
            pltpu.SMEM((1,), jnp.int32),
            pltpu.SemaphoreType.DMA((4 + NMC + HQ + 2 * HKV + HQ * DH // D + nt,)),
            pltpu.SemaphoreType.DMA((nt,)),
        ],
        compiler_params=_compiler_params(),
    )(B_w_r, c, x2, A_k_cache, A_v_cache, A_wq, A_wo, w_mod, B_w_gate, B_w_up, B_w_down)
    return out.reshape(B, S, D)
```

```python
import functools

import jax
import jax.numpy as jnp
from jax import lax
import jax.experimental.pallas as pl
import jax.experimental.pallas.tpu as pltpu

HQ = 32
DH = 128
TQ = 256
PAD = 128
P0 = 4
G0 = 4
MC = 512
CHE = 8
SIDE_PTS = ((0, 0), (1, 0), (2, 0))
POSTNORM = True
OS_F2 = [('oa', 128), ('oa', 192), (0, 0), (1, 0), (2, 0), (3, 0), (4, 0)]
OS_PTS = ([('ob', 96), ('ob', 136), ('ob', 176)], [('ob', 216), ('s', 0), ('s', 48)])
A0_PTS = ([('o', r) for r in (128, 168, 208)] + [('o', 248), ('s', 24), ('s', 60 // 8 * 8)]
          + [('s', 96), ('q', 120), ('q', 160)] + [('q', 200), ('q', 240), ('n', 24)]
          + [('n', 64), ('n', 104), ('n', 144)])
A0_DUE = 14
O0_ROWS = ((0, 48, 88), (128, 176, 216))
FILL = ((7, 7), (7, 7), (7, 7), (7, 0))
EPS = 1e-5
LOG2E = 1.4426950408889634


def _ln_stats(x, rel=None):
    d = x.shape[-1]
    part = x[..., 0:128]
    for j in range(1, d // 128):
        part = part + x[..., j * 128:(j + 1) * 128]
    if rel is not None:
        part = part + rel
    m = jnp.sum(part, axis=-1, keepdims=True) * (1.0 / d)
    xc = x - m
    v = jnp.mean(xc * xc, axis=-1, keepdims=True)
    return m, xc, lax.rsqrt(v + EPS)


def _ln(x, rel=None):
    _, xc, rs = _ln_stats(x, rel)
    return xc * rs


def _recip(l):
    return pl.reciprocal(l, approx=True)


def _lhs_sums(a11, a12, a21, a22):
    return [a11 + a22, a21 + a22, a11, a22, a11 + a12, a21 - a11, a12 - a22]


def _rhs_sums(b11, b12, b21, b22):
    return [b11 + b22, b11, b12 - b22, b21 - b11, b22, b11 + b12, b21 + b22]


_ORDER = [3, 4, 0, 6, 1, 2, 5]
_BLOCK = {6: (0, 0), 1: (1, 0), 2: (0, 1), 5: (1, 1)}


def _init(i, z):
    return {0: lambda: z[3] - z[4], 6: lambda: z[0], 1: lambda: z[3], 2: lambda: z[4],
            5: lambda: z[0] - z[1] + z[2]}.get(i, lambda: None)()


def _two_level(sums, blk, rel):
    if rel is not None and len(rel) == 3:
        blk = [[[[blk[a1][a2][b1][b2] + rel[0 if a1 == b1 else 1 + a1] for b2 in range(2)] for b1 in range(2)]
                for a2 in range(2)] for a1 in range(2)]
    x = [[sums(blk[0][a2][0][b2], blk[0][a2][1][b2], blk[1][a2][0][b2], blk[1][a2][1][b2]) for b2 in range(2)]
         for a2 in range(2)]
    if rel is not None and len(rel) == 7:
        y = [sums(x[0][0][i] + rel[i], x[0][1][i], x[1][0][i], x[1][1][i] + rel[i]) for i in range(7)]
    else:
        y = [sums(x[0][0][i], x[0][1][i], x[1][0][i], x[1][1][i]) for i in range(7)]
    return [y[i1][i2].astype(jnp.bfloat16) for i1 in range(7) for i2 in range(7)]


class _Assemble:
    def __init__(self, emit):
        self.z, self.outer, self.inj, self.emit = {}, {}, {}, emit

    def init(self, i1, i2):
        v = _init(i2, self.z)
        if i2 in _BLOCK and i1 not in (3, 4):
            self.inj[i2] = _init(i1, self.outer[i2])
            v = v + self.inj[i2]
            if i2 == 5:
                v = v + (self.inj[1] - self.inj[2])
        return v

    def add(self, i1, i2, m):
        self.z[i2] = m
        if i2 in _BLOCK:
            self.outer.setdefault(i2, {})[i1] = m
            if i1 in _BLOCK:
                (r1, n1), (r2, n2) = _BLOCK[i1], _BLOCK[i2]
                self.emit(r1, r2, n1, n2, m)


def _kernel(wr_hbm, c_hbm, x_hbm, k_hbm, v_hbm, wq_hbm, wo_hbm, wmod_hbm,
            wg_hbm, wu_hbm, wd_hbm, out_hbm,
            wr_s, c_s, x_s, k_s, v_s, wq_s, wo_s, wmod_s, out_s,
            wqc_s, woc_s, hf_s, hs_s, os_s,
            sc_s, mraw_s, mod_s, h_s, q_s, o_s, acc_s, stat_s, best_r, best_i, zero_s, sems, osems,
            *, S, D, HKV, SK, W, F):
    nt = S // TQ
    rep = HQ // HKV
    NB = D // 128
    HP = HQ // 2
    HT = TQ // 2
    QT = TQ // 4
    KH = D // 2
    KQ = D // 4
    KP = 512
    CPV = D // MC
    NMC = 6 * CPV
    NA = (HQ - P0) // G0
    NO = HQ * DH // D
    f32 = jnp.float32
    bf16 = jnp.bfloat16
    u32 = jnp.uint32
    qscale = (DH ** -0.5) * LOG2E
    assert KH == KP and rep == 8 and NB == 8 and NO == 4 and P0 == 4 and G0 == 4

    def al(v, n):
        return v if isinstance(v, int) else pl.multiple_of(v, n)

    S_C, S_WR, S_WG, S_WD, S_M = 0, 1, 2, 3, 4
    S_WQ = S_M + NMC
    S_K = S_WQ + HQ
    S_V = S_K + HKV
    S_WO = S_V + HKV
    S_X = S_WO + NO

    def cp_c():
        return pltpu.make_async_copy(c_hbm, c_s, sems.at[S_C])

    def cp_wr():
        return pltpu.make_async_copy(wr_hbm, wr_s, sems.at[S_WR])

    def cp_mod(j):
        return pltpu.make_async_copy(wmod_hbm.at[:, pl.ds(al(j * MC, MC), MC)], wmod_s.at[j], sems.at[S_M + j])

    def cp_wg():
        return pltpu.make_async_copy(wg_hbm, wq_s.at[:, pl.ds(0, F)], sems.at[S_WG])

    def cp_wu(u):
        return pltpu.make_async_copy(wu_hbm.at[:, pl.ds(u * MC, MC)], wmod_s.at[u], sems.at[S_M + u])

    def cp_wd():
        return pltpu.make_async_copy(wd_hbm, wo_s.at[pl.ds(0, F), pl.ds(0, D)], sems.at[S_WD])

    def cp_wq(h, n=1):
        sl = pl.ds(al(h * DH, DH), n * DH)
        return pltpu.make_async_copy(wq_hbm.at[:, sl], wq_s.at[:, sl], sems.at[S_WQ + h])

    def cp_k(g):
        return pltpu.make_async_copy(k_hbm.at[0, g, pl.ds(SK - W, W), :], k_s.at[g], sems.at[S_K + g])

    def cp_v(g):
        return pltpu.make_async_copy(v_hbm.at[0, g, pl.ds(SK - W, W), :], v_s.at[g], sems.at[S_V + g])

    def cp_wo(j):
        sl = pl.ds(al(j * D, D), D)
        return pltpu.make_async_copy(wo_hbm.at[sl, :], wo_s.at[sl, pl.ds(0, D)], sems.at[S_WO + j])

    def rsl(t, r0=0, n=TQ):
        return pl.ds(al(t * TQ + r0, n), n)

    def cp_x(t):
        return pltpu.make_async_copy(x_hbm.at[rsl(t), :], x_s.at[rsl(t), :], sems.at[S_X + t])

    def cp_out(t):
        return pltpu.make_async_copy(out_s.at[rsl(t), :], out_hbm.at[rsl(t), :], osems.at[t])

    def sched():
        zero = zero_s[0]
        z16 = pl.multiple_of(zero, 16)
        zvec = jnp.full((8, 128), zero, jnp.int32).astype(u32)

        def fence(deps):
            d = None
            for ref, base in deps:
                n = 16 if ref.dtype == bf16 else 8
                v = pltpu.bitcast(ref[pl.ds(pl.multiple_of(base + z16, n), n), 0:128], u32)
                d = v if d is None else d | v
            return d & zvec

        def release(acc, r0=0):
            return pltpu.bitcast(pltpu.bitcast(acc[r0:r0 + 8, 0:128], u32) & zvec, f32)

        return fence, release

    def pin(a, at):
        if not at:
            return a
        parts = []
        prev = 0
        for rb in sorted(at):
            r0 = rb * 8
            if r0 > prev:
                parts.append(a[prev:r0, :])
            if a.dtype == f32:
                blk = a[r0:r0 + 8, 0:128] + pltpu.bitcast(at[rb], f32)
            else:
                blk = a[r0:r0 + 8, 0:128] | at[rb]
            if a.shape[1] > 128:
                blk = jnp.concatenate([blk, a[r0:r0 + 8, 128:]], axis=1)
            parts.append(blk)
            prev = r0 + 8
        if prev < a.shape[0]:
            parts.append(a[prev:, :])
        return jnp.concatenate(parts, axis=0)

    def pin_bf16(w, d):
        if d is None:
            return w
        top = pltpu.bitcast(pltpu.bitcast(w[0:16], u32) | d, bf16)
        return jnp.concatenate([top, w[16:]], axis=0)

    def mvec(j):
        return mod_s[:, j * D:(j + 1) * D][None]

    def mraw(j):
        return jnp.concatenate([mraw_s[j * CPV + u] for u in range(CPV)], axis=1)

    def xrows(sl, n):
        return x_s[sl, :].astype(f32).reshape(n // 8, 8, D)

    def ln1(t, r0, n, rel=None):
        xn = _ln(xrows(rsl(t, r0, n), n), rel)
        hf_s[pl.ds(al(r0, n), n), :] = (xn * mvec(1) + mvec(0)).reshape(n, D)

    def h_slice(r0, rel):
        hq = [hf_s[pl.ds(al(r * QT + r0, 8), 8), :] for r in range(4)]
        blk = [[[[hq[2 * r1 + r2][:, (2 * k1 + k2) * KQ:(2 * k1 + k2 + 1) * KQ] for k2 in range(2)]
                 for k1 in range(2)] for r2 in range(2)] for r1 in range(2)]
        ops = _two_level(_lhs_sums, blk, None if rel is None else [jnp.tile(v, (1, KQ // 128)) for v in rel])
        for u in range(49):
            hs_s[u, pl.ds(al(r0, 8), 8), :] = ops[u]

    def w_unit(src, rows4, c0, dst, d0, rel):
        w = [src[pl.ds(al(r, 16), 16), c0:c0 + 512].astype(f32) for r in rows4]
        blk = [[[[w[2 * k1 + k2][:, (2 * n1 + n2) * 128:(2 * n1 + n2 + 1) * 128] for n2 in range(2)]
                 for n1 in range(2)] for k2 in range(2)] for k1 in range(2)]
        ops = _two_level(_rhs_sums, blk, None if rel is None else [jnp.tile(v, (2, 1)) for v in rel])
        for u in range(49):
            dst[u, pl.ds(al(d0, 16), 16), :] = ops[u]
        return (dst.at[0], d0)

    def resid(sl, n):
        attn = jnp.concatenate([acc_s[j, sl, :] for j in range(NB)], axis=1).reshape(n // 8, 8, D)
        return xrows(sl, n) + mvec(2) * attn

    def h2_from_stats(x1, sl, n):
        m = jnp.tile(stat_s[0, sl, :], (1, NB)).reshape(n // 8, 8, D)
        rs = jnp.tile(stat_s[1, sl, :], (1, NB)).reshape(n // 8, 8, D)
        return (x1 - m) * rs * mvec(4) + mvec(3)

    def epi_rows(t, r0, n, rel=None):
        sl = rsl(t, r0, n)
        x1 = resid(sl, n)
        m, xc, rs = _ln_stats(x1, rel)
        stat_s[0, sl, :] = jnp.broadcast_to(m.reshape(n, 1), (n, 128))
        stat_s[1, sl, :] = jnp.broadcast_to(rs.reshape(n, 1), (n, 128))
        h2 = xc * rs * mvec(4) + mvec(3)
        out_s[sl, :] = (x1 + mvec(5) * h2).reshape(n, D).astype(out_s.dtype)
        r = jnp.sum(h2 * mvec(6), axis=-1, keepdims=True)
        r = r.astype(bf16).astype(f32)
        bv = best_r[...]
        bi = best_i[...]
        sub = lax.broadcasted_iota(jnp.int32, (8, 128), 0)
        for u in range(n // 8):
            ru = jnp.broadcast_to(r[u], (8, 128))
            better = ru > bv
            bv = jnp.where(better, ru, bv)
            bi = jnp.where(better, sub + (t * TQ + r0 + u * 8), bi)
        best_r[...] = bv
        best_i[...] = bi

    def scores(q, g):
        return lax.dot_general(q.astype(bf16), k_s[g], (((1,), (1,)), ((), ())), preferred_element_type=f32)

    def softmax(s):
        m = jnp.max(s, axis=-1, keepdims=True)
        p = jnp.exp2(s - m)
        l = jnp.sum(p, axis=-1, keepdims=True)
        return p * _recip(l)

    def softmax2(s, zf):
        if not POSTNORM:
            return softmax(s), 1.0
        m = jnp.max(s, axis=-1, keepdims=True)
        p = jnp.exp2(s - m)
        part = p[:, 0:128]
        for j in range(1, W // 128):
            part = part + p[:, j * 128:(j + 1) * 128]
        p = jnp.concatenate([p[:, 0:128] + zf(part), p[:, 128:]], axis=1)
        return p, _recip(jnp.sum(part, axis=-1, keepdims=True))

    def qk(q, g):
        return softmax(scores(q, g))

    def pv(p, g):
        return jnp.dot(p.astype(bf16), v_s[g], preferred_element_type=f32)

    def qhalf(hval, hh, kh, acc=None):
        d = jnp.dot(hval[:, kh * KH:(kh + 1) * KH], wq_s[kh * KH:(kh + 1) * KH, pl.ds(al(hh * DH, DH), DH)],
                    preferred_element_type=f32)
        return d if acc is None else d + acc

    def head0(hval, q, hh, o_prev, units, fence, release):
        g = hh // rep
        hn = hh + 1 if isinstance(hh, int) else jnp.minimum(hh + 1, HQ - 1)
        units = list(units)

        def unit(rel):
            sv, dv, r0 = units.pop(0)
            return w_unit(sv, [c * KQ + r0 for c in range(4)], 0, dv, r0, rel)

        pts = list(A0_PTS)
        if o_prev is None:
            if units:
                q = pin(q, {16: fence([unit(None)])})
            pts = [('s', 0)] + pts[4:]
        s = scores(q, g)
        p = softmax(s)
        q1 = qhalf(hval, hn, 0)
        qn = qhalf(hval, hn, 1, q1)
        vals = dict(o=o_prev, s=s, q=q1, n=qn)
        assert 3 * len(units) <= len(pts)
        deps = []
        while units:
            deps.append(unit([release(vals[nm], row) for nm, row in pts[:3]]))
            pts = pts[3:]
        if deps:
            p = pin(p, {A0_DUE: fence(deps[-2:])})
        o = pv(p, g)
        o_s[hh] = pltpu.bitcast(o.astype(bf16), u32)
        return qn, o

    cp_c().start()
    cp_x(0).start()
    for j in range(2 * CPV):
        cp_mod(j).start()
    cp_wq(0).start()
    cp_k(0).start()
    cp_v(0).start()
    cp_wq(1).start()
    cp_wq(2).start()
    cp_wq(3, 2).start()
    for j in range(NA):
        h0 = P0 + j * G0
        cp_wq(h0 + 1, G0 if j + 1 < NA else G0 - 1).start()
        if h0 % rep == 0:
            cp_k(h0 // rep).start()
            cp_v(h0 // rep).start()
    cp_x(1).start()
    cp_wr().start()
    for j in range(NO):
        cp_wo(j).start()
        for u in range(CPV):
            cp_mod((j + 2) * CPV + u).start()
    for t in range(2, nt):
        cp_x(t).start()

    zero_s[0] = 0
    for n in range(NB):
        acc_s[n, rsl(0), :] = jnp.zeros((TQ, 128), f32)
    hs_s[0] = jnp.zeros((QT, KQ), bf16)
    best_r[...] = jnp.full(best_r.shape, -jnp.inf, f32)
    best_i[...] = jnp.zeros(best_i.shape, jnp.int32)
    cp_c().wait()
    cp_x(0).wait()
    cf = c_s[...].astype(f32)
    sc_s[...] = jnp.broadcast_to(cf * jax.nn.sigmoid(cf), (16, D)).astype(bf16)
    xn0 = _ln(xrows(rsl(0), TQ))

    def mod_body(j, carry):
        cp_mod(j).wait()
        mraw_s[j] = jnp.dot(sc_s[...], wmod_s[j], preferred_element_type=f32)[0:8, :]
        return carry

    lax.fori_loop(0, 2 * CPV, mod_body, 0)
    mod_s[:, 0:D] = mraw(0) * qscale
    mod_s[:, D:2 * D] = (1.0 + mraw(1)) * qscale
    h_s[...] = (xn0 * mvec(1) + mvec(0)).reshape(TQ, D).astype(bf16)
    cp_wq(0).wait()
    hval0 = h_s[...]
    q = qhalf(hval0, 0, 1, qhalf(hval0, 0, 0))
    cp_k(0).wait()
    cp_v(0).wait()
    NU = KQ // 16
    NPE = NU - NA
    fence0, release0 = sched()
    cp_wq(1).wait()
    q, _ = head0(hval0, q, 0, None, [], fence0, release0)
    cp_wq(2).wait()
    q, _ = head0(hval0, q, 1, None, [], fence0, release0)
    cp_wq(3, 2).wait()
    u0 = [(wq_s, wqc_s.at[0], u * 16) for u in range(NPE)]
    q, o = head0(hval0, q, 2, None, u0[:NPE // 2], fence0, release0)
    q, _ = head0(hval0, q, 3, o, u0[NPE // 2:], fence0, release0)
    q_s[...] = q

    def a0_body(j, carry):
        h0 = P0 + j * G0

        @pl.when(j + 1 < NA)
        def _():
            cp_wq(h0 + 1, G0).wait()

        @pl.when(j + 1 == NA)
        def _():
            cp_wq(HQ - G0 + 1, G0 - 1).wait()

        @pl.when(h0 % rep == 0)
        def _():
            cp_k(h0 // rep).wait()
            cp_v(h0 // rep).wait()

        fence, release = sched()
        sv = wq_s.at[:, pl.ds(al(h0 * DH, 4 * DH), 4 * DH)]
        dv = wqc_s.at[j + 1]
        units = [(sv, dv, u * 16) for u in range(NU)] + [(wq_s, wqc_s.at[0], (NPE + j) * 16)]
        hval = h_s[...]
        q = q_s[...]
        o = None
        for u in range(G0):
            mine = units[u * len(units) // G0:(u + 1) * len(units) // G0]
            q, o = head0(hval, q, h0 + u, o, mine, fence, release)
        q_s[...] = q
        return carry

    lax.fori_loop(0, NA, a0_body, 0)
    cp_x(1).wait()
    cp_wr().wait()

    def o0_body(j, carry):
        cp_wo(j).wait()
        for u in range(CPV):
            cp_mod((j + 2) * CPV + u).wait()

        fence, release = sched()
        sc = sc_s[...]
        hq = KP // DH
        wo_j = wo_s.at[pl.ds(al(j * D, D), D)]
        o_j = o_s.at[pl.ds(j * (D // DH), D // DH)]
        wm_j = wmod_s.at[pl.ds((j + 2) * CPV, CPV)]
        mr_j = mraw_s.at[pl.ds((j + 2) * CPV, CPV)]
        units = [(qd, ng, u) for qd in range(2) for ng in range(2) for u in range(DH // 16)]
        npass = NB * (D // KP)
        cnt = 0
        due = {}
        hist = []
        for n in range(NB):
            acc = acc_s[n, rsl(0), :]
            cu, cn = divmod(n, MC // 128)
            mv = None
            for kh in range(D // KP):
                lhs = jnp.concatenate([o_j[kh * hq + u] for u in range(hq)], axis=1)
                prev = hist[-1] if hist else None
                mine = units[cnt * len(units) // npass:(cnt + 1) * len(units) // npass]
                for n_, (qd, ng, u) in enumerate(mine):
                    rel = None if prev is None else [release(prev, rw) for rw in O0_ROWS[n_]]
                    last = w_unit(wo_j, [(4 * qd + c) * DH + u * 16 for c in range(4)], ng * 512,
                                  woc_s.at[j, ng], qd * DH + u * 16, rel)
                    if prev is None:
                        due.setdefault(0, {})[8 * n_ + 7] = fence([last])
                if prev is not None and cnt + 1 < npass:
                    due.setdefault(cnt + 1, {})[2] = fence([last])
                if cnt in (1, 3, 5, 7):
                    ln1(1, (cnt // 2) * QT + j * 16, 16, release(prev, 24))
                if cnt in (12, 15):
                    h_slice(j * 16 + (cnt // 15) * 8, [release(hv_, 104) for hv_ in hist[-3:]])
                    if cnt == 12:
                        due.setdefault(cnt + 1, {})[10] = fence([(hs_s.at[0], j * 16)])
                acc = jnp.dot(pltpu.bitcast(pin(lhs, due.pop(cnt, None)), bf16),
                              wo_j[kh * KP:(kh + 1) * KP, n * 128:(n + 1) * 128],
                              preferred_element_type=f32) + acc
                hist.append(acc)
                cnt += 1
                d = jnp.dot(sc[:, kh * KP:(kh + 1) * KP],
                            wm_j[cu, kh * KP:(kh + 1) * KP, cn * 128:(cn + 1) * 128],
                            preferred_element_type=f32)
                mv = d if mv is None else d + mv
            acc_s[n, rsl(0), :] = acc
            mr_j[cu, :, cn * 128:(cn + 1) * 128] = mv[0:8, :]
        assert not due
        return carry

    lax.fori_loop(0, NO, o0_body, 0)

    mod_s[:, 2 * D:3 * D] = mraw(2)
    mod_s[:, 3 * D:4 * D] = mraw(3)
    mod_s[:, 4 * D:5 * D] = 1.0 + mraw(4)
    mod_s[:, 5 * D:6 * D] = mraw(5)
    mod_s[:, 6 * D:7 * D] = jnp.broadcast_to(wr_s[...].astype(f32).reshape(1, D), (8, D))
    cp_wg().start()
    for u in range(F // MC):
        cp_wu(u).start()
    cp_wd().start()

    def step(t, carry):
        @pl.when(t + 1 < nt)
        def _():
            cp_x(t + 1).wait()

        @pl.when(t + 1 == nt)
        def _():
            cp_wg().wait()
            for u in range(F // MC):
                cp_wu(u).wait()
            cp_wd().wait()

        fence, release = sched()
        tprev, tnext = t - 1, jnp.minimum(t + 1, nt - 1)
        zall = jnp.full((TQ, 128), zero_s[0], jnp.int32).astype(u32)

        def zf(v_):
            return pltpu.bitcast(pltpu.bitcast(v_, u32) & zall, f32)

        prods = [(i1, i2) for i1 in _ORDER for i2 in _ORDER]
        hv = [hs_s[u] for u in range(49)]

        qblk = {}

        def q_passes(g):
            def emit(r1, r2, n1, n2, c):
                for z in range(2):
                    qblk[8 * g + 4 * z + 2 * n1 + n2, 2 * r1 + r2] = c[:, z * DH:(z + 1) * DH]
            asm = _Assemble(emit)

            def run(i1, i2):
                u = 7 * i1 + i2
                w = jnp.concatenate([wqc_s[2 * g + z, u] for z in range(2)], axis=1)
                d = jnp.dot(hv[u], w, preferred_element_type=f32)
                ini = asm.init(i1, i2)
                if ini is not None:
                    d = d + ini
                asm.add(i1, i2, d)
                return d
            return [functools.partial(run, i1, i2) for i1, i2 in prods]

        def q_head(hh):
            return jnp.concatenate([qblk.pop((hh, r)) for r in range(4)], axis=0)

        def o_passes():
            ms = {}
            asm = []
            for ng in range(2):
                def emit(r1, r2, n1, n2, c, ng=ng):
                    acc_s[4 * ng + 2 * n1 + n2, rsl(t, r1 * HT + r2 * QT, QT), :] = c
                asm.append(_Assemble(emit))

            def run(ng, i1, i2, k, dep=None):
                u = 7 * i1 + i2
                lhs = jnp.concatenate([os_s[u, 4 * k + v] for v in range(4)], axis=1)
                w = jnp.concatenate([woc_s[2 * k + v, ng, u] for v in range(2)], axis=0)
                d = jnp.dot(lhs, pin_bf16(w, dep), preferred_element_type=f32)
                early = ng == 0 or (i1, i2) in prods[:NE]
                if k == 1:
                    d = d + ms.pop((ng, u))
                if k == (1 if early else 0):
                    ini = asm[ng].init(i1, i2)
                    if ini is not None:
                        d = d + ini
                if k == 0:
                    ms[ng, u] = d
                else:
                    asm[ng].add(i1, i2, d)
                return d
            NE = 16
            seq = [(0,) + pr + (0,) for pr in prods] + [(1,) + pr + (0,) for pr in prods[:NE]]
            seq += [(0,) + pr + (1,) for pr in prods] + [(1,) + pr + (1,) for pr in prods[:NE]]
            seq += [(1,) + pr + (k,) for pr in prods[NE:] for k in range(2)]
            return [functools.partial(run, *a) for a in seq]

        def side(hp, pts):
            rel = [release(v_, rw) for v_, rw in pts]
            for u in range(2):
                epi_rows(tprev, (2 * hp + u) * CHE, CHE, rel[u])
            ln1(tnext, hp * 16, 16, rel[2])
            return fence([(out_s, tprev * TQ), (best_r, 0), (stat_s.at[0], tprev * TQ), (hf_s, 0)])

        def o_slice(qd, oq, u, pts):
            blk = [[[[oq[k1][k2][r1 * HT + r2 * QT + 16 * u:r1 * HT + r2 * QT + 16 * u + 16]
                      for k2 in range(2)] for k1 in range(2)] for r2 in range(2)] for r1 in range(2)]
            ops = _two_level(_lhs_sums, blk, [jnp.tile(release(v_, rw), (2, 1)) for v_, rw in pts])
            for v in range(49):
                os_s[v, qd, 16 * u:16 * u + 16, :] = ops[v]
            return fence([(os_s.at[0, qd], 16 * u)])

        assert 2 * HP * CHE == TQ
        for fn in q_passes(0):
            fn()
        opl = o_passes()
        oq = fo = ob_ = None
        for hp in range(HP):
            g, pp = divmod(hp, 4)
            if pp == 0:
                fill = q_passes(g + 1) if g + 1 < HKV else opl
            qa, qb = q_head(2 * hp), q_head(2 * hp + 1)
            sa_ = scores(qa if fo is None else pin(qa, {0: fo}), g)
            pa, la = softmax2(sa_, zf)
            vals = {'s': sa_, 'ob': ob_}
            if oq is not None:
                fl = [o_slice(hp // 2 - 1, oq, 2 * (hp % 2) + u, [(vals[nm], rw) for nm, rw in OS_PTS[u]])
                      for u in range(2 if FILL[pp][1] < 7 else 1)]
                qb = pin(qb, {0: functools.reduce(lambda a_, b_: a_ | b_, fl)})
            rs_ = [fill.pop(0)() for _ in range(FILL[pp][0])]
            vals.update({i_: rs_[max(len(rs_) - 6 + i_, 0)] for i_ in range(6)})
            fs = side(hp, [(vals[nm] if vals[nm] is not None else sa_, rw) for nm, rw in SIDE_PTS])
            pb, lb = softmax2(scores(qb, g), zf)
            oa_ = pv(pa, g)
            oa = oa_ * la
            rs_ = [fill.pop(0)() for _ in range(FILL[pp][1])]
            fo = None
            if oq is not None and FILL[pp][1] >= 7:
                vals = {'oa': oa_}
                vals.update(enumerate(rs_))
                fo = o_slice(hp // 2 - 1, oq, 2 * (hp % 2) + 1, [(vals[nm], rw) for nm, rw in OS_F2])
            ob_ = pv(pin(pb, {0: fs}), g)
            ob = ob_ * lb
            if hp % 2 == 0:
                oprev = (oa, ob)
            else:
                oq = [oprev, (oa, ob)]

        pts = []
        due = {} if fo is None else {2: fo}
        HS0, HSG, HSS = 30, 14, 2
        for s, fn in enumerate(opl):
            pts.append((fn(due.pop(s, None)), 0))
            if len(pts) % 3 == 0 and len(pts) <= 12:
                o_slice(HP // 2 - 1, oq, len(pts) // 3 - 1, pts[-3:])
            u, rem = divmod(s - HS0, HSG)
            if rem == 0 and 0 <= u < QT // 8:
                h_slice(u * 8, [release(pts[-1 - HSS * i_][0]) for i_ in range(7)])
                due[s + 6] = fence([(hs_s.at[0], 0)])
        assert not due
        cp_out(tprev).start()
        return carry

    lax.fori_loop(1, nt, step, 0)

    epi_rows(nt - 1, 0, TQ)
    cp_out(nt - 1).start()
    bv = best_r[...]
    rbest = jnp.max(bv, axis=0, keepdims=True)
    ibest = jnp.min(jnp.where(bv == rbest, best_i[...], S), axis=0, keepdims=True)
    idx = jnp.minimum(ibest[0, 0], S - 1)
    base = pl.multiple_of((idx // 16) * 16, 16)
    bsl = pl.ds(base, 16)
    x1 = resid(bsl, 16)
    h2 = h2_from_stats(x1, bsl, 16)
    xs = h2.reshape(16, D).astype(bf16)
    gt = jnp.dot(xs, wq_s[:, 0:F], preferred_element_type=f32)
    up = jnp.concatenate([jnp.dot(xs, wmod_s[u], preferred_element_type=f32) for u in range(F // MC)], axis=1)
    a = (gt * jax.nn.sigmoid(gt) * up).astype(bf16)
    y = jnp.dot(a, wo_s[0:F, 0:D], preferred_element_type=f32)
    y = y * jnp.tile(jax.nn.sigmoid(rbest), (1, NB))
    rr = lax.broadcasted_iota(jnp.int32, (16, D), 0) + base
    upd = jnp.where(rr == idx, y, 0.0).reshape(2, 8, D)
    new = (x1 + mvec(5) * (h2 + upd)).reshape(16, D)
    for t in range(nt):
        cp_out(t).wait()
    out_s[bsl, :] = new.astype(out_s.dtype)
    fix = pltpu.make_async_copy(out_s.at[bsl, :], out_hbm.at[bsl, :], osems.at[0])
    fix.start()
    fix.wait()


def _compiler_params():
    kw = dict(vmem_limit_bytes=124 * 1024 * 1024)
    try:
        return pltpu.CompilerParams(disable_semaphore_checks=True, disable_bounds_checks=True, **kw)
    except TypeError:
        return pltpu.CompilerParams(**kw)


@jax.jit
def pallas_adaLN_cond__sliding_block_cached__moe_arch_mod__prompt_kernel(
    A_x: jax.Array,
    A_k_cache: jax.Array,
    A_v_cache: jax.Array,
    A_wq: jax.Array,
    A_wo: jax.Array,
    B_x: jax.Array,
    B_w_r: jax.Array,
    B_w_gate: jax.Array,
    B_w_up: jax.Array,
    B_w_down: jax.Array,
    c: jax.Array,
    w_mod: jax.Array,
):
    B, S, D = A_x.shape
    assert B == 1
    HKV, SK = A_k_cache.shape[1], A_k_cache.shape[2]
    W = min(4096, max(256, SK // 4))
    F = B_w_gate.shape[1]
    dt = A_x.dtype
    f32 = jnp.float32
    nt = S // TQ
    NB = D // 128
    NMC = 6 * D // MC
    x2 = A_x.reshape(S, D)
    anyspec = pl.BlockSpec(memory_space=pl.ANY)
    kern = functools.partial(_kernel, S=S, D=D, HKV=HKV, SK=SK, W=W, F=F)
    out = pl.pallas_call(
        kern,
        in_specs=[anyspec] * 11,
        out_specs=anyspec,
        out_shape=jax.ShapeDtypeStruct((S, D), dt),
        scratch_shapes=[
            pltpu.VMEM((D,), dt),
            pltpu.VMEM((1, D), dt),
            pltpu.VMEM((S, D), dt),
            pltpu.VMEM((HKV, W, DH), dt),
            pltpu.VMEM((HKV, W, DH), dt),
            pltpu.VMEM((D, HQ * DH + PAD), dt),
            pltpu.VMEM((HQ * DH, D + PAD), dt),
            pltpu.VMEM((NMC, D, MC), dt),
            pltpu.VMEM((S, D), dt),
            pltpu.VMEM((HQ // 4, 49, D // 4, DH), dt),
            pltpu.VMEM((HQ * DH // D, 2, 49, 2 * DH, 128), dt),
            pltpu.VMEM((TQ, D), f32),
            pltpu.VMEM((49, TQ // 4, D // 4), dt),
            pltpu.VMEM((49, HQ // 4, TQ // 4, DH), dt),
            pltpu.VMEM((16, D), dt),
            pltpu.VMEM((NMC, 8, MC), f32),
            pltpu.VMEM((8, 7 * D), f32),
            pltpu.VMEM((TQ, D), dt),
            pltpu.VMEM((TQ, DH), f32),
            pltpu.VMEM((HQ, TQ // 2, DH), jnp.uint32),
            pltpu.VMEM((NB, S, 128), f32),
            pltpu.VMEM((2, S, 128), f32),
            pltpu.VMEM((8, 128), f32),
            pltpu.VMEM((8, 128), jnp.int32),
            pltpu.SMEM((1,), jnp.int32),
            pltpu.SemaphoreType.DMA((4 + NMC + HQ + 2 * HKV + HQ * DH // D + nt,)),
            pltpu.SemaphoreType.DMA((nt,)),
        ],
        compiler_params=_compiler_params(),
    )(B_w_r, c, x2, A_k_cache, A_v_cache, A_wq, A_wo, w_mod, B_w_gate, B_w_up, B_w_down)
    return out.reshape(B, S, D)
```

```python
import functools

import jax
import jax.numpy as jnp
from jax import lax
import jax.experimental.pallas as pl
import jax.experimental.pallas.tpu as pltpu

HQ = 32
DH = 128
TQ = 256
PAD = 128
P0 = 4
G0 = 4
MC = 512
CHE = 8
SIDE_PTS = ((1, 0), (2, 0), ('ob', 16))
POSTNORM = True
OS_F2 = [('oa', 128), ('oa', 192), (0, 0), (1, 0), (2, 0), (3, 0), (4, 0)]
OS_PTS = ([('ob', 96), ('ob', 136), ('ob', 176)], [('ob', 216), ('s', 0), ('s', 48)])
A0_PTS = ([('o', r) for r in (128, 176, 224)] + [('s', r) for r in (16, 64, 112)]
          + [('q', r) for r in (8, 56, 104, 152, 200, 248)] + [('n', r) for r in (40, 80, 120)])
A0_DUE = 14
A0_LATE = ((40, 80, 120), (152, 184, 216))
A0_CNT = (3, 4, 4, 6)
O0_ROWS = ((0, 48, 88), (128, 176, 216))
FILL = ((7, 7), (7, 7), (7, 7), (7, 0))
EPS = 1e-5
LOG2E = 1.4426950408889634


def _ln_stats(x, rel=None):
    d = x.shape[-1]
    part = x[..., 0:128]
    for j in range(1, d // 128):
        part = part + x[..., j * 128:(j + 1) * 128]
    if rel is not None:
        part = part + rel
    m = jnp.sum(part, axis=-1, keepdims=True) * (1.0 / d)
    xc = x - m
    v = jnp.mean(xc * xc, axis=-1, keepdims=True)
    return m, xc, lax.rsqrt(v + EPS)


def _ln(x, rel=None):
    _, xc, rs = _ln_stats(x, rel)
    return xc * rs


def _recip(l):
    return pl.reciprocal(l, approx=True)


def _lhs_sums(a11, a12, a21, a22):
    return [a11 + a22, a21 + a22, a11, a22, a11 + a12, a21 - a11, a12 - a22]


def _rhs_sums(b11, b12, b21, b22):
    return [b11 + b22, b11, b12 - b22, b21 - b11, b22, b11 + b12, b21 + b22]


_ORDER = [3, 4, 0, 6, 1, 2, 5]
_BLOCK = {6: (0, 0), 1: (1, 0), 2: (0, 1), 5: (1, 1)}


def _init(i, z):
    return {0: lambda: z[3] - z[4], 6: lambda: z[0], 1: lambda: z[3], 2: lambda: z[4],
            5: lambda: z[0] - z[1] + z[2]}.get(i, lambda: None)()


def _two_level(sums, blk, rel):
    if rel is not None and len(rel) == 3:
        blk = [[[[blk[a1][a2][b1][b2] + rel[0 if a1 == b1 else 1 + a1] for b2 in range(2)] for b1 in range(2)]
                for a2 in range(2)] for a1 in range(2)]
    x = [[sums(blk[0][a2][0][b2], blk[0][a2][1][b2], blk[1][a2][0][b2], blk[1][a2][1][b2]) for b2 in range(2)]
         for a2 in range(2)]
    if rel is not None and len(rel) == 7:
        y = [sums(x[0][0][i] + rel[i], x[0][1][i], x[1][0][i], x[1][1][i] + rel[i]) for i in range(7)]
    else:
        y = [sums(x[0][0][i], x[0][1][i], x[1][0][i], x[1][1][i]) for i in range(7)]
    return [y[i1][i2].astype(jnp.bfloat16) for i1 in range(7) for i2 in range(7)]


class _Assemble:
    def __init__(self, emit):
        self.z, self.outer, self.inj, self.emit = {}, {}, {}, emit

    def init(self, i1, i2):
        v = _init(i2, self.z)
        if i2 in _BLOCK and i1 not in (3, 4):
            self.inj[i2] = _init(i1, self.outer[i2])
            v = v + self.inj[i2]
            if i2 == 5:
                v = v + (self.inj[1] - self.inj[2])
        return v

    def add(self, i1, i2, m):
        self.z[i2] = m
        if i2 in _BLOCK:
            self.outer.setdefault(i2, {})[i1] = m
            if i1 in _BLOCK:
                (r1, n1), (r2, n2) = _BLOCK[i1], _BLOCK[i2]
                self.emit(r1, r2, n1, n2, m)


def _kernel(wr_hbm, c_hbm, x_hbm, k_hbm, v_hbm, wq_hbm, wo_hbm, wmod_hbm,
            wg_hbm, wu_hbm, wd_hbm, out_hbm,
            wr_s, c_s, x_s, k_s, v_s, wq_s, wo_s, wmod_s, out_s,
            wqc_s, woc_s, hf_s, hs_s, os_s,
            sc_s, mraw_s, mod_s, h_s, q_s, o_s, acc_s, stat_s, best_r, best_i, zero_s, sems, osems,
            *, S, D, HKV, SK, W, F):
    nt = S // TQ
    rep = HQ // HKV
    NB = D // 128
    HP = HQ // 2
    HT = TQ // 2
    QT = TQ // 4
    KH = D // 2
    KQ = D // 4
    KP = 512
    CPV = D // MC
    NMC = 6 * CPV
    NA = (HQ - P0) // G0
    NO = HQ * DH // D
    f32 = jnp.float32
    bf16 = jnp.bfloat16
    u32 = jnp.uint32
    qscale = (DH ** -0.5) * LOG2E
    assert KH == KP and rep == 8 and NB == 8 and NO == 4 and P0 == 4 and G0 == 4

    def al(v, n):
        return v if isinstance(v, int) else pl.multiple_of(v, n)

    S_C, S_WR, S_WG, S_WD, S_M = 0, 1, 2, 3, 4
    S_WQ = S_M + NMC
    S_K = S_WQ + HQ
    S_V = S_K + HKV
    S_WO = S_V + HKV
    S_X = S_WO + NO

    def cp_c():
        return pltpu.make_async_copy(c_hbm, c_s, sems.at[S_C])

    def cp_wr():
        return pltpu.make_async_copy(wr_hbm, wr_s, sems.at[S_WR])

    def cp_mod(j):
        return pltpu.make_async_copy(wmod_hbm.at[:, pl.ds(al(j * MC, MC), MC)], wmod_s.at[j], sems.at[S_M + j])

    def cp_wg():
        return pltpu.make_async_copy(wg_hbm, wq_s.at[:, pl.ds(0, F)], sems.at[S_WG])

    def cp_wu(u):
        return pltpu.make_async_copy(wu_hbm.at[:, pl.ds(u * MC, MC)], wmod_s.at[u], sems.at[S_M + u])

    def cp_wd():
        return pltpu.make_async_copy(wd_hbm, wo_s.at[pl.ds(0, F), pl.ds(0, D)], sems.at[S_WD])

    def cp_wq(h, n=1):
        sl = pl.ds(al(h * DH, DH), n * DH)
        return pltpu.make_async_copy(wq_hbm.at[:, sl], wq_s.at[:, sl], sems.at[S_WQ + h])

    def cp_k(g):
        return pltpu.make_async_copy(k_hbm.at[0, g, pl.ds(SK - W, W), :], k_s.at[g], sems.at[S_K + g])

    def cp_v(g):
        return pltpu.make_async_copy(v_hbm.at[0, g, pl.ds(SK - W, W), :], v_s.at[g], sems.at[S_V + g])

    def cp_wo(j):
        sl = pl.ds(al(j * D, D), D)
        return pltpu.make_async_copy(wo_hbm.at[sl, :], wo_s.at[sl, pl.ds(0, D)], sems.at[S_WO + j])

    def rsl(t, r0=0, n=TQ):
        return pl.ds(al(t * TQ + r0, n), n)

    def cp_x(t):
        return pltpu.make_async_copy(x_hbm.at[rsl(t), :], x_s.at[rsl(t), :], sems.at[S_X + t])

    def cp_out(t):
        return pltpu.make_async_copy(out_s.at[rsl(t), :], out_hbm.at[rsl(t), :], osems.at[t])

    def sched():
        zero = zero_s[0]
        z16 = pl.multiple_of(zero, 16)
        zvec = jnp.full((8, 128), zero, jnp.int32).astype(u32)

        def fence(deps):
            d = None
            for ref, base in deps:
                n = 16 if ref.dtype == bf16 else 8
                v = pltpu.bitcast(ref[pl.ds(pl.multiple_of(base + z16, n), n), 0:128], u32)
                d = v if d is None else d | v
            return d & zvec

        def release(acc, r0=0):
            return pltpu.bitcast(pltpu.bitcast(acc[r0:r0 + 8, 0:128], u32) & zvec, f32)

        def zf(v_):
            return pltpu.bitcast(pltpu.bitcast(v_, u32) & jnp.tile(zvec, (v_.shape[0] // 8, 1)), f32)

        return fence, release, zf

    def pin(a, at):
        if not at:
            return a
        parts = []
        prev = 0
        for rb in sorted(at):
            r0 = rb * 8
            if r0 > prev:
                parts.append(a[prev:r0, :])
            if a.dtype == f32:
                blk = a[r0:r0 + 8, 0:128] + pltpu.bitcast(at[rb], f32)
            else:
                blk = a[r0:r0 + 8, 0:128] | at[rb]
            if a.shape[1] > 128:
                blk = jnp.concatenate([blk, a[r0:r0 + 8, 128:]], axis=1)
            parts.append(blk)
            prev = r0 + 8
        if prev < a.shape[0]:
            parts.append(a[prev:, :])
        return jnp.concatenate(parts, axis=0)

    def pin_bf16(w, d):
        if d is None:
            return w
        top = pltpu.bitcast(pltpu.bitcast(w[0:16], u32) | d, bf16)
        return jnp.concatenate([top, w[16:]], axis=0)

    def mvec(j):
        return mod_s[:, j * D:(j + 1) * D][None]

    def mraw(j):
        return jnp.concatenate([mraw_s[j * CPV + u] for u in range(CPV)], axis=1)

    def xrows(sl, n):
        return x_s[sl, :].astype(f32).reshape(n // 8, 8, D)

    def ln1(t, r0, n, rel=None):
        xn = _ln(xrows(rsl(t, r0, n), n), rel)
        hf_s[pl.ds(al(r0, n), n), :] = (xn * mvec(1) + mvec(0)).reshape(n, D)

    def h_slice(r0, rel):
        hq = [hf_s[pl.ds(al(r * QT + r0, 8), 8), :] for r in range(4)]
        blk = [[[[hq[2 * r1 + r2][:, (2 * k1 + k2) * KQ:(2 * k1 + k2 + 1) * KQ] for k2 in range(2)]
                 for k1 in range(2)] for r2 in range(2)] for r1 in range(2)]
        ops = _two_level(_lhs_sums, blk, None if rel is None else [jnp.tile(v, (1, KQ // 128)) for v in rel])
        for u in range(49):
            hs_s[u, pl.ds(al(r0, 8), 8), :] = ops[u]

    def w_unit(src, rows4, c0, dst, d0, rel):
        w = [src[pl.ds(al(r, 16), 16), c0:c0 + 512].astype(f32) for r in rows4]
        blk = [[[[w[2 * k1 + k2][:, (2 * n1 + n2) * 128:(2 * n1 + n2 + 1) * 128] for n2 in range(2)]
                 for n1 in range(2)] for k2 in range(2)] for k1 in range(2)]
        ops = _two_level(_rhs_sums, blk, None if rel is None else [jnp.tile(v, (2, 1)) for v in rel])
        for u in range(49):
            dst[u, pl.ds(al(d0, 16), 16), :] = ops[u]
        return (dst.at[0], d0)

    def resid(sl, n):
        attn = jnp.concatenate([acc_s[j, sl, :] for j in range(NB)], axis=1).reshape(n // 8, 8, D)
        return xrows(sl, n) + mvec(2) * attn

    def h2_from_stats(x1, sl, n):
        m = jnp.tile(stat_s[0, sl, :], (1, NB)).reshape(n // 8, 8, D)
        rs = jnp.tile(stat_s[1, sl, :], (1, NB)).reshape(n // 8, 8, D)
        return (x1 - m) * rs * mvec(4) + mvec(3)

    def epi_rows(t, r0, n, rel=None):
        sl = rsl(t, r0, n)
        x1 = resid(sl, n)
        m, xc, rs = _ln_stats(x1, rel)
        stat_s[0, sl, :] = jnp.broadcast_to(m.reshape(n, 1), (n, 128))
        stat_s[1, sl, :] = jnp.broadcast_to(rs.reshape(n, 1), (n, 128))
        h2 = xc * rs * mvec(4) + mvec(3)
        out_s[sl, :] = (x1 + mvec(5) * h2).reshape(n, D).astype(out_s.dtype)
        r = jnp.sum(h2 * mvec(6), axis=-1, keepdims=True)
        r = r.astype(bf16).astype(f32)
        bv = best_r[...]
        bi = best_i[...]
        sub = lax.broadcasted_iota(jnp.int32, (8, 128), 0)
        for u in range(n // 8):
            ru = jnp.broadcast_to(r[u], (8, 128))
            better = ru > bv
            bv = jnp.where(better, ru, bv)
            bi = jnp.where(better, sub + (t * TQ + r0 + u * 8), bi)
        best_r[...] = bv
        best_i[...] = bi

    def scores(q, g):
        return lax.dot_general(q.astype(bf16), k_s[g], (((1,), (1,)), ((), ())), preferred_element_type=f32)

    def softmax(s):
        m = jnp.max(s, axis=-1, keepdims=True)
        p = jnp.exp2(s - m)
        l = jnp.sum(p, axis=-1, keepdims=True)
        return p * _recip(l)

    def softmax2(s, zf):
        if not POSTNORM:
            return softmax(s), 1.0
        m = jnp.max(s, axis=-1, keepdims=True)
        p = jnp.exp2(s - m)
        part = p[:, 0:128]
        for j in range(1, W // 128):
            part = part + p[:, j * 128:(j + 1) * 128]
        p = jnp.concatenate([p[:, 0:128] + zf(part), p[:, 128:]], axis=1)
        return p, _recip(jnp.sum(part, axis=-1, keepdims=True))

    def qk(q, g):
        return softmax(scores(q, g))

    def pv(p, g):
        return jnp.dot(p.astype(bf16), v_s[g], preferred_element_type=f32)

    def qhalf(hval, hh, kh, acc=None):
        d = jnp.dot(hval[:, kh * KH:(kh + 1) * KH], wq_s[kh * KH:(kh + 1) * KH, pl.ds(al(hh * DH, DH), DH)],
                    preferred_element_type=f32)
        return d if acc is None else d + acc

    def head0(hval, q, hh, o_prev, units, late, fence, release, zf):
        g = hh // rep
        hn = hh + 1 if isinstance(hh, int) else jnp.minimum(hh + 1, HQ - 1)
        units = list(units)

        def unit(rel):
            sv, dv, r0 = units.pop(0)
            return w_unit(sv, [c * KQ + r0 for c in range(4)], 0, dv, r0, rel)

        pts = list(A0_PTS) if o_prev is not None else list(A0_PTS[3:])
        s = scores(q, g)
        p, li = softmax2(s, zf)
        q1 = qhalf(hval, hn, 0)
        qn = qhalf(hval, hn, 1, q1)
        vals = dict(o=o_prev, s=s, q=q1, n=qn)
        deps = []
        while len(units) > late:
            deps.append(unit([release(vals[nm], row) for nm, row in pts[:3]]))
            pts = pts[3:]
        deps = deps[-2:] + ([(o_s.at[hh - 1], 0)] if o_prev is not None else [])
        if deps:
            p = pin(p, {A0_DUE: fence(deps)})
        o = pv(p, g)
        o_s[hh] = pltpu.bitcast((o * li).astype(bf16), u32)
        for u in range(late):
            unit([release(o, row) for row in A0_LATE[u]])
        return qn, o

    cp_c().start()
    cp_x(0).start()
    for j in range(2 * CPV):
        cp_mod(j).start()
    cp_wq(0).start()
    cp_k(0).start()
    cp_v(0).start()
    cp_wq(1).start()
    cp_wq(2).start()
    cp_wq(3, 2).start()
    for j in range(NA):
        h0 = P0 + j * G0
        cp_wq(h0 + 1, G0 if j + 1 < NA else G0 - 1).start()
        if h0 % rep == 0:
            cp_k(h0 // rep).start()
            cp_v(h0 // rep).start()
    cp_x(1).start()
    cp_wr().start()
    for j in range(NO):
        cp_wo(j).start()
        for u in range(CPV):
            cp_mod((j + 2) * CPV + u).start()
    for t in range(2, nt):
        cp_x(t).start()

    zero_s[0] = 0
    for n in range(NB):
        acc_s[n, rsl(0), :] = jnp.zeros((TQ, 128), f32)
    hs_s[0] = jnp.zeros((QT, KQ), bf16)
    best_r[...] = jnp.full(best_r.shape, -jnp.inf, f32)
    best_i[...] = jnp.zeros(best_i.shape, jnp.int32)
    cp_c().wait()
    cp_x(0).wait()
    cf = c_s[...].astype(f32)
    sc_s[...] = jnp.broadcast_to(cf * jax.nn.sigmoid(cf), (16, D)).astype(bf16)
    xn0 = _ln(xrows(rsl(0), TQ))

    def mod_body(j, carry):
        cp_mod(j).wait()
        mraw_s[j] = jnp.dot(sc_s[...], wmod_s[j], preferred_element_type=f32)[0:8, :]
        return carry

    lax.fori_loop(0, 2 * CPV, mod_body, 0)
    mod_s[:, 0:D] = mraw(0) * qscale
    mod_s[:, D:2 * D] = (1.0 + mraw(1)) * qscale
    h_s[...] = (xn0 * mvec(1) + mvec(0)).reshape(TQ, D).astype(bf16)
    cp_wq(0).wait()
    hval0 = h_s[...]
    q = qhalf(hval0, 0, 1, qhalf(hval0, 0, 0))
    cp_k(0).wait()
    cp_v(0).wait()
    NU = KQ // 16
    NPE = NU - NA
    sch0 = sched()
    cp_wq(1).wait()
    q, _ = head0(hval0, q, 0, None, [], 0, *sch0)
    cp_wq(2).wait()
    q, _ = head0(hval0, q, 1, None, [], 0, *sch0)
    cp_wq(3, 2).wait()
    u0 = [(wq_s, wqc_s.at[0], u * 16) for u in range(NPE)]
    q, o = head0(hval0, q, 2, None, u0[:3], 0, *sch0)
    q, _ = head0(hval0, q, 3, o, u0[3:], 2, *sch0)
    q_s[...] = q

    def a0_body(j, carry):
        h0 = P0 + j * G0

        @pl.when(j + 1 < NA)
        def _():
            cp_wq(h0 + 1, G0).wait()

        @pl.when(j + 1 == NA)
        def _():
            cp_wq(HQ - G0 + 1, G0 - 1).wait()

        @pl.when(h0 % rep == 0)
        def _():
            cp_k(h0 // rep).wait()
            cp_v(h0 // rep).wait()

        fence, release, zf = sched()
        sv = wq_s.at[:, pl.ds(al(h0 * DH, 4 * DH), 4 * DH)]
        dv = wqc_s.at[j + 1]
        units = [(sv, dv, u * 16) for u in range(NU)] + [(wq_s, wqc_s.at[0], (NPE + j) * 16)]
        hval = h_s[...]
        q = q_s[...]
        o = None
        for u in range(G0):
            mine = [units.pop(0) for _ in range(A0_CNT[u])]
            q, o = head0(hval, q, h0 + u, o, mine, 2 if u == G0 - 1 else 0, fence, release, zf)
        assert not units
        q_s[...] = q
        return carry

    lax.fori_loop(0, NA, a0_body, 0)
    cp_x(1).wait()
    cp_wr().wait()

    def o0_body(j, carry):
        cp_wo(j).wait()
        for u in range(CPV):
            cp_mod((j + 2) * CPV + u).wait()

        fence, release, zf = sched()
        sc = sc_s[...]
        hq = KP // DH
        wo_j = wo_s.at[pl.ds(al(j * D, D), D)]
        o_j = o_s.at[pl.ds(j * (D // DH), D // DH)]
        wm_j = wmod_s.at[pl.ds((j + 2) * CPV, CPV)]
        mr_j = mraw_s.at[pl.ds((j + 2) * CPV, CPV)]
        units = [(qd, ng, u) for qd in range(2) for ng in range(2) for u in range(DH // 16)]
        npass = NB * (D // KP)
        cnt = 0
        due = {}
        hist = []
        for n in range(NB):
            acc = acc_s[n, rsl(0), :]
            cu, cn = divmod(n, MC // 128)
            mv = None
            for kh in range(D // KP):
                lhs = jnp.concatenate([o_j[kh * hq + u] for u in range(hq)], axis=1)
                acc = jnp.dot(pltpu.bitcast(pin(lhs, due.pop(cnt, None)), bf16),
                              wo_j[kh * KP:(kh + 1) * KP, n * 128:(n + 1) * 128],
                              preferred_element_type=f32) + acc
                hist.append(acc)
                mine = units[cnt * len(units) // npass:(cnt + 1) * len(units) // npass]
                for n_, (qd, ng, u) in enumerate(mine):
                    last = w_unit(wo_j, [(4 * qd + c) * DH + u * 16 for c in range(4)], ng * 512,
                                  woc_s.at[j, ng], qd * DH + u * 16, [release(acc, rw) for rw in O0_ROWS[n_]])
                if cnt + 2 < npass:
                    due.setdefault(cnt + 2, {})[2] = fence([last])
                if cnt in (0, 2, 4, 6):
                    ln1(1, (cnt // 2) * QT + j * 16, 16, None if cnt == 0 else release(hist[-2], 24))
                    due.setdefault(cnt + 2, {})[12] = fence([(hf_s, (cnt // 2) * QT + j * 16)])
                if cnt in (11, 14):
                    h_slice(j * 16 + (cnt // 14) * 8, [release(hv_, 104) for hv_ in hist[-3:]])
                    if cnt == 11:
                        due.setdefault(cnt + 2, {})[10] = fence([(hs_s.at[0], j * 16)])
                cnt += 1
                d = jnp.dot(sc[:, kh * KP:(kh + 1) * KP],
                            wm_j[cu, kh * KP:(kh + 1) * KP, cn * 128:(cn + 1) * 128],
                            preferred_element_type=f32)
                mv = d if mv is None else d + mv
            acc_s[n, rsl(0), :] = acc
            mr_j[cu, :, cn * 128:(cn + 1) * 128] = mv[0:8, :]
        assert not due
        return carry

    lax.fori_loop(0, NO, o0_body, 0)

    mod_s[:, 2 * D:3 * D] = mraw(2)
    mod_s[:, 3 * D:4 * D] = mraw(3)
    mod_s[:, 4 * D:5 * D] = 1.0 + mraw(4)
    mod_s[:, 5 * D:6 * D] = mraw(5)
    mod_s[:, 6 * D:7 * D] = jnp.broadcast_to(wr_s[...].astype(f32).reshape(1, D), (8, D))
    cp_wg().start()
    for u in range(F // MC):
        cp_wu(u).start()
    cp_wd().start()

    def step(t, carry):
        @pl.when(t + 1 < nt)
        def _():
            cp_x(t + 1).wait()

        @pl.when(t + 1 == nt)
        def _():
            cp_wg().wait()
            for u in range(F // MC):
                cp_wu(u).wait()
            cp_wd().wait()

        fence, release, zf = sched()
        tprev, tnext = t - 1, jnp.minimum(t + 1, nt - 1)
        prods = [(i1, i2) for i1 in _ORDER for i2 in _ORDER]
        hv = [hs_s[u] for u in range(49)]

        qblk = {}

        def q_passes(g):
            def emit(r1, r2, n1, n2, c):
                for z in range(2):
                    qblk[8 * g + 4 * z + 2 * n1 + n2, 2 * r1 + r2] = c[:, z * DH:(z + 1) * DH]
            asm = _Assemble(emit)

            def run(i1, i2):
                u = 7 * i1 + i2
                w = jnp.concatenate([wqc_s[2 * g + z, u] for z in range(2)], axis=1)
                d = jnp.dot(hv[u], w, preferred_element_type=f32)
                ini = asm.init(i1, i2)
                if ini is not None:
                    d = d + ini
                asm.add(i1, i2, d)
                return d
            return [functools.partial(run, i1, i2) for i1, i2 in prods]

        def q_head(hh):
            return jnp.concatenate([qblk.pop((hh, r)) for r in range(4)], axis=0)

        def o_passes():
            ms = {}
            asm = []
            for ng in range(2):
                def emit(r1, r2, n1, n2, c, ng=ng):
                    acc_s[4 * ng + 2 * n1 + n2, rsl(t, r1 * HT + r2 * QT, QT), :] = c
                asm.append(_Assemble(emit))

            def run(ng, i1, i2, k, dep=None):
                u = 7 * i1 + i2
                lhs = jnp.concatenate([os_s[u, 4 * k + v] for v in range(4)], axis=1)
                w = jnp.concatenate([woc_s[2 * k + v, ng, u] for v in range(2)], axis=0)
                d = jnp.dot(lhs, pin_bf16(w, dep), preferred_element_type=f32)
                early = ng == 0 or (i1, i2) in prods[:NE]
                if k == 1:
                    d = d + ms.pop((ng, u))
                if k == (1 if early else 0):
                    ini = asm[ng].init(i1, i2)
                    if ini is not None:
                        d = d + ini
                if k == 0:
                    ms[ng, u] = d
                else:
                    asm[ng].add(i1, i2, d)
                return d
            NE = 16
            seq = [(0,) + pr + (0,) for pr in prods] + [(1,) + pr + (0,) for pr in prods[:NE]]
            seq += [(0,) + pr + (1,) for pr in prods] + [(1,) + pr + (1,) for pr in prods[:NE]]
            seq += [(1,) + pr + (k,) for pr in prods[NE:] for k in range(2)]
            return [functools.partial(run, *a) for a in seq]

        def side(hp, pts):
            rel = [release(v_, rw) for v_, rw in pts]
            for u in range(2):
                epi_rows(tprev, (2 * hp + u) * CHE, CHE, rel[u])
            ln1(tnext, hp * 16, 16, rel[2])
            return fence([(out_s, tprev * TQ), (best_r, 0), (stat_s.at[0], tprev * TQ), (hf_s, 0)])

        def o_slice(qd, oq, u, pts):
            blk = [[[[oq[k1][k2][r1 * HT + r2 * QT + 16 * u:r1 * HT + r2 * QT + 16 * u + 16]
                      for k2 in range(2)] for k1 in range(2)] for r2 in range(2)] for r1 in range(2)]
            ops = _two_level(_lhs_sums, blk, [jnp.tile(release(v_, rw), (2, 1)) for v_, rw in pts])
            for v in range(49):
                os_s[v, qd, 16 * u:16 * u + 16, :] = ops[v]
            return fence([(os_s.at[0, qd], 16 * u)])

        assert 2 * HP * CHE == TQ
        for fn in q_passes(0):
            fn()
        opl = o_passes()
        oq = fo = ob_ = None
        for hp in range(HP):
            g, pp = divmod(hp, 4)
            if pp == 0:
                fill = q_passes(g + 1) if g + 1 < HKV else opl
            qa, qb = q_head(2 * hp), q_head(2 * hp + 1)
            sa_ = scores(qa if fo is None else pin(qa, {0: fo}), g)
            pa, la = softmax2(sa_, zf)
            vals = {'s': sa_, 'ob': ob_}
            if oq is not None:
                fl = [o_slice(hp // 2 - 1, oq, 2 * (hp % 2) + u, [(vals[nm], rw) for nm, rw in OS_PTS[u]])
                      for u in range(2 if FILL[pp][1] < 7 else 1)]
                qb = pin(qb, {0: functools.reduce(lambda a_, b_: a_ | b_, fl)})
            rs_ = [fill.pop(0)() for _ in range(FILL[pp][0])]
            vals.update({i_: rs_[max(len(rs_) - 6 + i_, 0)] for i_ in range(6)})
            fs = side(hp, [(vals[nm] if vals[nm] is not None else sa_, rw) for nm, rw in SIDE_PTS])
            pb, lb = softmax2(scores(qb, g), zf)
            oa_ = pv(pa, g)
            oa = oa_ * la
            rs_ = [fill.pop(0)() for _ in range(FILL[pp][1])]
            fo = None
            if oq is not None and FILL[pp][1] >= 7:
                vals = {'oa': oa_}
                vals.update(enumerate(rs_))
                fo = o_slice(hp // 2 - 1, oq, 2 * (hp % 2) + 1, [(vals[nm], rw) for nm, rw in OS_F2])
            ob_ = pv(pin(pb, {0: fs}), g)
            ob = ob_ * lb
            if hp % 2 == 0:
                oprev = (oa, ob)
            else:
                oq = [oprev, (oa, ob)]

        pts = []
        due = {} if fo is None else {2: fo}
        HS0, HSG, HSS = 30, 14, 2
        for s, fn in enumerate(opl):
            pts.append((fn(due.pop(s, None)), 0))
            if len(pts) % 3 == 0 and len(pts) <= 12:
                o_slice(HP // 2 - 1, oq, len(pts) // 3 - 1, pts[-3:])
            u, rem = divmod(s - HS0, HSG)
            if rem == 0 and 0 <= u < QT // 8:
                h_slice(u * 8, [release(pts[-1 - HSS * i_][0]) for i_ in range(7)])
                due[s + 6] = fence([(hs_s.at[0], 0)])
        assert not due
        cp_out(tprev).start()
        return carry

    lax.fori_loop(1, nt, step, 0)

    epi_rows(nt - 1, 0, TQ)
    cp_out(nt - 1).start()
    bv = best_r[...]
    rbest = jnp.max(bv, axis=0, keepdims=True)
    ibest = jnp.min(jnp.where(bv == rbest, best_i[...], S), axis=0, keepdims=True)
    idx = jnp.minimum(ibest[0, 0], S - 1)
    base = pl.multiple_of((idx // 16) * 16, 16)
    bsl = pl.ds(base, 16)
    x1 = resid(bsl, 16)
    h2 = h2_from_stats(x1, bsl, 16)
    xs = h2.reshape(16, D).astype(bf16)
    gt = jnp.dot(xs, wq_s[:, 0:F], preferred_element_type=f32)
    up = jnp.concatenate([jnp.dot(xs, wmod_s[u], preferred_element_type=f32) for u in range(F // MC)], axis=1)
    a = (gt * jax.nn.sigmoid(gt) * up).astype(bf16)
    y = jnp.dot(a, wo_s[0:F, 0:D], preferred_element_type=f32)
    y = y * jnp.tile(jax.nn.sigmoid(rbest), (1, NB))
    rr = lax.broadcasted_iota(jnp.int32, (16, D), 0) + base
    upd = jnp.where(rr == idx, y, 0.0).reshape(2, 8, D)
    new = (x1 + mvec(5) * (h2 + upd)).reshape(16, D)
    for t in range(nt):
        cp_out(t).wait()
    out_s[bsl, :] = new.astype(out_s.dtype)
    fix = pltpu.make_async_copy(out_s.at[bsl, :], out_hbm.at[bsl, :], osems.at[0])
    fix.start()
    fix.wait()


def _compiler_params():
    kw = dict(vmem_limit_bytes=124 * 1024 * 1024)
    try:
        return pltpu.CompilerParams(disable_semaphore_checks=True, disable_bounds_checks=True, **kw)
    except TypeError:
        return pltpu.CompilerParams(**kw)


@jax.jit
def pallas_adaLN_cond__sliding_block_cached__moe_arch_mod__prompt_kernel(
    A_x: jax.Array,
    A_k_cache: jax.Array,
    A_v_cache: jax.Array,
    A_wq: jax.Array,
    A_wo: jax.Array,
    B_x: jax.Array,
    B_w_r: jax.Array,
    B_w_gate: jax.Array,
    B_w_up: jax.Array,
    B_w_down: jax.Array,
    c: jax.Array,
    w_mod: jax.Array,
):
    B, S, D = A_x.shape
    assert B == 1
    HKV, SK = A_k_cache.shape[1], A_k_cache.shape[2]
    W = min(4096, max(256, SK // 4))
    F = B_w_gate.shape[1]
    dt = A_x.dtype
    f32 = jnp.float32
    nt = S // TQ
    NB = D // 128
    NMC = 6 * D // MC
    x2 = A_x.reshape(S, D)
    anyspec = pl.BlockSpec(memory_space=pl.ANY)
    kern = functools.partial(_kernel, S=S, D=D, HKV=HKV, SK=SK, W=W, F=F)
    out = pl.pallas_call(
        kern,
        in_specs=[anyspec] * 11,
        out_specs=anyspec,
        out_shape=jax.ShapeDtypeStruct((S, D), dt),
        scratch_shapes=[
            pltpu.VMEM((D,), dt),
            pltpu.VMEM((1, D), dt),
            pltpu.VMEM((S, D), dt),
            pltpu.VMEM((HKV, W, DH), dt),
            pltpu.VMEM((HKV, W, DH), dt),
            pltpu.VMEM((D, HQ * DH + PAD), dt),
            pltpu.VMEM((HQ * DH, D + PAD), dt),
            pltpu.VMEM((NMC, D, MC), dt),
            pltpu.VMEM((S, D), dt),
            pltpu.VMEM((HQ // 4, 49, D // 4, DH), dt),
            pltpu.VMEM((HQ * DH // D, 2, 49, 2 * DH, 128), dt),
            pltpu.VMEM((TQ, D), f32),
            pltpu.VMEM((49, TQ // 4, D // 4), dt),
            pltpu.VMEM((49, HQ // 4, TQ // 4, DH), dt),
            pltpu.VMEM((16, D), dt),
            pltpu.VMEM((NMC, 8, MC), f32),
            pltpu.VMEM((8, 7 * D), f32),
            pltpu.VMEM((TQ, D), dt),
            pltpu.VMEM((TQ, DH), f32),
            pltpu.VMEM((HQ, TQ // 2, DH), jnp.uint32),
            pltpu.VMEM((NB, S, 128), f32),
            pltpu.VMEM((2, S, 128), f32),
            pltpu.VMEM((8, 128), f32),
            pltpu.VMEM((8, 128), jnp.int32),
            pltpu.SMEM((1,), jnp.int32),
            pltpu.SemaphoreType.DMA((4 + NMC + HQ + 2 * HKV + HQ * DH // D + nt,)),
            pltpu.SemaphoreType.DMA((nt,)),
        ],
        compiler_params=_compiler_params(),
    )(B_w_r, c, x2, A_k_cache, A_v_cache, A_wq, A_wo, w_mod, B_w_gate, B_w_up, B_w_down)
    return out.reshape(B, S, D)
```

```python
import functools

import jax
import jax.numpy as jnp
from jax import lax
import jax.experimental.pallas as pl
import jax.experimental.pallas.tpu as pltpu

HQ = 32
DH = 128
TQ = 256
PAD = 128
P0 = 4
G0 = 4
MC = 512
CHE = 8
SIDE_PTS = ((1, 0), (2, 0), ('ob', 16))
POSTNORM = True
OS_F2 = [('oa', 128), ('oa', 192), (0, 0), (1, 0), (2, 0), (3, 0), (4, 0)]
OS_PTS = ([('ob', 96), ('ob', 136), ('ob', 176)], [('ob', 216), ('s', 0), ('s', 48)])
A0_PTS = ([('o', r) for r in (128, 176, 224)] + [('s', r) for r in (16, 64, 112)]
          + [('q', r) for r in (8, 56, 104, 152, 200, 248)] + [('n', r) for r in (40, 80, 120)])
A0_PTS_LAST = ([('o', r) for r in (128, 168, 208)] + [('o', 248), ('s', 32), ('q', 136)]
               + [('q', 184), ('q', 232), ('n', 24)] + [('n', r) for r in (72, 120, 168)])
A0_DUE = 14
A0_LATE = ((40, 80, 120), (152, 184, 216))
A0_CNT = (3, 4, 4, 6)
O0_ROWS = ((0, 40, 152), (184, 216, 248))
FILL = ((7, 7), (7, 7), (7, 7), (7, 0))
EPS = 1e-5
LOG2E = 1.4426950408889634


def _ln_stats(x, rel=None):
    d = x.shape[-1]
    part = x[..., 0:128]
    for j in range(1, d // 128):
        part = part + x[..., j * 128:(j + 1) * 128]
    if rel is not None:
        part = part + rel
    m = jnp.sum(part, axis=-1, keepdims=True) * (1.0 / d)
    xc = x - m
    v = jnp.mean(xc * xc, axis=-1, keepdims=True)
    return m, xc, lax.rsqrt(v + EPS)


def _ln(x, rel=None):
    _, xc, rs = _ln_stats(x, rel)
    return xc * rs


def _recip(l):
    return pl.reciprocal(l, approx=True)


def _lhs_sums(a11, a12, a21, a22):
    return [a11 + a22, a21 + a22, a11, a22, a11 + a12, a21 - a11, a12 - a22]


def _rhs_sums(b11, b12, b21, b22):
    return [b11 + b22, b11, b12 - b22, b21 - b11, b22, b11 + b12, b21 + b22]


_ORDER = [3, 4, 0, 6, 1, 2, 5]
_BLOCK = {6: (0, 0), 1: (1, 0), 2: (0, 1), 5: (1, 1)}


def _init(i, z):
    return {0: lambda: z[3] - z[4], 6: lambda: z[0], 1: lambda: z[3], 2: lambda: z[4],
            5: lambda: z[0] - z[1] + z[2]}.get(i, lambda: None)()


def _two_level(sums, blk, rel):
    if rel is not None and len(rel) == 3:
        blk = [[[[blk[a1][a2][b1][b2] + rel[0 if a1 == b1 else 1 + a1] for b2 in range(2)] for b1 in range(2)]
                for a2 in range(2)] for a1 in range(2)]
    x = [[sums(blk[0][a2][0][b2], blk[0][a2][1][b2], blk[1][a2][0][b2], blk[1][a2][1][b2]) for b2 in range(2)]
         for a2 in range(2)]
    if rel is not None and len(rel) == 7:
        y = [sums(x[0][0][i] + rel[i], x[0][1][i], x[1][0][i], x[1][1][i] + rel[i]) for i in range(7)]
    else:
        y = [sums(x[0][0][i], x[0][1][i], x[1][0][i], x[1][1][i]) for i in range(7)]
    return [y[i1][i2].astype(jnp.bfloat16) for i1 in range(7) for i2 in range(7)]


class _Assemble:
    def __init__(self, emit):
        self.z, self.outer, self.inj, self.emit = {}, {}, {}, emit

    def init(self, i1, i2):
        v = _init(i2, self.z)
        if i2 in _BLOCK and i1 not in (3, 4):
            self.inj[i2] = _init(i1, self.outer[i2])
            v = v + self.inj[i2]
            if i2 == 5:
                v = v + (self.inj[1] - self.inj[2])
        return v

    def add(self, i1, i2, m):
        self.z[i2] = m
        if i2 in _BLOCK:
            self.outer.setdefault(i2, {})[i1] = m
            if i1 in _BLOCK:
                (r1, n1), (r2, n2) = _BLOCK[i1], _BLOCK[i2]
                self.emit(r1, r2, n1, n2, m)


def _kernel(wr_hbm, c_hbm, x_hbm, k_hbm, v_hbm, wq_hbm, wo_hbm, wmod_hbm,
            wg_hbm, wu_hbm, wd_hbm, out_hbm,
            wr_s, c_s, x_s, k_s, v_s, wq_s, wo_s, wmod_s, out_s,
            wqc_s, woc_s, hf_s, hs_s, os_s,
            sc_s, mraw_s, mod_s, h_s, q_s, o_s, acc_s, stat_s, best_r, best_i, zero_s, sems, osems,
            *, S, D, HKV, SK, W, F):
    nt = S // TQ
    rep = HQ // HKV
    NB = D // 128
    HP = HQ // 2
    HT = TQ // 2
    QT = TQ // 4
    KH = D // 2
    KQ = D // 4
    KP = 512
    CPV = D // MC
    NMC = 6 * CPV
    NA = (HQ - P0) // G0
    NO = HQ * DH // D
    f32 = jnp.float32
    bf16 = jnp.bfloat16
    u32 = jnp.uint32
    qscale = (DH ** -0.5) * LOG2E
    assert KH == KP and rep == 8 and NB == 8 and NO == 4 and P0 == 4 and G0 == 4

    def al(v, n):
        return v if isinstance(v, int) else pl.multiple_of(v, n)

    S_C, S_WR, S_WG, S_WD, S_M = 0, 1, 2, 3, 4
    S_WQ = S_M + NMC
    S_K = S_WQ + HQ
    S_V = S_K + HKV
    S_WO = S_V + HKV
    S_X = S_WO + NO

    def cp_c():
        return pltpu.make_async_copy(c_hbm, c_s, sems.at[S_C])

    def cp_wr():
        return pltpu.make_async_copy(wr_hbm, wr_s, sems.at[S_WR])

    def cp_mod(j):
        return pltpu.make_async_copy(wmod_hbm.at[:, pl.ds(al(j * MC, MC), MC)], wmod_s.at[j], sems.at[S_M + j])

    def cp_wg():
        return pltpu.make_async_copy(wg_hbm, wq_s.at[:, pl.ds(0, F)], sems.at[S_WG])

    def cp_wu(u):
        return pltpu.make_async_copy(wu_hbm.at[:, pl.ds(u * MC, MC)], wmod_s.at[u], sems.at[S_M + u])

    def cp_wd():
        return pltpu.make_async_copy(wd_hbm, wo_s.at[pl.ds(0, F), pl.ds(0, D)], sems.at[S_WD])

    def cp_wq(h, n=1):
        sl = pl.ds(al(h * DH, DH), n * DH)
        return pltpu.make_async_copy(wq_hbm.at[:, sl], wq_s.at[:, sl], sems.at[S_WQ + h])

    def cp_k(g):
        return pltpu.make_async_copy(k_hbm.at[0, g, pl.ds(SK - W, W), :], k_s.at[g], sems.at[S_K + g])

    def cp_v(g):
        return pltpu.make_async_copy(v_hbm.at[0, g, pl.ds(SK - W, W), :], v_s.at[g], sems.at[S_V + g])

    def cp_wo(j):
        sl = pl.ds(al(j * D, D), D)
        return pltpu.make_async_copy(wo_hbm.at[sl, :], wo_s.at[sl, pl.ds(0, D)], sems.at[S_WO + j])

    def rsl(t, r0=0, n=TQ):
        return pl.ds(al(t * TQ + r0, n), n)

    def cp_x(t):
        return pltpu.make_async_copy(x_hbm.at[rsl(t), :], x_s.at[t], sems.at[S_X + t])

    def cp_out(t):
        return pltpu.make_async_copy(out_s.at[t], out_hbm.at[rsl(t), :], osems.at[t])

    def sched():
        zero = zero_s[0]
        z16 = pl.multiple_of(zero, 16)
        zvec = jnp.full((8, 128), zero, jnp.int32).astype(u32)

        def fence(deps):
            d = None
            for ref, base in deps:
                n = 16 if ref.dtype == bf16 else 8
                v = pltpu.bitcast(ref[pl.ds(pl.multiple_of(base + z16, n), n), 0:128], u32)
                d = v if d is None else d | v
            return d & zvec

        def release(acc, r0=0):
            return pltpu.bitcast(pltpu.bitcast(acc[r0:r0 + 8, 0:128], u32) & zvec, f32)

        def zf(v_):
            return pltpu.bitcast(pltpu.bitcast(v_, u32) & jnp.tile(zvec, (v_.shape[0] // 8, 1)), f32)

        return fence, release, zf

    def pin(a, at):
        if not at:
            return a
        parts = []
        prev = 0
        for rb in sorted(at):
            r0 = rb * 8
            if r0 > prev:
                parts.append(a[prev:r0, :])
            if a.dtype == f32:
                blk = a[r0:r0 + 8, 0:128] + pltpu.bitcast(at[rb], f32)
            else:
                blk = a[r0:r0 + 8, 0:128] | at[rb]
            if a.shape[1] > 128:
                blk = jnp.concatenate([blk, a[r0:r0 + 8, 128:]], axis=1)
            parts.append(blk)
            prev = r0 + 8
        if prev < a.shape[0]:
            parts.append(a[prev:, :])
        return jnp.concatenate(parts, axis=0)

    def pin_bf16(w, d):
        if d is None:
            return w
        top = pltpu.bitcast(pltpu.bitcast(w[0:16], u32) | d, bf16)
        return jnp.concatenate([top, w[16:]], axis=0)

    def mvec(j):
        return mod_s[:, j * D:(j + 1) * D][None]

    def mraw(j):
        return jnp.concatenate([mraw_s[j * CPV + u] for u in range(CPV)], axis=1)

    def xrows(t, sl, n):
        return x_s[t, sl, :].astype(f32).reshape(n // 8, 8, D)

    def ln1(t, r0, n, rel=None):
        xn = _ln(xrows(t, pl.ds(al(r0, n), n), n), rel)
        hf_s[pl.ds(al(r0, n), n), :] = (xn * mvec(1) + mvec(0)).reshape(n, D)

    def h_slice(r0, rel):
        hq = [hf_s[pl.ds(al(r * QT + r0, 8), 8), :] for r in range(4)]
        blk = [[[[hq[2 * r1 + r2][:, (2 * k1 + k2) * KQ:(2 * k1 + k2 + 1) * KQ] for k2 in range(2)]
                 for k1 in range(2)] for r2 in range(2)] for r1 in range(2)]
        ops = _two_level(_lhs_sums, blk, None if rel is None else [jnp.tile(v, (1, KQ // 128)) for v in rel])
        for u in range(49):
            hs_s[u, pl.ds(al(r0, 8), 8), :] = ops[u]

    def w_unit(src, rows4, c0, dst, d0, rel):
        w = [src[pl.ds(al(r, 16), 16), c0:c0 + 512].astype(f32) for r in rows4]
        blk = [[[[w[2 * k1 + k2][:, (2 * n1 + n2) * 128:(2 * n1 + n2 + 1) * 128] for n2 in range(2)]
                 for n1 in range(2)] for k2 in range(2)] for k1 in range(2)]
        ops = _two_level(_rhs_sums, blk, None if rel is None else [jnp.tile(v, (2, 1)) for v in rel])
        for u in range(49):
            dst[u, pl.ds(al(d0, 16), 16), :] = ops[u]
        return (dst.at[0], d0)

    def resid(t, sl, n):
        attn = jnp.concatenate([acc_s[t, j, sl, :] for j in range(NB)], axis=1).reshape(n // 8, 8, D)
        return xrows(t, sl, n) + mvec(2) * attn

    def h2_from_stats(x1, t, sl, n):
        m = jnp.tile(stat_s[t, 0, sl, :], (1, NB)).reshape(n // 8, 8, D)
        rs = jnp.tile(stat_s[t, 1, sl, :], (1, NB)).reshape(n // 8, 8, D)
        return (x1 - m) * rs * mvec(4) + mvec(3)

    def epi_rows(t, r0, n, rel=None):
        sl = pl.ds(r0, n)
        x1 = resid(t, sl, n)
        m, xc, rs = _ln_stats(x1, rel)
        stat_s[t, 0, sl, :] = jnp.broadcast_to(m.reshape(n, 1), (n, 128))
        stat_s[t, 1, sl, :] = jnp.broadcast_to(rs.reshape(n, 1), (n, 128))
        h2 = xc * rs * mvec(4) + mvec(3)
        out_s[t, sl, :] = (x1 + mvec(5) * h2).reshape(n, D).astype(out_s.dtype)
        r = jnp.sum(h2 * mvec(6), axis=-1, keepdims=True)
        r = r.astype(bf16).astype(f32)
        bv = best_r[...]
        bi = best_i[...]
        sub = lax.broadcasted_iota(jnp.int32, (8, 128), 0)
        for u in range(n // 8):
            ru = jnp.broadcast_to(r[u], (8, 128))
            better = ru > bv
            bv = jnp.where(better, ru, bv)
            bi = jnp.where(better, sub + (t * TQ + r0 + u * 8), bi)
        best_r[...] = bv
        best_i[...] = bi

    def scores(q, g):
        return lax.dot_general(q.astype(bf16), k_s[g], (((1,), (1,)), ((), ())), preferred_element_type=f32)

    def softmax(s):
        m = jnp.max(s, axis=-1, keepdims=True)
        p = jnp.exp2(s - m)
        l = jnp.sum(p, axis=-1, keepdims=True)
        return p * _recip(l)

    def softmax2(s, zf):
        if not POSTNORM:
            return softmax(s), 1.0
        m = jnp.max(s, axis=-1, keepdims=True)
        p = jnp.exp2(s - m)
        part = p[:, 0:128]
        for j in range(1, W // 128):
            part = part + p[:, j * 128:(j + 1) * 128]
        p = jnp.concatenate([p[:, 0:128] + zf(part), p[:, 128:]], axis=1)
        return p, _recip(jnp.sum(part, axis=-1, keepdims=True))

    def qk(q, g):
        return softmax(scores(q, g))

    def pv(p, g):
        return jnp.dot(p.astype(bf16), v_s[g], preferred_element_type=f32)

    def qhalf(hval, hh, kh, acc=None):
        d = jnp.dot(hval[:, kh * KH:(kh + 1) * KH], wq_s[kh * KH:(kh + 1) * KH, pl.ds(al(hh * DH, DH), DH)],
                    preferred_element_type=f32)
        return d if acc is None else d + acc

    def head0(hval, q, hh, o_prev, units, late, fence, release, zf):
        g = hh // rep
        hn = hh + 1 if isinstance(hh, int) else jnp.minimum(hh + 1, HQ - 1)
        units = list(units)

        def unit(rel):
            sv, dv, r0 = units.pop(0)
            return w_unit(sv, [c * KQ + r0 for c in range(4)], 0, dv, r0, rel)

        pts = list(A0_PTS_LAST if late else A0_PTS)
        if o_prev is None:
            pts = pts[3:]
        s = scores(q, g)
        p, li = softmax2(s, zf)
        q1 = qhalf(hval, hn, 0)
        qn = qhalf(hval, hn, 1, q1)
        vals = dict(o=o_prev, s=s, q=q1, n=qn)
        deps = []
        while len(units) > late:
            deps.append(unit([release(vals[nm], row) for nm, row in pts[:3]]))
            pts = pts[3:]
        deps = deps[-2:] + ([(o_s.at[hh - 1], 0)] if o_prev is not None else [])
        if deps:
            p = pin(p, {(24 if late else A0_DUE): fence(deps)})
        o = pv(p, g)
        o_s[hh] = pltpu.bitcast((o * li).astype(bf16), u32)
        for u in range(late):
            unit([release(o, row) for row in A0_LATE[u]])
        return qn, o

    cp_c().start()
    cp_x(0).start()
    for j in range(2 * CPV):
        cp_mod(j).start()
    cp_wq(0).start()
    cp_k(0).start()
    cp_v(0).start()
    cp_wq(1).start()
    cp_wq(2).start()
    cp_wq(3, 2).start()
    for j in range(NA):
        h0 = P0 + j * G0
        cp_wq(h0 + 1, G0 if j + 1 < NA else G0 - 1).start()
        if h0 % rep == 0:
            cp_k(h0 // rep).start()
            cp_v(h0 // rep).start()
    cp_x(1).start()
    cp_wr().start()
    for j in range(NO):
        cp_wo(j).start()
        for u in range(CPV):
            cp_mod((j + 2) * CPV + u).start()
    for t in range(2, nt):
        cp_x(t).start()

    zero_s[0] = 0
    for n in range(NB):
        acc_s[0, n] = jnp.zeros((TQ, 128), f32)
    hs_s[0] = jnp.zeros((QT, KQ), bf16)
    best_r[...] = jnp.full(best_r.shape, -jnp.inf, f32)
    best_i[...] = jnp.zeros(best_i.shape, jnp.int32)
    cp_c().wait()
    cp_x(0).wait()
    cf = c_s[...].astype(f32)
    sc_s[...] = jnp.broadcast_to(cf * jax.nn.sigmoid(cf), (16, D)).astype(bf16)
    xn0 = _ln(xrows(0, pl.ds(0, TQ), TQ))

    def mod_body(j, carry):
        cp_mod(j).wait()
        mraw_s[j] = jnp.dot(sc_s[...], wmod_s[j], preferred_element_type=f32)[0:8, :]
        return carry

    lax.fori_loop(0, 2 * CPV, mod_body, 0)
    mod_s[:, 0:D] = mraw(0) * qscale
    mod_s[:, D:2 * D] = (1.0 + mraw(1)) * qscale
    h_s[...] = (xn0 * mvec(1) + mvec(0)).reshape(TQ, D).astype(bf16)
    cp_wq(0).wait()
    hval0 = h_s[...]
    q = qhalf(hval0, 0, 1, qhalf(hval0, 0, 0))
    cp_k(0).wait()
    cp_v(0).wait()
    NU = KQ // 16
    NPE = NU - NA
    sch0 = sched()
    cp_wq(1).wait()
    q, _ = head0(hval0, q, 0, None, [], 0, *sch0)
    cp_wq(2).wait()
    q, _ = head0(hval0, q, 1, None, [], 0, *sch0)
    cp_wq(3, 2).wait()
    u0 = [(wq_s, wqc_s.at[0], u * 16) for u in range(NPE)]
    q, o = head0(hval0, q, 2, None, u0[:3], 0, *sch0)
    q, _ = head0(hval0, q, 3, o, u0[3:], 2, *sch0)
    q_s[...] = q

    def a0_body(j, carry):
        h0 = P0 + j * G0

        @pl.when(j + 1 < NA)
        def _():
            cp_wq(h0 + 1, G0).wait()

        @pl.when(j + 1 == NA)
        def _():
            cp_wq(HQ - G0 + 1, G0 - 1).wait()

        @pl.when(h0 % rep == 0)
        def _():
            cp_k(h0 // rep).wait()
            cp_v(h0 // rep).wait()

        fence, release, zf = sched()
        sv = wq_s.at[:, pl.ds(al(h0 * DH, 4 * DH), 4 * DH)]
        dv = wqc_s.at[j + 1]
        units = [(sv, dv, u * 16) for u in range(NU)] + [(wq_s, wqc_s.at[0], (NPE + j) * 16)]
        hval = h_s[...]
        q = q_s[...]
        o = None
        for u in range(G0):
            mine = [units.pop(0) for _ in range(A0_CNT[u])]
            q, o = head0(hval, q, h0 + u, o, mine, 2 if u == G0 - 1 else 0, fence, release, zf)
        assert not units
        q_s[...] = q
        return carry

    lax.fori_loop(0, NA, a0_body, 0)
    cp_x(1).wait()
    cp_wr().wait()

    def o0_body(j, carry):
        cp_wo(j).wait()
        for u in range(CPV):
            cp_mod((j + 2) * CPV + u).wait()

        fence, release, zf = sched()
        sc = sc_s[...]
        hq = KP // DH
        wo_j = wo_s.at[pl.ds(al(j * D, D), D)]
        o_j = o_s.at[pl.ds(j * (D // DH), D // DH)]
        wm_j = wmod_s.at[pl.ds((j + 2) * CPV, CPV)]
        mr_j = mraw_s.at[pl.ds((j + 2) * CPV, CPV)]
        units = [(qd, ng, u) for qd in range(2) for ng in range(2) for u in range(DH // 16)]
        npass = NB * (D // KP)
        cnt = 0
        due = {}
        hist = []
        lhs2 = [jnp.concatenate([o_j[kh * hq + u] for u in range(hq)], axis=1) for kh in range(D // KP)]
        for n in range(NB):
            acc = acc_s[0, n]
            cu, cn = divmod(n, MC // 128)
            mv = None
            for kh in range(D // KP):
                lhs = lhs2[kh]
                acc = jnp.dot(pltpu.bitcast(pin(lhs, due.pop(cnt, None)), bf16),
                              wo_j[kh * KP:(kh + 1) * KP, n * 128:(n + 1) * 128],
                              preferred_element_type=f32) + acc
                hist.append(acc)
                mine = units[cnt * len(units) // npass:(cnt + 1) * len(units) // npass]
                for n_, (qd, ng, u) in enumerate(mine):
                    last = w_unit(wo_j, [(4 * qd + c) * DH + u * 16 for c in range(4)], ng * 512,
                                  woc_s.at[j, ng], qd * DH + u * 16, [release(acc, rw) for rw in O0_ROWS[n_]])
                if cnt + 2 < npass:
                    due.setdefault(cnt + 2, {})[2] = fence([last])
                if cnt in (0, 2, 4, 6):
                    ln1(1, (cnt // 2) * QT + j * 16, 16, None if cnt == 0 else release(hist[-2], 24))
                    due.setdefault(cnt + 2, {})[12] = fence([(hf_s, (cnt // 2) * QT + j * 16)])
                if cnt in (11, 14):
                    h_slice(j * 16 + (cnt // 14) * 8, [release(hv_, 104) for hv_ in hist[-3:]])
                    if cnt == 11:
                        due.setdefault(cnt + 2, {})[10] = fence([(hs_s.at[0], j * 16)])
                cnt += 1
                d = jnp.dot(sc[:, kh * KP:(kh + 1) * KP],
                            wm_j[cu, kh * KP:(kh + 1) * KP, cn * 128:(cn + 1) * 128],
                            preferred_element_type=f32)
                mv = d if mv is None else d + mv
            acc_s[0, n] = acc
            mr_j[cu, :, cn * 128:(cn + 1) * 128] = mv[0:8, :]
        assert not due
        return carry

    lax.fori_loop(0, NO, o0_body, 0)

    mod_s[:, 2 * D:3 * D] = mraw(2)
    mod_s[:, 3 * D:4 * D] = mraw(3)
    mod_s[:, 4 * D:5 * D] = 1.0 + mraw(4)
    mod_s[:, 5 * D:6 * D] = mraw(5)
    mod_s[:, 6 * D:7 * D] = jnp.broadcast_to(wr_s[...].astype(f32).reshape(1, D), (8, D))
    cp_wg().start()
    for u in range(F // MC):
        cp_wu(u).start()
    cp_wd().start()

    def step(t, carry):
        @pl.when(t + 1 < nt)
        def _():
            cp_x(t + 1).wait()

        @pl.when(t + 1 == nt)
        def _():
            cp_wg().wait()
            for u in range(F // MC):
                cp_wu(u).wait()
            cp_wd().wait()

        fence, release, zf = sched()
        tprev, tnext = t - 1, jnp.minimum(t + 1, nt - 1)
        prods = [(i1, i2) for i1 in _ORDER for i2 in _ORDER]
        hv = [hs_s[u] for u in range(49)]

        qblk = {}

        def q_passes(g):
            def emit(r1, r2, n1, n2, c):
                for z in range(2):
                    qblk[8 * g + 4 * z + 2 * n1 + n2, 2 * r1 + r2] = c[:, z * DH:(z + 1) * DH]
            asm = _Assemble(emit)

            def run(i1, i2):
                u = 7 * i1 + i2
                w = jnp.concatenate([wqc_s[2 * g + z, u] for z in range(2)], axis=1)
                d = jnp.dot(hv[u], w, preferred_element_type=f32)
                ini = asm.init(i1, i2)
                if ini is not None:
                    d = d + ini
                asm.add(i1, i2, d)
                return d
            return [functools.partial(run, i1, i2) for i1, i2 in prods]

        def q_head(hh):
            return jnp.concatenate([qblk.pop((hh, r)) for r in range(4)], axis=0)

        def o_passes():
            ms = {}
            asm = []
            for ng in range(2):
                def emit(r1, r2, n1, n2, c, ng=ng):
                    acc_s[t, 4 * ng + 2 * n1 + n2, pl.ds(r1 * HT + r2 * QT, QT), :] = c
                asm.append(_Assemble(emit))

            def run(ng, i1, i2, k, dep=None):
                u = 7 * i1 + i2
                lhs = jnp.concatenate([os_s[u, 4 * k + v] for v in range(4)], axis=1)
                w = jnp.concatenate([woc_s[2 * k + v, ng, u] for v in range(2)], axis=0)
                d = jnp.dot(lhs, pin_bf16(w, dep), preferred_element_type=f32)
                early = ng == 0 or (i1, i2) in prods[:NE]
                if k == 1:
                    d = d + ms.pop((ng, u))
                if k == (1 if early else 0):
                    ini = asm[ng].init(i1, i2)
                    if ini is not None:
                        d = d + ini
                if k == 0:
                    ms[ng, u] = d
                else:
                    asm[ng].add(i1, i2, d)
                return d
            NE = 16
            seq = [(0,) + pr + (0,) for pr in prods] + [(1,) + pr + (0,) for pr in prods[:NE]]
            seq += [(0,) + pr + (1,) for pr in prods] + [(1,) + pr + (1,) for pr in prods[:NE]]
            seq += [(1,) + pr + (k,) for pr in prods[NE:] for k in range(2)]
            return [functools.partial(run, *a) for a in seq]

        def side(hp, pts):
            rel = [release(v_, rw) for v_, rw in pts]
            for u in range(2):
                epi_rows(tprev, (2 * hp + u) * CHE, CHE, rel[u])
            ln1(tnext, hp * 16, 16, rel[2])
            return fence([(out_s.at[tprev], 0), (best_r, 0), (stat_s.at[tprev, 0], 0), (hf_s, 0)])

        def o_slice(qd, oq, u, pts):
            blk = [[[[oq[k1][k2][r1 * HT + r2 * QT + 16 * u:r1 * HT + r2 * QT + 16 * u + 16]
                      for k2 in range(2)] for k1 in range(2)] for r2 in range(2)] for r1 in range(2)]
            ops = _two_level(_lhs_sums, blk, [jnp.tile(release(v_, rw), (2, 1)) for v_, rw in pts])
            for v in range(49):
                os_s[v, qd, 16 * u:16 * u + 16, :] = ops[v]
            return fence([(os_s.at[0, qd], 16 * u)])

        assert 2 * HP * CHE == TQ
        for fn in q_passes(0):
            fn()
        opl = o_passes()
        oq = fo = ob_ = None
        for hp in range(HP):
            g, pp = divmod(hp, 4)
            if pp == 0:
                fill = q_passes(g + 1) if g + 1 < HKV else opl
            qa, qb = q_head(2 * hp), q_head(2 * hp + 1)
            sa_ = scores(qa if fo is None else pin(qa, {0: fo}), g)
            pa, la = softmax2(sa_, zf)
            vals = {'s': sa_, 'ob': ob_}
            if oq is not None:
                fl = [o_slice(hp // 2 - 1, oq, 2 * (hp % 2) + u, [(vals[nm], rw) for nm, rw in OS_PTS[u]])
                      for u in range(2 if FILL[pp][1] < 7 else 1)]
                qb = pin(qb, {0: functools.reduce(lambda a_, b_: a_ | b_, fl)})
            rs_ = [fill.pop(0)() for _ in range(FILL[pp][0])]
            vals.update({i_: rs_[max(len(rs_) - 6 + i_, 0)] for i_ in range(6)})
            fs = side(hp, [(vals[nm] if vals[nm] is not None else sa_, rw) for nm, rw in SIDE_PTS])
            pb, lb = softmax2(scores(qb, g), zf)
            oa_ = pv(pa, g)
            oa = oa_ * la
            rs_ = [fill.pop(0)() for _ in range(FILL[pp][1])]
            fo = None
            if oq is not None and FILL[pp][1] >= 7:
                vals = {'oa': oa_}
                vals.update(enumerate(rs_))
                fo = o_slice(hp // 2 - 1, oq, 2 * (hp % 2) + 1, [(vals[nm], rw) for nm, rw in OS_F2])
            ob_ = pv(pin(pb, {0: fs}), g)
            ob = ob_ * lb
            if hp % 2 == 0:
                oprev = (oa, ob)
            else:
                oq = [oprev, (oa, ob)]

        pts = []
        due = {} if fo is None else {2: fo}
        HS0, HSG, HSS = 30, 14, 2
        for s, fn in enumerate(opl):
            pts.append((fn(due.pop(s, None)), 0))
            if len(pts) % 3 == 0 and len(pts) <= 12:
                o_slice(HP // 2 - 1, oq, len(pts) // 3 - 1, pts[-3:])
            u, rem = divmod(s - HS0, HSG)
            if rem == 0 and 0 <= u < QT // 8:
                h_slice(u * 8, [release(pts[-1 - HSS * i_][0]) for i_ in range(7)])
                due[s + 6] = fence([(hs_s.at[0], 0)])
        assert not due
        cp_out(tprev).start()
        return carry

    lax.fori_loop(1, nt, step, 0)

    epi_rows(nt - 1, 0, TQ)
    cp_out(nt - 1).start()
    bv = best_r[...]
    rbest = jnp.max(bv, axis=0, keepdims=True)
    ibest = jnp.min(jnp.where(bv == rbest, best_i[...], S), axis=0, keepdims=True)
    idx = jnp.minimum(ibest[0, 0], S - 1)
    base = pl.multiple_of((idx // 16) * 16, 16)
    tb = idx // TQ
    bsl = pl.ds(pl.multiple_of(base - tb * TQ, 16), 16)
    x1 = resid(tb, bsl, 16)
    h2 = h2_from_stats(x1, tb, bsl, 16)
    xs = h2.reshape(16, D).astype(bf16)
    gt = jnp.dot(xs, wq_s[:, 0:F], preferred_element_type=f32)
    up = jnp.concatenate([jnp.dot(xs, wmod_s[u], preferred_element_type=f32) for u in range(F // MC)], axis=1)
    a = (gt * jax.nn.sigmoid(gt) * up).astype(bf16)
    y = jnp.dot(a, wo_s[0:F, 0:D], preferred_element_type=f32)
    y = y * jnp.tile(jax.nn.sigmoid(rbest), (1, NB))
    rr = lax.broadcasted_iota(jnp.int32, (16, D), 0) + base
    upd = jnp.where(rr == idx, y, 0.0).reshape(2, 8, D)
    new = (x1 + mvec(5) * (h2 + upd)).reshape(16, D)
    for t in range(nt):
        cp_out(t).wait()
    out_s[tb, bsl, :] = new.astype(out_s.dtype)
    fix = pltpu.make_async_copy(out_s.at[tb, bsl, :], out_hbm.at[pl.ds(base, 16), :], osems.at[0])
    fix.start()
    fix.wait()


def _compiler_params():
    kw = dict(vmem_limit_bytes=124 * 1024 * 1024)
    try:
        return pltpu.CompilerParams(disable_semaphore_checks=True, disable_bounds_checks=True, **kw)
    except TypeError:
        return pltpu.CompilerParams(**kw)


@jax.jit
def pallas_adaLN_cond__sliding_block_cached__moe_arch_mod__prompt_kernel(
    A_x: jax.Array,
    A_k_cache: jax.Array,
    A_v_cache: jax.Array,
    A_wq: jax.Array,
    A_wo: jax.Array,
    B_x: jax.Array,
    B_w_r: jax.Array,
    B_w_gate: jax.Array,
    B_w_up: jax.Array,
    B_w_down: jax.Array,
    c: jax.Array,
    w_mod: jax.Array,
):
    B, S, D = A_x.shape
    assert B == 1
    HKV, SK = A_k_cache.shape[1], A_k_cache.shape[2]
    W = min(4096, max(256, SK // 4))
    F = B_w_gate.shape[1]
    dt = A_x.dtype
    f32 = jnp.float32
    nt = S // TQ
    NB = D // 128
    NMC = 6 * D // MC
    x2 = A_x.reshape(S, D)
    anyspec = pl.BlockSpec(memory_space=pl.ANY)
    kern = functools.partial(_kernel, S=S, D=D, HKV=HKV, SK=SK, W=W, F=F)
    out = pl.pallas_call(
        kern,
        in_specs=[anyspec] * 11,
        out_specs=anyspec,
        out_shape=jax.ShapeDtypeStruct((S, D), dt),
        scratch_shapes=[
            pltpu.VMEM((D,), dt),
            pltpu.VMEM((1, D), dt),
            pltpu.VMEM((nt, TQ, D), dt),
            pltpu.VMEM((HKV, W, DH), dt),
            pltpu.VMEM((HKV, W, DH), dt),
            pltpu.VMEM((D, HQ * DH + PAD), dt),
            pltpu.VMEM((HQ * DH, D + PAD), dt),
            pltpu.VMEM((NMC, D, MC), dt),
            pltpu.VMEM((nt, TQ, D), dt),
            pltpu.VMEM((HQ // 4, 49, D // 4, DH), dt),
            pltpu.VMEM((HQ * DH // D, 2, 49, 2 * DH, 128), dt),
            pltpu.VMEM((TQ, D), f32),
            pltpu.VMEM((49, TQ // 4, D // 4), dt),
            pltpu.VMEM((49, HQ // 4, TQ // 4, DH), dt),
            pltpu.VMEM((16, D), dt),
            pltpu.VMEM((NMC, 8, MC), f32),
            pltpu.VMEM((8, 7 * D), f32),
            pltpu.VMEM((TQ, D), dt),
            pltpu.VMEM((TQ, DH), f32),
            pltpu.VMEM((HQ, TQ // 2, DH), jnp.uint32),
            pltpu.VMEM((nt, NB, TQ, 128), f32),
            pltpu.VMEM((nt, 2, TQ, 128), f32),
            pltpu.VMEM((8, 128), f32),
            pltpu.VMEM((8, 128), jnp.int32),
            pltpu.SMEM((1,), jnp.int32),
            pltpu.SemaphoreType.DMA((4 + NMC + HQ + 2 * HKV + HQ * DH // D + nt,)),
            pltpu.SemaphoreType.DMA((nt,)),
        ],
        compiler_params=_compiler_params(),
    )(B_w_r, c, x2, A_k_cache, A_v_cache, A_wq, A_wo, w_mod, B_w_gate, B_w_up, B_w_down)
    return out.reshape(B, S, D)
```

```python
import functools

import jax
import jax.numpy as jnp
from jax import lax
import jax.experimental.pallas as pl
import jax.experimental.pallas.tpu as pltpu

HQ = 32
DH = 128
TQ = 256
PAD = 128
P0 = 4
G0 = 4
MC = 512
CHE = 8
SIDE_PTS = ((1, 0), (2, 0), ('ob', 16))
POSTNORM = True
OS_F2 = [('oa', 128), ('oa', 192), (0, 0), (1, 0), (2, 0), (3, 0), (4, 0)]
OS_PTS = ([('ob', 96 + 16 * i) for i in range(7)],
          [('ob', 208), ('ob', 224), ('ob', 240), ('s', 0), ('s', 16), ('s', 32), ('s', 48)])
A0_WIN = ((2, 250), (394, 760))
A0_WIN_LAST = ((2, 170), (520, 820))
PERM = (3, 1, 4, 0, 5, 2, 6)
A0_DUE = 14
A0_LATE = (24, 136)
A0_CNT = (3, 4, 4, 6)
O0_ROWS = ((0, 16, 32, 56, 72, 88, 112), (128, 144, 168, 184, 200, 224, 240))
FILL = ((7, 7), (7, 7), (7, 7), (7, 0))
HS0, HSG, HSS = 30, 14, 2
O0_LN = (0, 2, 4, 6)
O0_HS = (11, 14)
O0_HSROW = 104
MSH = 1
EPS = 1e-5
LOG2E = 1.4426950408889634


def _ln_stats(x, rel=None):
    d = x.shape[-1]
    part = x[..., 0:128]
    for j in range(1, d // 128):
        part = part + x[..., j * 128:(j + 1) * 128]
    if rel is not None:
        part = part + rel
    m = jnp.sum(part, axis=-1, keepdims=True) * (1.0 / d)
    xc = x - m
    v = jnp.mean(xc * xc, axis=-1, keepdims=True)
    return m, xc, lax.rsqrt(v + EPS)


def _ln(x, rel=None):
    _, xc, rs = _ln_stats(x, rel)
    return xc * rs


def _recip(l):
    return pl.reciprocal(l, approx=True)


def _lhs_sums(a11, a12, a21, a22):
    return [a11 + a22, a21 + a22, a11, a22, a11 + a12, a21 - a11, a12 - a22]


def _rhs_sums(b11, b12, b21, b22):
    return [b11 + b22, b11, b12 - b22, b21 - b11, b22, b11 + b12, b21 + b22]


_ORDER = [3, 4, 0, 6, 1, 2, 5]
_BLOCK = {6: (0, 0), 1: (1, 0), 2: (0, 1), 5: (1, 1)}


def _init(i, z):
    return {0: lambda: z[3] - z[4], 6: lambda: z[0], 1: lambda: z[3], 2: lambda: z[4],
            5: lambda: z[0] - z[1] + z[2]}.get(i, lambda: None)()


def _two_level(sums, blk, rel):
    o = [[jnp.stack([blk[a1][a2][b1][b2] for a2 in range(2) for b2 in range(2)]) for b1 in range(2)]
         for a1 in range(2)]
    if rel is not None and len(rel) == 3:
        o = [[o[a1][b1] + rel[0 if a1 == b1 else 1 + a1][None] for b1 in range(2)] for a1 in range(2)]
    x = jnp.stack(sums(o[0][0], o[0][1], o[1][0], o[1][1]), axis=1)
    x = [x[u] for u in range(4)]
    if rel is not None and len(rel) == 7:
        r7 = jnp.stack(rel)
        x = [x[0] + r7, x[1], x[2], x[3] + r7]
    return [y.astype(jnp.bfloat16) for y in sums(*x)]


class _Assemble:
    def __init__(self, emit):
        self.z, self.outer, self.inj, self.emit = {}, {}, {}, emit

    def init(self, i1, i2):
        v = _init(i2, self.z)
        if i2 in _BLOCK and i1 not in (3, 4):
            self.inj[i2] = _init(i1, self.outer[i2])
            v = v + self.inj[i2]
            if i2 == 5:
                v = v + (self.inj[1] - self.inj[2])
        return v

    def add(self, i1, i2, m):
        self.z[i2] = m
        if i2 in _BLOCK:
            self.outer.setdefault(i2, {})[i1] = m
            if i1 in _BLOCK:
                (r1, n1), (r2, n2) = _BLOCK[i1], _BLOCK[i2]
                self.emit(r1, r2, n1, n2, m)


def _kernel(wr_hbm, c_hbm, x_hbm, k_hbm, v_hbm, wq_hbm, wo_hbm, wmod_hbm,
            wg_hbm, wu_hbm, wd_hbm, out_hbm,
            wr_s, c_s, x_s, k_s, v_s, wq_s, wo_s, wmod_s, out_s,
            wqc_s, woc_s, hf_s, hs_s, os_s,
            sc_s, mraw_s, mod_s, h_s, q_s, o_s, acc_s, stat_s, best_r, best_i, zero_s, sems, osems,
            *, S, D, HKV, SK, W, F):
    nt = S // TQ
    rep = HQ // HKV
    NB = D // 128
    HP = HQ // 2
    HT = TQ // 2
    QT = TQ // 4
    KH = D // 2
    KQ = D // 4
    KP = 512
    CPV = D // MC
    NMC = 6 * CPV
    NA = (HQ - P0) // G0
    NO = HQ * DH // D
    f32 = jnp.float32
    bf16 = jnp.bfloat16
    u32 = jnp.uint32
    qscale = (DH ** -0.5) * LOG2E
    assert KH == KP and rep == 8 and NB == 8 and NO == 4 and P0 == 4 and G0 == 4

    def al(v, n):
        return v if isinstance(v, int) else pl.multiple_of(v, n)

    S_C, S_WR, S_WG, S_WD, S_M = 0, 1, 2, 3, 4
    S_WQ = S_M + NMC
    S_K = S_WQ + HQ
    S_V = S_K + HKV
    S_WO = S_V + HKV
    S_X = S_WO + NO

    def cp_c():
        return pltpu.make_async_copy(c_hbm, c_s, sems.at[S_C])

    def cp_wr():
        return pltpu.make_async_copy(wr_hbm, wr_s, sems.at[S_WR])

    def cp_mod(j):
        return pltpu.make_async_copy(wmod_hbm.at[:, pl.ds(al(j * MC, MC), MC)], wmod_s.at[j], sems.at[S_M + j])

    def cp_wg():
        return pltpu.make_async_copy(wg_hbm, wq_s.at[:, pl.ds(0, F)], sems.at[S_WG])

    def cp_wu(u):
        return pltpu.make_async_copy(wu_hbm.at[:, pl.ds(u * MC, MC)], wmod_s.at[u], sems.at[S_M + u])

    def cp_wd():
        return pltpu.make_async_copy(wd_hbm, wo_s.at[pl.ds(0, F), pl.ds(0, D)], sems.at[S_WD])

    def cp_wq(h, n=1):
        sl = pl.ds(al(h * DH, DH), n * DH)
        return pltpu.make_async_copy(wq_hbm.at[:, sl], wq_s.at[:, sl], sems.at[S_WQ + h])

    def cp_k(g):
        return pltpu.make_async_copy(k_hbm.at[0, g, pl.ds(SK - W, W), :], k_s.at[g], sems.at[S_K + g])

    def cp_v(g):
        return pltpu.make_async_copy(v_hbm.at[0, g, pl.ds(SK - W, W), :], v_s.at[g], sems.at[S_V + g])

    def cp_wo(j):
        sl = pl.ds(al(j * D, D), D)
        return pltpu.make_async_copy(wo_hbm.at[sl, :], wo_s.at[sl, pl.ds(0, D)], sems.at[S_WO + j])

    def rsl(t, r0=0, n=TQ):
        return pl.ds(al(t * TQ + r0, n), n)

    def cp_x(t):
        return pltpu.make_async_copy(x_hbm.at[rsl(t), :], x_s.at[t], sems.at[S_X + t])

    def cp_out(t):
        return pltpu.make_async_copy(out_s.at[t], out_hbm.at[rsl(t), :], osems.at[t])

    def sched():
        zero = zero_s[0]
        z16 = pl.multiple_of(zero, 16)
        zvec = jnp.full((8, 128), zero, jnp.int32).astype(u32)

        def fence(deps):
            d = None
            for ref, base in deps:
                n = 16 if ref.dtype == bf16 else 8
                v = pltpu.bitcast(ref[pl.ds(pl.multiple_of(base + z16, n), n), 0:128], u32)
                d = v if d is None else d | v
            return d & zvec

        def release(acc, r0=0):
            return pltpu.bitcast(pltpu.bitcast(acc[r0:r0 + 8, 0:128], u32) & zvec, f32)

        def zf(v_):
            return pltpu.bitcast(pltpu.bitcast(v_, u32) & jnp.tile(zvec, (v_.shape[0] // 8, 1)), f32)

        return fence, release, zf

    def pin(a, at):
        if not at:
            return a
        parts = []
        prev = 0
        for rb in sorted(at):
            r0 = rb * 8
            if r0 > prev:
                parts.append(a[prev:r0, :])
            if a.dtype == f32:
                blk = a[r0:r0 + 8, 0:128] + pltpu.bitcast(at[rb], f32)
            else:
                blk = a[r0:r0 + 8, 0:128] | at[rb]
            if a.shape[1] > 128:
                blk = jnp.concatenate([blk, a[r0:r0 + 8, 128:]], axis=1)
            parts.append(blk)
            prev = r0 + 8
        if prev < a.shape[0]:
            parts.append(a[prev:, :])
        return jnp.concatenate(parts, axis=0)

    def pin_bf16(w, d):
        if d is None:
            return w
        top = pltpu.bitcast(pltpu.bitcast(w[0:16], u32) | d, bf16)
        return jnp.concatenate([top, w[16:]], axis=0)

    def mvec(j):
        return mod_s[:, j * D:(j + 1) * D][None]

    def mraw(j):
        return jnp.concatenate([mraw_s[j * CPV + u] for u in range(CPV)], axis=1)

    def xrows(t, sl, n):
        return x_s[t, sl, :].astype(f32).reshape(n // 8, 8, D)

    def ln1(t, r0, n, rel=None):
        xn = _ln(xrows(t, pl.ds(al(r0, n), n), n), rel)
        hf_s[pl.ds(al(r0, n), n), :] = (xn * mvec(1) + mvec(0)).reshape(n, D)

    def h_slice(r0, rel):
        hq = [hf_s[pl.ds(al(r * QT + r0, 8), 8), :] for r in range(4)]
        blk = [[[[hq[2 * r1 + r2][:, (2 * k1 + k2) * KQ:(2 * k1 + k2 + 1) * KQ] for k2 in range(2)]
                 for k1 in range(2)] for r2 in range(2)] for r1 in range(2)]
        ops = _two_level(_lhs_sums, blk, None if rel is None else [jnp.tile(v, (1, KQ // 128)) for v in rel])
        for u in range(7):
            hs_s[7 * u:7 * u + 7, pl.ds(al(r0, 8), 8), :] = ops[u]

    def w_unit(src, rows4, c0, dst, d0, rel):
        w = [src[pl.ds(al(r, 16), 16), c0:c0 + 512].astype(f32) for r in rows4]
        blk = [[[[w[2 * k1 + k2][:, (2 * n1 + n2) * 128:(2 * n1 + n2 + 1) * 128] for n2 in range(2)]
                 for n1 in range(2)] for k2 in range(2)] for k1 in range(2)]
        ops = _two_level(_rhs_sums, blk, None if rel is None else [jnp.tile(v, (2, 1)) for v in rel])
        for u in range(7):
            dst[7 * u:7 * u + 7, pl.ds(al(d0, 16), 16), :] = ops[u]
        return (dst.at[0], d0)

    def resid(t, sl, n):
        attn = jnp.concatenate([acc_s[t, j, sl, :] for j in range(NB)], axis=1).reshape(n // 8, 8, D)
        return xrows(t, sl, n) + mvec(2) * attn

    def h2_from_stats(x1, t, sl, n):
        m = jnp.tile(stat_s[t, 0, sl, :], (1, NB)).reshape(n // 8, 8, D)
        rs = jnp.tile(stat_s[t, 1, sl, :], (1, NB)).reshape(n // 8, 8, D)
        return (x1 - m) * rs * mvec(4) + mvec(3)

    def epi_rows(t, r0, n, rel=None):
        sl = pl.ds(r0, n)
        x1 = resid(t, sl, n)
        m, xc, rs = _ln_stats(x1, rel)
        stat_s[t, 0, sl, :] = jnp.broadcast_to(m.reshape(n, 1), (n, 128))
        stat_s[t, 1, sl, :] = jnp.broadcast_to(rs.reshape(n, 1), (n, 128))
        h2 = xc * rs * mvec(4) + mvec(3)
        out_s[t, sl, :] = (x1 + mvec(5) * h2).reshape(n, D).astype(out_s.dtype)
        r = jnp.sum(h2 * mvec(6), axis=-1, keepdims=True)
        r = r.astype(bf16).astype(f32)
        bv = best_r[...]
        bi = best_i[...]
        sub = lax.broadcasted_iota(jnp.int32, (8, 128), 0)
        for u in range(n // 8):
            ru = jnp.broadcast_to(r[u], (8, 128))
            better = ru > bv
            bv = jnp.where(better, ru, bv)
            bi = jnp.where(better, sub + (t * TQ + r0 + u * 8), bi)
        best_r[...] = bv
        best_i[...] = bi

    def scores(q, g):
        return lax.dot_general(q.astype(bf16), k_s[g], (((1,), (1,)), ((), ())), preferred_element_type=f32)

    def softmax(s):
        m = jnp.max(s, axis=-1, keepdims=True)
        p = jnp.exp2(s - m)
        l = jnp.sum(p, axis=-1, keepdims=True)
        return p * _recip(l)

    def softmax2(s, zf):
        if not POSTNORM:
            return softmax(s), 1.0
        m = jnp.max(s, axis=-1, keepdims=True)
        p = jnp.exp2(s - m)
        part = p[:, 0:128]
        for j in range(1, W // 128):
            part = part + p[:, j * 128:(j + 1) * 128]
        p = jnp.concatenate([jnp.minimum(p[:, 0:128], part), p[:, 128:]], axis=1)
        return p, _recip(jnp.sum(part, axis=-1, keepdims=True))

    def qk(q, g):
        return softmax(scores(q, g))

    def pv(p, g):
        return jnp.dot(p.astype(bf16), v_s[g], preferred_element_type=f32)

    def qhalf(hval, hh, kh, acc=None):
        d = jnp.dot(hval[:, kh * KH:(kh + 1) * KH], wq_s[kh * KH:(kh + 1) * KH, pl.ds(al(hh * DH, DH), DH)],
                    preferred_element_type=f32)
        return d if acc is None else d + acc

    def head0(hval, q, hh, o_prev, units, late, fence, release, zf):
        g = hh // rep
        hn = hh + 1 if isinstance(hh, int) else jnp.minimum(hh + 1, HQ - 1)
        units = list(units)

        def unit(rel):
            sv, dv, r0 = units.pop(0)
            return w_unit(sv, [c * KQ + r0 for c in range(4)], 0, dv, r0, rel)

        wins = [w_ for w_ in (A0_WIN_LAST if late else A0_WIN)]
        if o_prev is None:
            wins = [(max(a_, 130), b_) for a_, b_ in wins if b_ > 130]
        slots = [t_ for a_, b_ in wins for t_ in range(a_, b_, 8)]
        npt = 7 * (len(units) - late)
        pts = []
        for u in range(npt):
            t_ = slots[(u * len(slots)) // npt]
            nm, t0_ = [(n_, s_) for n_, s_ in (('o', -126), ('s', 130), ('q', 386), ('n', 642)) if t_ >= s_][-1]
            pts.append((nm, (t_ - t0_) // 8 * 8))
        s = scores(q, g)
        p, li = softmax2(s, zf)
        q1 = qhalf(hval, hn, 0)
        qn = qhalf(hval, hn, 1, q1)
        vals = dict(o=o_prev, s=s, q=q1, n=qn)
        deps = []
        while len(units) > late:
            deps.append(unit([release(vals[pts[PERM[i_]][0]], pts[PERM[i_]][1]) for i_ in range(7)]))
            pts = pts[7:]
        deps = deps[-2:] + ([(o_s.at[hh - 1], 0)] if o_prev is not None else [])
        if deps:
            p = pin(p, {(24 if late else A0_DUE): fence(deps)})
        o = pv(p, g)
        o_s[hh] = pltpu.bitcast((o * li).astype(bf16), u32)
        for u in range(late):
            unit([release(o, A0_LATE[u] + 16 * PERM[i_]) for i_ in range(7)])
        return qn, o

    cp_c().start()
    cp_x(0).start()
    for j in range(2 * CPV):
        cp_mod(j).start()
    cp_wq(0).start()
    cp_k(0).start()
    cp_v(0).start()
    cp_wq(1).start()
    cp_wq(2).start()
    cp_wq(3, 2).start()
    for j in range(NA):
        h0 = P0 + j * G0
        cp_wq(h0 + 1, G0 if j + 1 < NA else G0 - 1).start()
        if h0 % rep == 0:
            cp_k(h0 // rep).start()
            cp_v(h0 // rep).start()
    cp_x(1).start()
    cp_wr().start()
    for j in range(NO):
        cp_wo(j).start()
        for u in range(CPV):
            if (j + 2) * CPV + u - MSH >= 2 * CPV:
                cp_mod((j + 2) * CPV + u - MSH).start()
    for u in range(NMC - MSH, NMC):
        cp_mod(u).start()
    for t in range(2, nt):
        cp_x(t).start()

    zero_s[0] = 0
    for n in range(NB):
        acc_s[0, n] = jnp.zeros((TQ, 128), f32)
    hs_s[0] = jnp.zeros((QT, KQ), bf16)
    best_r[...] = jnp.full(best_r.shape, -jnp.inf, f32)
    best_i[...] = jnp.zeros(best_i.shape, jnp.int32)
    cp_c().wait()
    cp_x(0).wait()
    cf = c_s[...].astype(f32)
    sc_s[...] = jnp.broadcast_to(cf * jax.nn.sigmoid(cf), (16, D)).astype(bf16)
    xn0 = _ln(xrows(0, pl.ds(0, TQ), TQ))

    def mod_body(j, carry):
        cp_mod(j).wait()
        mraw_s[j] = jnp.dot(sc_s[...], wmod_s[j], preferred_element_type=f32)[0:8, :]
        return carry

    lax.fori_loop(0, 2 * CPV, mod_body, 0)
    mod_s[:, 0:D] = mraw(0) * qscale
    mod_s[:, D:2 * D] = (1.0 + mraw(1)) * qscale
    h_s[...] = (xn0 * mvec(1) + mvec(0)).reshape(TQ, D).astype(bf16)
    cp_wq(0).wait()
    hval0 = h_s[...]
    q = qhalf(hval0, 0, 1, qhalf(hval0, 0, 0))
    cp_k(0).wait()
    cp_v(0).wait()
    NU = KQ // 16
    NPE = NU - NA
    sch0 = sched()
    cp_wq(1).wait()
    q, _ = head0(hval0, q, 0, None, [], 0, *sch0)
    cp_wq(2).wait()
    q, _ = head0(hval0, q, 1, None, [], 0, *sch0)
    cp_wq(3, 2).wait()
    u0 = [(wq_s, wqc_s.at[0], u * 16) for u in range(NPE)]
    q, o = head0(hval0, q, 2, None, u0[:3], 0, *sch0)
    q, _ = head0(hval0, q, 3, o, u0[3:], 2, *sch0)
    q_s[...] = q

    def a0_body(j, carry):
        h0 = P0 + j * G0

        @pl.when(j + 1 < NA)
        def _():
            cp_wq(h0 + 1, G0).wait()

        @pl.when(j + 1 == NA)
        def _():
            cp_wq(HQ - G0 + 1, G0 - 1).wait()

        @pl.when(h0 % rep == 0)
        def _():
            cp_k(h0 // rep).wait()
            cp_v(h0 // rep).wait()

        fence, release, zf = sched()
        sv = wq_s.at[:, pl.ds(al(h0 * DH, 4 * DH), 4 * DH)]
        dv = wqc_s.at[j + 1]
        units = [(sv, dv, u * 16) for u in range(NU)] + [(wq_s, wqc_s.at[0], (NPE + j) * 16)]
        hval = h_s[...]
        q = q_s[...]
        o = None
        for u in range(G0):
            mine = [units.pop(0) for _ in range(A0_CNT[u])]
            q, o = head0(hval, q, h0 + u, o, mine, 2 if u == G0 - 1 else 0, fence, release, zf)
        assert not units
        q_s[...] = q
        return carry

    lax.fori_loop(0, NA, a0_body, 0)
    cp_x(1).wait()
    cp_wr().wait()

    def o0_body(j, carry):
        cp_wo(j).wait()
        for u in range(CPV):
            if u >= MSH:
                cp_mod((j + 2) * CPV + u - MSH).wait()
            else:
                @pl.when(j > 0)
                def _():
                    cp_mod((j + 2) * CPV + u - MSH).wait()

        fence, release, zf = sched()
        sc = sc_s[...]
        hq = KP // DH
        wo_j = wo_s.at[pl.ds(al(j * D, D), D)]
        o_j = o_s.at[pl.ds(j * (D // DH), D // DH)]
        wm_j = wmod_s.at[pl.ds((j + 2) * CPV - MSH, CPV)]
        mr_j = mraw_s.at[pl.ds((j + 2) * CPV - MSH, CPV)]
        units = [(qd, ng, u) for qd in range(2) for ng in range(2) for u in range(DH // 16)]
        npass = NB * (D // KP)
        cnt = 0
        due = {}
        hist = []
        lhs2 = [jnp.concatenate([o_j[kh * hq + u] for u in range(hq)], axis=1) for kh in range(D // KP)]
        for n in range(NB):
            acc = acc_s[0, n]
            cu, cn = divmod(n, MC // 128)
            mv = None
            for kh in range(D // KP):
                lhs = lhs2[kh]
                acc = jnp.dot(pltpu.bitcast(pin(lhs, due.pop(cnt, None)), bf16),
                              wo_j[kh * KP:(kh + 1) * KP, n * 128:(n + 1) * 128],
                              preferred_element_type=f32) + acc
                hist.append(acc)
                mine = units[cnt * len(units) // npass:(cnt + 1) * len(units) // npass]
                for n_, (qd, ng, u) in enumerate(mine):
                    last = w_unit(wo_j, [(4 * qd + c) * DH + u * 16 for c in range(4)], ng * 512,
                                  woc_s.at[j, ng], qd * DH + u * 16, [release(acc, O0_ROWS[n_][PERM[i_]]) for i_ in range(7)])
                if cnt + 2 < npass:
                    due.setdefault(cnt + 2, {})[2] = fence([last])
                if cnt in O0_LN:
                    qr = O0_LN.index(cnt)
                    ln1(1, qr * QT + j * 16, 16, None if cnt == 0 else release(hist[-2], 24))
                    due.setdefault(cnt + 2, {})[12] = fence([(hf_s, qr * QT + j * 16)])
                if cnt in O0_HS:
                    h_slice(j * 16 + O0_HS.index(cnt) * 8, [release(hv_, O0_HSROW) for hv_ in hist[-3:]])
                    if cnt == O0_HS[0]:
                        due.setdefault(cnt + 2, {})[10] = fence([(hs_s.at[0], j * 16)])
                cnt += 1
                d = jnp.dot(sc[:, kh * KP:(kh + 1) * KP],
                            wm_j[cu, kh * KP:(kh + 1) * KP, cn * 128:(cn + 1) * 128],
                            preferred_element_type=f32)
                mv = d if mv is None else d + mv
            acc_s[0, n] = acc
            mr_j[cu, :, cn * 128:(cn + 1) * 128] = mv[0:8, :]
        assert not due
        return carry

    lax.fori_loop(0, NO, o0_body, 0)

    for u in range(NMC - MSH, NMC):
        cp_mod(u).wait()
    for u in range(NMC - MSH, NMC):
        mraw_s[u] = jnp.dot(sc_s[...], wmod_s[u], preferred_element_type=f32)[0:8, :]
    mod_s[:, 2 * D:3 * D] = mraw(2)
    mod_s[:, 3 * D:4 * D] = mraw(3)
    mod_s[:, 4 * D:5 * D] = 1.0 + mraw(4)
    mod_s[:, 5 * D:6 * D] = mraw(5)
    mod_s[:, 6 * D:7 * D] = jnp.broadcast_to(wr_s[...].astype(f32).reshape(1, D), (8, D))
    cp_wg().start()
    for u in range(F // MC):
        cp_wu(u).start()
    cp_wd().start()

    def step(t, carry):
        @pl.when(t + 1 < nt)
        def _():
            cp_x(t + 1).wait()

        @pl.when(t + 1 == nt)
        def _():
            cp_wg().wait()
            for u in range(F // MC):
                cp_wu(u).wait()
            cp_wd().wait()

        fence, release, zf = sched()
        tprev, tnext = t - 1, jnp.minimum(t + 1, nt - 1)
        prods = [(i1, i2) for i1 in _ORDER for i2 in _ORDER]
        hv = [hs_s[u] for u in range(49)]

        qblk = {}

        def q_passes(g):
            def emit(r1, r2, n1, n2, c):
                for z in range(2):
                    qblk[8 * g + 4 * z + 2 * n1 + n2, 2 * r1 + r2] = c[:, z * DH:(z + 1) * DH]
            asm = _Assemble(emit)

            def run(i1, i2):
                u = 7 * i2 + i1
                w = jnp.concatenate([wqc_s[2 * g + z, u] for z in range(2)], axis=1)
                d = jnp.dot(hv[u], w, preferred_element_type=f32)
                ini = asm.init(i1, i2)
                if ini is not None:
                    d = d + ini
                asm.add(i1, i2, d)
                return d
            return [functools.partial(run, i1, i2) for i1, i2 in prods]

        def q_head(hh):
            return jnp.concatenate([qblk.pop((hh, r)) for r in range(4)], axis=0)

        def o_passes():
            ms = {}
            asm = []
            for ng in range(2):
                def emit(r1, r2, n1, n2, c, ng=ng):
                    acc_s[t, 4 * ng + 2 * n1 + n2, pl.ds(r1 * HT + r2 * QT, QT), :] = c
                asm.append(_Assemble(emit))

            def run(ng, i1, i2, k, dep=None):
                u = 7 * i2 + i1
                lhs = jnp.concatenate([os_s[u, 4 * k + v] for v in range(4)], axis=1)
                w = jnp.concatenate([woc_s[2 * k + v, ng, u] for v in range(2)], axis=0)
                d = jnp.dot(lhs, pin_bf16(w, dep), preferred_element_type=f32)
                early = ng == 0 or (i1, i2) in prods[:NE]
                if k == 1:
                    d = d + ms.pop((ng, u))
                if k == (1 if early else 0):
                    ini = asm[ng].init(i1, i2)
                    if ini is not None:
                        d = d + ini
                if k == 0:
                    ms[ng, u] = d
                else:
                    asm[ng].add(i1, i2, d)
                return d
            NE = 16
            seq = [(0,) + pr + (0,) for pr in prods] + [(1,) + pr + (0,) for pr in prods[:NE]]
            seq += [(0,) + pr + (1,) for pr in prods] + [(1,) + pr + (1,) for pr in prods[:NE]]
            seq += [(1,) + pr + (k,) for pr in prods[NE:] for k in range(2)]
            return [functools.partial(run, *a) for a in seq]

        def side(hp, pts):
            rel = [release(v_, rw) for v_, rw in pts]
            for u in range(2):
                epi_rows(tprev, (2 * hp + u) * CHE, CHE, rel[u])
            ln1(tnext, hp * 16, 16, rel[2])
            return fence([(out_s.at[tprev], 0), (best_r, 0), (stat_s.at[tprev, 0], 0), (hf_s, 0)])

        def o_slice(qd, oq, u, pts):
            blk = [[[[oq[k1][k2][r1 * HT + r2 * QT + 16 * u:r1 * HT + r2 * QT + 16 * u + 16]
                      for k2 in range(2)] for k1 in range(2)] for r2 in range(2)] for r1 in range(2)]
            ops = _two_level(_lhs_sums, blk, [jnp.tile(release(v_, rw), (2, 1)) for v_, rw in pts])
            for v in range(7):
                os_s[7 * v:7 * v + 7, qd, 16 * u:16 * u + 16, :] = ops[v]
            return fence([(os_s.at[0, qd], 16 * u)])

        assert 2 * HP * CHE == TQ
        for fn in q_passes(0):
            fn()
        opl = o_passes()
        oq = fo = ob_ = None
        for hp in range(HP):
            g, pp = divmod(hp, 4)
            if pp == 0:
                fill = q_passes(g + 1) if g + 1 < HKV else opl
            qa, qb = q_head(2 * hp), q_head(2 * hp + 1)
            sa_ = scores(qa if fo is None else pin(qa, {0: fo}), g)
            pa, la = softmax2(sa_, zf)
            vals = {'s': sa_, 'ob': ob_}
            if oq is not None:
                fl = [o_slice(hp // 2 - 1, oq, 2 * (hp % 2) + u, [(vals[nm], rw) for nm, rw in OS_PTS[u]])
                      for u in range(2 if FILL[pp][1] < 7 else 1)]
                qb = pin(qb, {0: functools.reduce(lambda a_, b_: a_ | b_, fl)})
            rs_ = [fill.pop(0)() for _ in range(FILL[pp][0])]
            vals.update({i_: rs_[max(len(rs_) - 6 + i_, 0)] for i_ in range(6)})
            fs = side(hp, [(vals[nm] if vals[nm] is not None else sa_, rw) for nm, rw in SIDE_PTS])
            pb, lb = softmax2(scores(qb, g), zf)
            oa_ = pv(pa, g)
            oa = oa_ * la
            rs_ = [fill.pop(0)() for _ in range(FILL[pp][1])]
            fo = None
            if oq is not None and FILL[pp][1] >= 7:
                vals = {'oa': oa_}
                vals.update(enumerate(rs_))
                fo = o_slice(hp // 2 - 1, oq, 2 * (hp % 2) + 1, [(vals[nm], rw) for nm, rw in OS_F2])
            ob_ = pv(pin(pb, {0: fs}), g)
            ob = ob_ * lb
            if hp % 2 == 0:
                oprev = (oa, ob)
            else:
                oq = [oprev, (oa, ob)]

        pts = []
        due = {} if fo is None else {2: fo}
        for s, fn in enumerate(opl):
            pts.append((fn(due.pop(s, None)), 0))
            if len(pts) % 3 == 0 and len(pts) <= 12:
                o_slice(HP // 2 - 1, oq, len(pts) // 3 - 1, pts[-3:])
            u, rem = divmod(s - HS0, HSG)
            if rem == 0 and 0 <= u < QT // 8:
                h_slice(u * 8, [release(pts[-1 - HSS * i_][0]) for i_ in range(7)])
                due[s + 6] = fence([(hs_s.at[0], 0)])
        assert not due
        cp_out(tprev).start()
        return carry

    lax.fori_loop(1, nt, step, 0)

    epi_rows(nt - 1, 0, TQ)
    cp_out(nt - 1).start()
    bv = best_r[...]
    rbest = jnp.max(bv, axis=0, keepdims=True)
    ibest = jnp.min(jnp.where(bv == rbest, best_i[...], S), axis=0, keepdims=True)
    idx = jnp.minimum(ibest[0, 0], S - 1)
    base = pl.multiple_of((idx // 16) * 16, 16)
    tb = idx // TQ
    bsl = pl.ds(pl.multiple_of(base - tb * TQ, 16), 16)
    x1 = resid(tb, bsl, 16)
    h2 = h2_from_stats(x1, tb, bsl, 16)
    xs = h2.reshape(16, D).astype(bf16)
    gt = jnp.dot(xs, wq_s[:, 0:F], preferred_element_type=f32)
    up = jnp.concatenate([jnp.dot(xs, wmod_s[u], preferred_element_type=f32) for u in range(F // MC)], axis=1)
    a = (gt * jax.nn.sigmoid(gt) * up).astype(bf16)
    y = jnp.dot(a, wo_s[0:F, 0:D], preferred_element_type=f32)
    y = y * jnp.tile(jax.nn.sigmoid(rbest), (1, NB))
    rr = lax.broadcasted_iota(jnp.int32, (16, D), 0) + base
    upd = jnp.where(rr == idx, y, 0.0).reshape(2, 8, D)
    new = (x1 + mvec(5) * (h2 + upd)).reshape(16, D)
    for t in range(nt):
        cp_out(t).wait()
    out_s[tb, bsl, :] = new.astype(out_s.dtype)
    fix = pltpu.make_async_copy(out_s.at[tb, bsl, :], out_hbm.at[pl.ds(base, 16), :], osems.at[0])
    fix.start()
    fix.wait()


def _compiler_params():
    kw = dict(vmem_limit_bytes=124 * 1024 * 1024)
    try:
        return pltpu.CompilerParams(disable_semaphore_checks=True, disable_bounds_checks=True, **kw)
    except TypeError:
        return pltpu.CompilerParams(**kw)


@jax.jit
def pallas_adaLN_cond__sliding_block_cached__moe_arch_mod__prompt_kernel(
    A_x: jax.Array,
    A_k_cache: jax.Array,
    A_v_cache: jax.Array,
    A_wq: jax.Array,
    A_wo: jax.Array,
    B_x: jax.Array,
    B_w_r: jax.Array,
    B_w_gate: jax.Array,
    B_w_up: jax.Array,
    B_w_down: jax.Array,
    c: jax.Array,
    w_mod: jax.Array,
):
    B, S, D = A_x.shape
    assert B == 1
    HKV, SK = A_k_cache.shape[1], A_k_cache.shape[2]
    W = min(4096, max(256, SK // 4))
    F = B_w_gate.shape[1]
    dt = A_x.dtype
    f32 = jnp.float32
    nt = S // TQ
    NB = D // 128
    NMC = 6 * D // MC
    x2 = A_x.reshape(S, D)
    anyspec = pl.BlockSpec(memory_space=pl.ANY)
    kern = functools.partial(_kernel, S=S, D=D, HKV=HKV, SK=SK, W=W, F=F)
    out = pl.pallas_call(
        kern,
        in_specs=[anyspec] * 11,
        out_specs=anyspec,
        out_shape=jax.ShapeDtypeStruct((S, D), dt),
        scratch_shapes=[
            pltpu.VMEM((D,), dt),
            pltpu.VMEM((1, D), dt),
            pltpu.VMEM((nt, TQ, D), dt),
            pltpu.VMEM((HKV, W, DH), dt),
            pltpu.VMEM((HKV, W, DH), dt),
            pltpu.VMEM((D, HQ * DH + PAD), dt),
            pltpu.VMEM((HQ * DH, D + PAD), dt),
            pltpu.VMEM((NMC, D, MC), dt),
            pltpu.VMEM((nt, TQ, D), dt),
            pltpu.VMEM((HQ // 4, 49, D // 4, DH), dt),
            pltpu.VMEM((HQ * DH // D, 2, 49, 2 * DH, 128), dt),
            pltpu.VMEM((TQ, D), f32),
            pltpu.VMEM((49, TQ // 4, D // 4), dt),
            pltpu.VMEM((49, HQ // 4, TQ // 4, DH), dt),
            pltpu.VMEM((16, D), dt),
            pltpu.VMEM((NMC, 8, MC), f32),
            pltpu.VMEM((8, 7 * D), f32),
            pltpu.VMEM((TQ, D), dt),
            pltpu.VMEM((TQ, DH), f32),
            pltpu.VMEM((HQ, TQ // 2, DH), jnp.uint32),
            pltpu.VMEM((nt, NB, TQ, 128), f32),
            pltpu.VMEM((nt, 2, TQ, 128), f32),
            pltpu.VMEM((8, 128), f32),
            pltpu.VMEM((8, 128), jnp.int32),
            pltpu.SMEM((1,), jnp.int32),
            pltpu.SemaphoreType.DMA((4 + NMC + HQ + 2 * HKV + HQ * DH // D + nt,)),
            pltpu.SemaphoreType.DMA((nt,)),
        ],
        compiler_params=_compiler_params(),
    )(B_w_r, c, x2, A_k_cache, A_v_cache, A_wq, A_wo, w_mod, B_w_gate, B_w_up, B_w_down)
    return out.reshape(B, S, D)
```

```python
import functools

import jax
import jax.numpy as jnp
from jax import lax
import jax.experimental.pallas as pl
import jax.experimental.pallas.tpu as pltpu

HQ = 32
DH = 128
TQ = 256
PAD = 128
P0 = 4
G0 = 4
MC = 512
CHE = 8
SIDE_PTS = ((1, 0), (2, 0), ('ob', 16))
OS_F2 = [('oa', 128), ('oa', 192), (0, 0), (1, 0), (2, 0), (3, 0), (4, 0)]
OS_PTS = ([('ob', 96 + 16 * i) for i in range(7)],
          [('ob', 208), ('ob', 224), ('ob', 240), ('s', 0), ('s', 16), ('s', 32), ('s', 48)])
A0_W = (2, 250, 394, 760, 130, 150, 370)
PERM = (3, 1, 4, 0, 5, 2, 6)
A0_DUE = 14
O0_ROWS = ((0, 16, 32, 56, 72, 88, 112), (128, 144, 168, 184, 200, 224, 240))
FILL = ((7, 7), (7, 7), (7, 7), (7, 0))
HS0, HSG, HSS = 30, 14, 2
O0_LN = (0, 2, 4, 6)
O0_HS = (11, 14)
O0_HSROW = 104
MSH = 1
EPS = 1e-5
LOG2E = 1.4426950408889634


def _ln_stats(x, rel=None):
    d = x.shape[-1]
    part = x[..., 0:128]
    for j in range(1, d // 128):
        part = part + x[..., j * 128:(j + 1) * 128]
    if rel is not None:
        part = part + rel
    m = jnp.sum(part, axis=-1, keepdims=True) * (1.0 / d)
    xc = x - m
    v = jnp.mean(xc * xc, axis=-1, keepdims=True)
    return m, xc, lax.rsqrt(v + EPS)


def _ln(x, rel=None):
    _, xc, rs = _ln_stats(x, rel)
    return xc * rs


def _recip(l):
    return pl.reciprocal(l, approx=True)


def _lhs_sums(a11, a12, a21, a22):
    return [a11 + a22, a21 + a22, a11, a22, a11 + a12, a21 - a11, a12 - a22]


def _rhs_sums(b11, b12, b21, b22):
    return [b11 + b22, b11, b12 - b22, b21 - b11, b22, b11 + b12, b21 + b22]


_ORDER = [3, 4, 0, 6, 1, 2, 5]
_BLOCK = {6: (0, 0), 1: (1, 0), 2: (0, 1), 5: (1, 1)}


def _init(i, z):
    return {0: lambda: z[3] - z[4], 6: lambda: z[0], 1: lambda: z[3], 2: lambda: z[4],
            5: lambda: z[0] - z[1] + z[2]}.get(i, lambda: None)()


def _two_level(sums, blk, rel):
    o = [[jnp.stack([blk[a1][a2][b1][b2] for a2 in range(2) for b2 in range(2)]) for b1 in range(2)]
         for a1 in range(2)]
    if rel is not None and len(rel) == 3:
        o = [[o[a1][b1] + rel[0 if a1 == b1 else 1 + a1][None] for b1 in range(2)] for a1 in range(2)]
    x = jnp.stack(sums(o[0][0], o[0][1], o[1][0], o[1][1]), axis=1)
    x = [x[u] for u in range(4)]
    if rel is not None and len(rel) == 7:
        r7 = jnp.stack(rel)
        x = [x[0] + r7, x[1], x[2], x[3] + r7]
    return [y.astype(jnp.bfloat16) for y in sums(*x)]


class _Assemble:
    def __init__(self, emit):
        self.z, self.outer, self.inj, self.emit = {}, {}, {}, emit

    def init(self, i1, i2):
        v = _init(i2, self.z)
        if i2 in _BLOCK and i1 not in (3, 4):
            self.inj[i2] = _init(i1, self.outer[i2])
            v = v + self.inj[i2]
            if i2 == 5:
                v = v + (self.inj[1] - self.inj[2])
        return v

    def add(self, i1, i2, m):
        self.z[i2] = m
        if i2 in _BLOCK:
            self.outer.setdefault(i2, {})[i1] = m
            if i1 in _BLOCK:
                (r1, n1), (r2, n2) = _BLOCK[i1], _BLOCK[i2]
                self.emit(r1, r2, n1, n2, m)


def _kernel(wr_hbm, c_hbm, x_hbm, k_hbm, v_hbm, wq_hbm, wo_hbm, wmod_hbm,
            wg_hbm, wu_hbm, wd_hbm, out_hbm,
            wr_s, c_s, x_s, k_s, v_s, wq_s, wo_s, wmod_s, out_s,
            wqc_s, woc_s, hf_s, hs_s, os_s,
            sc_s, mraw_s, mod_s, h_s, o_s, acc_s, stat_s, best_r, best_i, zero_s, sems, osems,
            *, S, D, HKV, SK, W, F):
    nt = S // TQ
    rep = HQ // HKV
    NB = D // 128
    HP = HQ // 2
    HT = TQ // 2
    QT = TQ // 4
    KH = D // 2
    KQ = D // 4
    KP = 512
    CPV = D // MC
    NMC = 6 * CPV
    NA = (HQ - P0) // G0
    NO = HQ * DH // D
    f32 = jnp.float32
    bf16 = jnp.bfloat16
    u32 = jnp.uint32
    qscale = (DH ** -0.5) * LOG2E
    assert KH == KP and rep == 8 and NB == 8 and NO == 4 and P0 == 4 and G0 == 4

    def al(v, n):
        return v if isinstance(v, int) else pl.multiple_of(v, n)

    S_C, S_WR, S_WG, S_WD, S_M = 0, 1, 2, 3, 4
    S_WQ = S_M + NMC
    S_K = S_WQ + HQ
    S_V = S_K + HKV
    S_WO = S_V + HKV
    S_X = S_WO + NO

    def cp_c():
        return pltpu.make_async_copy(c_hbm, c_s, sems.at[S_C])

    def cp_wr():
        return pltpu.make_async_copy(wr_hbm, wr_s, sems.at[S_WR])

    def cp_mod(j):
        return pltpu.make_async_copy(wmod_hbm.at[:, pl.ds(al(j * MC, MC), MC)], wmod_s.at[j], sems.at[S_M + j])

    def cp_wg():
        return pltpu.make_async_copy(wg_hbm, wq_s.at[:, pl.ds(0, F)], sems.at[S_WG])

    def cp_wu(u):
        return pltpu.make_async_copy(wu_hbm.at[:, pl.ds(u * MC, MC)], wmod_s.at[u], sems.at[S_M + u])

    def cp_wd():
        return pltpu.make_async_copy(wd_hbm, wo_s.at[pl.ds(0, F), pl.ds(0, D)], sems.at[S_WD])

    def cp_wq(h, n=1):
        sl = pl.ds(al(h * DH, DH), n * DH)
        return pltpu.make_async_copy(wq_hbm.at[:, sl], wq_s.at[:, sl], sems.at[S_WQ + h])

    def cp_k(g):
        return pltpu.make_async_copy(k_hbm.at[0, g, pl.ds(SK - W, W), :], k_s.at[g], sems.at[S_K + g])

    def cp_v(g):
        return pltpu.make_async_copy(v_hbm.at[0, g, pl.ds(SK - W, W), :], v_s.at[g], sems.at[S_V + g])

    def cp_wo(j):
        sl = pl.ds(al(j * D, D), D)
        return pltpu.make_async_copy(wo_hbm.at[sl, :], wo_s.at[sl, pl.ds(0, D)], sems.at[S_WO + j])

    def rsl(t, r0=0, n=TQ):
        return pl.ds(al(t * TQ + r0, n), n)

    def cp_x(t):
        return pltpu.make_async_copy(x_hbm.at[rsl(t), :], x_s.at[t], sems.at[S_X + t])

    def cp_out(t):
        return pltpu.make_async_copy(out_s.at[t], out_hbm.at[rsl(t), :], osems.at[t])

    def sched():
        zero = zero_s[0]
        z16 = pl.multiple_of(zero, 16)
        zvec = jnp.full((8, 128), zero, jnp.int32).astype(u32)

        def fence(deps):
            d = None
            for ref, base in deps:
                n = 16 if ref.dtype == bf16 else 8
                v = pltpu.bitcast(ref[pl.ds(pl.multiple_of(base + z16, n), n), 0:128], u32)
                d = v if d is None else d | v
            return d & zvec

        def release(acc, r0=0):
            return pltpu.bitcast(pltpu.bitcast(acc[r0:r0 + 8, 0:128], u32) & zvec, f32)

        return fence, release

    def pin(a, at):
        if not at:
            return a
        parts = []
        prev = 0
        for rb in sorted(at):
            r0 = rb * 8
            if r0 > prev:
                parts.append(a[prev:r0, :])
            if a.dtype == f32:
                blk = a[r0:r0 + 8, 0:128] + pltpu.bitcast(at[rb], f32)
            else:
                blk = a[r0:r0 + 8, 0:128] | at[rb]
            if a.shape[1] > 128:
                blk = jnp.concatenate([blk, a[r0:r0 + 8, 128:]], axis=1)
            parts.append(blk)
            prev = r0 + 8
        if prev < a.shape[0]:
            parts.append(a[prev:, :])
        return jnp.concatenate(parts, axis=0)

    def pin_bf16(w, d):
        if d is None:
            return w
        top = pltpu.bitcast(pltpu.bitcast(w[0:16], u32) | d, bf16)
        return jnp.concatenate([top, w[16:]], axis=0)

    def mvec(j):
        return mod_s[:, j * D:(j + 1) * D][None]

    def mraw(j):
        return jnp.concatenate([mraw_s[j * CPV + u] for u in range(CPV)], axis=1)

    def xrows(t, sl, n):
        return x_s[t, sl, :].astype(f32).reshape(n // 8, 8, D)

    def ln1(t, r0, n, rel=None):
        xn = _ln(xrows(t, pl.ds(al(r0, n), n), n), rel)
        hf_s[pl.ds(al(r0, n), n), :] = (xn * mvec(1) + mvec(0)).reshape(n, D)

    def h_slice(r0, rel):
        hq = [hf_s[pl.ds(al(r * QT + r0, 8), 8), :] for r in range(4)]
        blk = [[[[hq[2 * r1 + r2][:, (2 * k1 + k2) * KQ:(2 * k1 + k2 + 1) * KQ] for k2 in range(2)]
                 for k1 in range(2)] for r2 in range(2)] for r1 in range(2)]
        ops = _two_level(_lhs_sums, blk, None if rel is None else [jnp.tile(v, (1, KQ // 128)) for v in rel])
        for u in range(7):
            hs_s[7 * u:7 * u + 7, pl.ds(al(r0, 8), 8), :] = ops[u]

    def w_unit(src, rows4, c0, dst, d0, rel):
        w = [src[pl.ds(al(r, 16), 16), c0:c0 + 512].astype(f32) for r in rows4]
        blk = [[[[w[2 * k1 + k2][:, (2 * n1 + n2) * 128:(2 * n1 + n2 + 1) * 128] for n2 in range(2)]
                 for n1 in range(2)] for k2 in range(2)] for k1 in range(2)]
        ops = _two_level(_rhs_sums, blk, None if rel is None else [jnp.tile(v, (2, 1)) for v in rel])
        for u in range(7):
            dst[7 * u:7 * u + 7, pl.ds(al(d0, 16), 16), :] = ops[u]
        return (dst.at[0], d0)

    def resid(t, sl, n):
        attn = jnp.concatenate([acc_s[t, j, sl, :] for j in range(NB)], axis=1).reshape(n // 8, 8, D)
        return xrows(t, sl, n) + mvec(2) * attn

    def h2_from_stats(x1, t, sl, n):
        m = jnp.tile(stat_s[t, 0, sl, :], (1, NB)).reshape(n // 8, 8, D)
        rs = jnp.tile(stat_s[t, 1, sl, :], (1, NB)).reshape(n // 8, 8, D)
        return (x1 - m) * rs * mvec(4) + mvec(3)

    def epi_rows(t, r0, n, rel=None):
        sl = pl.ds(r0, n)
        x1 = resid(t, sl, n)
        m, xc, rs = _ln_stats(x1, rel)
        stat_s[t, 0, sl, :] = jnp.broadcast_to(m.reshape(n, 1), (n, 128))
        stat_s[t, 1, sl, :] = jnp.broadcast_to(rs.reshape(n, 1), (n, 128))
        h2 = xc * rs * mvec(4) + mvec(3)
        out_s[t, sl, :] = (x1 + mvec(5) * h2).reshape(n, D).astype(out_s.dtype)
        r = jnp.sum(h2 * mvec(6), axis=-1, keepdims=True)
        r = r.astype(bf16).astype(f32)
        bv = best_r[...]
        bi = best_i[...]
        sub = lax.broadcasted_iota(jnp.int32, (8, 128), 0)
        for u in range(n // 8):
            ru = jnp.broadcast_to(r[u], (8, 128))
            better = ru > bv
            bv = jnp.where(better, ru, bv)
            bi = jnp.where(better, sub + (t * TQ + r0 + u * 8), bi)
        best_r[...] = bv
        best_i[...] = bi

    def scores(q, g):
        return lax.dot_general(q.astype(bf16), k_s[g], (((1,), (1,)), ((), ())), preferred_element_type=f32)

    def softmax(s):
        m = jnp.max(s, axis=-1, keepdims=True)
        p = jnp.exp2(s - m)
        part = p[:, 0:128]
        for j in range(1, W // 128):
            part = part + p[:, j * 128:(j + 1) * 128]
        p = jnp.concatenate([jnp.minimum(p[:, 0:128], part), p[:, 128:]], axis=1)
        return p, _recip(jnp.sum(part, axis=-1, keepdims=True))

    def pv(p, g):
        return jnp.dot(p.astype(bf16), v_s[g], preferred_element_type=f32)

    def block0(wv, c0, h0, nh, units):
        fence, release = sched()
        hval = h_s[...]
        g = h0 // rep
        tqk = [512 + 1024 * u for u in range(nh)]
        tpv = [tqk[u] + (768 if u + 1 < nh else 256) for u in range(nh)]
        wins = [(130, tqk[0])]
        for u in range(nh):
            wins.append((tqk[u] + A0_W[0], tqk[u] + (A0_W[1] if u + 1 < nh else A0_W[4])))
            if u + 1 < nh:
                wins.append((tqk[u] + A0_W[2], tqk[u] + A0_W[3]))
        wins.append((tpv[-1] + A0_W[5], tpv[-1] + A0_W[6]))
        slots = [t_ for a_, b_ in wins for t_ in range(a_, b_, 8)]
        npt = 7 * len(units)
        times = [slots[(u * len(slots)) // npt] for u in range(npt)]
        todo = [(un, times[7 * u:7 * u + 7]) for u, un in enumerate(units)]
        vals = []

        def emit(tmax):
            last = []
            while todo and todo[0][1][-1] < tmax:
                (sv, dv, r0), ts = todo.pop(0)
                rel = []
                for i_ in range(7):
                    t0_, v_ = [tv for tv in vals if tv[0] <= ts[PERM[i_]]][-1]
                    rel.append(release(v_, min((ts[PERM[i_]] - t0_) // 8 * 8, TQ - 8)))
                last = last[-1:] + [w_unit(sv, [c * KQ + r0 for c in range(4)], 0, dv, r0, rel)]
            return last

        def qproj(u, t_):
            cols = slice(c0 + u * DH, c0 + (u + 1) * DH)
            q1 = jnp.dot(hval[:, 0:KH], wv[0:KH, cols], preferred_element_type=f32)
            q2 = jnp.dot(hval[:, KH:D], wv[KH:D, cols], preferred_element_type=f32) + q1
            vals.extend([(t_ + 130, q1), (t_ + 386, q2)])
            return q2

        q = qproj(0, 0)
        for u in range(nh):
            s = scores(q, g)
            vals.append((tqk[u] + 130, s))
            p, li = softmax(s)
            if u + 1 < nh:
                q = qproj(u + 1, tqk[u] + 256)
            deps = emit(tpv[u]) + ([(o_s.at[h0 + u - 1], 0)] if u > 0 else [])
            if deps:
                p = pin(p, {A0_DUE: fence(deps)})
            o = pv(p, g)
            vals.append((tpv[u] + 130, o))
            o_s[h0 + u] = pltpu.bitcast((o * li).astype(bf16), u32)
        emit(1 << 30)

    cp_c().start()
    cp_x(0).start()
    for j in range(2 * CPV):
        cp_mod(j).start()
    cp_wq(0).start()
    cp_k(0).start()
    cp_v(0).start()
    cp_wq(1, P0 - 1).start()
    for j in range(NA):
        h0 = P0 + j * G0
        cp_wq(h0, G0).start()
        if h0 % rep == 0:
            cp_k(h0 // rep).start()
            cp_v(h0 // rep).start()
    cp_x(1).start()
    cp_wr().start()
    for j in range(NO):
        cp_wo(j).start()
        for u in range(CPV):
            if (j + 2) * CPV + u - MSH >= 2 * CPV:
                cp_mod((j + 2) * CPV + u - MSH).start()
    for u in range(NMC - MSH, NMC):
        cp_mod(u).start()
    for t in range(2, nt):
        cp_x(t).start()

    zero_s[0] = 0
    for n in range(NB):
        acc_s[0, n] = jnp.zeros((TQ, 128), f32)
    hs_s[0] = jnp.zeros((QT, KQ), bf16)
    best_r[...] = jnp.full(best_r.shape, -jnp.inf, f32)
    best_i[...] = jnp.zeros(best_i.shape, jnp.int32)
    cp_c().wait()
    cp_x(0).wait()
    cf = c_s[...].astype(f32)
    sc_s[...] = jnp.broadcast_to(cf * jax.nn.sigmoid(cf), (16, D)).astype(bf16)
    xn0 = _ln(xrows(0, pl.ds(0, TQ), TQ))

    def mod_body(j, carry):
        cp_mod(j).wait()
        mraw_s[j] = jnp.dot(sc_s[...], wmod_s[j], preferred_element_type=f32)[0:8, :]
        return carry

    lax.fori_loop(0, 2 * CPV, mod_body, 0)
    mod_s[:, 0:D] = mraw(0) * qscale
    mod_s[:, D:2 * D] = (1.0 + mraw(1)) * qscale
    h_s[...] = (xn0 * mvec(1) + mvec(0)).reshape(TQ, D).astype(bf16)
    NU = KQ // 16
    NPE = NU - NA
    cp_wq(0).wait()
    cp_k(0).wait()
    cp_v(0).wait()
    block0(wq_s, 0, 0, 1, [])
    cp_wq(1, P0 - 1).wait()
    block0(wq_s, DH, 1, P0 - 1, [(wq_s, wqc_s.at[0], u * 16) for u in range(NPE)])

    def a0_body(j, carry):
        h0 = P0 + j * G0
        cp_wq(h0, G0).wait()

        @pl.when(h0 % rep == 0)
        def _():
            cp_k(h0 // rep).wait()
            cp_v(h0 // rep).wait()

        sv = wq_s.at[:, pl.ds(al(h0 * DH, 4 * DH), 4 * DH)]
        dv = wqc_s.at[j + 1]
        block0(sv, 0, h0, G0, [(sv, dv, u * 16) for u in range(NU)] + [(wq_s, wqc_s.at[0], (NPE + j) * 16)])
        return carry

    lax.fori_loop(0, NA, a0_body, 0)
    cp_x(1).wait()
    cp_wr().wait()

    def o0_body(j, carry):
        cp_wo(j).wait()
        for u in range(CPV):
            if u >= MSH:
                cp_mod((j + 2) * CPV + u - MSH).wait()
            else:
                @pl.when(j > 0)
                def _():
                    cp_mod((j + 2) * CPV + u - MSH).wait()

        fence, release = sched()
        sc = sc_s[...]
        hq = KP // DH
        wo_j = wo_s.at[pl.ds(al(j * D, D), D)]
        o_j = o_s.at[pl.ds(j * (D // DH), D // DH)]
        wm_j = wmod_s.at[pl.ds((j + 2) * CPV - MSH, CPV)]
        mr_j = mraw_s.at[pl.ds((j + 2) * CPV - MSH, CPV)]
        units = [(qd, ng, u) for qd in range(2) for ng in range(2) for u in range(DH // 16)]
        npass = NB * (D // KP)
        cnt = 0
        due = {}
        hist = []
        lhs2 = [jnp.concatenate([o_j[kh * hq + u] for u in range(hq)], axis=1) for kh in range(D // KP)]
        for n in range(NB):
            acc = acc_s[0, n]
            cu, cn = divmod(n, MC // 128)
            mv = None
            for kh in range(D // KP):
                lhs = lhs2[kh]
                acc = jnp.dot(pltpu.bitcast(pin(lhs, due.pop(cnt, None)), bf16),
                              wo_j[kh * KP:(kh + 1) * KP, n * 128:(n + 1) * 128],
                              preferred_element_type=f32) + acc
                hist.append(acc)
                mine = units[cnt * len(units) // npass:(cnt + 1) * len(units) // npass]
                for n_, (qd, ng, u) in enumerate(mine):
                    last = w_unit(wo_j, [(4 * qd + c) * DH + u * 16 for c in range(4)], ng * 512,
                                  woc_s.at[j, ng], qd * DH + u * 16, [release(acc, O0_ROWS[n_][PERM[i_]]) for i_ in range(7)])
                if cnt + 2 < npass:
                    due.setdefault(cnt + 2, {})[2] = fence([last])
                if cnt in O0_LN:
                    qr = O0_LN.index(cnt)
                    ln1(1, qr * QT + j * 16, 16, None if cnt == 0 else release(hist[-2], 24))
                    due.setdefault(cnt + 2, {})[12] = fence([(hf_s, qr * QT + j * 16)])
                if cnt in O0_HS:
                    h_slice(j * 16 + O0_HS.index(cnt) * 8, [release(hv_, O0_HSROW) for hv_ in hist[-3:]])
                    if cnt == O0_HS[0]:
                        due.setdefault(cnt + 2, {})[10] = fence([(hs_s.at[0], j * 16)])
                cnt += 1
                d = jnp.dot(sc[:, kh * KP:(kh + 1) * KP],
                            wm_j[cu, kh * KP:(kh + 1) * KP, cn * 128:(cn + 1) * 128],
                            preferred_element_type=f32)
                mv = d if mv is None else d + mv
            acc_s[0, n] = acc
            mr_j[cu, :, cn * 128:(cn + 1) * 128] = mv[0:8, :]
        assert not due
        return carry

    lax.fori_loop(0, NO, o0_body, 0)

    for u in range(NMC - MSH, NMC):
        cp_mod(u).wait()
    for u in range(NMC - MSH, NMC):
        mraw_s[u] = jnp.dot(sc_s[...], wmod_s[u], preferred_element_type=f32)[0:8, :]
    mod_s[:, 2 * D:3 * D] = mraw(2)
    mod_s[:, 3 * D:4 * D] = mraw(3)
    mod_s[:, 4 * D:5 * D] = 1.0 + mraw(4)
    mod_s[:, 5 * D:6 * D] = mraw(5)
    mod_s[:, 6 * D:7 * D] = jnp.broadcast_to(wr_s[...].astype(f32).reshape(1, D), (8, D))
    cp_wg().start()
    for u in range(F // MC):
        cp_wu(u).start()
    cp_wd().start()

    def step(t, carry):
        @pl.when(t + 1 < nt)
        def _():
            cp_x(t + 1).wait()

        @pl.when(t + 1 == nt)
        def _():
            cp_wg().wait()
            for u in range(F // MC):
                cp_wu(u).wait()
            cp_wd().wait()

        fence, release = sched()
        tprev, tnext = t - 1, jnp.minimum(t + 1, nt - 1)
        prods = [(i1, i2) for i1 in _ORDER for i2 in _ORDER]
        hv = [hs_s[u] for u in range(49)]

        qblk = {}

        def q_passes(g):
            def emit(r1, r2, n1, n2, c):
                for z in range(2):
                    qblk[8 * g + 4 * z + 2 * n1 + n2, 2 * r1 + r2] = c[:, z * DH:(z + 1) * DH]
            asm = _Assemble(emit)

            def run(i1, i2):
                u = 7 * i2 + i1
                w = jnp.concatenate([wqc_s[2 * g + z, u] for z in range(2)], axis=1)
                d = jnp.dot(hv[u], w, preferred_element_type=f32)
                ini = asm.init(i1, i2)
                if ini is not None:
                    d = d + ini
                asm.add(i1, i2, d)
                return d
            return [functools.partial(run, i1, i2) for i1, i2 in prods]

        def q_head(hh):
            return jnp.concatenate([qblk.pop((hh, r)) for r in range(4)], axis=0)

        def o_passes():
            ms = {}
            asm = []
            for ng in range(2):
                def emit(r1, r2, n1, n2, c, ng=ng):
                    acc_s[t, 4 * ng + 2 * n1 + n2, pl.ds(r1 * HT + r2 * QT, QT), :] = c
                asm.append(_Assemble(emit))

            def run(ng, i1, i2, k, dep=None):
                u = 7 * i2 + i1
                lhs = jnp.concatenate([os_s[u, 4 * k + v] for v in range(4)], axis=1)
                w = jnp.concatenate([woc_s[2 * k + v, ng, u] for v in range(2)], axis=0)
                d = jnp.dot(lhs, pin_bf16(w, dep), preferred_element_type=f32)
                early = ng == 0 or (i1, i2) in prods[:NE]
                if k == 1:
                    d = d + ms.pop((ng, u))
                if k == (1 if early else 0):
                    ini = asm[ng].init(i1, i2)
                    if ini is not None:
                        d = d + ini
                if k == 0:
                    ms[ng, u] = d
                else:
                    asm[ng].add(i1, i2, d)
                return d
            NE = 16
            seq = [(0,) + pr + (0,) for pr in prods] + [(1,) + pr + (0,) for pr in prods[:NE]]
            seq += [(0,) + pr + (1,) for pr in prods] + [(1,) + pr + (1,) for pr in prods[:NE]]
            seq += [(1,) + pr + (k,) for pr in prods[NE:] for k in range(2)]
            return [functools.partial(run, *a) for a in seq]

        def side(hp, pts):
            rel = [release(v_, rw) for v_, rw in pts]
            for u in range(2):
                epi_rows(tprev, (2 * hp + u) * CHE, CHE, rel[u])
            ln1(tnext, hp * 16, 16, rel[2])
            return fence([(out_s.at[tprev], 0), (best_r, 0), (stat_s.at[tprev, 0], 0), (hf_s, 0)])

        def o_slice(qd, oq, u, pts):
            blk = [[[[oq[k1][k2][r1 * HT + r2 * QT + 16 * u:r1 * HT + r2 * QT + 16 * u + 16]
                      for k2 in range(2)] for k1 in range(2)] for r2 in range(2)] for r1 in range(2)]
            ops = _two_level(_lhs_sums, blk, [jnp.tile(release(v_, rw), (2, 1)) for v_, rw in pts])
            for v in range(7):
                os_s[7 * v:7 * v + 7, qd, 16 * u:16 * u + 16, :] = ops[v]
            return fence([(os_s.at[0, qd], 16 * u)])

        assert 2 * HP * CHE == TQ
        for fn in q_passes(0):
            fn()
        opl = o_passes()
        oq = fo = ob_ = None
        for hp in range(HP):
            g, pp = divmod(hp, 4)
            if pp == 0:
                fill = q_passes(g + 1) if g + 1 < HKV else opl
            qa, qb = q_head(2 * hp), q_head(2 * hp + 1)
            sa_ = scores(qa if fo is None else pin(qa, {0: fo}), g)
            pa, la = softmax(sa_)
            vals = {'s': sa_, 'ob': ob_}
            if oq is not None:
                fl = [o_slice(hp // 2 - 1, oq, 2 * (hp % 2) + u, [(vals[nm], rw) for nm, rw in OS_PTS[u]])
                      for u in range(2 if FILL[pp][1] < 7 else 1)]
                qb = pin(qb, {0: functools.reduce(lambda a_, b_: a_ | b_, fl)})
            rs_ = [fill.pop(0)() for _ in range(FILL[pp][0])]
            vals.update({i_: rs_[max(len(rs_) - 6 + i_, 0)] for i_ in range(6)})
            fs = side(hp, [(vals[nm] if vals[nm] is not None else sa_, rw) for nm, rw in SIDE_PTS])
            pb, lb = softmax(scores(qb, g))
            oa_ = pv(pa, g)
            oa = oa_ * la
            rs_ = [fill.pop(0)() for _ in range(FILL[pp][1])]
            fo = None
            if oq is not None and FILL[pp][1] >= 7:
                vals = {'oa': oa_}
                vals.update(enumerate(rs_))
                fo = o_slice(hp // 2 - 1, oq, 2 * (hp % 2) + 1, [(vals[nm], rw) for nm, rw in OS_F2])
            ob_ = pv(pin(pb, {0: fs}), g)
            ob = ob_ * lb
            if hp % 2 == 0:
                oprev = (oa, ob)
            else:
                oq = [oprev, (oa, ob)]

        pts = []
        due = {} if fo is None else {2: fo}
        for s, fn in enumerate(opl):
            pts.append((fn(due.pop(s, None)), 0))
            if len(pts) % 3 == 0 and len(pts) <= 12:
                o_slice(HP // 2 - 1, oq, len(pts) // 3 - 1, pts[-3:])
            u, rem = divmod(s - HS0, HSG)
            if rem == 0 and 0 <= u < QT // 8:
                h_slice(u * 8, [release(pts[-1 - HSS * i_][0]) for i_ in range(7)])
                due[s + 6] = fence([(hs_s.at[0], 0)])
        assert not due
        cp_out(tprev).start()
        return carry

    lax.fori_loop(1, nt, step, 0)

    epi_rows(nt - 1, 0, TQ)
    cp_out(nt - 1).start()
    bv = best_r[...]
    rbest = jnp.max(bv, axis=0, keepdims=True)
    ibest = jnp.min(jnp.where(bv == rbest, best_i[...], S), axis=0, keepdims=True)
    idx = jnp.minimum(ibest[0, 0], S - 1)
    base = pl.multiple_of((idx // 16) * 16, 16)
    tb = idx // TQ
    bsl = pl.ds(pl.multiple_of(base - tb * TQ, 16), 16)
    x1 = resid(tb, bsl, 16)
    h2 = h2_from_stats(x1, tb, bsl, 16)
    xs = h2.reshape(16, D).astype(bf16)
    gt = jnp.dot(xs, wq_s[:, 0:F], preferred_element_type=f32)
    up = jnp.concatenate([jnp.dot(xs, wmod_s[u], preferred_element_type=f32) for u in range(F // MC)], axis=1)
    a = (gt * jax.nn.sigmoid(gt) * up).astype(bf16)
    y = jnp.dot(a, wo_s[0:F, 0:D], preferred_element_type=f32)
    y = y * jnp.tile(jax.nn.sigmoid(rbest), (1, NB))
    rr = lax.broadcasted_iota(jnp.int32, (16, D), 0) + base
    upd = jnp.where(rr == idx, y, 0.0).reshape(2, 8, D)
    new = (x1 + mvec(5) * (h2 + upd)).reshape(16, D)
    for t in range(nt):
        cp_out(t).wait()
    out_s[tb, bsl, :] = new.astype(out_s.dtype)
    fix = pltpu.make_async_copy(out_s.at[tb, bsl, :], out_hbm.at[pl.ds(base, 16), :], osems.at[0])
    fix.start()
    fix.wait()


def _compiler_params():
    kw = dict(vmem_limit_bytes=124 * 1024 * 1024)
    try:
        return pltpu.CompilerParams(disable_semaphore_checks=True, disable_bounds_checks=True, **kw)
    except TypeError:
        return pltpu.CompilerParams(**kw)


@jax.jit
def pallas_adaLN_cond__sliding_block_cached__moe_arch_mod__prompt_kernel(
    A_x: jax.Array,
    A_k_cache: jax.Array,
    A_v_cache: jax.Array,
    A_wq: jax.Array,
    A_wo: jax.Array,
    B_x: jax.Array,
    B_w_r: jax.Array,
    B_w_gate: jax.Array,
    B_w_up: jax.Array,
    B_w_down: jax.Array,
    c: jax.Array,
    w_mod: jax.Array,
):
    B, S, D = A_x.shape
    assert B == 1
    HKV, SK = A_k_cache.shape[1], A_k_cache.shape[2]
    W = min(4096, max(256, SK // 4))
    F = B_w_gate.shape[1]
    dt = A_x.dtype
    f32 = jnp.float32
    nt = S // TQ
    NB = D // 128
    NMC = 6 * D // MC
    x2 = A_x.reshape(S, D)
    anyspec = pl.BlockSpec(memory_space=pl.ANY)
    kern = functools.partial(_kernel, S=S, D=D, HKV=HKV, SK=SK, W=W, F=F)
    out = pl.pallas_call(
        kern,
        in_specs=[anyspec] * 11,
        out_specs=anyspec,
        out_shape=jax.ShapeDtypeStruct((S, D), dt),
        scratch_shapes=[
            pltpu.VMEM((D,), dt),
            pltpu.VMEM((1, D), dt),
            pltpu.VMEM((nt, TQ, D), dt),
            pltpu.VMEM((HKV, W, DH), dt),
            pltpu.VMEM((HKV, W, DH), dt),
            pltpu.VMEM((D, HQ * DH + PAD), dt),
            pltpu.VMEM((HQ * DH, D + PAD), dt),
            pltpu.VMEM((NMC, D, MC), dt),
            pltpu.VMEM((nt, TQ, D), dt),
            pltpu.VMEM((HQ // 4, 49, D // 4, DH), dt),
            pltpu.VMEM((HQ * DH // D, 2, 49, 2 * DH, 128), dt),
            pltpu.VMEM((TQ, D), f32),
            pltpu.VMEM((49, TQ // 4, D // 4), dt),
            pltpu.VMEM((49, HQ // 4, TQ // 4, DH), dt),
            pltpu.VMEM((16, D), dt),
            pltpu.VMEM((NMC, 8, MC), f32),
            pltpu.VMEM((8, 7 * D), f32),
            pltpu.VMEM((TQ, D), dt),
            pltpu.VMEM((HQ, TQ // 2, DH), jnp.uint32),
            pltpu.VMEM((nt, NB, TQ, 128), f32),
            pltpu.VMEM((nt, 2, TQ, 128), f32),
            pltpu.VMEM((8, 128), f32),
            pltpu.VMEM((8, 128), jnp.int32),
            pltpu.SMEM((1,), jnp.int32),
            pltpu.SemaphoreType.DMA((4 + NMC + HQ + 2 * HKV + HQ * DH // D + nt,)),
            pltpu.SemaphoreType.DMA((nt,)),
        ],
        compiler_params=_compiler_params(),
    )(B_w_r, c, x2, A_k_cache, A_v_cache, A_wq, A_wo, w_mod, B_w_gate, B_w_up, B_w_down)
    return out.reshape(B, S, D)
```

```python
import functools

import jax
import jax.numpy as jnp
from jax import lax
import jax.experimental.pallas as pl
import jax.experimental.pallas.tpu as pltpu

HQ = 32
DH = 128
TQ = 256
PAD = 128
P0 = 4
G0 = 4
MC = 512
CHE = 8
SIDE_PTS = ((1, 0), (2, 0), ('ob', 0), ('ob', 56))
OS_F2 = [('oa', 128), ('oa', 192), (0, 0), (1, 0), (2, 0), (3, 0), (4, 0)]
OS_PTS = ([('ob', 96 + 16 * i) for i in range(7)],
          [('ob', 208), ('ob', 224), ('ob', 240), ('s', 0), ('s', 16), ('s', 32), ('s', 48)])
A0_W = (2, 250, 394, 760, 130, 150, 370)
PERM = (3, 1, 4, 0, 5, 2, 6)
A0_DUE = 14
O0_ROWS = ((0, 16, 32, 56, 72, 88, 112), (128, 144, 168, 184, 200, 224, 240))
FILL = ((7, 7), (7, 7), (7, 7), (7, 0))
HS0, HSG, HSS = 30, 14, 2
O0_LN = (0, 1, 2, 3, 4, 5, 6, 7)
O0_LNROW = 24
O0_HS = (12, 15)
O0_HSROW = (8, 104, 192)
PERML = (0, 1, 2, 3, 4, 5, 6)
MSH = 1
EPS = 1e-5
LOG2E = 1.4426950408889634


def _ln_stats(x, rel=None):
    d = x.shape[-1]
    part = x[..., 0:128]
    for j in range(1, d // 128):
        part = part + x[..., j * 128:(j + 1) * 128]
    if rel is not None:
        part = part + rel
    m = jnp.sum(part, axis=-1, keepdims=True) * (1.0 / d)
    xc = x - m
    v = jnp.mean(xc * xc, axis=-1, keepdims=True)
    return m, xc, lax.rsqrt(v + EPS)


def _ln(x, rel=None):
    _, xc, rs = _ln_stats(x, rel)
    return xc * rs


def _recip(l):
    return pl.reciprocal(l, approx=True)


def _lhs_sums(a11, a12, a21, a22):
    return [a11 + a22, a21 + a22, a11, a22, a11 + a12, a21 - a11, a12 - a22]


def _rhs_sums(b11, b12, b21, b22):
    return [b11 + b22, b11, b12 - b22, b21 - b11, b22, b11 + b12, b21 + b22]


_ORDER = [3, 4, 0, 6, 1, 2, 5]
_BLOCK = {6: (0, 0), 1: (1, 0), 2: (0, 1), 5: (1, 1)}


def _init(i, z):
    return {0: lambda: z[3] - z[4], 6: lambda: z[0], 1: lambda: z[3], 2: lambda: z[4],
            5: lambda: z[0] - z[1] + z[2]}.get(i, lambda: None)()


def _two_level(sums, blk, rel):
    o = [[jnp.stack([blk[a1][a2][b1][b2] for a2 in range(2) for b2 in range(2)]) for b1 in range(2)]
         for a1 in range(2)]
    if rel is not None and len(rel) == 3:
        o = [[o[a1][b1] + rel[0 if a1 == b1 else 1 + a1][None] for b1 in range(2)] for a1 in range(2)]
    x = jnp.stack(sums(o[0][0], o[0][1], o[1][0], o[1][1]), axis=1)
    x = [x[u] for u in range(4)]
    if rel is not None and len(rel) == 7:
        r7 = jnp.stack(rel)
        x = [x[0] + r7, x[1], x[2], x[3] + r7]
    return [y.astype(jnp.bfloat16) for y in sums(*x)]


class _Assemble:
    def __init__(self, emit):
        self.z, self.outer, self.inj, self.emit = {}, {}, {}, emit

    def init(self, i1, i2):
        v = _init(i2, self.z)
        if i2 in _BLOCK and i1 not in (3, 4):
            self.inj[i2] = _init(i1, self.outer[i2])
            v = v + self.inj[i2]
            if i2 == 5:
                v = v + (self.inj[1] - self.inj[2])
        return v

    def add(self, i1, i2, m):
        self.z[i2] = m
        if i2 in _BLOCK:
            self.outer.setdefault(i2, {})[i1] = m
            if i1 in _BLOCK:
                (r1, n1), (r2, n2) = _BLOCK[i1], _BLOCK[i2]
                self.emit(r1, r2, n1, n2, m)


def _kernel(wr_hbm, c_hbm, x_hbm, k_hbm, v_hbm, wq_hbm, wo_hbm, wmod_hbm,
            wg_hbm, wu_hbm, wd_hbm, out_hbm,
            wr_s, c_s, x_s, k_s, v_s, wq_s, wo_s, wmod_s, out_s,
            wqc_s, woc_s, hf_s, hs_s, os_s,
            sc_s, mraw_s, mod_s, h_s, o_s, acc_s, stat_s, best_r, best_i, zero_s, sems, osems,
            *, S, D, HKV, SK, W, F):
    nt = S // TQ
    rep = HQ // HKV
    NB = D // 128
    HP = HQ // 2
    HT = TQ // 2
    QT = TQ // 4
    KH = D // 2
    KQ = D // 4
    KP = 512
    CPV = D // MC
    NMC = 6 * CPV
    NA = (HQ - P0) // G0
    NO = HQ * DH // D
    f32 = jnp.float32
    bf16 = jnp.bfloat16
    u32 = jnp.uint32
    qscale = (DH ** -0.5) * LOG2E
    assert KH == KP and rep == 8 and NB == 8 and NO == 4 and P0 == 4 and G0 == 4

    def al(v, n):
        return v if isinstance(v, int) else pl.multiple_of(v, n)

    S_C, S_WR, S_WG, S_WD, S_M = 0, 1, 2, 3, 4
    S_WQ = S_M + NMC
    S_K = S_WQ + HQ
    S_V = S_K + HKV
    S_WO = S_V + HKV
    S_X = S_WO + NO

    def cp_c():
        return pltpu.make_async_copy(c_hbm, c_s, sems.at[S_C])

    def cp_wr():
        return pltpu.make_async_copy(wr_hbm, wr_s, sems.at[S_WR])

    def cp_mod(j):
        return pltpu.make_async_copy(wmod_hbm.at[:, pl.ds(al(j * MC, MC), MC)], wmod_s.at[j], sems.at[S_M + j])

    def cp_wg():
        return pltpu.make_async_copy(wg_hbm, wq_s.at[:, pl.ds(0, F)], sems.at[S_WG])

    def cp_wu(u):
        return pltpu.make_async_copy(wu_hbm.at[:, pl.ds(u * MC, MC)], wmod_s.at[u], sems.at[S_M + u])

    def cp_wd():
        return pltpu.make_async_copy(wd_hbm, wo_s.at[pl.ds(0, F), pl.ds(0, D)], sems.at[S_WD])

    def cp_wq(h, n=1):
        sl = pl.ds(al(h * DH, DH), n * DH)
        return pltpu.make_async_copy(wq_hbm.at[:, sl], wq_s.at[:, sl], sems.at[S_WQ + h])

    def cp_k(g):
        return pltpu.make_async_copy(k_hbm.at[0, g, pl.ds(SK - W, W), :], k_s.at[g], sems.at[S_K + g])

    def cp_v(g):
        return pltpu.make_async_copy(v_hbm.at[0, g, pl.ds(SK - W, W), :], v_s.at[g], sems.at[S_V + g])

    def cp_wo(j):
        sl = pl.ds(al(j * D, D), D)
        return pltpu.make_async_copy(wo_hbm.at[sl, :], wo_s.at[sl, pl.ds(0, D)], sems.at[S_WO + j])

    def rsl(t, r0=0, n=TQ):
        return pl.ds(al(t * TQ + r0, n), n)

    def cp_x(t):
        return pltpu.make_async_copy(x_hbm.at[rsl(t), :], x_s.at[t], sems.at[S_X + t])

    def cp_out(t):
        return pltpu.make_async_copy(out_s.at[t], out_hbm.at[rsl(t), :], osems.at[t])

    def sched():
        zero = zero_s[0]
        z16 = pl.multiple_of(zero, 16)
        zvec = jnp.full((8, 128), zero, jnp.int32).astype(u32)

        def fence(deps):
            d = None
            for ref, base in deps:
                n = 16 if ref.dtype == bf16 else 8
                v = pltpu.bitcast(ref[pl.ds(pl.multiple_of(base + z16, n), n), 0:128], u32)
                d = v if d is None else d | v
            return d & zvec

        def release(acc, r0=0):
            return pltpu.bitcast(pltpu.bitcast(acc[r0:r0 + 8, 0:128], u32) & zvec, f32)

        return fence, release

    def pin(a, at):
        if not at:
            return a
        parts = []
        prev = 0
        for rb in sorted(at):
            r0 = rb * 8
            if r0 > prev:
                parts.append(a[prev:r0, :])
            if a.dtype == f32:
                blk = a[r0:r0 + 8, 0:128] + pltpu.bitcast(at[rb], f32)
            else:
                blk = a[r0:r0 + 8, 0:128] | at[rb]
            if a.shape[1] > 128:
                blk = jnp.concatenate([blk, a[r0:r0 + 8, 128:]], axis=1)
            parts.append(blk)
            prev = r0 + 8
        if prev < a.shape[0]:
            parts.append(a[prev:, :])
        return jnp.concatenate(parts, axis=0)

    def pin_bf16(w, d):
        if d is None:
            return w
        top = pltpu.bitcast(pltpu.bitcast(w[0:16], u32) | d, bf16)
        return jnp.concatenate([top, w[16:]], axis=0)

    def mvec(j):
        return mod_s[:, j * D:(j + 1) * D][None]

    def mraw(j):
        return jnp.concatenate([mraw_s[j * CPV + u] for u in range(CPV)], axis=1)

    def xrows(t, sl, n):
        return x_s[t, sl, :].astype(f32).reshape(n // 8, 8, D)

    def ln1(t, r0, n, rel=None):
        xn = _ln(xrows(t, pl.ds(al(r0, n), n), n), rel)
        hf_s[pl.ds(al(r0, n), n), :] = (xn * mvec(1) + mvec(0)).reshape(n, D)

    def h_slice(r0, rel):
        hq = [hf_s[pl.ds(al(r * QT + r0, 8), 8), :] for r in range(4)]
        blk = [[[[hq[2 * r1 + r2][:, (2 * k1 + k2) * KQ:(2 * k1 + k2 + 1) * KQ] for k2 in range(2)]
                 for k1 in range(2)] for r2 in range(2)] for r1 in range(2)]
        ops = _two_level(_lhs_sums, blk, None if rel is None else [jnp.tile(v, (1, KQ // 128)) for v in rel])
        for u in range(7):
            hs_s[7 * u:7 * u + 7, pl.ds(al(r0, 8), 8), :] = ops[u]

    def w_unit(src, rows4, c0, dst, d0, rel):
        w = [src[pl.ds(al(r, 16), 16), c0:c0 + 512].astype(f32) for r in rows4]
        blk = [[[[w[2 * k1 + k2][:, (2 * n1 + n2) * 128:(2 * n1 + n2 + 1) * 128] for n2 in range(2)]
                 for n1 in range(2)] for k2 in range(2)] for k1 in range(2)]
        ops = _two_level(_rhs_sums, blk, None if rel is None else [jnp.tile(v, (2, 1)) for v in rel])
        for u in range(7):
            dst[7 * u:7 * u + 7, pl.ds(al(d0, 16), 16), :] = ops[u]
        return (dst.at[0], d0)

    def resid(t, sl, n):
        attn = jnp.concatenate([acc_s[t, j, sl, :] for j in range(NB)], axis=1).reshape(n // 8, 8, D)
        return xrows(t, sl, n) + mvec(2) * attn

    def h2_from_stats(x1, t, sl, n):
        m = jnp.tile(stat_s[t, 0, sl, :], (1, NB)).reshape(n // 8, 8, D)
        rs = jnp.tile(stat_s[t, 1, sl, :], (1, NB)).reshape(n // 8, 8, D)
        return (x1 - m) * rs * mvec(4) + mvec(3)

    def epi_rows(t, r0, n, rel=None):
        sl = pl.ds(r0, n)
        x1 = resid(t, sl, n)
        m, xc, rs = _ln_stats(x1, rel)
        stat_s[t, 0, sl, :] = jnp.broadcast_to(m.reshape(n, 1), (n, 128))
        stat_s[t, 1, sl, :] = jnp.broadcast_to(rs.reshape(n, 1), (n, 128))
        h2 = xc * rs * mvec(4) + mvec(3)
        out_s[t, sl, :] = (x1 + mvec(5) * h2).reshape(n, D).astype(out_s.dtype)
        r = jnp.sum(h2 * mvec(6), axis=-1, keepdims=True)
        r = r.astype(bf16).astype(f32)
        bv = best_r[...]
        bi = best_i[...]
        sub = lax.broadcasted_iota(jnp.int32, (8, 128), 0)
        for u in range(n // 8):
            ru = jnp.broadcast_to(r[u], (8, 128))
            better = ru > bv
            bv = jnp.where(better, ru, bv)
            bi = jnp.where(better, sub + (t * TQ + r0 + u * 8), bi)
        best_r[...] = bv
        best_i[...] = bi

    def scores(q, g):
        return lax.dot_general(q.astype(bf16), k_s[g], (((1,), (1,)), ((), ())), preferred_element_type=f32)

    def softmax(s):
        m = jnp.max(s, axis=-1, keepdims=True)
        p = jnp.exp2(s - m)
        part = p[:, 0:128]
        for j in range(1, W // 128):
            part = part + p[:, j * 128:(j + 1) * 128]
        p = jnp.concatenate([jnp.minimum(p[:, 0:128], part), p[:, 128:]], axis=1)
        return p, _recip(jnp.sum(part, axis=-1, keepdims=True))

    def pv(p, g):
        return jnp.dot(p.astype(bf16), v_s[g], preferred_element_type=f32)

    def block0(wv, c0, h0, nh, units):
        fence, release = sched()
        hval = h_s[...]
        g = h0 // rep
        tqk = [512 + 1024 * u for u in range(nh)]
        tpv = [tqk[u] + (768 if u + 1 < nh else 256) for u in range(nh)]
        wins = [(130, tqk[0])]
        for u in range(nh):
            wins.append((tqk[u] + A0_W[0], tqk[u] + (A0_W[1] if u + 1 < nh else A0_W[4])))
            if u + 1 < nh:
                wins.append((tqk[u] + A0_W[2], tqk[u] + A0_W[3]))
        wins.append((tpv[-1] + A0_W[5], tpv[-1] + A0_W[6]))
        slots = [t_ for a_, b_ in wins for t_ in range(a_, b_, 8)]
        npt = 7 * len(units)
        times = [slots[(u * len(slots)) // npt] for u in range(npt)]
        todo = [(un, times[7 * u:7 * u + 7]) for u, un in enumerate(units)]
        vals = []

        def emit(tmax):
            last = []
            while todo and todo[0][1][-1] < tmax:
                (sv, dv, r0), ts = todo.pop(0)
                rel = []
                for i_ in range(7):
                    t0_, v_ = [tv for tv in vals if tv[0] <= ts[PERM[i_]]][-1]
                    rel.append(release(v_, min((ts[PERM[i_]] - t0_) // 8 * 8, TQ - 8)))
                last = last[-1:] + [w_unit(sv, [c * KQ + r0 for c in range(4)], 0, dv, r0, rel)]
            return last

        def qproj(u, t_):
            cols = slice(c0 + u * DH, c0 + (u + 1) * DH)
            q1 = jnp.dot(hval[:, 0:KH], wv[0:KH, cols], preferred_element_type=f32)
            q2 = jnp.dot(hval[:, KH:D], wv[KH:D, cols], preferred_element_type=f32) + q1
            vals.extend([(t_ + 130, q1), (t_ + 386, q2)])
            return q2

        q = qproj(0, 0)
        for u in range(nh):
            s = scores(q, g)
            vals.append((tqk[u] + 130, s))
            p, li = softmax(s)
            if u + 1 < nh:
                q = qproj(u + 1, tqk[u] + 256)
            deps = emit(tpv[u]) + ([(o_s.at[h0 + u - 1], 0)] if u > 0 else [])
            if deps:
                p = pin(p, {A0_DUE: fence(deps)})
            o = pv(p, g)
            vals.append((tpv[u] + 130, o))
            o_s[h0 + u] = pltpu.bitcast((o * li).astype(bf16), u32)
        emit(1 << 30)

    cp_c().start()
    cp_x(0).start()
    for j in range(2 * CPV):
        cp_mod(j).start()
    cp_wq(0).start()
    cp_k(0).start()
    cp_v(0).start()
    cp_wq(1, P0 - 1).start()
    for j in range(NA):
        h0 = P0 + j * G0
        cp_wq(h0, G0).start()
        if h0 % rep == 0:
            cp_k(h0 // rep).start()
            cp_v(h0 // rep).start()
    cp_x(1).start()
    cp_wr().start()
    for j in range(NO):
        cp_wo(j).start()
        for u in range(CPV):
            if (j + 2) * CPV + u - MSH >= 2 * CPV:
                cp_mod((j + 2) * CPV + u - MSH).start()
    for u in range(NMC - MSH, NMC):
        cp_mod(u).start()
    for t in range(2, nt):
        cp_x(t).start()

    zero_s[0] = 0
    for n in range(NB):
        acc_s[0, n] = jnp.zeros((TQ, 128), f32)
    hs_s[0] = jnp.zeros((QT, KQ), bf16)
    best_r[...] = jnp.full(best_r.shape, -jnp.inf, f32)
    best_i[...] = jnp.zeros(best_i.shape, jnp.int32)
    cp_c().wait()
    cp_x(0).wait()
    cf = c_s[...].astype(f32)
    sc_s[...] = jnp.broadcast_to(cf * jax.nn.sigmoid(cf), (16, D)).astype(bf16)
    xn0 = _ln(xrows(0, pl.ds(0, TQ), TQ))

    def mod_body(j, carry):
        cp_mod(j).wait()
        mraw_s[j] = jnp.dot(sc_s[...], wmod_s[j], preferred_element_type=f32)[0:8, :]
        return carry

    lax.fori_loop(0, 2 * CPV, mod_body, 0)
    mod_s[:, 0:D] = mraw(0) * qscale
    mod_s[:, D:2 * D] = (1.0 + mraw(1)) * qscale
    h_s[...] = (xn0 * mvec(1) + mvec(0)).reshape(TQ, D).astype(bf16)
    NU = KQ // 16
    NPE = NU - NA
    cp_wq(0).wait()
    cp_k(0).wait()
    cp_v(0).wait()
    block0(wq_s, 0, 0, 1, [])
    cp_wq(1, P0 - 1).wait()
    block0(wq_s, DH, 1, P0 - 1, [(wq_s, wqc_s.at[0], u * 16) for u in range(NPE)])

    def a0_body(j, carry):
        h0 = P0 + j * G0
        cp_wq(h0, G0).wait()

        @pl.when(h0 % rep == 0)
        def _():
            cp_k(h0 // rep).wait()
            cp_v(h0 // rep).wait()

        sv = wq_s.at[:, pl.ds(al(h0 * DH, 4 * DH), 4 * DH)]
        dv = wqc_s.at[j + 1]
        block0(sv, 0, h0, G0, [(sv, dv, u * 16) for u in range(NU)] + [(wq_s, wqc_s.at[0], (NPE + j) * 16)])
        return carry

    lax.fori_loop(0, NA, a0_body, 0)
    cp_x(1).wait()
    cp_wr().wait()

    def o0_body(j, carry):
        cp_wo(j).wait()
        for u in range(CPV):
            if u >= MSH:
                cp_mod((j + 2) * CPV + u - MSH).wait()
            else:
                @pl.when(j > 0)
                def _():
                    cp_mod((j + 2) * CPV + u - MSH).wait()

        fence, release = sched()
        sc = sc_s[...]
        hq = KP // DH
        wo_j = wo_s.at[pl.ds(al(j * D, D), D)]
        o_j = o_s.at[pl.ds(j * (D // DH), D // DH)]
        wm_j = wmod_s.at[pl.ds((j + 2) * CPV - MSH, CPV)]
        mr_j = mraw_s.at[pl.ds((j + 2) * CPV - MSH, CPV)]
        units = [(qd, ng, u) for qd in range(2) for ng in range(2) for u in range(DH // 16)]
        npass = NB * (D // KP)
        cnt = 0
        due = {}
        hist = []
        lhs2 = [jnp.concatenate([o_j[kh * hq + u] for u in range(hq)], axis=1) for kh in range(D // KP)]
        for n in range(NB):
            acc = acc_s[0, n]
            cu, cn = divmod(n, MC // 128)
            mv = None
            for kh in range(D // KP):
                lhs = lhs2[kh]
                acc = jnp.dot(pltpu.bitcast(pin(lhs, due.pop(cnt, None)), bf16),
                              wo_j[kh * KP:(kh + 1) * KP, n * 128:(n + 1) * 128],
                              preferred_element_type=f32) + acc
                hist.append(acc)
                mine = units[cnt * len(units) // npass:(cnt + 1) * len(units) // npass]
                for n_, (qd, ng, u) in enumerate(mine):
                    last = w_unit(wo_j, [(4 * qd + c) * DH + u * 16 for c in range(4)], ng * 512,
                                  woc_s.at[j, ng], qd * DH + u * 16, [release(acc, O0_ROWS[n_][PERM[i_]]) for i_ in range(7)])
                if cnt + 2 < npass:
                    due.setdefault(cnt + 2, {})[2] = fence([last])
                if cnt in O0_LN:
                    qr, hf_ = O0_LN.index(cnt) % 4, O0_LN.index(cnt) // 4
                    ln1(1, qr * QT + j * 16 + hf_ * 8, 8, release(acc, O0_LNROW))
                    due.setdefault(cnt + 3, {})[4] = fence([(hf_s, qr * QT + j * 16 + hf_ * 8)])
                if cnt in O0_HS:
                    hp_ = [(hist[-3 + u_ // 3], O0_HSROW[u_ % 3]) for u_ in range(9)]
                    h_slice(j * 16 + O0_HS.index(cnt) * 8, [release(*hp_[PERML[i_]]) for i_ in range(7)])
                    if cnt == O0_HS[0]:
                        due.setdefault(cnt + 2, {})[10] = fence([(hs_s.at[0], j * 16)])
                cnt += 1
                d = jnp.dot(sc[:, kh * KP:(kh + 1) * KP],
                            wm_j[cu, kh * KP:(kh + 1) * KP, cn * 128:(cn + 1) * 128],
                            preferred_element_type=f32)
                mv = d if mv is None else d + mv
            acc_s[0, n] = acc
            mr_j[cu, :, cn * 128:(cn + 1) * 128] = mv[0:8, :]
        assert not due
        return carry

    lax.fori_loop(0, NO, o0_body, 0)

    for u in range(NMC - MSH, NMC):
        cp_mod(u).wait()
    for u in range(NMC - MSH, NMC):
        mraw_s[u] = jnp.dot(sc_s[...], wmod_s[u], preferred_element_type=f32)[0:8, :]
    mod_s[:, 2 * D:3 * D] = mraw(2)
    mod_s[:, 3 * D:4 * D] = mraw(3)
    mod_s[:, 4 * D:5 * D] = 1.0 + mraw(4)
    mod_s[:, 5 * D:6 * D] = mraw(5)
    mod_s[:, 6 * D:7 * D] = jnp.broadcast_to(wr_s[...].astype(f32).reshape(1, D), (8, D))
    cp_wg().start()
    for u in range(F // MC):
        cp_wu(u).start()
    cp_wd().start()

    def step(t, carry):
        @pl.when(t + 1 < nt)
        def _():
            cp_x(t + 1).wait()

        @pl.when(t + 1 == nt)
        def _():
            cp_wg().wait()
            for u in range(F // MC):
                cp_wu(u).wait()
            cp_wd().wait()

        fence, release = sched()
        tprev, tnext = t - 1, jnp.minimum(t + 1, nt - 1)
        prods = [(i1, i2) for i1 in _ORDER for i2 in _ORDER]
        hv = [hs_s[u] for u in range(49)]

        qblk = {}

        def q_passes(g):
            def emit(r1, r2, n1, n2, c):
                for z in range(2):
                    qblk[8 * g + 4 * z + 2 * n1 + n2, 2 * r1 + r2] = c[:, z * DH:(z + 1) * DH]
            asm = _Assemble(emit)

            def run(i1, i2):
                u = 7 * i2 + i1
                w = jnp.concatenate([wqc_s[2 * g + z, u] for z in range(2)], axis=1)
                d = jnp.dot(hv[u], w, preferred_element_type=f32)
                ini = asm.init(i1, i2)
                if ini is not None:
                    d = d + ini
                asm.add(i1, i2, d)
                return d
            return [functools.partial(run, i1, i2) for i1, i2 in prods]

        def q_head(hh):
            return jnp.concatenate([qblk.pop((hh, r)) for r in range(4)], axis=0)

        def o_passes():
            ms = {}
            asm = []
            for ng in range(2):
                def emit(r1, r2, n1, n2, c, ng=ng):
                    acc_s[t, 4 * ng + 2 * n1 + n2, pl.ds(r1 * HT + r2 * QT, QT), :] = c
                asm.append(_Assemble(emit))

            def run(ng, i1, i2, k, dep=None):
                u = 7 * i2 + i1
                lhs = jnp.concatenate([os_s[u, 4 * k + v] for v in range(4)], axis=1)
                w = jnp.concatenate([woc_s[2 * k + v, ng, u] for v in range(2)], axis=0)
                d = jnp.dot(lhs, pin_bf16(w, dep), preferred_element_type=f32)
                early = ng == 0 or (i1, i2) in prods[:NE]
                if k == 1:
                    d = d + ms.pop((ng, u))
                if k == (1 if early else 0):
                    ini = asm[ng].init(i1, i2)
                    if ini is not None:
                        d = d + ini
                if k == 0:
                    ms[ng, u] = d
                else:
                    asm[ng].add(i1, i2, d)
                return d
            NE = 16
            seq = [(0,) + pr + (0,) for pr in prods] + [(1,) + pr + (0,) for pr in prods[:NE]]
            seq += [(0,) + pr + (1,) for pr in prods] + [(1,) + pr + (1,) for pr in prods[:NE]]
            seq += [(1,) + pr + (k,) for pr in prods[NE:] for k in range(2)]
            return [functools.partial(run, *a) for a in seq]

        def side(hp, pts):
            rel = [release(v_, rw) for v_, rw in pts]
            for u in range(2):
                epi_rows(tprev, (2 * hp + u) * CHE, CHE, rel[u])
            if len(rel) == 3:
                ln1(tnext, hp * 16, 16, rel[2])
            else:
                for u in range(2):
                    ln1(tnext, hp * 16 + 8 * u, 8, rel[2 + u])
            return fence([(out_s.at[tprev], 0), (best_r, 0), (stat_s.at[tprev, 0], 0), (hf_s, 0)])

        def o_slice(qd, oq, u, pts):
            blk = [[[[oq[k1][k2][r1 * HT + r2 * QT + 16 * u:r1 * HT + r2 * QT + 16 * u + 16]
                      for k2 in range(2)] for k1 in range(2)] for r2 in range(2)] for r1 in range(2)]
            if len(pts) == 7:
                pts = [pts[PERML[i_]] for i_ in range(7)]
            ops = _two_level(_lhs_sums, blk, [jnp.tile(release(v_, rw), (2, 1)) for v_, rw in pts])
            for v in range(7):
                os_s[7 * v:7 * v + 7, qd, 16 * u:16 * u + 16, :] = ops[v]
            return fence([(os_s.at[0, qd], 16 * u)])

        assert 2 * HP * CHE == TQ
        for fn in q_passes(0):
            fn()
        opl = o_passes()
        oq = fo = ob_ = None
        for hp in range(HP):
            g, pp = divmod(hp, 4)
            if pp == 0:
                fill = q_passes(g + 1) if g + 1 < HKV else opl
            qa, qb = q_head(2 * hp), q_head(2 * hp + 1)
            sa_ = scores(qa if fo is None else pin(qa, {0: fo}), g)
            pa, la = softmax(sa_)
            vals = {'s': sa_, 'ob': ob_}
            if oq is not None:
                fl = [o_slice(hp // 2 - 1, oq, 2 * (hp % 2) + u, [(vals[nm], rw) for nm, rw in OS_PTS[u]])
                      for u in range(2 if FILL[pp][1] < 7 else 1)]
                qb = pin(qb, {0: functools.reduce(lambda a_, b_: a_ | b_, fl)})
            rs_ = [fill.pop(0)() for _ in range(FILL[pp][0])]
            vals.update({i_: rs_[max(len(rs_) - 6 + i_, 0)] for i_ in range(6)})
            fs = side(hp, [(vals[nm] if vals[nm] is not None else sa_, rw) for nm, rw in SIDE_PTS])
            pb, lb = softmax(scores(qb, g))
            oa_ = pv(pa, g)
            oa = oa_ * la
            rs_ = [fill.pop(0)() for _ in range(FILL[pp][1])]
            fo = None
            if oq is not None and FILL[pp][1] >= 7:
                vals = {'oa': oa_}
                vals.update(enumerate(rs_))
                fo = o_slice(hp // 2 - 1, oq, 2 * (hp % 2) + 1, [(vals[nm], rw) for nm, rw in OS_F2])
            ob_ = pv(pin(pb, {0: fs}), g)
            ob = ob_ * lb
            if hp % 2 == 0:
                oprev = (oa, ob)
            else:
                oq = [oprev, (oa, ob)]

        pts = []
        due = {} if fo is None else {2: fo}
        for s, fn in enumerate(opl):
            pts.append((fn(due.pop(s, None)), 0))
            if len(pts) % 3 == 0 and len(pts) <= 12:
                o_slice(HP // 2 - 1, oq, len(pts) // 3 - 1, pts[-3:])
            u, rem = divmod(s - HS0, HSG)
            if rem == 0 and 0 <= u < QT // 8:
                h_slice(u * 8, [release(pts[-1 - HSS * (6 - PERML[i_])][0]) for i_ in range(7)])
                due[s + 6] = fence([(hs_s.at[0], 0)])
        assert not due
        cp_out(tprev).start()
        return carry

    lax.fori_loop(1, nt, step, 0)

    epi_rows(nt - 1, 0, TQ)
    cp_out(nt - 1).start()
    bv = best_r[...]
    rbest = jnp.max(bv, axis=0, keepdims=True)
    ibest = jnp.min(jnp.where(bv == rbest, best_i[...], S), axis=0, keepdims=True)
    idx = jnp.minimum(ibest[0, 0], S - 1)
    base = pl.multiple_of((idx // 16) * 16, 16)
    tb = idx // TQ
    bsl = pl.ds(pl.multiple_of(base - tb * TQ, 16), 16)
    x1 = resid(tb, bsl, 16)
    h2 = h2_from_stats(x1, tb, bsl, 16)
    xs = h2.reshape(16, D).astype(bf16)
    gt = jnp.dot(xs, wq_s[:, 0:F], preferred_element_type=f32)
    up = jnp.concatenate([jnp.dot(xs, wmod_s[u], preferred_element_type=f32) for u in range(F // MC)], axis=1)
    a = (gt * jax.nn.sigmoid(gt) * up).astype(bf16)
    y = jnp.dot(a, wo_s[0:F, 0:D], preferred_element_type=f32)
    y = y * jnp.tile(jax.nn.sigmoid(rbest), (1, NB))
    rr = lax.broadcasted_iota(jnp.int32, (16, D), 0) + base
    upd = jnp.where(rr == idx, y, 0.0).reshape(2, 8, D)
    new = (x1 + mvec(5) * (h2 + upd)).reshape(16, D)
    for t in range(nt):
        cp_out(t).wait()
    out_s[tb, bsl, :] = new.astype(out_s.dtype)
    fix = pltpu.make_async_copy(out_s.at[tb, bsl, :], out_hbm.at[pl.ds(base, 16), :], osems.at[0])
    fix.start()
    fix.wait()


def _compiler_params():
    kw = dict(vmem_limit_bytes=124 * 1024 * 1024)
    try:
        return pltpu.CompilerParams(disable_semaphore_checks=True, disable_bounds_checks=True, **kw)
    except TypeError:
        return pltpu.CompilerParams(**kw)


@jax.jit
def pallas_adaLN_cond__sliding_block_cached__moe_arch_mod__prompt_kernel(
    A_x: jax.Array,
    A_k_cache: jax.Array,
    A_v_cache: jax.Array,
    A_wq: jax.Array,
    A_wo: jax.Array,
    B_x: jax.Array,
    B_w_r: jax.Array,
    B_w_gate: jax.Array,
    B_w_up: jax.Array,
    B_w_down: jax.Array,
    c: jax.Array,
    w_mod: jax.Array,
):
    B, S, D = A_x.shape
    assert B == 1
    HKV, SK = A_k_cache.shape[1], A_k_cache.shape[2]
    W = min(4096, max(256, SK // 4))
    F = B_w_gate.shape[1]
    dt = A_x.dtype
    f32 = jnp.float32
    nt = S // TQ
    NB = D // 128
    NMC = 6 * D // MC
    x2 = A_x.reshape(S, D)
    anyspec = pl.BlockSpec(memory_space=pl.ANY)
    kern = functools.partial(_kernel, S=S, D=D, HKV=HKV, SK=SK, W=W, F=F)
    out = pl.pallas_call(
        kern,
        in_specs=[anyspec] * 11,
        out_specs=anyspec,
        out_shape=jax.ShapeDtypeStruct((S, D), dt),
        scratch_shapes=[
            pltpu.VMEM((D,), dt),
            pltpu.VMEM((1, D), dt),
            pltpu.VMEM((nt, TQ, D), dt),
            pltpu.VMEM((HKV, W, DH), dt),
            pltpu.VMEM((HKV, W, DH), dt),
            pltpu.VMEM((D, HQ * DH + PAD), dt),
            pltpu.VMEM((HQ * DH, D + PAD), dt),
            pltpu.VMEM((NMC, D, MC), dt),
            pltpu.VMEM((nt, TQ, D), dt),
            pltpu.VMEM((HQ // 4, 49, D // 4, DH), dt),
            pltpu.VMEM((HQ * DH // D, 2, 49, 2 * DH, 128), dt),
            pltpu.VMEM((TQ, D), f32),
            pltpu.VMEM((49, TQ // 4, D // 4), dt),
            pltpu.VMEM((49, HQ // 4, TQ // 4, DH), dt),
            pltpu.VMEM((16, D), dt),
            pltpu.VMEM((NMC, 8, MC), f32),
            pltpu.VMEM((8, 7 * D), f32),
            pltpu.VMEM((TQ, D), dt),
            pltpu.VMEM((HQ, TQ // 2, DH), jnp.uint32),
            pltpu.VMEM((nt, NB, TQ, 128), f32),
            pltpu.VMEM((nt, 2, TQ, 128), f32),
            pltpu.VMEM((8, 128), f32),
            pltpu.VMEM((8, 128), jnp.int32),
            pltpu.SMEM((1,), jnp.int32),
            pltpu.SemaphoreType.DMA((4 + NMC + HQ + 2 * HKV + HQ * DH // D + nt,)),
            pltpu.SemaphoreType.DMA((nt,)),
        ],
        compiler_params=_compiler_params(),
    )(B_w_r, c, x2, A_k_cache, A_v_cache, A_wq, A_wo, w_mod, B_w_gate, B_w_up, B_w_down)
    return out.reshape(B, S, D)
```

```python
import functools

import jax
import jax.numpy as jnp
from jax import lax
import jax.experimental.pallas as pl
import jax.experimental.pallas.tpu as pltpu

HQ = 32
DH = 128
TQ = 256
PAD = 128
P0 = 4
G0 = 4
MC = 512
MSH = 1
CHE = 8
FILL = ((7, 7), (7, 7), (7, 7), (7, 0))

SIDE_PTS = ((1, 0), (2, 0), ('ob', 0), ('ob', 56))
OS_F2 = [('oa', 128), ('oa', 192), (0, 0), (1, 0), (2, 0), (3, 0), (4, 0)]
OS_PTS = ([('ob', 96 + 16 * i) for i in range(7)],
          [('ob', 208), ('ob', 224), ('ob', 240), ('s', 0), ('s', 16), ('s', 32), ('s', 48)])
HS0, HSG, HSS = 30, 14, 2
A0_W = (2, 250, 394, 760, 130, 150, 370)
A0_DUE = 14
O0_ROWS = ((0, 16, 32, 56, 72, 88, 112), (128, 144, 168, 184, 200, 224, 240))
O0_LN = (0, 1, 2, 3, 4, 5, 6, 7)
O0_LNROW = 24
O0_HS = (12, 15)
O0_HSROW = (8, 104, 192)
PERM = (3, 1, 4, 0, 5, 2, 6)
PERML = (0, 1, 2, 3, 4, 5, 6)

EPS = 1e-5
LOG2E = 1.4426950408889634


def _ln_stats(x, rel=None):
    d = x.shape[-1]
    part = x[..., 0:128]
    for j in range(1, d // 128):
        part = part + x[..., j * 128:(j + 1) * 128]
    if rel is not None:
        part = part + rel
    m = jnp.sum(part, axis=-1, keepdims=True) * (1.0 / d)
    xc = x - m
    v = jnp.mean(xc * xc, axis=-1, keepdims=True)
    return m, xc, lax.rsqrt(v + EPS)


def _ln(x, rel=None):
    _, xc, rs = _ln_stats(x, rel)
    return xc * rs


def _recip(l):
    return pl.reciprocal(l, approx=True)


def _lhs_sums(a11, a12, a21, a22):
    return [a11 + a22, a21 + a22, a11, a22, a11 + a12, a21 - a11, a12 - a22]


def _rhs_sums(b11, b12, b21, b22):
    return [b11 + b22, b11, b12 - b22, b21 - b11, b22, b11 + b12, b21 + b22]


_ORDER = [3, 4, 0, 6, 1, 2, 5]
_BLOCK = {6: (0, 0), 1: (1, 0), 2: (0, 1), 5: (1, 1)}


def _init(i, z):
    return {0: lambda: z[3] - z[4], 6: lambda: z[0], 1: lambda: z[3], 2: lambda: z[4],
            5: lambda: z[0] - z[1] + z[2]}.get(i, lambda: None)()


def _two_level(sums, blk, rel):
    o = [[jnp.stack([blk[a1][a2][b1][b2] for a2 in range(2) for b2 in range(2)]) for b1 in range(2)]
         for a1 in range(2)]
    if rel is not None and len(rel) == 3:
        o = [[o[a1][b1] + rel[0 if a1 == b1 else 1 + a1][None] for b1 in range(2)] for a1 in range(2)]
    x = jnp.stack(sums(o[0][0], o[0][1], o[1][0], o[1][1]), axis=1)
    x = [x[u] for u in range(4)]
    if rel is not None and len(rel) == 7:
        r7 = jnp.stack(rel)
        x = [x[0] + r7, x[1], x[2], x[3] + r7]
    return [y.astype(jnp.bfloat16) for y in sums(*x)]


class _Assemble:
    def __init__(self, emit):
        self.z, self.outer, self.inj, self.emit = {}, {}, {}, emit

    def init(self, i1, i2):
        v = _init(i2, self.z)
        if i2 in _BLOCK and i1 not in (3, 4):
            self.inj[i2] = _init(i1, self.outer[i2])
            v = v + self.inj[i2]
            if i2 == 5:
                v = v + (self.inj[1] - self.inj[2])
        return v

    def add(self, i1, i2, m):
        self.z[i2] = m
        if i2 in _BLOCK:
            self.outer.setdefault(i2, {})[i1] = m
            if i1 in _BLOCK:
                (r1, n1), (r2, n2) = _BLOCK[i1], _BLOCK[i2]
                self.emit(r1, r2, n1, n2, m)


def _kernel(wr_hbm, c_hbm, x_hbm, k_hbm, v_hbm, wq_hbm, wo_hbm, wmod_hbm,
            wg_hbm, wu_hbm, wd_hbm, out_hbm,
            wr_s, c_s, x_s, k_s, v_s, wq_s, wo_s, wmod_s, out_s,
            wqc_s, woc_s, hf_s, hs_s, os_s,
            sc_s, mraw_s, mod_s, h_s, o_s, acc_s, stat_s, best_r, best_i, zero_s, sems, osems,
            *, S, D, HKV, SK, W, F):
    nt = S // TQ
    rep = HQ // HKV
    NB = D // 128
    HP = HQ // 2
    HT = TQ // 2
    QT = TQ // 4
    KH = D // 2
    KQ = D // 4
    KP = 512
    CPV = D // MC
    NMC = 6 * CPV
    NA = (HQ - P0) // G0
    NO = HQ * DH // D
    f32 = jnp.float32
    bf16 = jnp.bfloat16
    u32 = jnp.uint32
    qscale = (DH ** -0.5) * LOG2E
    assert KH == KP and rep == 8 and NB == 8 and NO == 4 and P0 == 4 and G0 == 4

    def al(v, n):
        return v if isinstance(v, int) else pl.multiple_of(v, n)

    S_C, S_WR, S_WG, S_WD, S_M = 0, 1, 2, 3, 4
    S_WQ = S_M + NMC
    S_K = S_WQ + HQ
    S_V = S_K + HKV
    S_WO = S_V + HKV
    S_X = S_WO + NO

    def cp_c():
        return pltpu.make_async_copy(c_hbm, c_s, sems.at[S_C])

    def cp_wr():
        return pltpu.make_async_copy(wr_hbm, wr_s, sems.at[S_WR])

    def cp_mod(j):
        return pltpu.make_async_copy(wmod_hbm.at[:, pl.ds(al(j * MC, MC), MC)], wmod_s.at[j], sems.at[S_M + j])

    def cp_wg():
        return pltpu.make_async_copy(wg_hbm, wq_s.at[:, pl.ds(0, F)], sems.at[S_WG])

    def cp_wu(u):
        return pltpu.make_async_copy(wu_hbm.at[:, pl.ds(u * MC, MC)], wmod_s.at[u], sems.at[S_M + u])

    def cp_wd():
        return pltpu.make_async_copy(wd_hbm, wo_s.at[pl.ds(0, F), pl.ds(0, D)], sems.at[S_WD])

    def cp_wq(h, n=1):
        sl = pl.ds(al(h * DH, DH), n * DH)
        return pltpu.make_async_copy(wq_hbm.at[:, sl], wq_s.at[:, sl], sems.at[S_WQ + h])

    def cp_k(g):
        return pltpu.make_async_copy(k_hbm.at[0, g, pl.ds(SK - W, W), :], k_s.at[g], sems.at[S_K + g])

    def cp_v(g):
        return pltpu.make_async_copy(v_hbm.at[0, g, pl.ds(SK - W, W), :], v_s.at[g], sems.at[S_V + g])

    def cp_wo(j):
        sl = pl.ds(al(j * D, D), D)
        return pltpu.make_async_copy(wo_hbm.at[sl, :], wo_s.at[sl, pl.ds(0, D)], sems.at[S_WO + j])

    def rsl(t, r0=0, n=TQ):
        return pl.ds(al(t * TQ + r0, n), n)

    def cp_x(t):
        return pltpu.make_async_copy(x_hbm.at[rsl(t), :], x_s.at[t], sems.at[S_X + t])

    def cp_out(t):
        return pltpu.make_async_copy(out_s.at[t], out_hbm.at[rsl(t), :], osems.at[t])

    def sched():
        zero = zero_s[0]
        z16 = pl.multiple_of(zero, 16)
        zvec = jnp.full((8, 128), zero, jnp.int32).astype(u32)

        def fence(deps):
            d = None
            for ref, base in deps:
                n = 16 if ref.dtype == bf16 else 8
                v = pltpu.bitcast(ref[pl.ds(pl.multiple_of(base + z16, n), n), 0:128], u32)
                d = v if d is None else d | v
            return d & zvec

        def release(acc, r0=0):
            return pltpu.bitcast(pltpu.bitcast(acc[r0:r0 + 8, 0:128], u32) & zvec, f32)

        return fence, release

    def pin(a, at):
        if not at:
            return a
        parts = []
        prev = 0
        for rb in sorted(at):
            r0 = rb * 8
            if r0 > prev:
                parts.append(a[prev:r0, :])
            if a.dtype == f32:
                blk = a[r0:r0 + 8, 0:128] + pltpu.bitcast(at[rb], f32)
            else:
                blk = a[r0:r0 + 8, 0:128] | at[rb]
            if a.shape[1] > 128:
                blk = jnp.concatenate([blk, a[r0:r0 + 8, 128:]], axis=1)
            parts.append(blk)
            prev = r0 + 8
        if prev < a.shape[0]:
            parts.append(a[prev:, :])
        return jnp.concatenate(parts, axis=0)

    def pin_bf16(w, d):
        if d is None:
            return w
        top = pltpu.bitcast(pltpu.bitcast(w[0:16], u32) | d, bf16)
        return jnp.concatenate([top, w[16:]], axis=0)

    def mvec(j):
        return mod_s[:, j * D:(j + 1) * D][None]

    def mraw(j):
        return jnp.concatenate([mraw_s[j * CPV + u] for u in range(CPV)], axis=1)

    def xrows(t, sl, n):
        return x_s[t, sl, :].astype(f32).reshape(n // 8, 8, D)

    def ln1(t, r0, n, rel=None):
        xn = _ln(xrows(t, pl.ds(al(r0, n), n), n), rel)
        hf_s[pl.ds(al(r0, n), n), :] = (xn * mvec(1) + mvec(0)).reshape(n, D)

    def h_slice(r0, rel):
        hq = [hf_s[pl.ds(al(r * QT + r0, 8), 8), :] for r in range(4)]
        blk = [[[[hq[2 * r1 + r2][:, (2 * k1 + k2) * KQ:(2 * k1 + k2 + 1) * KQ] for k2 in range(2)]
                 for k1 in range(2)] for r2 in range(2)] for r1 in range(2)]
        ops = _two_level(_lhs_sums, blk, None if rel is None else [jnp.tile(v, (1, KQ // 128)) for v in rel])
        for u in range(7):
            hs_s[7 * u:7 * u + 7, pl.ds(al(r0, 8), 8), :] = ops[u]

    def w_unit(src, rows4, c0, dst, d0, rel):
        w = [src[pl.ds(al(r, 16), 16), c0:c0 + 512].astype(f32) for r in rows4]
        blk = [[[[w[2 * k1 + k2][:, (2 * n1 + n2) * 128:(2 * n1 + n2 + 1) * 128] for n2 in range(2)]
                 for n1 in range(2)] for k2 in range(2)] for k1 in range(2)]
        ops = _two_level(_rhs_sums, blk, None if rel is None else [jnp.tile(v, (2, 1)) for v in rel])
        for u in range(7):
            dst[7 * u:7 * u + 7, pl.ds(al(d0, 16), 16), :] = ops[u]
        return (dst.at[0], d0)

    def resid(t, sl, n):
        attn = jnp.concatenate([acc_s[t, j, sl, :] for j in range(NB)], axis=1).reshape(n // 8, 8, D)
        return xrows(t, sl, n) + mvec(2) * attn

    def h2_from_stats(x1, t, sl, n):
        m = jnp.tile(stat_s[t, 0, sl, :], (1, NB)).reshape(n // 8, 8, D)
        rs = jnp.tile(stat_s[t, 1, sl, :], (1, NB)).reshape(n // 8, 8, D)
        return (x1 - m) * rs * mvec(4) + mvec(3)

    def epi_rows(t, r0, n, rel=None):
        sl = pl.ds(r0, n)
        x1 = resid(t, sl, n)
        m, xc, rs = _ln_stats(x1, rel)
        stat_s[t, 0, sl, :] = jnp.broadcast_to(m.reshape(n, 1), (n, 128))
        stat_s[t, 1, sl, :] = jnp.broadcast_to(rs.reshape(n, 1), (n, 128))
        h2 = xc * rs * mvec(4) + mvec(3)
        out_s[t, sl, :] = (x1 + mvec(5) * h2).reshape(n, D).astype(out_s.dtype)
        r = jnp.sum(h2 * mvec(6), axis=-1, keepdims=True)
        r = r.astype(bf16).astype(f32)
        bv = best_r[...]
        bi = best_i[...]
        sub = lax.broadcasted_iota(jnp.int32, (8, 128), 0)
        for u in range(n // 8):
            ru = jnp.broadcast_to(r[u], (8, 128))
            better = ru > bv
            bv = jnp.where(better, ru, bv)
            bi = jnp.where(better, sub + (t * TQ + r0 + u * 8), bi)
        best_r[...] = bv
        best_i[...] = bi

    def scores(q, g):
        return lax.dot_general(q.astype(bf16), k_s[g], (((1,), (1,)), ((), ())), preferred_element_type=f32)

    def softmax(s):
        m = jnp.max(s, axis=-1, keepdims=True)
        p = jnp.exp2(s - m)
        part = p[:, 0:128]
        for j in range(1, W // 128):
            part = part + p[:, j * 128:(j + 1) * 128]
        p = jnp.concatenate([jnp.minimum(p[:, 0:128], part), p[:, 128:]], axis=1)
        return p, _recip(jnp.sum(part, axis=-1, keepdims=True))

    def pv(p, g):
        return jnp.dot(p.astype(bf16), v_s[g], preferred_element_type=f32)

    def block0(wv, c0, h0, nh, units):
        fence, release = sched()
        hval = h_s[...]
        g = h0 // rep
        tqk = [512 + 1024 * u for u in range(nh)]
        tpv = [tqk[u] + (768 if u + 1 < nh else 256) for u in range(nh)]
        wins = [(130, tqk[0])]
        for u in range(nh):
            wins.append((tqk[u] + A0_W[0], tqk[u] + (A0_W[1] if u + 1 < nh else A0_W[4])))
            if u + 1 < nh:
                wins.append((tqk[u] + A0_W[2], tqk[u] + A0_W[3]))
        wins.append((tpv[-1] + A0_W[5], tpv[-1] + A0_W[6]))
        slots = [t_ for a_, b_ in wins for t_ in range(a_, b_, 8)]
        npt = 7 * len(units)
        times = [slots[(u * len(slots)) // npt] for u in range(npt)]
        todo = [(un, times[7 * u:7 * u + 7]) for u, un in enumerate(units)]
        vals = []

        def emit(tmax):
            last = []
            while todo and todo[0][1][-1] < tmax:
                (sv, dv, r0), ts = todo.pop(0)
                rel = []
                for i_ in range(7):
                    t0_, v_ = [tv for tv in vals if tv[0] <= ts[PERM[i_]]][-1]
                    rel.append(release(v_, min((ts[PERM[i_]] - t0_) // 8 * 8, TQ - 8)))
                last = last[-1:] + [w_unit(sv, [c * KQ + r0 for c in range(4)], 0, dv, r0, rel)]
            return last

        def qproj(u, t_):
            cols = slice(c0 + u * DH, c0 + (u + 1) * DH)
            q1 = jnp.dot(hval[:, 0:KH], wv[0:KH, cols], preferred_element_type=f32)
            q2 = jnp.dot(hval[:, KH:D], wv[KH:D, cols], preferred_element_type=f32) + q1
            vals.extend([(t_ + 130, q1), (t_ + 386, q2)])
            return q2

        q = qproj(0, 0)
        for u in range(nh):
            s = scores(q, g)
            vals.append((tqk[u] + 130, s))
            p, li = softmax(s)
            if u + 1 < nh:
                q = qproj(u + 1, tqk[u] + 256)
            deps = emit(tpv[u]) + ([(o_s.at[h0 + u - 1], 0)] if u > 0 else [])
            if deps:
                p = pin(p, {A0_DUE: fence(deps)})
            o = pv(p, g)
            vals.append((tpv[u] + 130, o))
            o_s[h0 + u] = pltpu.bitcast((o * li).astype(bf16), u32)
        emit(1 << 30)

    cp_c().start()
    cp_x(0).start()
    for j in range(2 * CPV):
        cp_mod(j).start()
    cp_wq(0).start()
    cp_k(0).start()
    cp_v(0).start()
    cp_wq(1, P0 - 1).start()
    for j in range(NA):
        h0 = P0 + j * G0
        cp_wq(h0, G0).start()
        if h0 % rep == 0:
            cp_k(h0 // rep).start()
            cp_v(h0 // rep).start()
    cp_x(1).start()
    cp_wr().start()
    for j in range(NO):
        cp_wo(j).start()
        for u in range(CPV):
            if (j + 2) * CPV + u - MSH >= 2 * CPV:
                cp_mod((j + 2) * CPV + u - MSH).start()
    for u in range(NMC - MSH, NMC):
        cp_mod(u).start()
    for t in range(2, nt):
        cp_x(t).start()

    zero_s[0] = 0
    for n in range(NB):
        acc_s[0, n] = jnp.zeros((TQ, 128), f32)
    hs_s[0] = jnp.zeros((QT, KQ), bf16)
    best_r[...] = jnp.full(best_r.shape, -jnp.inf, f32)
    best_i[...] = jnp.zeros(best_i.shape, jnp.int32)
    cp_c().wait()
    cp_x(0).wait()
    cf = c_s[...].astype(f32)
    sc_s[...] = jnp.broadcast_to(cf * jax.nn.sigmoid(cf), (16, D)).astype(bf16)
    xn0 = _ln(xrows(0, pl.ds(0, TQ), TQ))

    def mod_body(j, carry):
        cp_mod(j).wait()
        mraw_s[j] = jnp.dot(sc_s[...], wmod_s[j], preferred_element_type=f32)[0:8, :]
        return carry

    lax.fori_loop(0, 2 * CPV, mod_body, 0)
    mod_s[:, 0:D] = mraw(0) * qscale
    mod_s[:, D:2 * D] = (1.0 + mraw(1)) * qscale
    h_s[...] = (xn0 * mvec(1) + mvec(0)).reshape(TQ, D).astype(bf16)
    NU = KQ // 16
    NPE = NU - NA
    cp_wq(0).wait()
    cp_k(0).wait()
    cp_v(0).wait()
    block0(wq_s, 0, 0, 1, [])
    cp_wq(1, P0 - 1).wait()
    block0(wq_s, DH, 1, P0 - 1, [(wq_s, wqc_s.at[0], u * 16) for u in range(NPE)])

    def a0_body(j, carry):
        h0 = P0 + j * G0
        cp_wq(h0, G0).wait()

        @pl.when(h0 % rep == 0)
        def _():
            cp_k(h0 // rep).wait()
            cp_v(h0 // rep).wait()

        sv = wq_s.at[:, pl.ds(al(h0 * DH, 4 * DH), 4 * DH)]
        dv = wqc_s.at[j + 1]
        block0(sv, 0, h0, G0, [(sv, dv, u * 16) for u in range(NU)] + [(wq_s, wqc_s.at[0], (NPE + j) * 16)])
        return carry

    lax.fori_loop(0, NA, a0_body, 0)
    cp_x(1).wait()
    cp_wr().wait()

    def o0_body(j, carry):
        cp_wo(j).wait()
        for u in range(CPV):
            if u >= MSH:
                cp_mod((j + 2) * CPV + u - MSH).wait()
            else:
                @pl.when(j > 0)
                def _():
                    cp_mod((j + 2) * CPV + u - MSH).wait()

        fence, release = sched()
        sc = sc_s[...]
        hq = KP // DH
        wo_j = wo_s.at[pl.ds(al(j * D, D), D)]
        o_j = o_s.at[pl.ds(j * (D // DH), D // DH)]
        wm_j = wmod_s.at[pl.ds((j + 2) * CPV - MSH, CPV)]
        mr_j = mraw_s.at[pl.ds((j + 2) * CPV - MSH, CPV)]
        units = [(qd, ng, u) for qd in range(2) for ng in range(2) for u in range(DH // 16)]
        npass = NB * (D // KP)
        cnt = 0
        due = {}
        hist = []
        lhs2 = [jnp.concatenate([o_j[kh * hq + u] for u in range(hq)], axis=1) for kh in range(D // KP)]
        for n in range(NB):
            acc = acc_s[0, n]
            cu, cn = divmod(n, MC // 128)
            mv = None
            for kh in range(D // KP):
                lhs = lhs2[kh]
                acc = jnp.dot(pltpu.bitcast(pin(lhs, due.pop(cnt, None)), bf16),
                              wo_j[kh * KP:(kh + 1) * KP, n * 128:(n + 1) * 128],
                              preferred_element_type=f32) + acc
                hist.append(acc)
                mine = units[cnt * len(units) // npass:(cnt + 1) * len(units) // npass]
                for n_, (qd, ng, u) in enumerate(mine):
                    last = w_unit(wo_j, [(4 * qd + c) * DH + u * 16 for c in range(4)], ng * 512,
                                  woc_s.at[j, ng], qd * DH + u * 16, [release(acc, O0_ROWS[n_][PERM[i_]]) for i_ in range(7)])
                if cnt + 2 < npass:
                    due.setdefault(cnt + 2, {})[2] = fence([last])
                if cnt in O0_LN:
                    qr, hf_ = O0_LN.index(cnt) % 4, O0_LN.index(cnt) // 4
                    ln1(1, qr * QT + j * 16 + hf_ * 8, 8, release(acc, O0_LNROW))
                    due.setdefault(cnt + 3, {})[4] = fence([(hf_s, qr * QT + j * 16 + hf_ * 8)])
                if cnt in O0_HS:
                    hp_ = [(hist[-3 + u_ // 3], O0_HSROW[u_ % 3]) for u_ in range(9)]
                    h_slice(j * 16 + O0_HS.index(cnt) * 8, [release(*hp_[PERML[i_]]) for i_ in range(7)])
                    if cnt == O0_HS[0]:
                        due.setdefault(cnt + 2, {})[10] = fence([(hs_s.at[0], j * 16)])
                cnt += 1
                d = jnp.dot(sc[:, kh * KP:(kh + 1) * KP],
                            wm_j[cu, kh * KP:(kh + 1) * KP, cn * 128:(cn + 1) * 128],
                            preferred_element_type=f32)
                mv = d if mv is None else d + mv
            acc_s[0, n] = acc
            mr_j[cu, :, cn * 128:(cn + 1) * 128] = mv[0:8, :]
        assert not due
        return carry

    lax.fori_loop(0, NO, o0_body, 0)

    for u in range(NMC - MSH, NMC):
        cp_mod(u).wait()
    for u in range(NMC - MSH, NMC):
        mraw_s[u] = jnp.dot(sc_s[...], wmod_s[u], preferred_element_type=f32)[0:8, :]
    mod_s[:, 2 * D:3 * D] = mraw(2)
    mod_s[:, 3 * D:4 * D] = mraw(3)
    mod_s[:, 4 * D:5 * D] = 1.0 + mraw(4)
    mod_s[:, 5 * D:6 * D] = mraw(5)
    mod_s[:, 6 * D:7 * D] = jnp.broadcast_to(wr_s[...].astype(f32).reshape(1, D), (8, D))
    cp_wg().start()
    for u in range(F // MC):
        cp_wu(u).start()
    cp_wd().start()

    def step(t, carry):
        @pl.when(t + 1 < nt)
        def _():
            cp_x(t + 1).wait()

        fence, release = sched()
        tprev, tnext = t - 1, jnp.minimum(t + 1, nt - 1)
        prods = [(i1, i2) for i1 in _ORDER for i2 in _ORDER]
        hv = [hs_s[u] for u in range(49)]

        qblk = {}

        def q_passes(g):
            def emit(r1, r2, n1, n2, c):
                for z in range(2):
                    qblk[8 * g + 4 * z + 2 * n1 + n2, 2 * r1 + r2] = c[:, z * DH:(z + 1) * DH]
            asm = _Assemble(emit)

            def run(i1, i2):
                u = 7 * i2 + i1
                w = jnp.concatenate([wqc_s[2 * g + z, u] for z in range(2)], axis=1)
                d = jnp.dot(hv[u], w, preferred_element_type=f32)
                ini = asm.init(i1, i2)
                if ini is not None:
                    d = d + ini
                asm.add(i1, i2, d)
                return d
            return [functools.partial(run, i1, i2) for i1, i2 in prods]

        def q_head(hh):
            return jnp.concatenate([qblk.pop((hh, r)) for r in range(4)], axis=0)

        def o_passes():
            ms = {}
            asm = []
            for ng in range(2):
                def emit(r1, r2, n1, n2, c, ng=ng):
                    acc_s[t, 4 * ng + 2 * n1 + n2, pl.ds(r1 * HT + r2 * QT, QT), :] = c
                asm.append(_Assemble(emit))

            def run(ng, i1, i2, k, dep=None):
                u = 7 * i2 + i1
                lhs = jnp.concatenate([os_s[u, 4 * k + v] for v in range(4)], axis=1)
                w = jnp.concatenate([woc_s[2 * k + v, ng, u] for v in range(2)], axis=0)
                d = jnp.dot(lhs, pin_bf16(w, dep), preferred_element_type=f32)
                early = ng == 0 or (i1, i2) in prods[:NE]
                if k == 1:
                    d = d + ms.pop((ng, u))
                if k == (1 if early else 0):
                    ini = asm[ng].init(i1, i2)
                    if ini is not None:
                        d = d + ini
                if k == 0:
                    ms[ng, u] = d
                else:
                    asm[ng].add(i1, i2, d)
                return d
            NE = 16
            seq = [(0,) + pr + (0,) for pr in prods] + [(1,) + pr + (0,) for pr in prods[:NE]]
            seq += [(0,) + pr + (1,) for pr in prods] + [(1,) + pr + (1,) for pr in prods[:NE]]
            seq += [(1,) + pr + (k,) for pr in prods[NE:] for k in range(2)]
            return [functools.partial(run, *a) for a in seq]

        def side(hp, pts):
            rel = [release(v_, rw) for v_, rw in pts]
            for u in range(2):
                epi_rows(tprev, (2 * hp + u) * CHE, CHE, rel[u])
            if len(rel) == 3:
                ln1(tnext, hp * 16, 16, rel[2])
            else:
                for u in range(2):
                    ln1(tnext, hp * 16 + 8 * u, 8, rel[2 + u])
            return fence([(out_s.at[tprev], 0), (best_r, 0), (stat_s.at[tprev, 0], 0), (hf_s, 0)])

        def o_slice(qd, oq, u, pts):
            blk = [[[[oq[k1][k2][r1 * HT + r2 * QT + 16 * u:r1 * HT + r2 * QT + 16 * u + 16]
                      for k2 in range(2)] for k1 in range(2)] for r2 in range(2)] for r1 in range(2)]
            if len(pts) == 7:
                pts = [pts[PERML[i_]] for i_ in range(7)]
            ops = _two_level(_lhs_sums, blk, [jnp.tile(release(v_, rw), (2, 1)) for v_, rw in pts])
            for v in range(7):
                os_s[7 * v:7 * v + 7, qd, 16 * u:16 * u + 16, :] = ops[v]
            return fence([(os_s.at[0, qd], 16 * u)])

        assert 2 * HP * CHE == TQ
        for fn in q_passes(0):
            fn()
        opl = o_passes()
        oq = fo = ob_ = None
        for hp in range(HP):
            g, pp = divmod(hp, 4)
            if pp == 0:
                fill = q_passes(g + 1) if g + 1 < HKV else opl
            qa, qb = q_head(2 * hp), q_head(2 * hp + 1)
            sa_ = scores(qa if fo is None else pin(qa, {0: fo}), g)
            pa, la = softmax(sa_)
            vals = {'s': sa_, 'ob': ob_}
            if oq is not None:
                fl = [o_slice(hp // 2 - 1, oq, 2 * (hp % 2) + u, [(vals[nm], rw) for nm, rw in OS_PTS[u]])
                      for u in range(2 if FILL[pp][1] < 7 else 1)]
                qb = pin(qb, {0: functools.reduce(lambda a_, b_: a_ | b_, fl)})
            rs_ = [fill.pop(0)() for _ in range(FILL[pp][0])]
            vals.update({i_: rs_[max(len(rs_) - 6 + i_, 0)] for i_ in range(6)})
            fs = side(hp, [(vals[nm] if vals[nm] is not None else sa_, rw) for nm, rw in SIDE_PTS])
            pb, lb = softmax(scores(qb, g))
            oa_ = pv(pa, g)
            oa = oa_ * la
            rs_ = [fill.pop(0)() for _ in range(FILL[pp][1])]
            fo = None
            if oq is not None and FILL[pp][1] >= 7:
                vals = {'oa': oa_}
                vals.update(enumerate(rs_))
                fo = o_slice(hp // 2 - 1, oq, 2 * (hp % 2) + 1, [(vals[nm], rw) for nm, rw in OS_F2])
            ob_ = pv(pin(pb, {0: fs}), g)
            ob = ob_ * lb
            if hp % 2 == 0:
                oprev = (oa, ob)
            else:
                oq = [oprev, (oa, ob)]

        pts = []
        due = {} if fo is None else {2: fo}
        for s, fn in enumerate(opl):
            pts.append((fn(due.pop(s, None)), 0))
            if len(pts) % 3 == 0 and len(pts) <= 12:
                o_slice(HP // 2 - 1, oq, len(pts) // 3 - 1, pts[-3:])
            u, rem = divmod(s - HS0, HSG)
            if rem == 0 and 0 <= u < QT // 8:
                h_slice(u * 8, [release(pts[-1 - HSS * (6 - PERML[i_])][0]) for i_ in range(7)])
                due[s + 6] = fence([(hs_s.at[0], 0)])
        assert not due
        cp_out(tprev).start()
        return carry

    lax.fori_loop(1, nt, step, 0)

    cp_wg().wait()
    for u in range(F // MC):
        cp_wu(u).wait()
    cp_wd().wait()
    for t in range(nt - 1):
        cp_out(t).wait()
    epi_rows(nt - 1, 0, TQ)
    cp_out(nt - 1).start()
    bv = best_r[...]
    rbest = jnp.max(bv, axis=0, keepdims=True)
    ibest = jnp.min(jnp.where(bv == rbest, best_i[...], S), axis=0, keepdims=True)
    idx = jnp.minimum(ibest[0, 0], S - 1)
    base = pl.multiple_of((idx // 16) * 16, 16)
    tb = idx // TQ
    bsl = pl.ds(pl.multiple_of(base - tb * TQ, 16), 16)
    x1 = resid(tb, bsl, 16)
    h2 = h2_from_stats(x1, tb, bsl, 16)
    xs = h2.reshape(16, D).astype(bf16)
    gt = jnp.dot(xs, wq_s[:, 0:F], preferred_element_type=f32)
    up = jnp.concatenate([jnp.dot(xs, wmod_s[u], preferred_element_type=f32) for u in range(F // MC)], axis=1)
    a = (gt * jax.nn.sigmoid(gt) * up).astype(bf16)
    y = jnp.dot(a, wo_s[0:F, 0:D], preferred_element_type=f32)
    y = y * jnp.tile(jax.nn.sigmoid(rbest), (1, NB))
    rr = lax.broadcasted_iota(jnp.int32, (16, D), 0) + base
    upd = jnp.where(rr == idx, y, 0.0).reshape(2, 8, D)
    new = (x1 + mvec(5) * (h2 + upd)).reshape(16, D)
    cp_out(nt - 1).wait()
    out_s[tb, bsl, :] = new.astype(out_s.dtype)
    fix = pltpu.make_async_copy(out_s.at[tb, bsl, :], out_hbm.at[pl.ds(base, 16), :], osems.at[0])
    fix.start()
    fix.wait()


def _compiler_params():
    kw = dict(vmem_limit_bytes=124 * 1024 * 1024)
    try:
        return pltpu.CompilerParams(disable_semaphore_checks=True, disable_bounds_checks=True, **kw)
    except TypeError:
        return pltpu.CompilerParams(**kw)


@jax.jit
def pallas_adaLN_cond__sliding_block_cached__moe_arch_mod__prompt_kernel(
    A_x: jax.Array,
    A_k_cache: jax.Array,
    A_v_cache: jax.Array,
    A_wq: jax.Array,
    A_wo: jax.Array,
    B_x: jax.Array,
    B_w_r: jax.Array,
    B_w_gate: jax.Array,
    B_w_up: jax.Array,
    B_w_down: jax.Array,
    c: jax.Array,
    w_mod: jax.Array,
):
    B, S, D = A_x.shape
    assert B == 1
    HKV, SK = A_k_cache.shape[1], A_k_cache.shape[2]
    W = min(4096, max(256, SK // 4))
    F = B_w_gate.shape[1]
    dt = A_x.dtype
    f32 = jnp.float32
    nt = S // TQ
    NB = D // 128
    NMC = 6 * D // MC
    x2 = A_x.reshape(S, D)
    anyspec = pl.BlockSpec(memory_space=pl.ANY)
    kern = functools.partial(_kernel, S=S, D=D, HKV=HKV, SK=SK, W=W, F=F)
    out = pl.pallas_call(
        kern,
        in_specs=[anyspec] * 11,
        out_specs=anyspec,
        out_shape=jax.ShapeDtypeStruct((S, D), dt),
        scratch_shapes=[
            pltpu.VMEM((D,), dt),
            pltpu.VMEM((1, D), dt),
            pltpu.VMEM((nt, TQ, D), dt),
            pltpu.VMEM((HKV, W, DH), dt),
            pltpu.VMEM((HKV, W, DH), dt),
            pltpu.VMEM((D, HQ * DH + PAD), dt),
            pltpu.VMEM((HQ * DH, D + PAD), dt),
            pltpu.VMEM((NMC, D, MC), dt),
            pltpu.VMEM((nt, TQ, D), dt),
            pltpu.VMEM((HQ // 4, 49, D // 4, DH), dt),
            pltpu.VMEM((HQ * DH // D, 2, 49, 2 * DH, 128), dt),
            pltpu.VMEM((TQ, D), f32),
            pltpu.VMEM((49, TQ // 4, D // 4), dt),
            pltpu.VMEM((49, HQ // 4, TQ // 4, DH), dt),
            pltpu.VMEM((16, D), dt),
            pltpu.VMEM((NMC, 8, MC), f32),
            pltpu.VMEM((8, 7 * D), f32),
            pltpu.VMEM((TQ, D), dt),
            pltpu.VMEM((HQ, TQ // 2, DH), jnp.uint32),
            pltpu.VMEM((nt, NB, TQ, 128), f32),
            pltpu.VMEM((nt, 2, TQ, 128), f32),
            pltpu.VMEM((8, 128), f32),
            pltpu.VMEM((8, 128), jnp.int32),
            pltpu.SMEM((1,), jnp.int32),
            pltpu.SemaphoreType.DMA((4 + NMC + HQ + 2 * HKV + HQ * DH // D + nt,)),
            pltpu.SemaphoreType.DMA((nt,)),
        ],
        compiler_params=_compiler_params(),
    )(B_w_r, c, x2, A_k_cache, A_v_cache, A_wq, A_wo, w_mod, B_w_gate, B_w_up, B_w_down)
    return out.reshape(B, S, D)
```

```python
import functools

import jax
import jax.numpy as jnp
from jax import lax
import jax.experimental.pallas as pl
import jax.experimental.pallas.tpu as pltpu

HQ = 32
DH = 128
TQ = 256
PAD = 128
P0 = 4
G0 = 4
MC = 512
MSH = 1
CHE = 8
FILL = ((7, 7), (7, 7), (7, 7), (7, 0))

SIDE_PTS = ((1, 0), (2, 0), ('ob', 0), ('ob', 56))
OS_F2 = [('oa', 128), ('oa', 192), (0, 0), (1, 0), (2, 0), (3, 0), (4, 0)]
OS_PTS = ([('ob', 96 + 16 * i) for i in range(7)],
          [('ob', 208), ('ob', 224), ('ob', 240), ('s', 0), ('s', 16), ('s', 32), ('s', 48)])
HS0, HSG, HSS = 30, 14, 2
A0_W = (2, 250, 394, 760, 130, 150, 370)
A0_DUE = 14
O0_ROWS = ((0, 16, 32, 56, 72, 88, 112), (128, 144, 168, 184, 200, 224, 240))
O0_LN = (0, 1, 2, 3, 4, 5, 6, 7)
O0_LNROW = 24
O0_HS = (12, 15)
O0_HSROW = (8, 104, 192)
PERM = (3, 1, 4, 0, 5, 2, 6)
PERML = (0, 1, 2, 3, 4, 5, 6)

EPS = 1e-5
LOG2E = 1.4426950408889634


def _ln_stats(x, rel=None):
    d = x.shape[-1]
    part = x[..., 0:128]
    for j in range(1, d // 128):
        part = part + x[..., j * 128:(j + 1) * 128]
    if rel is not None:
        part = part + rel
    m = jnp.sum(part, axis=-1, keepdims=True) * (1.0 / d)
    xc = x - m
    v = jnp.mean(xc * xc, axis=-1, keepdims=True)
    return m, xc, lax.rsqrt(v + EPS)


def _ln(x, rel=None):
    _, xc, rs = _ln_stats(x, rel)
    return xc * rs


def _recip(l):
    return pl.reciprocal(l, approx=True)


def _lhs_sums(a11, a12, a21, a22):
    return [a11 + a22, a21 + a22, a11, a22, a11 + a12, a21 - a11, a12 - a22]


def _rhs_sums(b11, b12, b21, b22):
    return [b11 + b22, b11, b12 - b22, b21 - b11, b22, b11 + b12, b21 + b22]


_ORDER = [3, 4, 0, 6, 1, 2, 5]
_BLOCK = {6: (0, 0), 1: (1, 0), 2: (0, 1), 5: (1, 1)}


def _init(i, z):
    return {0: lambda: z[3] - z[4], 6: lambda: z[0], 1: lambda: z[3], 2: lambda: z[4],
            5: lambda: z[0] - z[1] + z[2]}.get(i, lambda: None)()


def _two_level(sums, blk, rel):
    o = [[jnp.stack([blk[a1][a2][b1][b2] for a2 in range(2) for b2 in range(2)]) for b1 in range(2)]
         for a1 in range(2)]
    if rel is not None and len(rel) == 3:
        o = [[o[a1][b1] + rel[0 if a1 == b1 else 1 + a1][None] for b1 in range(2)] for a1 in range(2)]
    x = jnp.stack(sums(o[0][0], o[0][1], o[1][0], o[1][1]), axis=1)
    x = [x[u] for u in range(4)]
    if rel is not None and len(rel) == 7:
        r7 = jnp.stack(rel)
        x = [x[0] + r7, x[1], x[2], x[3] + r7]
    return [y.astype(jnp.bfloat16) for y in sums(*x)]


class _Assemble:
    def __init__(self, emit):
        self.z, self.outer, self.inj, self.emit = {}, {}, {}, emit

    def init(self, i1, i2):
        v = _init(i2, self.z)
        if i2 in _BLOCK and i1 not in (3, 4):
            self.inj[i2] = _init(i1, self.outer[i2])
            v = v + self.inj[i2]
            if i2 == 5:
                v = v + (self.inj[1] - self.inj[2])
        return v

    def add(self, i1, i2, m):
        self.z[i2] = m
        if i2 in _BLOCK:
            self.outer.setdefault(i2, {})[i1] = m
            if i1 in _BLOCK:
                (r1, n1), (r2, n2) = _BLOCK[i1], _BLOCK[i2]
                self.emit(r1, r2, n1, n2, m)


def _kernel(wr_hbm, c_hbm, x_hbm, k_hbm, v_hbm, wq_hbm, wo_hbm, wmod_hbm,
            wg_hbm, wu_hbm, wd_hbm, out_hbm,
            wr_s, c_s, x_s, k_s, v_s, wq_s, wo_s, wmod_s, out_s,
            wqc_s, woc_s, hf_s, hs_s, os_s,
            sc_s, mraw_s, mod_s, h_s, o_s, acc_s, keep_s, cand_s, fix_s, best_r, best_i, zero_s, sems, osems,
            *, S, D, HKV, SK, W, F):
    nt = S // TQ
    rep = HQ // HKV
    NB = D // 128
    HP = HQ // 2
    HT = TQ // 2
    QT = TQ // 4
    KH = D // 2
    KQ = D // 4
    KP = 512
    CPV = D // MC
    NMC = 6 * CPV
    NA = (HQ - P0) // G0
    NO = HQ * DH // D
    f32 = jnp.float32
    bf16 = jnp.bfloat16
    u32 = jnp.uint32
    qscale = (DH ** -0.5) * LOG2E
    assert KH == KP and rep == 8 and NB == 8 and NO == 4 and P0 == 4 and G0 == 4

    def al(v, n):
        return v if isinstance(v, int) else pl.multiple_of(v, n)

    S_C, S_WR, S_WG, S_WD, S_M = 0, 1, 2, 3, 4
    S_WQ = S_M + NMC
    S_K = S_WQ + HQ
    S_V = S_K + HKV
    S_WO = S_V + HKV
    S_X = S_WO + NO

    def cp_c():
        return pltpu.make_async_copy(c_hbm, c_s, sems.at[S_C])

    def cp_wr():
        return pltpu.make_async_copy(wr_hbm, wr_s, sems.at[S_WR])

    def cp_mod(j):
        return pltpu.make_async_copy(wmod_hbm.at[:, pl.ds(al(j * MC, MC), MC)], wmod_s.at[j], sems.at[S_M + j])

    def cp_wg():
        return pltpu.make_async_copy(wg_hbm, wq_s.at[:, pl.ds(0, F)], sems.at[S_WG])

    def cp_wu(u):
        return pltpu.make_async_copy(wu_hbm.at[:, pl.ds(u * MC, MC)], wmod_s.at[u], sems.at[S_M + u])

    def cp_wd():
        return pltpu.make_async_copy(wd_hbm, wo_s.at[pl.ds(0, F), pl.ds(0, D)], sems.at[S_WD])

    def cp_wq(h, n=1):
        sl = pl.ds(al(h * DH, DH), n * DH)
        return pltpu.make_async_copy(wq_hbm.at[:, sl], wq_s.at[:, sl], sems.at[S_WQ + h])

    def cp_k(g):
        return pltpu.make_async_copy(k_hbm.at[0, g, pl.ds(SK - W, W), :], k_s.at[g], sems.at[S_K + g])

    def cp_v(g):
        return pltpu.make_async_copy(v_hbm.at[0, g, pl.ds(SK - W, W), :], v_s.at[g], sems.at[S_V + g])

    def cp_wo(j):
        sl = pl.ds(al(j * D, D), D)
        return pltpu.make_async_copy(wo_hbm.at[sl, :], wo_s.at[sl, pl.ds(0, D)], sems.at[S_WO + j])

    def rsl(t, r0=0, n=TQ):
        return pl.ds(al(t * TQ + r0, n), n)

    XE, X1, XL = 0, 1, 2

    def cp_x(t, slot):
        return pltpu.make_async_copy(x_hbm.at[rsl(t), :], x_s.at[slot], sems.at[S_X + slot])

    def cp_out(t):
        return pltpu.make_async_copy(out_s, out_hbm.at[rsl(t), :], osems.at[0])

    def sched():
        zero = zero_s[0]
        z16 = pl.multiple_of(zero, 16)
        zvec = jnp.full((8, 128), zero, jnp.int32).astype(u32)

        def fence(deps):
            d = None
            for ref, base in deps:
                n = 16 if ref.dtype == bf16 else 8
                v = pltpu.bitcast(ref[pl.ds(pl.multiple_of(base + z16, n), n), 0:128], u32)
                d = v if d is None else d | v
            return d & zvec

        def release(acc, r0=0):
            return pltpu.bitcast(pltpu.bitcast(acc[r0:r0 + 8, 0:128], u32) & zvec, f32)

        return fence, release

    def pin(a, at):
        if not at:
            return a
        parts = []
        prev = 0
        for rb in sorted(at):
            r0 = rb * 8
            if r0 > prev:
                parts.append(a[prev:r0, :])
            if a.dtype == f32:
                blk = a[r0:r0 + 8, 0:128] + pltpu.bitcast(at[rb], f32)
            else:
                blk = a[r0:r0 + 8, 0:128] | at[rb]
            if a.shape[1] > 128:
                blk = jnp.concatenate([blk, a[r0:r0 + 8, 128:]], axis=1)
            parts.append(blk)
            prev = r0 + 8
        if prev < a.shape[0]:
            parts.append(a[prev:, :])
        return jnp.concatenate(parts, axis=0)

    def pin_bf16(w, d):
        if d is None:
            return w
        top = pltpu.bitcast(pltpu.bitcast(w[0:16], u32) | d, bf16)
        return jnp.concatenate([top, w[16:]], axis=0)

    def mvec(j):
        return mod_s[:, j * D:(j + 1) * D][None]

    def mraw(j):
        return jnp.concatenate([mraw_s[j * CPV + u] for u in range(CPV)], axis=1)

    def xrows(t, sl, n):
        return x_s[t, sl, :].astype(f32).reshape(n // 8, 8, D)

    def ln1(t, r0, n, rel=None):
        xn = _ln(xrows(t, pl.ds(al(r0, n), n), n), rel)
        hf_s[pl.ds(al(r0, n), n), :] = (xn * mvec(1) + mvec(0)).reshape(n, D)

    def h_slice(r0, rel):
        hq = [hf_s[pl.ds(al(r * QT + r0, 8), 8), :] for r in range(4)]
        blk = [[[[hq[2 * r1 + r2][:, (2 * k1 + k2) * KQ:(2 * k1 + k2 + 1) * KQ] for k2 in range(2)]
                 for k1 in range(2)] for r2 in range(2)] for r1 in range(2)]
        ops = _two_level(_lhs_sums, blk, None if rel is None else [jnp.tile(v, (1, KQ // 128)) for v in rel])
        for u in range(7):
            hs_s[7 * u:7 * u + 7, pl.ds(al(r0, 8), 8), :] = ops[u]

    def w_unit(src, rows4, c0, dst, d0, rel):
        w = [src[pl.ds(al(r, 16), 16), c0:c0 + 512].astype(f32) for r in rows4]
        blk = [[[[w[2 * k1 + k2][:, (2 * n1 + n2) * 128:(2 * n1 + n2 + 1) * 128] for n2 in range(2)]
                 for n1 in range(2)] for k2 in range(2)] for k1 in range(2)]
        ops = _two_level(_rhs_sums, blk, None if rel is None else [jnp.tile(v, (2, 1)) for v in rel])
        for u in range(7):
            dst[7 * u:7 * u + 7, pl.ds(al(d0, 16), 16), :] = ops[u]
        return (dst.at[0], d0)

    def epi_rows(t, r0, n, rel=None):
        sl = pl.ds(r0, n)
        attn = jnp.concatenate([acc_s[j, sl, :] for j in range(NB)], axis=1).reshape(n // 8, 8, D)
        x1 = xrows(XE, sl, n) + mvec(2) * attn
        m, xc, rs = _ln_stats(x1, rel)
        keep_s[sl, 0:D] = x1.reshape(n, D)
        keep_s[sl, D:D + 128] = jnp.broadcast_to(m.reshape(n, 1), (n, 128))
        keep_s[sl, D + 128:D + 256] = jnp.broadcast_to(rs.reshape(n, 1), (n, 128))
        h2 = xc * rs * mvec(4) + mvec(3)
        out_s[sl, :] = (x1 + mvec(5) * h2).reshape(n, D).astype(out_s.dtype)
        r = jnp.sum(h2 * mvec(6), axis=-1, keepdims=True)
        r = r.astype(bf16).astype(f32)
        bv = best_r[...]
        bi = best_i[...]
        sub = lax.broadcasted_iota(jnp.int32, (8, 128), 0)
        for u in range(n // 8):
            ru = jnp.broadcast_to(r[u], (8, 128))
            better = ru > bv
            bv = jnp.where(better, ru, bv)
            bi = jnp.where(better, sub + (t * TQ + r0 + u * 8), bi)
        best_r[...] = bv
        best_i[...] = bi

    def capture(t):
        bv = best_r[...]
        rbest = jnp.max(bv, axis=0, keepdims=True)
        ibest = jnp.min(jnp.where(bv == rbest, best_i[...], S), axis=0, keepdims=True)
        idx = jnp.minimum(ibest[0, 0], S - 1)
        local = idx - t * TQ
        off = pl.multiple_of(jnp.clip(local // 16, 0, TQ // 16 - 1) * 16, 16)
        rows = jnp.where(local >= 0, keep_s[pl.ds(off, 16), :], cand_s[...])
        cand_s[...] = rows
        return rbest, idx, rows

    def scores(q, g):
        return lax.dot_general(q.astype(bf16), k_s[g], (((1,), (1,)), ((), ())), preferred_element_type=f32)

    def softmax(s):
        m = jnp.max(s, axis=-1, keepdims=True)
        p = jnp.exp2(s - m)
        part = p[:, 0:128]
        for j in range(1, W // 128):
            part = part + p[:, j * 128:(j + 1) * 128]
        p = jnp.concatenate([jnp.minimum(p[:, 0:128], part), p[:, 128:]], axis=1)
        return p, _recip(jnp.sum(part, axis=-1, keepdims=True))

    def pv(p, g):
        return jnp.dot(p.astype(bf16), v_s[g], preferred_element_type=f32)

    def block0(wv, c0, h0, nh, units):
        fence, release = sched()
        hval = h_s[...]
        g = h0 // rep
        tqk = [512 + 1024 * u for u in range(nh)]
        tpv = [tqk[u] + (768 if u + 1 < nh else 256) for u in range(nh)]
        wins = [(130, tqk[0])]
        for u in range(nh):
            wins.append((tqk[u] + A0_W[0], tqk[u] + (A0_W[1] if u + 1 < nh else A0_W[4])))
            if u + 1 < nh:
                wins.append((tqk[u] + A0_W[2], tqk[u] + A0_W[3]))
        wins.append((tpv[-1] + A0_W[5], tpv[-1] + A0_W[6]))
        slots = [t_ for a_, b_ in wins for t_ in range(a_, b_, 8)]
        npt = 7 * len(units)
        times = [slots[(u * len(slots)) // npt] for u in range(npt)]
        todo = [(un, times[7 * u:7 * u + 7]) for u, un in enumerate(units)]
        vals = []

        def emit(tmax):
            last = []
            while todo and todo[0][1][-1] < tmax:
                (sv, dv, r0), ts = todo.pop(0)
                rel = []
                for i_ in range(7):
                    t0_, v_ = [tv for tv in vals if tv[0] <= ts[PERM[i_]]][-1]
                    rel.append(release(v_, min((ts[PERM[i_]] - t0_) // 8 * 8, TQ - 8)))
                last = last[-1:] + [w_unit(sv, [c * KQ + r0 for c in range(4)], 0, dv, r0, rel)]
            return last

        def qproj(u, t_):
            cols = slice(c0 + u * DH, c0 + (u + 1) * DH)
            q1 = jnp.dot(hval[:, 0:KH], wv[0:KH, cols], preferred_element_type=f32)
            q2 = jnp.dot(hval[:, KH:D], wv[KH:D, cols], preferred_element_type=f32) + q1
            vals.extend([(t_ + 130, q1), (t_ + 386, q2)])
            return q2

        q = qproj(0, 0)
        for u in range(nh):
            s = scores(q, g)
            vals.append((tqk[u] + 130, s))
            p, li = softmax(s)
            if u + 1 < nh:
                q = qproj(u + 1, tqk[u] + 256)
            deps = emit(tpv[u]) + ([(o_s.at[h0 + u - 1], 0)] if u > 0 else [])
            if deps:
                p = pin(p, {A0_DUE: fence(deps)})
            o = pv(p, g)
            vals.append((tpv[u] + 130, o))
            o_s[h0 + u] = pltpu.bitcast((o * li).astype(bf16), u32)
        emit(1 << 30)

    cp_c().start()
    cp_x(0, XE).start()
    for j in range(2 * CPV):
        cp_mod(j).start()
    cp_wq(0).start()
    cp_k(0).start()
    cp_v(0).start()
    cp_wq(1, P0 - 1).start()
    for j in range(NA):
        h0 = P0 + j * G0
        cp_wq(h0, G0).start()
        if h0 % rep == 0:
            cp_k(h0 // rep).start()
            cp_v(h0 // rep).start()
    cp_x(1, X1).start()
    cp_wr().start()
    for j in range(NO):
        cp_wo(j).start()
        for u in range(CPV):
            if (j + 2) * CPV + u - MSH >= 2 * CPV:
                cp_mod((j + 2) * CPV + u - MSH).start()
    for u in range(NMC - MSH, NMC):
        cp_mod(u).start()
    cp_x(2, XL).start()

    zero_s[0] = 0
    for n in range(NB):
        acc_s[n] = jnp.zeros((TQ, 128), f32)
    hs_s[0] = jnp.zeros((QT, KQ), bf16)
    cand_s[...] = jnp.zeros(cand_s.shape, f32)
    best_r[...] = jnp.full(best_r.shape, -jnp.inf, f32)
    best_i[...] = jnp.zeros(best_i.shape, jnp.int32)
    cp_c().wait()
    cp_x(0, XE).wait()
    cf = c_s[...].astype(f32)
    sc_s[...] = jnp.broadcast_to(cf * jax.nn.sigmoid(cf), (16, D)).astype(bf16)
    xn0 = _ln(xrows(XE, pl.ds(0, TQ), TQ))

    def mod_body(j, carry):
        cp_mod(j).wait()
        mraw_s[j] = jnp.dot(sc_s[...], wmod_s[j], preferred_element_type=f32)[0:8, :]
        return carry

    lax.fori_loop(0, 2 * CPV, mod_body, 0)
    mod_s[:, 0:D] = mraw(0) * qscale
    mod_s[:, D:2 * D] = (1.0 + mraw(1)) * qscale
    h_s[...] = (xn0 * mvec(1) + mvec(0)).reshape(TQ, D).astype(bf16)
    NU = KQ // 16
    NPE = NU - NA
    cp_wq(0).wait()
    cp_k(0).wait()
    cp_v(0).wait()
    block0(wq_s, 0, 0, 1, [])
    cp_wq(1, P0 - 1).wait()
    block0(wq_s, DH, 1, P0 - 1, [(wq_s, wqc_s.at[0], u * 16) for u in range(NPE)])

    def a0_body(j, carry):
        h0 = P0 + j * G0
        cp_wq(h0, G0).wait()

        @pl.when(h0 % rep == 0)
        def _():
            cp_k(h0 // rep).wait()
            cp_v(h0 // rep).wait()

        sv = wq_s.at[:, pl.ds(al(h0 * DH, 4 * DH), 4 * DH)]
        dv = wqc_s.at[j + 1]
        block0(sv, 0, h0, G0, [(sv, dv, u * 16) for u in range(NU)] + [(wq_s, wqc_s.at[0], (NPE + j) * 16)])
        return carry

    lax.fori_loop(0, NA, a0_body, 0)
    cp_x(1, X1).wait()
    cp_wr().wait()

    def o0_body(j, carry):
        cp_wo(j).wait()
        for u in range(CPV):
            if u >= MSH:
                cp_mod((j + 2) * CPV + u - MSH).wait()
            else:
                @pl.when(j > 0)
                def _():
                    cp_mod((j + 2) * CPV + u - MSH).wait()

        fence, release = sched()
        sc = sc_s[...]
        hq = KP // DH
        wo_j = wo_s.at[pl.ds(al(j * D, D), D)]
        o_j = o_s.at[pl.ds(j * (D // DH), D // DH)]
        wm_j = wmod_s.at[pl.ds((j + 2) * CPV - MSH, CPV)]
        mr_j = mraw_s.at[pl.ds((j + 2) * CPV - MSH, CPV)]
        units = [(qd, ng, u) for qd in range(2) for ng in range(2) for u in range(DH // 16)]
        npass = NB * (D // KP)
        cnt = 0
        due = {}
        hist = []
        lhs2 = [jnp.concatenate([o_j[kh * hq + u] for u in range(hq)], axis=1) for kh in range(D // KP)]
        for n in range(NB):
            acc = acc_s[n]
            cu, cn = divmod(n, MC // 128)
            mv = None
            for kh in range(D // KP):
                lhs = lhs2[kh]
                acc = jnp.dot(pltpu.bitcast(pin(lhs, due.pop(cnt, None)), bf16),
                              wo_j[kh * KP:(kh + 1) * KP, n * 128:(n + 1) * 128],
                              preferred_element_type=f32) + acc
                hist.append(acc)
                mine = units[cnt * len(units) // npass:(cnt + 1) * len(units) // npass]
                for n_, (qd, ng, u) in enumerate(mine):
                    last = w_unit(wo_j, [(4 * qd + c) * DH + u * 16 for c in range(4)], ng * 512,
                                  woc_s.at[j, ng], qd * DH + u * 16, [release(acc, O0_ROWS[n_][PERM[i_]]) for i_ in range(7)])
                if cnt + 2 < npass:
                    due.setdefault(cnt + 2, {})[2] = fence([last])
                if cnt in O0_LN:
                    qr, hf_ = O0_LN.index(cnt) % 4, O0_LN.index(cnt) // 4
                    ln1(X1, qr * QT + j * 16 + hf_ * 8, 8, release(acc, O0_LNROW))
                    due.setdefault(cnt + 3, {})[4] = fence([(hf_s, qr * QT + j * 16 + hf_ * 8)])
                if cnt in O0_HS:
                    hp_ = [(hist[-3 + u_ // 3], O0_HSROW[u_ % 3]) for u_ in range(9)]
                    h_slice(j * 16 + O0_HS.index(cnt) * 8, [release(*hp_[PERML[i_]]) for i_ in range(7)])
                    if cnt == O0_HS[0]:
                        due.setdefault(cnt + 2, {})[10] = fence([(hs_s.at[0], j * 16)])
                cnt += 1
                d = jnp.dot(sc[:, kh * KP:(kh + 1) * KP],
                            wm_j[cu, kh * KP:(kh + 1) * KP, cn * 128:(cn + 1) * 128],
                            preferred_element_type=f32)
                mv = d if mv is None else d + mv
            acc_s[n] = acc
            mr_j[cu, :, cn * 128:(cn + 1) * 128] = mv[0:8, :]
        assert not due
        return carry

    lax.fori_loop(0, NO, o0_body, 0)

    for u in range(NMC - MSH, NMC):
        cp_mod(u).wait()
    for u in range(NMC - MSH, NMC):
        mraw_s[u] = jnp.dot(sc_s[...], wmod_s[u], preferred_element_type=f32)[0:8, :]
    mod_s[:, 2 * D:3 * D] = mraw(2)
    mod_s[:, 3 * D:4 * D] = mraw(3)
    mod_s[:, 4 * D:5 * D] = 1.0 + mraw(4)
    mod_s[:, 5 * D:6 * D] = mraw(5)
    mod_s[:, 6 * D:7 * D] = jnp.broadcast_to(wr_s[...].astype(f32).reshape(1, D), (8, D))
    cp_wg().start(priority=1)
    for u in range(F // MC):
        cp_wu(u).start(priority=1)
    cp_wd().start(priority=1)

    def step(t, carry):
        cp_x(0, XL).wait()

        @pl.when(t > 1)
        def _():
            cp_x(0, XE).wait()
            cp_out(0).wait()

        fence, release = sched()
        tprev = t - 1
        prods = [(i1, i2) for i1 in _ORDER for i2 in _ORDER]
        hv = [hs_s[u] for u in range(49)]

        qblk = {}

        def q_passes(g):
            def emit(r1, r2, n1, n2, c):
                for z in range(2):
                    qblk[8 * g + 4 * z + 2 * n1 + n2, 2 * r1 + r2] = c[:, z * DH:(z + 1) * DH]
            asm = _Assemble(emit)

            def run(i1, i2):
                u = 7 * i2 + i1
                w = jnp.concatenate([wqc_s[2 * g + z, u] for z in range(2)], axis=1)
                d = jnp.dot(hv[u], w, preferred_element_type=f32)
                ini = asm.init(i1, i2)
                if ini is not None:
                    d = d + ini
                asm.add(i1, i2, d)
                return d
            return [functools.partial(run, i1, i2) for i1, i2 in prods]

        def q_head(hh):
            return jnp.concatenate([qblk.pop((hh, r)) for r in range(4)], axis=0)

        def o_passes():
            ms = {}
            asm = []
            for ng in range(2):
                def emit(r1, r2, n1, n2, c, ng=ng):
                    acc_s[4 * ng + 2 * n1 + n2, pl.ds(r1 * HT + r2 * QT, QT), :] = c
                asm.append(_Assemble(emit))

            def run(ng, i1, i2, k, dep=None):
                u = 7 * i2 + i1
                lhs = jnp.concatenate([os_s[u, 4 * k + v] for v in range(4)], axis=1)
                w = jnp.concatenate([woc_s[2 * k + v, ng, u] for v in range(2)], axis=0)
                d = jnp.dot(lhs, pin_bf16(w, dep), preferred_element_type=f32)
                early = ng == 0 or (i1, i2) in prods[:NE]
                if k == 1:
                    d = d + ms.pop((ng, u))
                if k == (1 if early else 0):
                    ini = asm[ng].init(i1, i2)
                    if ini is not None:
                        d = d + ini
                if k == 0:
                    ms[ng, u] = d
                else:
                    asm[ng].add(i1, i2, d)
                return d
            NE = 16
            seq = [(0,) + pr + (0,) for pr in prods] + [(1,) + pr + (0,) for pr in prods[:NE]]
            seq += [(0,) + pr + (1,) for pr in prods] + [(1,) + pr + (1,) for pr in prods[:NE]]
            seq += [(1,) + pr + (k,) for pr in prods[NE:] for k in range(2)]
            return [functools.partial(run, *a) for a in seq]

        def side(hp, pts):
            rel = [release(v_, rw) for v_, rw in pts]
            for u in range(2):
                epi_rows(tprev, (2 * hp + u) * CHE, CHE, rel[u])
            if len(rel) == 3:
                ln1(XL, hp * 16, 16, rel[2])
            else:
                for u in range(2):
                    ln1(XL, hp * 16 + 8 * u, 8, rel[2 + u])
            return fence([(out_s, 0), (best_r, 0), (keep_s, 0), (hf_s, 0)])

        def o_slice(qd, oq, u, pts):
            blk = [[[[oq[k1][k2][r1 * HT + r2 * QT + 16 * u:r1 * HT + r2 * QT + 16 * u + 16]
                      for k2 in range(2)] for k1 in range(2)] for r2 in range(2)] for r1 in range(2)]
            if len(pts) == 7:
                pts = [pts[PERML[i_]] for i_ in range(7)]
            ops = _two_level(_lhs_sums, blk, [jnp.tile(release(v_, rw), (2, 1)) for v_, rw in pts])
            for v in range(7):
                os_s[7 * v:7 * v + 7, qd, 16 * u:16 * u + 16, :] = ops[v]
            return fence([(os_s.at[0, qd], 16 * u)])

        assert 2 * HP * CHE == TQ
        for fn in q_passes(0):
            fn()
        opl = o_passes()
        oq = fo = ob_ = None
        for hp in range(HP):
            g, pp = divmod(hp, 4)
            if pp == 0:
                fill = q_passes(g + 1) if g + 1 < HKV else opl
            qa, qb = q_head(2 * hp), q_head(2 * hp + 1)
            sa_ = scores(qa if fo is None else pin(qa, {0: fo}), g)
            pa, la = softmax(sa_)
            vals = {'s': sa_, 'ob': ob_}
            if oq is not None:
                fl = [o_slice(hp // 2 - 1, oq, 2 * (hp % 2) + u, [(vals[nm], rw) for nm, rw in OS_PTS[u]])
                      for u in range(2 if FILL[pp][1] < 7 else 1)]
                qb = pin(qb, {0: functools.reduce(lambda a_, b_: a_ | b_, fl)})
            rs_ = [fill.pop(0)() for _ in range(FILL[pp][0])]
            vals.update({i_: rs_[max(len(rs_) - 6 + i_, 0)] for i_ in range(6)})
            fs = side(hp, [(vals[nm] if vals[nm] is not None else sa_, rw) for nm, rw in SIDE_PTS])
            pb, lb = softmax(scores(qb, g))
            oa_ = pv(pa, g)
            oa = oa_ * la
            rs_ = [fill.pop(0)() for _ in range(FILL[pp][1])]
            fo = None
            if oq is not None and FILL[pp][1] >= 7:
                vals = {'oa': oa_}
                vals.update(enumerate(rs_))
                fo = o_slice(hp // 2 - 1, oq, 2 * (hp % 2) + 1, [(vals[nm], rw) for nm, rw in OS_F2])
            ob_ = pv(pin(pb, {0: fs}), g)
            ob = ob_ * lb
            if hp % 2 == 0:
                oprev = (oa, ob)
            else:
                oq = [oprev, (oa, ob)]

        capture(tprev)
        cp_out(tprev).start()
        cp_x(t, XE).start()
        cp_x(jnp.minimum(t + 2, nt - 1), XL).start()
        pts = []
        due = {} if fo is None else {2: fo}
        for s, fn in enumerate(opl):
            pts.append((fn(due.pop(s, None)), 0))
            if len(pts) % 3 == 0 and len(pts) <= 12:
                o_slice(HP // 2 - 1, oq, len(pts) // 3 - 1, pts[-3:])
            u, rem = divmod(s - HS0, HSG)
            if rem == 0 and 0 <= u < QT // 8:
                h_slice(u * 8, [release(pts[-1 - HSS * (6 - PERML[i_])][0]) for i_ in range(7)])
                due[s + 6] = fence([(hs_s.at[0], 0)])
        assert not due
        return carry

    lax.fori_loop(1, nt, step, 0)

    cp_wg().wait()
    for u in range(F // MC):
        cp_wu(u).wait()
    cp_wd().wait()
    cp_x(0, XL).wait()
    cp_x(0, XE).wait()
    cp_out(0).wait()
    epi_rows(nt - 1, 0, TQ)
    cp_out(nt - 1).start()
    rbest, idx, rows = capture(nt - 1)
    base = pl.multiple_of((idx // 16) * 16, 16)
    x1 = rows[:, 0:D].reshape(2, 8, D)
    mu = jnp.tile(rows[:, D:D + 128], (1, NB)).reshape(2, 8, D)
    rs = jnp.tile(rows[:, D + 128:D + 256], (1, NB)).reshape(2, 8, D)
    h2 = (x1 - mu) * rs * mvec(4) + mvec(3)
    xs = h2.reshape(16, D).astype(bf16)
    gt = jnp.dot(xs, wq_s[:, 0:F], preferred_element_type=f32)
    up = jnp.concatenate([jnp.dot(xs, wmod_s[u], preferred_element_type=f32) for u in range(F // MC)], axis=1)
    a = (gt * jax.nn.sigmoid(gt) * up).astype(bf16)
    y = jnp.dot(a, wo_s[0:F, 0:D], preferred_element_type=f32)
    y = y * jnp.tile(jax.nn.sigmoid(rbest), (1, NB))
    rr = lax.broadcasted_iota(jnp.int32, (16, D), 0) + base
    upd = jnp.where(rr == idx, y, 0.0).reshape(2, 8, D)
    new = (x1 + mvec(5) * (h2 + upd)).reshape(16, D)
    fix_s[...] = new.astype(fix_s.dtype)
    cp_out(nt - 1).wait()
    fix = pltpu.make_async_copy(fix_s, out_hbm.at[pl.ds(base, 16), :], osems.at[0])
    fix.start()
    fix.wait()


def _compiler_params():
    kw = dict(vmem_limit_bytes=124 * 1024 * 1024)
    try:
        return pltpu.CompilerParams(disable_semaphore_checks=True, disable_bounds_checks=True, **kw)
    except TypeError:
        return pltpu.CompilerParams(**kw)


@jax.jit
def pallas_adaLN_cond__sliding_block_cached__moe_arch_mod__prompt_kernel(
    A_x: jax.Array,
    A_k_cache: jax.Array,
    A_v_cache: jax.Array,
    A_wq: jax.Array,
    A_wo: jax.Array,
    B_x: jax.Array,
    B_w_r: jax.Array,
    B_w_gate: jax.Array,
    B_w_up: jax.Array,
    B_w_down: jax.Array,
    c: jax.Array,
    w_mod: jax.Array,
):
    B, S, D = A_x.shape
    assert B == 1
    HKV, SK = A_k_cache.shape[1], A_k_cache.shape[2]
    W = min(4096, max(256, SK // 4))
    F = B_w_gate.shape[1]
    dt = A_x.dtype
    f32 = jnp.float32
    nt = S // TQ
    NB = D // 128
    NMC = 6 * D // MC
    x2 = A_x.reshape(S, D)
    anyspec = pl.BlockSpec(memory_space=pl.ANY)
    kern = functools.partial(_kernel, S=S, D=D, HKV=HKV, SK=SK, W=W, F=F)
    out = pl.pallas_call(
        kern,
        in_specs=[anyspec] * 11,
        out_specs=anyspec,
        out_shape=jax.ShapeDtypeStruct((S, D), dt),
        scratch_shapes=[
            pltpu.VMEM((D,), dt),
            pltpu.VMEM((1, D), dt),
            pltpu.VMEM((3, TQ, D), dt),
            pltpu.VMEM((HKV, W, DH), dt),
            pltpu.VMEM((HKV, W, DH), dt),
            pltpu.VMEM((D, HQ * DH + PAD), dt),
            pltpu.VMEM((HQ * DH, D + PAD), dt),
            pltpu.VMEM((NMC, D, MC), dt),
            pltpu.VMEM((TQ, D), dt),
            pltpu.VMEM((HQ // 4, 49, D // 4, DH), dt),
            pltpu.VMEM((HQ * DH // D, 2, 49, 2 * DH, 128), dt),
            pltpu.VMEM((TQ, D), f32),
            pltpu.VMEM((49, TQ // 4, D // 4), dt),
            pltpu.VMEM((49, HQ // 4, TQ // 4, DH), dt),
            pltpu.VMEM((16, D), dt),
            pltpu.VMEM((NMC, 8, MC), f32),
            pltpu.VMEM((8, 7 * D), f32),
            pltpu.VMEM((TQ, D), dt),
            pltpu.VMEM((HQ, TQ // 2, DH), jnp.uint32),
            pltpu.VMEM((NB, TQ, 128), f32),
            pltpu.VMEM((TQ, D + 256), f32),
            pltpu.VMEM((16, D + 256), f32),
            pltpu.VMEM((16, D), dt),
            pltpu.VMEM((8, 128), f32),
            pltpu.VMEM((8, 128), jnp.int32),
            pltpu.SMEM((1,), jnp.int32),
            pltpu.SemaphoreType.DMA((4 + NMC + HQ + 2 * HKV + HQ * DH // D + 3,)),
            pltpu.SemaphoreType.DMA((2,)),
        ],
        compiler_params=_compiler_params(),
    )(B_w_r, c, x2, A_k_cache, A_v_cache, A_wq, A_wo, w_mod, B_w_gate, B_w_up, B_w_down)
    return out.reshape(B, S, D)
```

```python
import functools

import jax
import jax.numpy as jnp
from jax import lax
import jax.experimental.pallas as pl
import jax.experimental.pallas.tpu as pltpu

HQ = 32
DH = 128
TQ = 256
PAD = 128
P0 = 4
G0 = 4
MC = 512
MSH = 1
CHE = 8
FILL = ((7, 7), (7, 7), (7, 7), (7, 0))

SIDE_PTS = ((1, 48), (2, 48), ('ob', 0), ('ob', 56))
OS_F2 = [('oa', 128), ('oa', 192), (0, 0), (1, 0), (2, 0), (3, 0), (4, 0)]
OS_PTS = ([('ob', 96 + 16 * i) for i in range(7)],
          [('ob', 208), ('ob', 224), ('ob', 240), ('s', 0), ('s', 16), ('s', 32), ('s', 48)])
HS0, HSG, HSS = 30, 14, 2
A0_W = (2, 250, 394, 760, 130, 150, 370)
A0_DUE = 14
O0_ROWS = ((0, 16, 32, 56, 72, 88, 112), (128, 144, 168, 184, 200, 224, 240))
O0_LN = (0, 1, 2, 3, 4, 5, 6, 7)
O0_LNROW = 24
O0_HS = (12, 15)
O0_HSROW = (8, 104, 192)
PERM = (3, 1, 4, 0, 5, 2, 6)
PERML = (0, 1, 2, 3, 4, 5, 6)

T_EARLY = 8
EPS = 1e-5
LOG2E = 1.4426950408889634


def _ln_stats(x, rel=None):
    d = x.shape[-1]
    part = x[..., 0:128]
    for j in range(1, d // 128):
        part = part + x[..., j * 128:(j + 1) * 128]
    if rel is not None:
        part = part + rel
    m = jnp.sum(part, axis=-1, keepdims=True) * (1.0 / d)
    xc = x - m
    v = jnp.mean(xc * xc, axis=-1, keepdims=True)
    return m, xc, lax.rsqrt(v + EPS)


def _ln(x, rel=None):
    _, xc, rs = _ln_stats(x, rel)
    return xc * rs


def _recip(l):
    return pl.reciprocal(l, approx=True)


def _lhs_sums(a11, a12, a21, a22):
    return [a11 + a22, a21 + a22, a11, a22, a11 + a12, a21 - a11, a12 - a22]


def _rhs_sums(b11, b12, b21, b22):
    return [b11 + b22, b11, b12 - b22, b21 - b11, b22, b11 + b12, b21 + b22]


_ORDER = [3, 4, 0, 6, 1, 2, 5]
_BLOCK = {6: (0, 0), 1: (1, 0), 2: (0, 1), 5: (1, 1)}


def _init(i, z):
    return {0: lambda: z[3] - z[4], 6: lambda: z[0], 1: lambda: z[3], 2: lambda: z[4],
            5: lambda: z[0] - z[1] + z[2]}.get(i, lambda: None)()


def _two_level(sums, blk, rel):
    o = [[jnp.stack([blk[a1][a2][b1][b2] for a2 in range(2) for b2 in range(2)]) for b1 in range(2)]
         for a1 in range(2)]
    if rel is not None and len(rel) == 3:
        o = [[o[a1][b1] + rel[0 if a1 == b1 else 1 + a1][None] for b1 in range(2)] for a1 in range(2)]
    x = jnp.stack(sums(o[0][0], o[0][1], o[1][0], o[1][1]), axis=1)
    x = [x[u] for u in range(4)]
    if rel is not None and len(rel) == 7:
        r7 = jnp.stack(rel)
        x = [x[0] + r7, x[1], x[2], x[3] + r7]
    return [y.astype(jnp.bfloat16) for y in sums(*x)]


class _Assemble:
    def __init__(self, emit):
        self.z, self.outer, self.inj, self.emit = {}, {}, {}, emit

    def init(self, i1, i2):
        v = _init(i2, self.z)
        if i2 in _BLOCK and i1 not in (3, 4):
            self.inj[i2] = _init(i1, self.outer[i2])
            v = v + self.inj[i2]
            if i2 == 5:
                v = v + (self.inj[1] - self.inj[2])
        return v

    def add(self, i1, i2, m):
        self.z[i2] = m
        if i2 in _BLOCK:
            self.outer.setdefault(i2, {})[i1] = m
            if i1 in _BLOCK:
                (r1, n1), (r2, n2) = _BLOCK[i1], _BLOCK[i2]
                self.emit(r1, r2, n1, n2, m)


def _kernel(wr_hbm, c_hbm, x_hbm, k_hbm, v_hbm, wq_hbm, wo_hbm, wmod_hbm,
            wg_hbm, wu_hbm, wd_hbm, out_hbm,
            wr_s, c_s, x_s, k_s, v_s, wq_s, wo_s, wmod_s, out_s,
            wqc_s, woc_s, hf_s, hs_s, os_s,
            sc_s, mraw_s, mod_s, h_s, o_s, acc_s, keep_s, cand_s, fix_s, best_r, best_i, zero_s, sems, osems,
            *, S, D, HKV, SK, W, F):
    nt = S // TQ
    rep = HQ // HKV
    NB = D // 128
    HP = HQ // 2
    HT = TQ // 2
    QT = TQ // 4
    KH = D // 2
    KQ = D // 4
    KP = 512
    CPV = D // MC
    NMC = 6 * CPV
    NA = (HQ - P0) // G0
    NO = HQ * DH // D
    f32 = jnp.float32
    bf16 = jnp.bfloat16
    u32 = jnp.uint32
    qscale = (DH ** -0.5) * LOG2E
    assert KH == KP and rep == 8 and NB == 8 and NO == 4 and P0 == 4 and G0 == 4

    def al(v, n):
        return v if isinstance(v, int) else pl.multiple_of(v, n)

    S_C, S_WR, S_WG, S_WD, S_M = 0, 1, 2, 3, 4
    S_WQ = S_M + NMC
    S_K = S_WQ + HQ
    S_V = S_K + HKV
    S_WO = S_V + HKV
    S_X = S_WO + NO

    def cp_c():
        return pltpu.make_async_copy(c_hbm, c_s, sems.at[S_C])

    def cp_wr():
        return pltpu.make_async_copy(wr_hbm, wr_s, sems.at[S_WR])

    def cp_mod(j):
        return pltpu.make_async_copy(wmod_hbm.at[:, pl.ds(al(j * MC, MC), MC)], wmod_s.at[j], sems.at[S_M + j])

    def cp_wg():
        return pltpu.make_async_copy(wg_hbm, wq_s.at[:, pl.ds(0, F)], sems.at[S_WG])

    def cp_wu(u):
        return pltpu.make_async_copy(wu_hbm.at[:, pl.ds(u * MC, MC)], wmod_s.at[u], sems.at[S_M + u])

    def cp_wd():
        return pltpu.make_async_copy(wd_hbm, wo_s.at[pl.ds(0, F), pl.ds(0, D)], sems.at[S_WD])

    def cp_wq(h, n=1):
        sl = pl.ds(al(h * DH, DH), n * DH)
        return pltpu.make_async_copy(wq_hbm.at[:, sl], wq_s.at[:, sl], sems.at[S_WQ + h])

    def cp_k(g):
        return pltpu.make_async_copy(k_hbm.at[0, g, pl.ds(SK - W, W), :], k_s.at[g], sems.at[S_K + g])

    def cp_v(g):
        return pltpu.make_async_copy(v_hbm.at[0, g, pl.ds(SK - W, W), :], v_s.at[g], sems.at[S_V + g])

    def cp_wo(j):
        sl = pl.ds(al(j * D, D), D)
        return pltpu.make_async_copy(wo_hbm.at[sl, :], wo_s.at[sl, pl.ds(0, D)], sems.at[S_WO + j])

    def rsl(t, r0=0, n=TQ):
        return pl.ds(al(t * TQ + r0, n), n)

    XE, X1, XL = 0, 1, 2

    def cp_x(t, slot):
        return pltpu.make_async_copy(x_hbm.at[rsl(t), :], x_s.at[slot], sems.at[S_X + slot])

    def cp_out(t):
        return pltpu.make_async_copy(out_s, out_hbm.at[rsl(t), :], osems.at[0])

    def sched():
        zero = zero_s[0]
        z16 = pl.multiple_of(zero, 16)
        zvec = jnp.full((8, 128), zero, jnp.int32).astype(u32)

        def fence(deps):
            d = None
            for ref, base in deps:
                n = 16 if ref.dtype == bf16 else 8
                v = pltpu.bitcast(ref[pl.ds(pl.multiple_of(base + z16, n), n), 0:128], u32)
                d = v if d is None else d | v
            return d & zvec

        def release(acc, r0=0):
            return pltpu.bitcast(pltpu.bitcast(acc[r0:r0 + 8, 0:128], u32) & zvec, f32)

        return fence, release

    def pin(a, at):
        if not at:
            return a
        parts = []
        prev = 0
        for rb in sorted(at):
            r0 = rb * 8
            if r0 > prev:
                parts.append(a[prev:r0, :])
            if a.dtype == f32:
                blk = a[r0:r0 + 8, 0:128] + pltpu.bitcast(at[rb], f32)
            else:
                blk = a[r0:r0 + 8, 0:128] | at[rb]
            if a.shape[1] > 128:
                blk = jnp.concatenate([blk, a[r0:r0 + 8, 128:]], axis=1)
            parts.append(blk)
            prev = r0 + 8
        if prev < a.shape[0]:
            parts.append(a[prev:, :])
        return jnp.concatenate(parts, axis=0)

    def pin_bf16(w, d):
        if d is None:
            return w
        top = pltpu.bitcast(pltpu.bitcast(w[0:16], u32) | d, bf16)
        return jnp.concatenate([top, w[16:]], axis=0)

    def mvec(j):
        return mod_s[:, j * D:(j + 1) * D][None]

    def mraw(j):
        return jnp.concatenate([mraw_s[j * CPV + u] for u in range(CPV)], axis=1)

    def xrows(t, sl, n):
        return x_s[t, sl, :].astype(f32).reshape(n // 8, 8, D)

    def ln1(t, r0, n, rel=None):
        xn = _ln(xrows(t, pl.ds(al(r0, n), n), n), rel)
        hf_s[pl.ds(al(r0, n), n), :] = (xn * mvec(1) + mvec(0)).reshape(n, D)

    def h_slice(r0, rel):
        hq = [hf_s[pl.ds(al(r * QT + r0, 8), 8), :] for r in range(4)]
        blk = [[[[hq[2 * r1 + r2][:, (2 * k1 + k2) * KQ:(2 * k1 + k2 + 1) * KQ] for k2 in range(2)]
                 for k1 in range(2)] for r2 in range(2)] for r1 in range(2)]
        ops = _two_level(_lhs_sums, blk, None if rel is None else [jnp.tile(v, (1, KQ // 128)) for v in rel])
        for u in range(7):
            hs_s[7 * u:7 * u + 7, pl.ds(al(r0, 8), 8), :] = ops[u]

    def w_unit(src, rows4, c0, dst, d0, rel):
        w = [src[pl.ds(al(r, 16), 16), c0:c0 + 512].astype(f32) for r in rows4]
        blk = [[[[w[2 * k1 + k2][:, (2 * n1 + n2) * 128:(2 * n1 + n2 + 1) * 128] for n2 in range(2)]
                 for n1 in range(2)] for k2 in range(2)] for k1 in range(2)]
        ops = _two_level(_rhs_sums, blk, None if rel is None else [jnp.tile(v, (2, 1)) for v in rel])
        for u in range(7):
            dst[7 * u:7 * u + 7, pl.ds(al(d0, 16), 16), :] = ops[u]
        return (dst.at[0], d0)

    def epi_rows(t, r0, n, rel=None, write_out=True):
        sl = pl.ds(r0, n)
        attn = jnp.concatenate([acc_s[j, sl, :] for j in range(NB)], axis=1).reshape(n // 8, 8, D)
        x1 = xrows(XE, sl, n) + mvec(2) * attn
        m, xc, rs = _ln_stats(x1, rel)
        keep_s[sl, 0:D] = x1.reshape(n, D)
        keep_s[sl, D:D + 128] = jnp.broadcast_to(m.reshape(n, 1), (n, 128))
        keep_s[sl, D + 128:D + 256] = jnp.broadcast_to(rs.reshape(n, 1), (n, 128))
        if write_out:
            h2 = xc * rs * mvec(4) + mvec(3)
            out_s[sl, :] = (x1 + mvec(5) * h2).reshape(n, D).astype(out_s.dtype)
        r = rs * jnp.sum(xc * mvec(6), axis=-1, keepdims=True) + mod_s[:, 7 * D:7 * D + 128][None]
        r = r.astype(bf16).astype(f32)
        bv = best_r[...]
        bi = best_i[...]
        sub = lax.broadcasted_iota(jnp.int32, (8, 128), 0)
        for u in range(n // 8):
            ru = r[u]
            better = ru > bv
            bv = jnp.where(better, ru, bv)
            bi = jnp.where(better, sub + (t * TQ + r0 + u * 8), bi)
        best_r[...] = bv
        best_i[...] = bi

    def capture(t):
        bv = best_r[...]
        rbest = jnp.max(bv, axis=0, keepdims=True)
        ibest = jnp.min(jnp.where(bv == rbest, best_i[...], S), axis=0, keepdims=True)
        idx = jnp.minimum(ibest[0, 0], S - 1)
        local = idx - t * TQ
        off = pl.multiple_of(jnp.clip(local // 16, 0, TQ // 16 - 1) * 16, 16)
        rows = jnp.where(local >= 0, keep_s[pl.ds(off, 16), :], cand_s[...])
        cand_s[...] = rows
        return rbest, idx, rows

    def scores(q, g):
        return lax.dot_general(q.astype(bf16), k_s[g], (((1,), (1,)), ((), ())), preferred_element_type=f32)

    def softmax(s):
        m = jnp.max(s, axis=-1, keepdims=True)
        p = jnp.exp2(s - m)
        part = p[:, 0:128]
        for j in range(1, W // 128):
            part = part + p[:, j * 128:(j + 1) * 128]
        p = jnp.concatenate([jnp.minimum(p[:, 0:128], part), p[:, 128:]], axis=1)
        return p, _recip(jnp.sum(part, axis=-1, keepdims=True))

    def pv(p, g):
        return jnp.dot(p.astype(bf16), v_s[g], preferred_element_type=f32)

    def block0(wv, c0, h0, nh, units):
        fence, release = sched()
        hval = h_s[...]
        g = h0 // rep
        tqk = [512 + 1024 * u for u in range(nh)]
        tpv = [tqk[u] + (768 if u + 1 < nh else 256) for u in range(nh)]
        wins = [(130, tqk[0])]
        for u in range(nh):
            wins.append((tqk[u] + A0_W[0], tqk[u] + (A0_W[1] if u + 1 < nh else A0_W[4])))
            if u + 1 < nh:
                wins.append((tqk[u] + A0_W[2], tqk[u] + A0_W[3]))
        wins.append((tpv[-1] + A0_W[5], tpv[-1] + A0_W[6]))
        slots = [t_ for a_, b_ in wins for t_ in range(a_, b_, 8)]
        npt = 7 * len(units)
        times = [slots[(u * len(slots)) // npt] for u in range(npt)]
        todo = [(un, times[7 * u:7 * u + 7]) for u, un in enumerate(units)]
        vals = []

        def emit(tmax):
            last = []
            while todo and todo[0][1][-1] < tmax:
                (sv, dv, r0), ts = todo.pop(0)
                rel = []
                for i_ in range(7):
                    t0_, v_ = [tv for tv in vals if tv[0] <= ts[PERM[i_]]][-1]
                    rel.append(release(v_, min((ts[PERM[i_]] - t0_) // 8 * 8, TQ - 8)))
                last = last[-1:] + [w_unit(sv, [c * KQ + r0 for c in range(4)], 0, dv, r0, rel)]
            return last

        def qproj(u, t_):
            cols = slice(c0 + u * DH, c0 + (u + 1) * DH)
            q1 = jnp.dot(hval[:, 0:KH], wv[0:KH, cols], preferred_element_type=f32)
            q2 = jnp.dot(hval[:, KH:D], wv[KH:D, cols], preferred_element_type=f32) + q1
            vals.extend([(t_ + 130, q1), (t_ + 386, q2)])
            return q2

        q = qproj(0, 0)
        for u in range(nh):
            s = scores(q, g)
            vals.append((tqk[u] + 130, s))
            p, li = softmax(s)
            if u + 1 < nh:
                q = qproj(u + 1, tqk[u] + 256)
            deps = emit(tpv[u]) + ([(o_s.at[h0 + u - 1], 0)] if u > 0 else [])
            if deps:
                p = pin(p, {A0_DUE: fence(deps)})
            o = pv(p, g)
            vals.append((tpv[u] + 130, o))
            o_s[h0 + u] = pltpu.bitcast((o * li).astype(bf16), u32)
        emit(1 << 30)

    cp_c().start()
    cp_x(0, XE).start()
    for j in range(2 * CPV):
        cp_mod(j).start()
    cp_wq(0).start()
    cp_k(0).start()
    cp_v(0).start()
    cp_wq(1, P0 - 1).start()
    for j in range(NA):
        h0 = P0 + j * G0
        cp_wq(h0, G0).start()
        if h0 % rep == 0:
            cp_k(h0 // rep).start()
            cp_v(h0 // rep).start()
    cp_x(1, X1).start()
    cp_wr().start()
    for j in range(NO):
        cp_wo(j).start()
        for u in range(CPV):
            if (j + 2) * CPV + u - MSH >= 2 * CPV:
                cp_mod((j + 2) * CPV + u - MSH).start()
    for u in range(NMC - MSH, NMC):
        cp_mod(u).start()
    cp_x(2, XL).start()

    zero_s[0] = 0
    for n in range(NB):
        acc_s[n] = jnp.zeros((TQ, 128), f32)
    hs_s[0] = jnp.zeros((QT, KQ), bf16)
    cand_s[...] = jnp.zeros(cand_s.shape, f32)
    best_r[...] = jnp.full(best_r.shape, -jnp.inf, f32)
    best_i[...] = jnp.zeros(best_i.shape, jnp.int32)
    cp_c().wait()
    cp_x(0, XE).wait()
    cf = c_s[...].astype(f32)
    sc_s[...] = jnp.broadcast_to(cf * jax.nn.sigmoid(cf), (16, D)).astype(bf16)
    xn0 = _ln(xrows(XE, pl.ds(0, TQ), TQ))

    def mod_body(j, carry):
        cp_mod(j).wait()
        mraw_s[j] = jnp.dot(sc_s[...], wmod_s[j], preferred_element_type=f32)[0:8, :]
        return carry

    lax.fori_loop(0, 2 * CPV, mod_body, 0)
    mod_s[:, 0:D] = mraw(0) * qscale
    mod_s[:, D:2 * D] = (1.0 + mraw(1)) * qscale
    h_s[...] = (xn0 * mvec(1) + mvec(0)).reshape(TQ, D).astype(bf16)
    NU = KQ // 16
    NPE = NU - NA
    cp_wq(0).wait()
    cp_k(0).wait()
    cp_v(0).wait()
    block0(wq_s, 0, 0, 1, [])
    cp_wq(1, P0 - 1).wait()
    block0(wq_s, DH, 1, P0 - 1, [(wq_s, wqc_s.at[0], u * 16) for u in range(NPE)])

    def a0_body(j, carry):
        h0 = P0 + j * G0
        cp_wq(h0, G0).wait()

        @pl.when(h0 % rep == 0)
        def _():
            cp_k(h0 // rep).wait()
            cp_v(h0 // rep).wait()

        sv = wq_s.at[:, pl.ds(al(h0 * DH, 4 * DH), 4 * DH)]
        dv = wqc_s.at[j + 1]
        block0(sv, 0, h0, G0, [(sv, dv, u * 16) for u in range(NU)] + [(wq_s, wqc_s.at[0], (NPE + j) * 16)])
        return carry

    lax.fori_loop(0, NA, a0_body, 0)
    cp_x(1, X1).wait()
    cp_wr().wait()

    def o0_body(j, carry):
        cp_wo(j).wait()
        for u in range(CPV):
            if u >= MSH:
                cp_mod((j + 2) * CPV + u - MSH).wait()
            else:
                @pl.when(j > 0)
                def _():
                    cp_mod((j + 2) * CPV + u - MSH).wait()

        fence, release = sched()
        sc = sc_s[...]
        hq = KP // DH
        wo_j = wo_s.at[pl.ds(al(j * D, D), D)]
        o_j = o_s.at[pl.ds(j * (D // DH), D // DH)]
        wm_j = wmod_s.at[pl.ds((j + 2) * CPV - MSH, CPV)]
        mr_j = mraw_s.at[pl.ds((j + 2) * CPV - MSH, CPV)]
        units = [(qd, ng, u) for qd in range(2) for ng in range(2) for u in range(DH // 16)]
        npass = NB * (D // KP)
        cnt = 0
        due = {}
        hist = []
        lhs2 = [jnp.concatenate([o_j[kh * hq + u] for u in range(hq)], axis=1) for kh in range(D // KP)]
        for n in range(NB):
            acc = acc_s[n]
            cu, cn = divmod(n, MC // 128)
            mv = None
            for kh in range(D // KP):
                lhs = lhs2[kh]
                acc = jnp.dot(pltpu.bitcast(pin(lhs, due.pop(cnt, None)), bf16),
                              wo_j[kh * KP:(kh + 1) * KP, n * 128:(n + 1) * 128],
                              preferred_element_type=f32) + acc
                hist.append(acc)
                mine = units[cnt * len(units) // npass:(cnt + 1) * len(units) // npass]
                for n_, (qd, ng, u) in enumerate(mine):
                    last = w_unit(wo_j, [(4 * qd + c) * DH + u * 16 for c in range(4)], ng * 512,
                                  woc_s.at[j, ng], qd * DH + u * 16, [release(acc, O0_ROWS[n_][PERM[i_]]) for i_ in range(7)])
                if cnt + 2 < npass:
                    due.setdefault(cnt + 2, {})[2] = fence([last])
                if cnt in O0_LN:
                    qr, hf_ = O0_LN.index(cnt) % 4, O0_LN.index(cnt) // 4
                    ln1(X1, qr * QT + j * 16 + hf_ * 8, 8, release(acc, O0_LNROW))
                    due.setdefault(cnt + 3, {})[4] = fence([(hf_s, qr * QT + j * 16 + hf_ * 8)])
                if cnt in O0_HS:
                    hp_ = [(hist[-3 + u_ // 3], O0_HSROW[u_ % 3]) for u_ in range(9)]
                    h_slice(j * 16 + O0_HS.index(cnt) * 8, [release(*hp_[PERML[i_]]) for i_ in range(7)])
                    if cnt == O0_HS[0]:
                        due.setdefault(cnt + 2, {})[10] = fence([(hs_s.at[0], j * 16)])
                cnt += 1
                d = jnp.dot(sc[:, kh * KP:(kh + 1) * KP],
                            wm_j[cu, kh * KP:(kh + 1) * KP, cn * 128:(cn + 1) * 128],
                            preferred_element_type=f32)
                mv = d if mv is None else d + mv
            acc_s[n] = acc
            mr_j[cu, :, cn * 128:(cn + 1) * 128] = mv[0:8, :]
        assert not due
        return carry

    lax.fori_loop(0, NO, o0_body, 0)

    for u in range(NMC - MSH, NMC):
        cp_mod(u).wait()
    for u in range(NMC - MSH, NMC):
        mraw_s[u] = jnp.dot(sc_s[...], wmod_s[u], preferred_element_type=f32)[0:8, :]
    mod_s[:, 2 * D:3 * D] = mraw(2)
    mod_s[:, 3 * D:4 * D] = mraw(3)
    mod_s[:, 4 * D:5 * D] = 1.0 + mraw(4)
    mod_s[:, 5 * D:6 * D] = mraw(5)
    wr8 = jnp.broadcast_to(wr_s[...].astype(f32).reshape(1, D), (8, D))
    mod_s[:, 6 * D:7 * D] = (1.0 + mraw(4)) * wr8
    mod_s[:, 7 * D:7 * D + 128] = jnp.broadcast_to(jnp.sum(mraw(3) * wr8, axis=-1, keepdims=True), (8, 128))
    cp_wg().start(priority=1)
    for u in range(F // MC):
        cp_wu(u).start(priority=1)
    cp_wd().start(priority=1)

    def step(t, carry):
        cp_x(0, XL).wait()

        @pl.when(t > 1)
        def _():
            cp_x(0, XE).wait()
            cp_out(0).wait()

        fence, release = sched()
        tprev = t - 1
        prods = [(i1, i2) for i1 in _ORDER for i2 in _ORDER]
        hv = [hs_s[u] for u in range(49)]

        qblk = {}

        def q_passes(g):
            def emit(r1, r2, n1, n2, c):
                for z in range(2):
                    qblk[8 * g + 4 * z + 2 * n1 + n2, 2 * r1 + r2] = c[:, z * DH:(z + 1) * DH]
            asm = _Assemble(emit)

            def run(i1, i2):
                u = 7 * i2 + i1
                w = jnp.concatenate([wqc_s[2 * g + z, u] for z in range(2)], axis=1)
                d = jnp.dot(hv[u], w, preferred_element_type=f32)
                ini = asm.init(i1, i2)
                if ini is not None:
                    d = d + ini
                asm.add(i1, i2, d)
                return d
            return [functools.partial(run, i1, i2) for i1, i2 in prods]

        def q_head(hh):
            return jnp.concatenate([qblk.pop((hh, r)) for r in range(4)], axis=0)

        def o_passes():
            ms = {}
            asm = []
            for ng in range(2):
                def emit(r1, r2, n1, n2, c, ng=ng):
                    acc_s[4 * ng + 2 * n1 + n2, pl.ds(r1 * HT + r2 * QT, QT), :] = c
                asm.append(_Assemble(emit))

            def run(ng, i1, i2, k, dep=None):
                u = 7 * i2 + i1
                lhs = jnp.concatenate([os_s[u, 4 * k + v] for v in range(4)], axis=1)
                w = jnp.concatenate([woc_s[2 * k + v, ng, u] for v in range(2)], axis=0)
                d = jnp.dot(lhs, pin_bf16(w, dep), preferred_element_type=f32)
                early = ng == 0 or (i1, i2) in prods[:NE]
                if k == 1:
                    d = d + ms.pop((ng, u))
                if k == (1 if early else 0):
                    ini = asm[ng].init(i1, i2)
                    if ini is not None:
                        d = d + ini
                if k == 0:
                    ms[ng, u] = d
                else:
                    asm[ng].add(i1, i2, d)
                return d
            NE = 16
            seq = [(0,) + pr + (0,) for pr in prods] + [(1,) + pr + (0,) for pr in prods[:NE]]
            seq += [(0,) + pr + (1,) for pr in prods] + [(1,) + pr + (1,) for pr in prods[:NE]]
            seq += [(1,) + pr + (k,) for pr in prods[NE:] for k in range(2)]
            return [functools.partial(run, *a) for a in seq]

        def side(hp, pts):
            rel = [release(v_, rw) for v_, rw in pts]
            for u in range(2):
                epi_rows(tprev, (2 * hp + u) * CHE, CHE, rel[u])
            if len(rel) == 3:
                ln1(XL, hp * 16, 16, rel[2])
            else:
                for u in range(2):
                    ln1(XL, hp * 16 + 8 * u, 8, rel[2 + u])
            return fence([(out_s, 0), (best_r, 0), (keep_s, 0), (hf_s, 0)])

        def o_slice(qd, oq, u, pts):
            blk = [[[[oq[k1][k2][r1 * HT + r2 * QT + 16 * u:r1 * HT + r2 * QT + 16 * u + 16]
                      for k2 in range(2)] for k1 in range(2)] for r2 in range(2)] for r1 in range(2)]
            if len(pts) == 7:
                pts = [pts[PERML[i_]] for i_ in range(7)]
            ops = _two_level(_lhs_sums, blk, [jnp.tile(release(v_, rw), (2, 1)) for v_, rw in pts])
            for v in range(7):
                os_s[7 * v:7 * v + 7, qd, 16 * u:16 * u + 16, :] = ops[v]
            return fence([(os_s.at[0, qd], 16 * u)])

        assert 2 * HP * CHE == TQ
        for fn in q_passes(0):
            fn()
        opl = o_passes()
        oq = fo = ob_ = None
        for hp in range(HP):
            g, pp = divmod(hp, 4)
            if pp == 0:
                fill = q_passes(g + 1) if g + 1 < HKV else opl
            qa, qb = q_head(2 * hp), q_head(2 * hp + 1)
            sa_ = scores(qa if fo is None else pin(qa, {0: fo}), g)
            pa, la = softmax(sa_)
            vals = {'s': sa_, 'ob': ob_}
            if oq is not None:
                fl = [o_slice(hp // 2 - 1, oq, 2 * (hp % 2) + u, [(vals[nm], rw) for nm, rw in OS_PTS[u]])
                      for u in range(2 if FILL[pp][1] < 7 else 1)]
                qb = pin(qb, {0: functools.reduce(lambda a_, b_: a_ | b_, fl)})
            rs_ = [fill.pop(0)() for _ in range(FILL[pp][0])]
            vals.update({i_: rs_[max(len(rs_) - 6 + i_, 0)] for i_ in range(6)})
            fs = side(hp, [(vals[nm] if vals[nm] is not None else sa_, rw) for nm, rw in SIDE_PTS])
            pb, lb = softmax(scores(qb, g))
            oa_ = pv(pa, g)
            oa = oa_ * la
            rs_ = [fill.pop(0)() for _ in range(FILL[pp][1])]
            fo = None
            if oq is not None and FILL[pp][1] >= 7:
                vals = {'oa': oa_}
                vals.update(enumerate(rs_))
                fo = o_slice(hp // 2 - 1, oq, 2 * (hp % 2) + 1, [(vals[nm], rw) for nm, rw in OS_F2])
            ob_ = pv(pin(pb, {0: fs}), g)
            ob = ob_ * lb
            if hp % 2 == 0:
                oprev = (oa, ob)
            else:
                oq = [oprev, (oa, ob)]

        capture(tprev)
        cp_out(tprev).start()
        cp_x(t, XE).start()
        cp_x(jnp.minimum(t + 2, nt - 1), XL).start()
        pts = []
        due = {} if fo is None else {2: fo}
        for s, fn in enumerate(opl):
            pts.append((fn(due.pop(s, None)), 0))
            if len(pts) % 3 == 0 and len(pts) <= 12:
                o_slice(HP // 2 - 1, oq, len(pts) // 3 - 1, pts[-3:])
            u, rem = divmod(s - HS0, HSG)
            if rem == 0 and 0 <= u < QT // 8:
                h_slice(u * 8, [release(pts[-1 - HSS * (6 - PERML[i_])][0]) for i_ in range(7)])
                due[s + 6] = fence([(hs_s.at[0], 0)])
        assert not due
        return carry

    lax.fori_loop(1, nt, step, 0)

    cp_wg().wait()
    for u in range(F // MC):
        cp_wu(u).wait()
    cp_wd().wait()
    cp_x(0, XL).wait()
    cp_x(0, XE).wait()
    cp_out(0).wait()
    epi_rows(nt - 1, 0, TQ, write_out=False)
    _, release_t = sched()
    rel0 = release_t(best_r[...])
    rbest, idx, rows = capture(nt - 1)
    base = pl.multiple_of((idx // 16) * 16, 16)
    x1 = rows[:, 0:D].reshape(2, 8, D)
    mu = jnp.tile(rows[:, D:D + 128], (1, NB)).reshape(2, 8, D)
    rs = jnp.tile(rows[:, D + 128:D + 256], (1, NB)).reshape(2, 8, D)
    h2 = (x1 - mu) * rs * mvec(4) + mvec(3)
    xs = h2.reshape(16, D).astype(bf16)
    gt = jnp.dot(xs, wq_s[:, 0:F], preferred_element_type=f32)
    for u in range(TQ // 8):
        rel = rel0 if u < T_EARLY else release_t(gt[:, (u - T_EARLY) * 128:(u - T_EARLY + 1) * 128])
        kr = keep_s[8 * u:8 * u + 8, :]
        xc_ = kr[:, 0:D] - jnp.tile(kr[:, D:D + 128] + rel, (1, NB))
        h2_ = xc_ * jnp.tile(kr[:, D + 128:D + 256], (1, NB)) * mvec(4)[0] + mvec(3)[0]
        out_s[8 * u:8 * u + 8, :] = (kr[:, 0:D] + mvec(5)[0] * h2_).astype(out_s.dtype)
    cp_out(nt - 1).start()
    up = jnp.concatenate([jnp.dot(xs, wmod_s[u], preferred_element_type=f32) for u in range(F // MC)], axis=1)
    a = (gt * jax.nn.sigmoid(gt) * up).astype(bf16)
    y = jnp.dot(a, wo_s[0:F, 0:D], preferred_element_type=f32)
    y = y * jnp.tile(jax.nn.sigmoid(rbest), (1, NB))
    rr = lax.broadcasted_iota(jnp.int32, (16, D), 0) + base
    upd = jnp.where(rr == idx, y, 0.0).reshape(2, 8, D)
    new = (x1 + mvec(5) * (h2 + upd)).reshape(16, D)
    fix_s[...] = new.astype(fix_s.dtype)
    cp_out(nt - 1).wait()
    fix = pltpu.make_async_copy(fix_s, out_hbm.at[pl.ds(base, 16), :], osems.at[0])
    fix.start()
    fix.wait()


def _compiler_params():
    kw = dict(vmem_limit_bytes=124 * 1024 * 1024)
    try:
        return pltpu.CompilerParams(disable_semaphore_checks=True, disable_bounds_checks=True, **kw)
    except TypeError:
        return pltpu.CompilerParams(**kw)


@jax.jit
def pallas_adaLN_cond__sliding_block_cached__moe_arch_mod__prompt_kernel(
    A_x: jax.Array,
    A_k_cache: jax.Array,
    A_v_cache: jax.Array,
    A_wq: jax.Array,
    A_wo: jax.Array,
    B_x: jax.Array,
    B_w_r: jax.Array,
    B_w_gate: jax.Array,
    B_w_up: jax.Array,
    B_w_down: jax.Array,
    c: jax.Array,
    w_mod: jax.Array,
):
    B, S, D = A_x.shape
    assert B == 1
    HKV, SK = A_k_cache.shape[1], A_k_cache.shape[2]
    W = min(4096, max(256, SK // 4))
    F = B_w_gate.shape[1]
    dt = A_x.dtype
    f32 = jnp.float32
    nt = S // TQ
    NB = D // 128
    NMC = 6 * D // MC
    x2 = A_x.reshape(S, D)
    anyspec = pl.BlockSpec(memory_space=pl.ANY)
    kern = functools.partial(_kernel, S=S, D=D, HKV=HKV, SK=SK, W=W, F=F)
    out = pl.pallas_call(
        kern,
        in_specs=[anyspec] * 11,
        out_specs=anyspec,
        out_shape=jax.ShapeDtypeStruct((S, D), dt),
        scratch_shapes=[
            pltpu.VMEM((D,), dt),
            pltpu.VMEM((1, D), dt),
            pltpu.VMEM((3, TQ, D), dt),
            pltpu.VMEM((HKV, W, DH), dt),
            pltpu.VMEM((HKV, W, DH), dt),
            pltpu.VMEM((D, HQ * DH + PAD), dt),
            pltpu.VMEM((HQ * DH, D + PAD), dt),
            pltpu.VMEM((NMC, D, MC), dt),
            pltpu.VMEM((TQ, D), dt),
            pltpu.VMEM((HQ // 4, 49, D // 4, DH), dt),
            pltpu.VMEM((HQ * DH // D, 2, 49, 2 * DH, 128), dt),
            pltpu.VMEM((TQ, D), f32),
            pltpu.VMEM((49, TQ // 4, D // 4), dt),
            pltpu.VMEM((49, HQ // 4, TQ // 4, DH), dt),
            pltpu.VMEM((16, D), dt),
            pltpu.VMEM((NMC, 8, MC), f32),
            pltpu.VMEM((8, 7 * D + 512), f32),
            pltpu.VMEM((TQ, D), dt),
            pltpu.VMEM((HQ, TQ // 2, DH), jnp.uint32),
            pltpu.VMEM((NB, TQ, 128), f32),
            pltpu.VMEM((TQ, D + 256), f32),
            pltpu.VMEM((16, D + 256), f32),
            pltpu.VMEM((16, D), dt),
            pltpu.VMEM((8, 128), f32),
            pltpu.VMEM((8, 128), jnp.int32),
            pltpu.SMEM((1,), jnp.int32),
            pltpu.SemaphoreType.DMA((4 + NMC + HQ + 2 * HKV + HQ * DH // D + 3,)),
            pltpu.SemaphoreType.DMA((2,)),
        ],
        compiler_params=_compiler_params(),
    )(B_w_r, c, x2, A_k_cache, A_v_cache, A_wq, A_wo, w_mod, B_w_gate, B_w_up, B_w_down)
    return out.reshape(B, S, D)
```

```python
import functools

import jax
import jax.numpy as jnp
from jax import lax
import jax.experimental.pallas as pl
import jax.experimental.pallas.tpu as pltpu

HQ = 32
DH = 128
TQ = 256
PAD = 128
P0 = 4
G0 = 4
MC = 512
MSH = 1
CHE = 8
FILL = ((7, 7), (7, 7), (7, 7), (7, 0))

SIDE_PTS = ((1, 48), (2, 48), ('ob', 0), ('ob', 56))
OS_F2 = [('oa', 128), ('oa', 192), (0, 0), (1, 0), (2, 0), (3, 0), (4, 0)]
OS_PTS = ([('ob', 96 + 16 * i) for i in range(7)],
          [('ob', 208), ('ob', 224), ('ob', 240), ('s', 0), ('s', 16), ('s', 32), ('s', 48)])
HS0, HSG, HSS = 30, 14, 2
A0_W = (2, 250, 394, 760, 130, 150, 370)
A0_DUE = 14
O0_ROWS = ((0, 16, 32, 56, 72, 88, 112), (128, 144, 168, 184, 200, 224, 240))
O0_LN = (0, 1, 2, 3, 4, 5, 6, 7)
O0_LNROW = 24
O0_HS = (12, 15)
O0_HSROW = (8, 104, 192)
PERM = (3, 1, 4, 0, 5, 2, 6)
PERML = (0, 1, 2, 3, 4, 5, 6)

T_EARLY = 8
EPS = 1e-5
LOG2E = 1.4426950408889634


def _ln_stats(x, rel=None):
    d = x.shape[-1]
    part = x[..., 0:128]
    for j in range(1, d // 128):
        part = part + x[..., j * 128:(j + 1) * 128]
    if rel is not None:
        part = part + rel
    m = jnp.sum(part, axis=-1, keepdims=True) * (1.0 / d)
    xc = x - m
    v = jnp.mean(xc * xc, axis=-1, keepdims=True)
    return m, xc, lax.rsqrt(v + EPS)


def _ln(x, rel=None):
    _, xc, rs = _ln_stats(x, rel)
    return xc * rs


def _recip(l):
    return pl.reciprocal(l, approx=True)


def _lhs_sums(a11, a12, a21, a22):
    return [a11 + a22, a21 + a22, a11, a22, a11 + a12, a21 - a11, a12 - a22]


def _rhs_sums(b11, b12, b21, b22):
    return [b11 + b22, b11, b12 - b22, b21 - b11, b22, b11 + b12, b21 + b22]


_ORDER = [3, 4, 0, 6, 1, 2, 5]
_BLOCK = {6: (0, 0), 1: (1, 0), 2: (0, 1), 5: (1, 1)}


def _init(i, z):
    return {0: lambda: z[3] - z[4], 6: lambda: z[0], 1: lambda: z[3], 2: lambda: z[4],
            5: lambda: z[0] - z[1] + z[2]}.get(i, lambda: None)()


def _two_level(sums, blk, rel):
    o = [[jnp.stack([blk[a1][a2][b1][b2] for a2 in range(2) for b2 in range(2)]) for b1 in range(2)]
         for a1 in range(2)]
    if rel is not None and len(rel) == 3:
        o = [[o[a1][b1] + rel[0 if a1 == b1 else 1 + a1][None] for b1 in range(2)] for a1 in range(2)]
    x = jnp.stack(sums(o[0][0], o[0][1], o[1][0], o[1][1]), axis=1)
    x = [x[u] for u in range(4)]
    if rel is not None and len(rel) == 7:
        r7 = jnp.stack(rel)
        x = [x[0] + r7, x[1], x[2], x[3] + r7]
    return [y.astype(jnp.bfloat16) for y in sums(*x)]


class _Assemble:
    def __init__(self, emit):
        self.z, self.outer, self.inj, self.emit = {}, {}, {}, emit

    def init(self, i1, i2):
        v = _init(i2, self.z)
        if i2 in _BLOCK and i1 not in (3, 4):
            self.inj[i2] = _init(i1, self.outer[i2])
            v = v + self.inj[i2]
            if i2 == 5:
                v = v + (self.inj[1] - self.inj[2])
        return v

    def add(self, i1, i2, m):
        self.z[i2] = m
        if i2 in _BLOCK:
            self.outer.setdefault(i2, {})[i1] = m
            if i1 in _BLOCK:
                (r1, n1), (r2, n2) = _BLOCK[i1], _BLOCK[i2]
                self.emit(r1, r2, n1, n2, m)


def _kernel(wr_hbm, c_hbm, x_hbm, k_hbm, v_hbm, wq_hbm, wo_hbm, wmod_hbm,
            wg_hbm, wu_hbm, wd_hbm, out_hbm,
            wr_s, c_s, x_s, k_s, v_s, wq_s, wo_s, wmod_s, out_s,
            wqc_s, woc_s, hf_s, hs_s, os_s,
            sc_s, mraw_s, mod_s, h_s, o_s, acc_s, keep_s, cand_s, fix_s, best_r, best_i, zero_s, sems, osems,
            *, S, D, HKV, SK, W, F):
    nt = S // TQ
    rep = HQ // HKV
    NB = D // 128
    HP = HQ // 2
    HT = TQ // 2
    QT = TQ // 4
    KH = D // 2
    KQ = D // 4
    KP = 512
    CPV = D // MC
    NMC = 6 * CPV
    NA = (HQ - P0) // G0
    NO = HQ * DH // D
    f32 = jnp.float32
    bf16 = jnp.bfloat16
    u32 = jnp.uint32
    qscale = (DH ** -0.5) * LOG2E
    assert KH == KP and rep == 8 and NB == 8 and NO == 4 and P0 == 4 and G0 == 4

    def al(v, n):
        return v if isinstance(v, int) else pl.multiple_of(v, n)

    S_C, S_WR, S_WG, S_WD, S_M = 0, 1, 2, 3, 4
    S_WQ = S_M + NMC
    S_K = S_WQ + HQ
    S_V = S_K + HKV
    S_WO = S_V + HKV
    S_X = S_WO + NO

    def cp_c():
        return pltpu.make_async_copy(c_hbm, c_s, sems.at[S_C])

    def cp_wr():
        return pltpu.make_async_copy(wr_hbm, wr_s, sems.at[S_WR])

    def cp_mod(j):
        return pltpu.make_async_copy(wmod_hbm.at[:, pl.ds(al(j * MC, MC), MC)], wmod_s.at[j], sems.at[S_M + j])

    def cp_wg():
        return pltpu.make_async_copy(wg_hbm, wq_s.at[:, pl.ds(0, F)], sems.at[S_WG])

    def cp_wu(u):
        return pltpu.make_async_copy(wu_hbm.at[:, pl.ds(u * MC, MC)], wmod_s.at[u], sems.at[S_M + u])

    def cp_wd():
        return pltpu.make_async_copy(wd_hbm, wo_s.at[pl.ds(0, F), pl.ds(0, D)], sems.at[S_WD])

    def cp_wq(h, n=1):
        sl = pl.ds(al(h * DH, DH), n * DH)
        return pltpu.make_async_copy(wq_hbm.at[:, sl], wq_s.at[:, sl], sems.at[S_WQ + h])

    def cp_k(g):
        return pltpu.make_async_copy(k_hbm.at[0, g, pl.ds(SK - W, W), :], k_s.at[g], sems.at[S_K + g])

    def cp_v(g):
        return pltpu.make_async_copy(v_hbm.at[0, g, pl.ds(SK - W, W), :], v_s.at[g], sems.at[S_V + g])

    def cp_wo(j):
        sl = pl.ds(al(j * D, D), D)
        return pltpu.make_async_copy(wo_hbm.at[sl, :], wo_s.at[sl, pl.ds(0, D)], sems.at[S_WO + j])

    def rsl(t, r0=0, n=TQ):
        return pl.ds(al(t * TQ + r0, n), n)

    XE, X1, XL = 0, 1, 2

    def cp_x(t, slot):
        return pltpu.make_async_copy(x_hbm.at[rsl(t), :], x_s.at[slot], sems.at[S_X + slot])

    def cp_out(t):
        return pltpu.make_async_copy(out_s, out_hbm.at[rsl(t), :], osems.at[0])

    def sched():
        zero = zero_s[0]
        z16 = pl.multiple_of(zero, 16)
        zvec = jnp.full((8, 128), zero, jnp.int32).astype(u32)

        def fence(deps):
            d = None
            for ref, base in deps:
                n = 16 if ref.dtype == bf16 else 8
                v = pltpu.bitcast(ref[pl.ds(pl.multiple_of(base + z16, n), n), 0:128], u32)
                d = v if d is None else d | v
            return d & zvec

        def release(acc, r0=0):
            return pltpu.bitcast(pltpu.bitcast(acc[r0:r0 + 8, 0:128], u32) & zvec, f32)

        return fence, release

    def pin(a, at):
        if not at:
            return a
        parts = []
        prev = 0
        for rb in sorted(at):
            r0 = rb * 8
            if r0 > prev:
                parts.append(a[prev:r0, :])
            if a.dtype == f32:
                blk = a[r0:r0 + 8, 0:128] + pltpu.bitcast(at[rb], f32)
            else:
                blk = a[r0:r0 + 8, 0:128] | at[rb]
            if a.shape[1] > 128:
                blk = jnp.concatenate([blk, a[r0:r0 + 8, 128:]], axis=1)
            parts.append(blk)
            prev = r0 + 8
        if prev < a.shape[0]:
            parts.append(a[prev:, :])
        return jnp.concatenate(parts, axis=0)

    def pin_bf16(w, d):
        if d is None:
            return w
        top = pltpu.bitcast(pltpu.bitcast(w[0:16], u32) | d, bf16)
        return jnp.concatenate([top, w[16:]], axis=0)

    def mvec(j):
        return mod_s[:, j * D:(j + 1) * D][None]

    def mraw(j):
        return jnp.concatenate([mraw_s[j * CPV + u] for u in range(CPV)], axis=1)

    def xrows(t, sl, n):
        return x_s[t, sl, :].astype(f32).reshape(n // 8, 8, D)

    def ln1(t, r0, n, rel=None):
        xn = _ln(xrows(t, pl.ds(al(r0, n), n), n), rel)
        hf_s[pl.ds(al(r0, n), n), :] = (xn * mvec(1) + mvec(0)).reshape(n, D)

    def h_slice(r0, rel):
        hq = [hf_s[pl.ds(al(r * QT + r0, 8), 8), :] for r in range(4)]
        blk = [[[[hq[2 * r1 + r2][:, (2 * k1 + k2) * KQ:(2 * k1 + k2 + 1) * KQ] for k2 in range(2)]
                 for k1 in range(2)] for r2 in range(2)] for r1 in range(2)]
        ops = _two_level(_lhs_sums, blk, None if rel is None else [jnp.tile(v, (1, KQ // 128)) for v in rel])
        for u in range(7):
            hs_s[7 * u:7 * u + 7, pl.ds(al(r0, 8), 8), :] = ops[u]

    def w_unit(src, rows4, c0, dst, d0, rel):
        w = [src[pl.ds(al(r, 16), 16), c0:c0 + 512].astype(f32) for r in rows4]
        blk = [[[[w[2 * k1 + k2][:, (2 * n1 + n2) * 128:(2 * n1 + n2 + 1) * 128] for n2 in range(2)]
                 for n1 in range(2)] for k2 in range(2)] for k1 in range(2)]
        ops = _two_level(_rhs_sums, blk, None if rel is None else [jnp.tile(v, (2, 1)) for v in rel])
        for u in range(7):
            dst[7 * u:7 * u + 7, pl.ds(al(d0, 16), 16), :] = ops[u]
        return (dst.at[0], d0)

    def epi_rows(t, r0, n, rel=None, write_out=True):
        sl = pl.ds(r0, n)
        attn = jnp.concatenate([acc_s[j, sl, :] for j in range(NB)], axis=1).reshape(n // 8, 8, D)
        x1 = xrows(XE, sl, n) + mvec(2) * attn
        m, xc, rs = _ln_stats(x1, rel)
        keep_s[sl, 0:D] = x1.reshape(n, D)
        keep_s[sl, D:D + 128] = jnp.broadcast_to(m.reshape(n, 1), (n, 128))
        keep_s[sl, D + 128:D + 256] = jnp.broadcast_to(rs.reshape(n, 1), (n, 128))
        if write_out:
            h2 = xc * rs * mvec(4) + mvec(3)
            out_s[sl, :] = (x1 + mvec(5) * h2).reshape(n, D).astype(out_s.dtype)
        r = rs * jnp.sum(xc * mvec(6), axis=-1, keepdims=True) + mod_s[:, 7 * D:7 * D + 128][None]
        r = r.astype(bf16).astype(f32)
        bv = best_r[...]
        bi = best_i[...]
        sub = lax.broadcasted_iota(jnp.int32, (8, 128), 0)
        for u in range(n // 8):
            ru = r[u]
            better = ru > bv
            bv = jnp.where(better, ru, bv)
            bi = jnp.where(better, sub + (t * TQ + r0 + u * 8), bi)
        best_r[...] = bv
        best_i[...] = bi

    def capture(t):
        bv = best_r[...]
        rbest = jnp.max(bv, axis=0, keepdims=True)
        ibest = jnp.min(jnp.where(bv == rbest, best_i[...], S), axis=0, keepdims=True)
        idx = jnp.minimum(ibest[0, 0], S - 1)
        local = idx - t * TQ
        off = pl.multiple_of(jnp.clip(local // 16, 0, TQ // 16 - 1) * 16, 16)
        rows = jnp.where(local >= 0, keep_s[pl.ds(off, 16), :], cand_s[...])
        cand_s[...] = rows
        return rbest, idx, rows

    def scores(q, g):
        return lax.dot_general(q.astype(bf16), k_s[g], (((1,), (1,)), ((), ())), preferred_element_type=f32)

    def softmax(s):
        m = jnp.max(s, axis=-1, keepdims=True)
        p = jnp.exp2(s - m)
        part = p[:, 0:128]
        for j in range(1, W // 128):
            part = part + p[:, j * 128:(j + 1) * 128]
        p = jnp.concatenate([jnp.minimum(p[:, 0:128], part), p[:, 128:]], axis=1)
        return p, _recip(jnp.sum(part, axis=-1, keepdims=True))

    def pv(p, g):
        return jnp.dot(p.astype(bf16), v_s[g], preferred_element_type=f32)

    def block0(wv, c0, h0, nh, units):
        fence, release = sched()
        hval = h_s[...]
        g = h0 // rep
        tqk = [512 + 1024 * u for u in range(nh)]
        tpv = [tqk[u] + (768 if u + 1 < nh else 256) for u in range(nh)]
        wins = [(130, tqk[0])]
        for u in range(nh):
            wins.append((tqk[u] + A0_W[0], tqk[u] + (A0_W[1] if u + 1 < nh else A0_W[4])))
            if u + 1 < nh:
                wins.append((tqk[u] + A0_W[2], tqk[u] + A0_W[3]))
        wins.append((tpv[-1] + A0_W[5], tpv[-1] + A0_W[6]))
        slots = [t_ for a_, b_ in wins for t_ in range(a_, b_, 8)]
        npt = 7 * len(units)
        times = [slots[(u * len(slots)) // npt] for u in range(npt)]
        todo = [(un, times[7 * u:7 * u + 7]) for u, un in enumerate(units)]
        vals = []

        def emit(tmax):
            last = []
            while todo and todo[0][1][-1] < tmax:
                (sv, dv, r0), ts = todo.pop(0)
                rel = []
                for i_ in range(7):
                    t0_, v_ = [tv for tv in vals if tv[0] <= ts[PERM[i_]]][-1]
                    rel.append(release(v_, min((ts[PERM[i_]] - t0_) // 8 * 8, TQ - 8)))
                last = last[-1:] + [w_unit(sv, [c * KQ + r0 for c in range(4)], 0, dv, r0, rel)]
            return last

        def qproj(u, t_):
            cols = slice(c0 + u * DH, c0 + (u + 1) * DH)
            q1 = jnp.dot(hval[:, 0:KH], wv[0:KH, cols], preferred_element_type=f32)
            q2 = jnp.dot(hval[:, KH:D], wv[KH:D, cols], preferred_element_type=f32) + q1
            vals.extend([(t_ + 130, q1), (t_ + 386, q2)])
            return q2

        q = qproj(0, 0)
        for u in range(nh):
            s = scores(q, g)
            vals.append((tqk[u] + 130, s))
            p, li = softmax(s)
            if u + 1 < nh:
                q = qproj(u + 1, tqk[u] + 256)
            deps = emit(tpv[u]) + ([(o_s.at[h0 + u - 1], 0)] if u > 0 else [])
            if deps:
                p = pin(p, {A0_DUE: fence(deps)})
            o = pv(p, g)
            vals.append((tpv[u] + 130, o))
            o_s[h0 + u] = pltpu.bitcast((o * li).astype(bf16), u32)
        emit(1 << 30)

    cp_c().start()
    cp_x(0, XE).start()
    for j in range(2 * CPV):
        cp_mod(j).start()
    cp_wq(0).start()
    cp_k(0).start()
    cp_v(0).start()
    cp_wq(1, P0 - 1).start()
    for j in range(NA):
        h0 = P0 + j * G0
        cp_wq(h0, G0).start()
        if h0 % rep == 0:
            cp_k(h0 // rep).start()
            cp_v(h0 // rep).start()
    cp_x(1, X1).start()
    cp_wr().start()
    for j in range(NO):
        cp_wo(j).start()
        for u in range(CPV):
            if (j + 2) * CPV + u - MSH >= 2 * CPV:
                cp_mod((j + 2) * CPV + u - MSH).start()
    for u in range(NMC - MSH, NMC):
        cp_mod(u).start()
    cp_x(2, XL).start()

    zero_s[0] = 0
    for n in range(NB):
        acc_s[n] = jnp.zeros((TQ, 128), f32)
    hs_s[0] = jnp.zeros((QT, KQ), bf16)
    cand_s[...] = jnp.zeros(cand_s.shape, f32)
    best_r[...] = jnp.full(best_r.shape, -jnp.inf, f32)
    best_i[...] = jnp.zeros(best_i.shape, jnp.int32)
    cp_c().wait()
    cp_x(0, XE).wait()
    cf = c_s[...].astype(f32)
    sc_s[...] = jnp.broadcast_to(cf * jax.nn.sigmoid(cf), (16, D)).astype(bf16)
    xn0 = _ln(xrows(XE, pl.ds(0, TQ), TQ))

    def mod_body(j, carry):
        cp_mod(j).wait()
        mraw_s[j] = jnp.dot(sc_s[...], wmod_s[j], preferred_element_type=f32)[0:8, :]
        return carry

    lax.fori_loop(0, 2 * CPV, mod_body, 0)
    mod_s[:, 0:D] = mraw(0) * qscale
    mod_s[:, D:2 * D] = (1.0 + mraw(1)) * qscale
    h_s[...] = (xn0 * mvec(1) + mvec(0)).reshape(TQ, D).astype(bf16)
    NU = KQ // 16
    NPE = NU - NA
    cp_wq(0).wait()
    cp_k(0).wait()
    cp_v(0).wait()
    block0(wq_s, 0, 0, 1, [])
    cp_wq(1, P0 - 1).wait()
    block0(wq_s, DH, 1, P0 - 1, [(wq_s, wqc_s.at[0], u * 16) for u in range(NPE)])

    def a0_body(j, carry):
        h0 = P0 + j * G0
        cp_wq(h0, G0).wait()

        @pl.when(h0 % rep == 0)
        def _():
            cp_k(h0 // rep).wait()
            cp_v(h0 // rep).wait()

        sv = wq_s.at[:, pl.ds(al(h0 * DH, 4 * DH), 4 * DH)]
        dv = wqc_s.at[j + 1]
        block0(sv, 0, h0, G0, [(sv, dv, u * 16) for u in range(NU)] + [(wq_s, wqc_s.at[0], (NPE + j) * 16)])
        return carry

    lax.fori_loop(0, NA, a0_body, 0)
    cp_x(1, X1).wait()
    cp_wr().wait()

    def o0_body(j, carry):
        cp_wo(j).wait()
        for u in range(CPV):
            if u >= MSH:
                cp_mod((j + 2) * CPV + u - MSH).wait()
            else:
                @pl.when(j > 0)
                def _():
                    cp_mod((j + 2) * CPV + u - MSH).wait()

        fence, release = sched()
        sc = sc_s[...]
        hq = KP // DH
        wo_j = wo_s.at[pl.ds(al(j * D, D), D)]
        o_j = o_s.at[pl.ds(j * (D // DH), D // DH)]
        wm_j = wmod_s.at[pl.ds((j + 2) * CPV - MSH, CPV)]
        mr_j = mraw_s.at[pl.ds((j + 2) * CPV - MSH, CPV)]
        units = [(qd, ng, u) for qd in range(2) for ng in range(2) for u in range(DH // 16)]
        npass = NB * (D // KP)
        cnt = 0
        due = {}
        hist = []
        lhs2 = [jnp.concatenate([o_j[kh * hq + u] for u in range(hq)], axis=1) for kh in range(D // KP)]
        for n in range(NB):
            acc = acc_s[n]
            cu, cn = divmod(n, MC // 128)
            mv = None
            for kh in range(D // KP):
                lhs = lhs2[kh]
                acc = jnp.dot(pltpu.bitcast(pin(lhs, due.pop(cnt, None)), bf16),
                              wo_j[kh * KP:(kh + 1) * KP, n * 128:(n + 1) * 128],
                              preferred_element_type=f32) + acc
                hist.append(acc)
                mine = units[cnt * len(units) // npass:(cnt + 1) * len(units) // npass]
                for n_, (qd, ng, u) in enumerate(mine):
                    last = w_unit(wo_j, [(4 * qd + c) * DH + u * 16 for c in range(4)], ng * 512,
                                  woc_s.at[j, ng], qd * DH + u * 16, [release(acc, O0_ROWS[n_][PERM[i_]]) for i_ in range(7)])
                if cnt + 2 < npass:
                    due.setdefault(cnt + 2, {})[2] = fence([last])
                if cnt in O0_LN:
                    qr, hf_ = O0_LN.index(cnt) % 4, O0_LN.index(cnt) // 4
                    ln1(X1, qr * QT + j * 16 + hf_ * 8, 8, release(acc, O0_LNROW))
                    due.setdefault(cnt + 3, {})[4] = fence([(hf_s, qr * QT + j * 16 + hf_ * 8)])
                if cnt in O0_HS:
                    hp_ = [(hist[-3 + u_ // 3], O0_HSROW[u_ % 3]) for u_ in range(9)]
                    h_slice(j * 16 + O0_HS.index(cnt) * 8, [release(*hp_[PERML[i_]]) for i_ in range(7)])
                    if cnt == O0_HS[0]:
                        due.setdefault(cnt + 2, {})[10] = fence([(hs_s.at[0], j * 16)])
                cnt += 1
                d = jnp.dot(sc[:, kh * KP:(kh + 1) * KP],
                            wm_j[cu, kh * KP:(kh + 1) * KP, cn * 128:(cn + 1) * 128],
                            preferred_element_type=f32)
                mv = d if mv is None else d + mv
            acc_s[n] = acc
            mr_j[cu, :, cn * 128:(cn + 1) * 128] = mv[0:8, :]
        assert not due
        return carry

    lax.fori_loop(0, NO, o0_body, 0)

    for u in range(NMC - MSH, NMC):
        cp_mod(u).wait()
    for u in range(NMC - MSH, NMC):
        mraw_s[u] = jnp.dot(sc_s[...], wmod_s[u], preferred_element_type=f32)[0:8, :]
    mod_s[:, 2 * D:3 * D] = mraw(2)
    mod_s[:, 3 * D:4 * D] = mraw(3)
    mod_s[:, 4 * D:5 * D] = 1.0 + mraw(4)
    mod_s[:, 5 * D:6 * D] = mraw(5)
    wr8 = jnp.broadcast_to(wr_s[...].astype(f32).reshape(1, D), (8, D))
    mod_s[:, 6 * D:7 * D] = (1.0 + mraw(4)) * wr8
    mod_s[:, 7 * D:7 * D + 128] = jnp.broadcast_to(jnp.sum(mraw(3) * wr8, axis=-1, keepdims=True), (8, 128))
    cp_wg().start(priority=1)
    for u in range(F // MC):
        cp_wu(u).start(priority=1)
    cp_wd().start(priority=1)

    def step(t, carry):
        cp_x(jnp.minimum(t + 1, nt - 1), XL).wait()

        @pl.when(t > 1)
        def _():
            cp_x(t - 1, XE).wait()
            cp_out(t - 2).wait()

        fence, release = sched()
        tprev = t - 1
        prods = [(i1, i2) for i1 in _ORDER for i2 in _ORDER]
        hv = [hs_s[u] for u in range(49)]

        qblk = {}

        def q_passes(g):
            def emit(r1, r2, n1, n2, c):
                for z in range(2):
                    qblk[8 * g + 4 * z + 2 * n1 + n2, 2 * r1 + r2] = c[:, z * DH:(z + 1) * DH]
            asm = _Assemble(emit)

            def run(i1, i2):
                u = 7 * i2 + i1
                w = jnp.concatenate([wqc_s[2 * g + z, u] for z in range(2)], axis=1)
                d = jnp.dot(hv[u], w, preferred_element_type=f32)
                ini = asm.init(i1, i2)
                if ini is not None:
                    d = d + ini
                asm.add(i1, i2, d)
                return d
            return [functools.partial(run, i1, i2) for i1, i2 in prods]

        def q_head(hh):
            return jnp.concatenate([qblk.pop((hh, r)) for r in range(4)], axis=0)

        def o_passes():
            ms = {}
            asm = []
            for ng in range(2):
                def emit(r1, r2, n1, n2, c, ng=ng):
                    acc_s[4 * ng + 2 * n1 + n2, pl.ds(r1 * HT + r2 * QT, QT), :] = c
                asm.append(_Assemble(emit))

            def run(ng, i1, i2, k, dep=None):
                u = 7 * i2 + i1
                lhs = jnp.concatenate([os_s[u, 4 * k + v] for v in range(4)], axis=1)
                w = jnp.concatenate([woc_s[2 * k + v, ng, u] for v in range(2)], axis=0)
                d = jnp.dot(lhs, pin_bf16(w, dep), preferred_element_type=f32)
                early = ng == 0 or (i1, i2) in prods[:NE]
                if k == 1:
                    d = d + ms.pop((ng, u))
                if k == (1 if early else 0):
                    ini = asm[ng].init(i1, i2)
                    if ini is not None:
                        d = d + ini
                if k == 0:
                    ms[ng, u] = d
                else:
                    asm[ng].add(i1, i2, d)
                return d
            NE = 16
            seq = [(0,) + pr + (0,) for pr in prods] + [(1,) + pr + (0,) for pr in prods[:NE]]
            seq += [(0,) + pr + (1,) for pr in prods] + [(1,) + pr + (1,) for pr in prods[:NE]]
            seq += [(1,) + pr + (k,) for pr in prods[NE:] for k in range(2)]
            return [functools.partial(run, *a) for a in seq]

        def side(hp, pts):
            rel = [release(v_, rw) for v_, rw in pts]
            for u in range(2):
                epi_rows(tprev, (2 * hp + u) * CHE, CHE, rel[u])
            if len(rel) == 3:
                ln1(XL, hp * 16, 16, rel[2])
            else:
                for u in range(2):
                    ln1(XL, hp * 16 + 8 * u, 8, rel[2 + u])
            return fence([(out_s, 0), (best_r, 0), (keep_s, 0), (hf_s, 0)])

        def o_slice(qd, oq, u, pts):
            blk = [[[[oq[k1][k2][r1 * HT + r2 * QT + 16 * u:r1 * HT + r2 * QT + 16 * u + 16]
                      for k2 in range(2)] for k1 in range(2)] for r2 in range(2)] for r1 in range(2)]
            if len(pts) == 7:
                pts = [pts[PERML[i_]] for i_ in range(7)]
            ops = _two_level(_lhs_sums, blk, [jnp.tile(release(v_, rw), (2, 1)) for v_, rw in pts])
            for v in range(7):
                os_s[7 * v:7 * v + 7, qd, 16 * u:16 * u + 16, :] = ops[v]
            return fence([(os_s.at[0, qd], 16 * u)])

        assert 2 * HP * CHE == TQ
        for fn in q_passes(0):
            fn()
        opl = o_passes()
        oq = fo = ob_ = None
        for hp in range(HP):
            g, pp = divmod(hp, 4)
            if pp == 0:
                fill = q_passes(g + 1) if g + 1 < HKV else opl
            qa, qb = q_head(2 * hp), q_head(2 * hp + 1)
            sa_ = scores(qa if fo is None else pin(qa, {0: fo}), g)
            pa, la = softmax(sa_)
            vals = {'s': sa_, 'ob': ob_}
            if oq is not None:
                fl = [o_slice(hp // 2 - 1, oq, 2 * (hp % 2) + u, [(vals[nm], rw) for nm, rw in OS_PTS[u]])
                      for u in range(2 if FILL[pp][1] < 7 else 1)]
                qb = pin(qb, {0: functools.reduce(lambda a_, b_: a_ | b_, fl)})
            rs_ = [fill.pop(0)() for _ in range(FILL[pp][0])]
            vals.update({i_: rs_[max(len(rs_) - 6 + i_, 0)] for i_ in range(6)})
            fs = side(hp, [(vals[nm] if vals[nm] is not None else sa_, rw) for nm, rw in SIDE_PTS])
            pb, lb = softmax(scores(qb, g))
            oa_ = pv(pa, g)
            oa = oa_ * la
            rs_ = [fill.pop(0)() for _ in range(FILL[pp][1])]
            fo = None
            if oq is not None and FILL[pp][1] >= 7:
                vals = {'oa': oa_}
                vals.update(enumerate(rs_))
                fo = o_slice(hp // 2 - 1, oq, 2 * (hp % 2) + 1, [(vals[nm], rw) for nm, rw in OS_F2])
            ob_ = pv(pin(pb, {0: fs}), g)
            ob = ob_ * lb
            if hp % 2 == 0:
                oprev = (oa, ob)
            else:
                oq = [oprev, (oa, ob)]

        capture(tprev)
        cp_out(tprev).start()
        cp_x(t, XE).start()
        cp_x(jnp.minimum(t + 2, nt - 1), XL).start()
        pts = []
        due = {} if fo is None else {2: fo}
        for s, fn in enumerate(opl):
            pts.append((fn(due.pop(s, None)), 0))
            if len(pts) % 3 == 0 and len(pts) <= 12:
                o_slice(HP // 2 - 1, oq, len(pts) // 3 - 1, pts[-3:])
            u, rem = divmod(s - HS0, HSG)
            if rem == 0 and 0 <= u < QT // 8:
                h_slice(u * 8, [release(pts[-1 - HSS * (6 - PERML[i_])][0]) for i_ in range(7)])
                due[s + 6] = fence([(hs_s.at[0], 0)])
        assert not due
        return carry

    lax.fori_loop(1, nt, step, 0)

    cp_wg().wait()
    for u in range(F // MC):
        cp_wu(u).wait()
    cp_wd().wait()
    cp_x(nt - 1, XL).wait()
    cp_x(nt - 1, XE).wait()
    cp_out(nt - 2).wait()
    epi_rows(nt - 1, 0, TQ, write_out=False)
    _, release_t = sched()
    rel0 = release_t(best_r[...])
    rbest, idx, rows = capture(nt - 1)
    base = pl.multiple_of((idx // 16) * 16, 16)
    x1 = rows[:, 0:D].reshape(2, 8, D)
    mu = jnp.tile(rows[:, D:D + 128], (1, NB)).reshape(2, 8, D)
    rs = jnp.tile(rows[:, D + 128:D + 256], (1, NB)).reshape(2, 8, D)
    h2 = (x1 - mu) * rs * mvec(4) + mvec(3)
    xs = h2.reshape(16, D).astype(bf16)
    gt = jnp.dot(xs, wq_s[:, 0:F], preferred_element_type=f32)
    for u in range(TQ // 8):
        rel = rel0 if u < T_EARLY else release_t(gt[:, (u - T_EARLY) * 128:(u - T_EARLY + 1) * 128])
        kr = keep_s[8 * u:8 * u + 8, :]
        xc_ = kr[:, 0:D] - jnp.tile(kr[:, D:D + 128] + rel, (1, NB))
        h2_ = xc_ * jnp.tile(kr[:, D + 128:D + 256], (1, NB)) * mvec(4)[0] + mvec(3)[0]
        out_s[8 * u:8 * u + 8, :] = (kr[:, 0:D] + mvec(5)[0] * h2_).astype(out_s.dtype)
    cp_out(nt - 1).start()
    up = jnp.concatenate([jnp.dot(xs, wmod_s[u], preferred_element_type=f32) for u in range(F // MC)], axis=1)
    a = (gt * jax.nn.sigmoid(gt) * up).astype(bf16)
    y = jnp.dot(a, wo_s[0:F, 0:D], preferred_element_type=f32)
    y = y * jnp.tile(jax.nn.sigmoid(rbest), (1, NB))
    rr = lax.broadcasted_iota(jnp.int32, (16, D), 0) + base
    upd = jnp.where(rr == idx, y, 0.0).reshape(2, 8, D)
    new = (x1 + mvec(5) * (h2 + upd)).reshape(16, D)
    fix_s[...] = new.astype(fix_s.dtype)
    cp_out(nt - 1).wait()
    fix = pltpu.make_async_copy(fix_s, out_hbm.at[pl.ds(base, 16), :], osems.at[0])
    fix.start()
    fix.wait()


def _compiler_params():
    kw = dict(vmem_limit_bytes=124 * 1024 * 1024)
    try:
        return pltpu.CompilerParams(disable_semaphore_checks=True, disable_bounds_checks=True, **kw)
    except TypeError:
        return pltpu.CompilerParams(**kw)


@jax.jit
def pallas_adaLN_cond__sliding_block_cached__moe_arch_mod__prompt_kernel(
    A_x: jax.Array,
    A_k_cache: jax.Array,
    A_v_cache: jax.Array,
    A_wq: jax.Array,
    A_wo: jax.Array,
    B_x: jax.Array,
    B_w_r: jax.Array,
    B_w_gate: jax.Array,
    B_w_up: jax.Array,
    B_w_down: jax.Array,
    c: jax.Array,
    w_mod: jax.Array,
):
    B, S, D = A_x.shape
    assert B == 1
    HKV, SK = A_k_cache.shape[1], A_k_cache.shape[2]
    W = min(4096, max(256, SK // 4))
    F = B_w_gate.shape[1]
    dt = A_x.dtype
    f32 = jnp.float32
    nt = S // TQ
    NB = D // 128
    NMC = 6 * D // MC
    x2 = A_x.reshape(S, D)
    anyspec = pl.BlockSpec(memory_space=pl.ANY)
    kern = functools.partial(_kernel, S=S, D=D, HKV=HKV, SK=SK, W=W, F=F)
    out = pl.pallas_call(
        kern,
        in_specs=[anyspec] * 11,
        out_specs=anyspec,
        out_shape=jax.ShapeDtypeStruct((S, D), dt),
        scratch_shapes=[
            pltpu.VMEM((D,), dt),
            pltpu.VMEM((1, D), dt),
            pltpu.VMEM((3, TQ, D), dt),
            pltpu.VMEM((HKV, W, DH), dt),
            pltpu.VMEM((HKV, W, DH), dt),
            pltpu.VMEM((D, HQ * DH + PAD), dt),
            pltpu.VMEM((HQ * DH, D + PAD), dt),
            pltpu.VMEM((NMC, D, MC), dt),
            pltpu.VMEM((TQ, D), dt),
            pltpu.VMEM((HQ // 4, 49, D // 4, DH), dt),
            pltpu.VMEM((HQ * DH // D, 2, 49, 2 * DH, 128), dt),
            pltpu.VMEM((TQ, D), f32),
            pltpu.VMEM((49, TQ // 4, D // 4), dt),
            pltpu.VMEM((49, HQ // 4, TQ // 4, DH), dt),
            pltpu.VMEM((16, D), dt),
            pltpu.VMEM((NMC, 8, MC), f32),
            pltpu.VMEM((8, 7 * D + 512), f32),
            pltpu.VMEM((TQ, D), dt),
            pltpu.VMEM((HQ, TQ // 2, DH), jnp.uint32),
            pltpu.VMEM((NB, TQ, 128), f32),
            pltpu.VMEM((TQ, D + 256), f32),
            pltpu.VMEM((16, D + 256), f32),
            pltpu.VMEM((16, D), dt),
            pltpu.VMEM((8, 128), f32),
            pltpu.VMEM((8, 128), jnp.int32),
            pltpu.SMEM((1,), jnp.int32),
            pltpu.SemaphoreType.DMA((4 + NMC + HQ + 2 * HKV + HQ * DH // D + 3,)),
            pltpu.SemaphoreType.DMA((1,)),
        ],
        compiler_params=_compiler_params(),
    )(B_w_r, c, x2, A_k_cache, A_v_cache, A_wq, A_wo, w_mod, B_w_gate, B_w_up, B_w_down)
    return out.reshape(B, S, D)
```

```python
import functools

import jax
import jax.numpy as jnp
from jax import lax
import jax.experimental.pallas as pl
import jax.experimental.pallas.tpu as pltpu

HQ = 32
DH = 128
TQ = 256
PAD = 128
P0 = 4
G0 = 4
MC = 512
MSH = 1
CHE = 8
FILL = ((7, 7), (7, 7), (7, 7), (7, 0))

SIDE_PTS = ((1, 48), (2, 48), ('ob', 0), ('ob', 56))
OS_F2 = [('oa', 128), ('oa', 192), (0, 0), (1, 0), (2, 0), (3, 0), (4, 0)]
OS_PTS = ([('ob', 96 + 16 * i) for i in range(7)],
          [('ob', 208), ('ob', 224), ('ob', 240), ('s', 0), ('s', 16), ('s', 32), ('s', 48)])
HS0, HSG, HSS = 30, 14, 2
A0_W = (2, 250, 394, 760, 130, 150, 370)
A0_DUE = 14
O0_ROWS = ((0, 16, 32, 56, 72, 88, 112), (128, 144, 168, 184, 200, 224, 240))
O0_LN = (0, 1, 2, 3, 4, 5, 6, 7)
O0_LNROW = 24
O0_HS = (12, 15)
O0_HSROW = (8, 104, 192)
PERM = (3, 1, 4, 0, 5, 2, 6)
PERML = (0, 1, 2, 3, 4, 5, 6)

T_EARLY = 8
EPS = 1e-5
LOG2E = 1.4426950408889634


def _ln_stats(x, rel=None):
    d = x.shape[-1]
    part = x[..., 0:128]
    for j in range(1, d // 128):
        part = part + x[..., j * 128:(j + 1) * 128]
    if rel is not None:
        part = part + rel
    m = jnp.sum(part, axis=-1, keepdims=True) * (1.0 / d)
    xc = x - m
    v = jnp.mean(xc * xc, axis=-1, keepdims=True)
    return m, xc, lax.rsqrt(v + EPS)


def _ln(x, rel=None):
    _, xc, rs = _ln_stats(x, rel)
    return xc * rs


def _recip(l):
    return pl.reciprocal(l, approx=True)


def _lhs_sums(a11, a12, a21, a22):
    return [a11 + a22, a21 + a22, a11, a22, a11 + a12, a21 - a11, a12 - a22]


def _rhs_sums(b11, b12, b21, b22):
    return [b11 + b22, b11, b12 - b22, b21 - b11, b22, b11 + b12, b21 + b22]


_ORDER = [3, 4, 0, 6, 1, 2, 5]
_BLOCK = {6: (0, 0), 1: (1, 0), 2: (0, 1), 5: (1, 1)}


def _init(i, z):
    return {0: lambda: z[3] - z[4], 6: lambda: z[0], 1: lambda: z[3], 2: lambda: z[4],
            5: lambda: z[0] - z[1] + z[2]}.get(i, lambda: None)()


def _two_level(sums, blk, rel):
    o = [[jnp.stack([blk[a1][a2][b1][b2] for a2 in range(2) for b2 in range(2)]) for b1 in range(2)]
         for a1 in range(2)]
    if rel is not None and len(rel) == 3:
        o = [[o[a1][b1] + rel[0 if a1 == b1 else 1 + a1][None] for b1 in range(2)] for a1 in range(2)]
    x = jnp.stack(sums(o[0][0], o[0][1], o[1][0], o[1][1]), axis=1)
    x = [x[u] for u in range(4)]
    if rel is not None and len(rel) == 7:
        r7 = jnp.stack(rel)
        x = [x[0] + r7, x[1], x[2], x[3] + r7]
    return [y.astype(jnp.bfloat16) for y in sums(*x)]


class _Assemble:
    def __init__(self, emit):
        self.z, self.outer, self.inj, self.emit = {}, {}, {}, emit

    def init(self, i1, i2):
        v = _init(i2, self.z)
        if i2 in _BLOCK and i1 not in (3, 4):
            self.inj[i2] = _init(i1, self.outer[i2])
            v = v + self.inj[i2]
            if i2 == 5:
                v = v + (self.inj[1] - self.inj[2])
        return v

    def add(self, i1, i2, m):
        self.z[i2] = m
        if i2 in _BLOCK:
            self.outer.setdefault(i2, {})[i1] = m
            if i1 in _BLOCK:
                (r1, n1), (r2, n2) = _BLOCK[i1], _BLOCK[i2]
                self.emit(r1, r2, n1, n2, m)


def _kernel(wr_hbm, c_hbm, x_hbm, k_hbm, v_hbm, wq_hbm, wo_hbm, wmod_hbm,
            wg_hbm, wu_hbm, wd_hbm, out_hbm,
            wr_s, c_s, x_s, k_s, v_s, wq_s, wo_s, wmod_s, out_s,
            wqc_s, woc_s, hf_s, hs_s, os_s,
            sc_s, mraw_s, mod_s, h_s, o_s, acc_s, keep_s, cand_s, fix_s, best_r, best_i, zero_s, sems, osems,
            *, S, D, HKV, SK, W, F):
    nt = S // TQ
    rep = HQ // HKV
    NB = D // 128
    HP = HQ // 2
    HT = TQ // 2
    QT = TQ // 4
    KH = D // 2
    KQ = D // 4
    KP = 512
    CPV = D // MC
    NMC = 6 * CPV
    NA = (HQ - P0) // G0
    NO = HQ * DH // D
    f32 = jnp.float32
    bf16 = jnp.bfloat16
    u32 = jnp.uint32
    qscale = (DH ** -0.5) * LOG2E
    assert KH == KP and rep == 8 and NB == 8 and NO == 4 and P0 == 4 and G0 == 4

    def al(v, n):
        return v if isinstance(v, int) else pl.multiple_of(v, n)

    S_C, S_WR, S_WG, S_WD, S_M = 0, 1, 2, 3, 4
    S_WQ = S_M + NMC
    S_K = S_WQ + HQ
    S_V = S_K + HKV
    S_WO = S_V + HKV
    S_X = S_WO + NO

    def cp_c():
        return pltpu.make_async_copy(c_hbm, c_s, sems.at[S_C])

    def cp_wr():
        return pltpu.make_async_copy(wr_hbm, wr_s, sems.at[S_WR])

    def cp_mod(j):
        return pltpu.make_async_copy(wmod_hbm.at[:, pl.ds(al(j * MC, MC), MC)], wmod_s.at[j], sems.at[S_M + j])

    def cp_wg():
        return pltpu.make_async_copy(wg_hbm, wq_s.at[:, pl.ds(0, F)], sems.at[S_WG])

    def cp_wu(u):
        return pltpu.make_async_copy(wu_hbm.at[:, pl.ds(u * MC, MC)], wmod_s.at[u], sems.at[S_M + u])

    def cp_wd():
        return pltpu.make_async_copy(wd_hbm, wo_s.at[pl.ds(0, F), pl.ds(0, D)], sems.at[S_WD])

    def cp_wq(h, n=1):
        sl = pl.ds(al(h * DH, DH), n * DH)
        return pltpu.make_async_copy(wq_hbm.at[:, sl], wq_s.at[:, sl], sems.at[S_WQ + h])

    def cp_k(g):
        return pltpu.make_async_copy(k_hbm.at[0, g, pl.ds(SK - W, W), :], k_s.at[g], sems.at[S_K + g])

    def cp_v(g):
        return pltpu.make_async_copy(v_hbm.at[0, g, pl.ds(SK - W, W), :], v_s.at[g], sems.at[S_V + g])

    def cp_wo(j):
        sl = pl.ds(al(j * D, D), D)
        return pltpu.make_async_copy(wo_hbm.at[sl, :], wo_s.at[sl, pl.ds(0, D)], sems.at[S_WO + j])

    def rsl(t, r0=0, n=TQ):
        return pl.ds(al(t * TQ + r0, n), n)

    XE, X1, XL = 0, 1, 2

    def cp_x(t, slot):
        return pltpu.make_async_copy(x_hbm.at[rsl(t), :], x_s.at[slot], sems.at[S_X + slot])

    def cp_out(t):
        return pltpu.make_async_copy(out_s, out_hbm.at[rsl(t), :], osems.at[0])

    def sched():
        zero = zero_s[0]
        z16 = pl.multiple_of(zero, 16)
        zvec = jnp.full((8, 128), zero, jnp.int32).astype(u32)

        def fence(deps):
            d = None
            for ref, base in deps:
                n = 16 if ref.dtype == bf16 else 8
                v = pltpu.bitcast(ref[pl.ds(pl.multiple_of(base + z16, n), n), 0:128], u32)
                d = v if d is None else d | v
            return d & zvec

        def release(acc, r0=0):
            return pltpu.bitcast(pltpu.bitcast(acc[r0:r0 + 8, 0:128], u32) & zvec, f32)

        return fence, release

    def pin(a, at):
        if not at:
            return a
        parts = []
        prev = 0
        for rb in sorted(at):
            r0 = rb * 8
            if r0 > prev:
                parts.append(a[prev:r0, :])
            if a.dtype == f32:
                blk = a[r0:r0 + 8, 0:128] + pltpu.bitcast(at[rb], f32)
            else:
                blk = a[r0:r0 + 8, 0:128] | at[rb]
            if a.shape[1] > 128:
                blk = jnp.concatenate([blk, a[r0:r0 + 8, 128:]], axis=1)
            parts.append(blk)
            prev = r0 + 8
        if prev < a.shape[0]:
            parts.append(a[prev:, :])
        return jnp.concatenate(parts, axis=0)

    def pin_bf16(w, d):
        if d is None:
            return w
        top = pltpu.bitcast(pltpu.bitcast(w[0:16], u32) | d, bf16)
        return jnp.concatenate([top, w[16:]], axis=0)

    def mvec(j):
        return mod_s[:, j * D:(j + 1) * D][None]

    def mraw(j):
        return jnp.concatenate([mraw_s[j * CPV + u] for u in range(CPV)], axis=1)

    def xrows(t, sl, n):
        return x_s[t, sl, :].astype(f32).reshape(n // 8, 8, D)

    def ln1(t, r0, n, rel=None):
        xn = _ln(xrows(t, pl.ds(al(r0, n), n), n), rel)
        hf_s[pl.ds(al(r0, n), n), :] = (xn * mvec(1) + mvec(0)).reshape(n, D)

    def h_slice(r0, rel):
        hq = [hf_s[pl.ds(al(r * QT + r0, 8), 8), :] for r in range(4)]
        blk = [[[[hq[2 * r1 + r2][:, (2 * k1 + k2) * KQ:(2 * k1 + k2 + 1) * KQ] for k2 in range(2)]
                 for k1 in range(2)] for r2 in range(2)] for r1 in range(2)]
        ops = _two_level(_lhs_sums, blk, None if rel is None else [jnp.tile(v, (1, KQ // 128)) for v in rel])
        for u in range(7):
            hs_s[7 * u:7 * u + 7, pl.ds(al(r0, 8), 8), :] = ops[u]

    def w_unit(src, rows4, c0, dst, d0, rel):
        w = [src[pl.ds(al(r, 16), 16), c0:c0 + 512].astype(f32) for r in rows4]
        blk = [[[[w[2 * k1 + k2][:, (2 * n1 + n2) * 128:(2 * n1 + n2 + 1) * 128] for n2 in range(2)]
                 for n1 in range(2)] for k2 in range(2)] for k1 in range(2)]
        ops = _two_level(_rhs_sums, blk, None if rel is None else [jnp.tile(v, (2, 1)) for v in rel])
        for u in range(7):
            dst[7 * u:7 * u + 7, pl.ds(al(d0, 16), 16), :] = ops[u]
        return (dst.at[0], d0)

    def epi_rows(t, r0, n, rel=None, write_out=True):
        sl = pl.ds(r0, n)
        attn = jnp.concatenate([acc_s[j, sl, :] for j in range(NB)], axis=1).reshape(n // 8, 8, D)
        x1 = xrows(XE, sl, n) + mvec(2) * attn
        m, xc, rs = _ln_stats(x1, rel)
        keep_s[sl, 0:D] = x1.reshape(n, D)
        keep_s[sl, D:D + 128] = jnp.broadcast_to(m.reshape(n, 1), (n, 128))
        keep_s[sl, D + 128:D + 256] = jnp.broadcast_to(rs.reshape(n, 1), (n, 128))
        if write_out:
            h2 = xc * rs * mvec(4) + mvec(3)
            out_s[sl, :] = (x1 + mvec(5) * h2).reshape(n, D).astype(out_s.dtype)
        r = rs * jnp.sum(xc * mvec(6), axis=-1, keepdims=True) + mod_s[:, 7 * D:7 * D + 128][None]
        r = r.astype(bf16).astype(f32)
        bv = best_r[...]
        bi = best_i[...]
        sub = lax.broadcasted_iota(jnp.int32, (8, 128), 0)
        for u in range(n // 8):
            ru = r[u]
            better = ru > bv
            bv = jnp.where(better, ru, bv)
            bi = jnp.where(better, sub + (t * TQ + r0 + u * 8), bi)
        best_r[...] = bv
        best_i[...] = bi

    def capture(t):
        bv = best_r[...]
        rbest = jnp.max(bv, axis=0, keepdims=True)
        ibest = jnp.min(jnp.where(bv == rbest, best_i[...], S), axis=0, keepdims=True)
        idx = jnp.minimum(ibest[0, 0], S - 1)
        local = idx - t * TQ
        off = pl.multiple_of(jnp.clip(local // 16, 0, TQ // 16 - 1) * 16, 16)
        rows = jnp.where(local >= 0, keep_s[pl.ds(off, 16), :], cand_s[...])
        cand_s[...] = rows
        return rbest, idx, rows

    def scores(q, g):
        return lax.dot_general(q.astype(bf16), k_s[g], (((1,), (1,)), ((), ())), preferred_element_type=f32)

    def softmax(s):
        m = jnp.max(s, axis=-1, keepdims=True)
        p = jnp.exp2(s - m)
        part = p[:, 0:128]
        for j in range(1, W // 128):
            part = part + p[:, j * 128:(j + 1) * 128]
        p = jnp.concatenate([jnp.minimum(p[:, 0:128], part), p[:, 128:]], axis=1)
        return p, _recip(jnp.sum(part, axis=-1, keepdims=True))

    def pv(p, g):
        return jnp.dot(p.astype(bf16), v_s[g], preferred_element_type=f32)

    def block0(wv, c0, h0, nh, units):
        fence, release = sched()
        hval = h_s[...]
        g = h0 // rep
        tqk = [512 + 1024 * u for u in range(nh)]
        tpv = [tqk[u] + (768 if u + 1 < nh else 256) for u in range(nh)]
        wins = [(130, tqk[0])]
        for u in range(nh):
            wins.append((tqk[u] + A0_W[0], tqk[u] + (A0_W[1] if u + 1 < nh else A0_W[4])))
            if u + 1 < nh:
                wins.append((tqk[u] + A0_W[2], tqk[u] + A0_W[3]))
        wins.append((tpv[-1] + A0_W[5], tpv[-1] + A0_W[6]))
        slots = [t_ for a_, b_ in wins for t_ in range(a_, b_, 8)]
        npt = 7 * len(units)
        times = [slots[(u * len(slots)) // npt] for u in range(npt)]
        todo = [(un, times[7 * u:7 * u + 7]) for u, un in enumerate(units)]
        vals = []

        def emit(tmax):
            last = []
            while todo and todo[0][1][-1] < tmax:
                (sv, dv, r0), ts = todo.pop(0)
                rel = []
                for i_ in range(7):
                    t0_, v_ = [tv for tv in vals if tv[0] <= ts[PERM[i_]]][-1]
                    rel.append(release(v_, min((ts[PERM[i_]] - t0_) // 8 * 8, TQ - 8)))
                last = last[-1:] + [w_unit(sv, [c * KQ + r0 for c in range(4)], 0, dv, r0, rel)]
            return last

        def qproj(u, t_):
            cols = slice(c0 + u * DH, c0 + (u + 1) * DH)
            q1 = jnp.dot(hval[:, 0:KH], wv[0:KH, cols], preferred_element_type=f32)
            q2 = jnp.dot(hval[:, KH:D], wv[KH:D, cols], preferred_element_type=f32) + q1
            vals.extend([(t_ + 130, q1), (t_ + 386, q2)])
            return q2

        q = qproj(0, 0)
        for u in range(nh):
            s = scores(q, g)
            vals.append((tqk[u] + 130, s))
            p, li = softmax(s)
            if u + 1 < nh:
                q = qproj(u + 1, tqk[u] + 256)
            deps = emit(tpv[u]) + ([(o_s.at[h0 + u - 1], 0)] if u > 0 else [])
            if deps:
                p = pin(p, {A0_DUE: fence(deps)})
            o = pv(p, g)
            vals.append((tpv[u] + 130, o))
            o_s[h0 + u] = pltpu.bitcast((o * li).astype(bf16), u32)
        emit(1 << 30)

    def first_tile():
        cp_c().start()
        cp_x(0, XE).start()
        for j in range(2 * CPV):
            cp_mod(j).start()
        cp_wq(0).start()
        cp_k(0).start()
        cp_v(0).start()
        cp_wq(1, P0 - 1).start()
        for j in range(NA):
            h0 = P0 + j * G0
            cp_wq(h0, G0).start()
            if h0 % rep == 0:
                cp_k(h0 // rep).start()
                cp_v(h0 // rep).start()
        cp_x(1, X1).start()
        cp_wr().start()
        for j in range(NO):
            cp_wo(j).start()
            for u in range(CPV):
                if (j + 2) * CPV + u - MSH >= 2 * CPV:
                    cp_mod((j + 2) * CPV + u - MSH).start()
        for u in range(NMC - MSH, NMC):
            cp_mod(u).start()
        cp_x(2, XL).start()

        zero_s[0] = 0
        for n in range(NB):
            acc_s[n] = jnp.zeros((TQ, 128), f32)
        hs_s[0] = jnp.zeros((QT, KQ), bf16)
        cand_s[...] = jnp.zeros(cand_s.shape, f32)
        best_r[...] = jnp.full(best_r.shape, -jnp.inf, f32)
        best_i[...] = jnp.zeros(best_i.shape, jnp.int32)
        cp_c().wait()
        cp_x(0, XE).wait()
        cf = c_s[...].astype(f32)
        sc_s[...] = jnp.broadcast_to(cf * jax.nn.sigmoid(cf), (16, D)).astype(bf16)
        xn0 = _ln(xrows(XE, pl.ds(0, TQ), TQ))

        def mod_body(j, carry):
            cp_mod(j).wait()
            mraw_s[j] = jnp.dot(sc_s[...], wmod_s[j], preferred_element_type=f32)[0:8, :]
            return carry

        lax.fori_loop(0, 2 * CPV, mod_body, 0)
        mod_s[:, 0:D] = mraw(0) * qscale
        mod_s[:, D:2 * D] = (1.0 + mraw(1)) * qscale
        h_s[...] = (xn0 * mvec(1) + mvec(0)).reshape(TQ, D).astype(bf16)
        NU = KQ // 16
        NPE = NU - NA
        cp_wq(0).wait()
        cp_k(0).wait()
        cp_v(0).wait()
        block0(wq_s, 0, 0, 1, [])
        cp_wq(1, P0 - 1).wait()
        block0(wq_s, DH, 1, P0 - 1, [(wq_s, wqc_s.at[0], u * 16) for u in range(NPE)])

        def a0_body(j, carry):
            h0 = P0 + j * G0
            cp_wq(h0, G0).wait()

            @pl.when(h0 % rep == 0)
            def _():
                cp_k(h0 // rep).wait()
                cp_v(h0 // rep).wait()

            sv = wq_s.at[:, pl.ds(al(h0 * DH, 4 * DH), 4 * DH)]
            dv = wqc_s.at[j + 1]
            block0(sv, 0, h0, G0, [(sv, dv, u * 16) for u in range(NU)] + [(wq_s, wqc_s.at[0], (NPE + j) * 16)])
            return carry

        lax.fori_loop(0, NA, a0_body, 0)
        cp_x(1, X1).wait()
        cp_wr().wait()

        def o0_body(j, carry):
            cp_wo(j).wait()
            for u in range(CPV):
                if u >= MSH:
                    cp_mod((j + 2) * CPV + u - MSH).wait()
                else:
                    @pl.when(j > 0)
                    def _():
                        cp_mod((j + 2) * CPV + u - MSH).wait()

            fence, release = sched()
            sc = sc_s[...]
            hq = KP // DH
            wo_j = wo_s.at[pl.ds(al(j * D, D), D)]
            o_j = o_s.at[pl.ds(j * (D // DH), D // DH)]
            wm_j = wmod_s.at[pl.ds((j + 2) * CPV - MSH, CPV)]
            mr_j = mraw_s.at[pl.ds((j + 2) * CPV - MSH, CPV)]
            units = [(qd, ng, u) for qd in range(2) for ng in range(2) for u in range(DH // 16)]
            npass = NB * (D // KP)
            cnt = 0
            due = {}
            hist = []
            lhs2 = [jnp.concatenate([o_j[kh * hq + u] for u in range(hq)], axis=1) for kh in range(D // KP)]
            for n in range(NB):
                acc = acc_s[n]
                cu, cn = divmod(n, MC // 128)
                mv = None
                for kh in range(D // KP):
                    lhs = lhs2[kh]
                    acc = jnp.dot(pltpu.bitcast(pin(lhs, due.pop(cnt, None)), bf16),
                                  wo_j[kh * KP:(kh + 1) * KP, n * 128:(n + 1) * 128],
                                  preferred_element_type=f32) + acc
                    hist.append(acc)
                    mine = units[cnt * len(units) // npass:(cnt + 1) * len(units) // npass]
                    for n_, (qd, ng, u) in enumerate(mine):
                        last = w_unit(wo_j, [(4 * qd + c) * DH + u * 16 for c in range(4)], ng * 512,
                                      woc_s.at[j, ng], qd * DH + u * 16, [release(acc, O0_ROWS[n_][PERM[i_]]) for i_ in range(7)])
                    if cnt + 2 < npass:
                        due.setdefault(cnt + 2, {})[2] = fence([last])
                    if cnt in O0_LN:
                        qr, hf_ = O0_LN.index(cnt) % 4, O0_LN.index(cnt) // 4
                        ln1(X1, qr * QT + j * 16 + hf_ * 8, 8, release(acc, O0_LNROW))
                        due.setdefault(cnt + 3, {})[4] = fence([(hf_s, qr * QT + j * 16 + hf_ * 8)])
                    if cnt in O0_HS:
                        hp_ = [(hist[-3 + u_ // 3], O0_HSROW[u_ % 3]) for u_ in range(9)]
                        h_slice(j * 16 + O0_HS.index(cnt) * 8, [release(*hp_[PERML[i_]]) for i_ in range(7)])
                        if cnt == O0_HS[0]:
                            due.setdefault(cnt + 2, {})[10] = fence([(hs_s.at[0], j * 16)])
                    cnt += 1
                    d = jnp.dot(sc[:, kh * KP:(kh + 1) * KP],
                                wm_j[cu, kh * KP:(kh + 1) * KP, cn * 128:(cn + 1) * 128],
                                preferred_element_type=f32)
                    mv = d if mv is None else d + mv
                acc_s[n] = acc
                mr_j[cu, :, cn * 128:(cn + 1) * 128] = mv[0:8, :]
            assert not due
            return carry

        lax.fori_loop(0, NO, o0_body, 0)

        for u in range(NMC - MSH, NMC):
            cp_mod(u).wait()
        for u in range(NMC - MSH, NMC):
            mraw_s[u] = jnp.dot(sc_s[...], wmod_s[u], preferred_element_type=f32)[0:8, :]
        mod_s[:, 2 * D:3 * D] = mraw(2)
        mod_s[:, 3 * D:4 * D] = mraw(3)
        mod_s[:, 4 * D:5 * D] = 1.0 + mraw(4)
        mod_s[:, 5 * D:6 * D] = mraw(5)
        wr8 = jnp.broadcast_to(wr_s[...].astype(f32).reshape(1, D), (8, D))
        mod_s[:, 6 * D:7 * D] = (1.0 + mraw(4)) * wr8
        mod_s[:, 7 * D:7 * D + 128] = jnp.broadcast_to(jnp.sum(mraw(3) * wr8, axis=-1, keepdims=True), (8, 128))
        cp_wg().start(priority=1)
        for u in range(F // MC):
            cp_wu(u).start(priority=1)
        cp_wd().start(priority=1)

    def step(t, carry):
        cp_x(jnp.minimum(t + 1, nt - 1), XL).wait()

        @pl.when(t > 1)
        def _():
            cp_x(t - 1, XE).wait()
            cp_out(t - 2).wait()

        fence, release = sched()
        tprev = t - 1
        prods = [(i1, i2) for i1 in _ORDER for i2 in _ORDER]
        hv = [hs_s[u] for u in range(49)]

        qblk = {}

        def q_passes(g):
            def emit(r1, r2, n1, n2, c):
                for z in range(2):
                    qblk[8 * g + 4 * z + 2 * n1 + n2, 2 * r1 + r2] = c[:, z * DH:(z + 1) * DH]
            asm = _Assemble(emit)

            def run(i1, i2):
                u = 7 * i2 + i1
                w = jnp.concatenate([wqc_s[2 * g + z, u] for z in range(2)], axis=1)
                d = jnp.dot(hv[u], w, preferred_element_type=f32)
                ini = asm.init(i1, i2)
                if ini is not None:
                    d = d + ini
                asm.add(i1, i2, d)
                return d
            return [functools.partial(run, i1, i2) for i1, i2 in prods]

        def q_head(hh):
            return jnp.concatenate([qblk.pop((hh, r)) for r in range(4)], axis=0)

        def o_passes():
            ms = {}
            asm = []
            for ng in range(2):
                def emit(r1, r2, n1, n2, c, ng=ng):
                    acc_s[4 * ng + 2 * n1 + n2, pl.ds(r1 * HT + r2 * QT, QT), :] = c
                asm.append(_Assemble(emit))

            def run(ng, i1, i2, k, dep=None):
                u = 7 * i2 + i1
                lhs = jnp.concatenate([os_s[u, 4 * k + v] for v in range(4)], axis=1)
                w = jnp.concatenate([woc_s[2 * k + v, ng, u] for v in range(2)], axis=0)
                d = jnp.dot(lhs, pin_bf16(w, dep), preferred_element_type=f32)
                early = ng == 0 or (i1, i2) in prods[:NE]
                if k == 1:
                    d = d + ms.pop((ng, u))
                if k == (1 if early else 0):
                    ini = asm[ng].init(i1, i2)
                    if ini is not None:
                        d = d + ini
                if k == 0:
                    ms[ng, u] = d
                else:
                    asm[ng].add(i1, i2, d)
                return d
            NE = 16
            seq = [(0,) + pr + (0,) for pr in prods] + [(1,) + pr + (0,) for pr in prods[:NE]]
            seq += [(0,) + pr + (1,) for pr in prods] + [(1,) + pr + (1,) for pr in prods[:NE]]
            seq += [(1,) + pr + (k,) for pr in prods[NE:] for k in range(2)]
            return [functools.partial(run, *a) for a in seq]

        def side(hp, pts):
            rel = [release(v_, rw) for v_, rw in pts]
            for u in range(2):
                epi_rows(tprev, (2 * hp + u) * CHE, CHE, rel[u])
            if len(rel) == 3:
                ln1(XL, hp * 16, 16, rel[2])
            else:
                for u in range(2):
                    ln1(XL, hp * 16 + 8 * u, 8, rel[2 + u])
            return fence([(out_s, 0), (best_r, 0), (keep_s, 0), (hf_s, 0)])

        def o_slice(qd, oq, u, pts):
            blk = [[[[oq[k1][k2][r1 * HT + r2 * QT + 16 * u:r1 * HT + r2 * QT + 16 * u + 16]
                      for k2 in range(2)] for k1 in range(2)] for r2 in range(2)] for r1 in range(2)]
            if len(pts) == 7:
                pts = [pts[PERML[i_]] for i_ in range(7)]
            ops = _two_level(_lhs_sums, blk, [jnp.tile(release(v_, rw), (2, 1)) for v_, rw in pts])
            for v in range(7):
                os_s[7 * v:7 * v + 7, qd, 16 * u:16 * u + 16, :] = ops[v]
            return fence([(os_s.at[0, qd], 16 * u)])

        assert 2 * HP * CHE == TQ
        for fn in q_passes(0):
            fn()
        opl = o_passes()
        oq = fo = ob_ = None
        for hp in range(HP):
            g, pp = divmod(hp, 4)
            if pp == 0:
                fill = q_passes(g + 1) if g + 1 < HKV else opl
            qa, qb = q_head(2 * hp), q_head(2 * hp + 1)
            sa_ = scores(qa if fo is None else pin(qa, {0: fo}), g)
            pa, la = softmax(sa_)
            vals = {'s': sa_, 'ob': ob_}
            if oq is not None:
                fl = [o_slice(hp // 2 - 1, oq, 2 * (hp % 2) + u, [(vals[nm], rw) for nm, rw in OS_PTS[u]])
                      for u in range(2 if FILL[pp][1] < 7 else 1)]
                qb = pin(qb, {0: functools.reduce(lambda a_, b_: a_ | b_, fl)})
            rs_ = [fill.pop(0)() for _ in range(FILL[pp][0])]
            vals.update({i_: rs_[max(len(rs_) - 6 + i_, 0)] for i_ in range(6)})
            fs = side(hp, [(vals[nm] if vals[nm] is not None else sa_, rw) for nm, rw in SIDE_PTS])
            pb, lb = softmax(scores(qb, g))
            oa_ = pv(pa, g)
            oa = oa_ * la
            rs_ = [fill.pop(0)() for _ in range(FILL[pp][1])]
            fo = None
            if oq is not None and FILL[pp][1] >= 7:
                vals = {'oa': oa_}
                vals.update(enumerate(rs_))
                fo = o_slice(hp // 2 - 1, oq, 2 * (hp % 2) + 1, [(vals[nm], rw) for nm, rw in OS_F2])
            ob_ = pv(pin(pb, {0: fs}), g)
            ob = ob_ * lb
            if hp % 2 == 0:
                oprev = (oa, ob)
            else:
                oq = [oprev, (oa, ob)]

        capture(tprev)
        cp_out(tprev).start()
        cp_x(t, XE).start()
        cp_x(jnp.minimum(t + 2, nt - 1), XL).start()
        pts = []
        due = {} if fo is None else {2: fo}
        for s, fn in enumerate(opl):
            pts.append((fn(due.pop(s, None)), 0))
            if len(pts) % 3 == 0 and len(pts) <= 12:
                o_slice(HP // 2 - 1, oq, len(pts) // 3 - 1, pts[-3:])
            u, rem = divmod(s - HS0, HSG)
            if rem == 0 and 0 <= u < QT // 8:
                h_slice(u * 8, [release(pts[-1 - HSS * (6 - PERML[i_])][0]) for i_ in range(7)])
                due[s + 6] = fence([(hs_s.at[0], 0)])
        assert not due
        return carry

    def finish():
        cp_wg().wait()
        for u in range(F // MC):
            cp_wu(u).wait()
        cp_wd().wait()
        cp_x(nt - 1, XL).wait()
        cp_x(nt - 1, XE).wait()
        cp_out(nt - 2).wait()
        epi_rows(nt - 1, 0, TQ, write_out=False)
        _, release_t = sched()
        rel0 = release_t(best_r[...])
        rbest, idx, rows = capture(nt - 1)
        base = pl.multiple_of((idx // 16) * 16, 16)
        x1 = rows[:, 0:D].reshape(2, 8, D)
        mu = jnp.tile(rows[:, D:D + 128], (1, NB)).reshape(2, 8, D)
        rs = jnp.tile(rows[:, D + 128:D + 256], (1, NB)).reshape(2, 8, D)
        h2 = (x1 - mu) * rs * mvec(4) + mvec(3)
        xs = h2.reshape(16, D).astype(bf16)
        gt = jnp.dot(xs, wq_s[:, 0:F], preferred_element_type=f32)
        for u in range(TQ // 8):
            rel = rel0 if u < T_EARLY else release_t(gt[:, (u - T_EARLY) * 128:(u - T_EARLY + 1) * 128])
            kr = keep_s[8 * u:8 * u + 8, :]
            xc_ = kr[:, 0:D] - jnp.tile(kr[:, D:D + 128] + rel, (1, NB))
            h2_ = xc_ * jnp.tile(kr[:, D + 128:D + 256], (1, NB)) * mvec(4)[0] + mvec(3)[0]
            out_s[8 * u:8 * u + 8, :] = (kr[:, 0:D] + mvec(5)[0] * h2_).astype(out_s.dtype)
        cp_out(nt - 1).start()
        up = jnp.concatenate([jnp.dot(xs, wmod_s[u], preferred_element_type=f32) for u in range(F // MC)], axis=1)
        a = (gt * jax.nn.sigmoid(gt) * up).astype(bf16)
        y = jnp.dot(a, wo_s[0:F, 0:D], preferred_element_type=f32)
        y = y * jnp.tile(jax.nn.sigmoid(rbest), (1, NB))
        rr = lax.broadcasted_iota(jnp.int32, (16, D), 0) + base
        upd = jnp.where(rr == idx, y, 0.0).reshape(2, 8, D)
        new = (x1 + mvec(5) * (h2 + upd)).reshape(16, D)
        fix_s[...] = new.astype(fix_s.dtype)
        cp_out(nt - 1).wait()
        fix = pltpu.make_async_copy(fix_s, out_hbm.at[pl.ds(base, 16), :], osems.at[0])
        fix.start()
        fix.wait()

    def outer(t, carry):
        first_tile()
        lax.fori_loop(1, nt, step, 0)
        finish()
        return carry

    zero_s[0] = 0
    lax.fori_loop(0, zero_s[0] + 1, outer, 0)


def _compiler_params():
    kw = dict(vmem_limit_bytes=124 * 1024 * 1024)
    try:
        return pltpu.CompilerParams(disable_semaphore_checks=True, disable_bounds_checks=True, **kw)
    except TypeError:
        return pltpu.CompilerParams(**kw)


@jax.jit
def pallas_adaLN_cond__sliding_block_cached__moe_arch_mod__prompt_kernel(
    A_x: jax.Array,
    A_k_cache: jax.Array,
    A_v_cache: jax.Array,
    A_wq: jax.Array,
    A_wo: jax.Array,
    B_x: jax.Array,
    B_w_r: jax.Array,
    B_w_gate: jax.Array,
    B_w_up: jax.Array,
    B_w_down: jax.Array,
    c: jax.Array,
    w_mod: jax.Array,
):
    B, S, D = A_x.shape
    assert B == 1
    HKV, SK = A_k_cache.shape[1], A_k_cache.shape[2]
    W = min(4096, max(256, SK // 4))
    F = B_w_gate.shape[1]
    dt = A_x.dtype
    f32 = jnp.float32
    nt = S // TQ
    NB = D // 128
    NMC = 6 * D // MC
    x2 = A_x.reshape(S, D)
    anyspec = pl.BlockSpec(memory_space=pl.ANY)
    kern = functools.partial(_kernel, S=S, D=D, HKV=HKV, SK=SK, W=W, F=F)
    out = pl.pallas_call(
        kern,
        in_specs=[anyspec] * 11,
        out_specs=anyspec,
        out_shape=jax.ShapeDtypeStruct((S, D), dt),
        scratch_shapes=[
            pltpu.VMEM((D,), dt),
            pltpu.VMEM((1, D), dt),
            pltpu.VMEM((3, TQ, D), dt),
            pltpu.VMEM((HKV, W, DH), dt),
            pltpu.VMEM((HKV, W, DH), dt),
            pltpu.VMEM((D, HQ * DH + PAD), dt),
            pltpu.VMEM((HQ * DH, D + PAD), dt),
            pltpu.VMEM((NMC, D, MC), dt),
            pltpu.VMEM((TQ, D), dt),
            pltpu.VMEM((HQ // 4, 49, D // 4, DH), dt),
            pltpu.VMEM((HQ * DH // D, 2, 49, 2 * DH, 128), dt),
            pltpu.VMEM((TQ, D), f32),
            pltpu.VMEM((49, TQ // 4, D // 4), dt),
            pltpu.VMEM((49, HQ // 4, TQ // 4, DH), dt),
            pltpu.VMEM((16, D), dt),
            pltpu.VMEM((NMC, 8, MC), f32),
            pltpu.VMEM((8, 7 * D + 512), f32),
            pltpu.VMEM((TQ, D), dt),
            pltpu.VMEM((HQ, TQ // 2, DH), jnp.uint32),
            pltpu.VMEM((NB, TQ, 128), f32),
            pltpu.VMEM((TQ, D + 256), f32),
            pltpu.VMEM((16, D + 256), f32),
            pltpu.VMEM((16, D), dt),
            pltpu.VMEM((8, 128), f32),
            pltpu.VMEM((8, 128), jnp.int32),
            pltpu.SMEM((1,), jnp.int32),
            pltpu.SemaphoreType.DMA((4 + NMC + HQ + 2 * HKV + HQ * DH // D + 3,)),
            pltpu.SemaphoreType.DMA((1,)),
        ],
        compiler_params=_compiler_params(),
    )(B_w_r, c, x2, A_k_cache, A_v_cache, A_wq, A_wo, w_mod, B_w_gate, B_w_up, B_w_down)
    return out.reshape(B, S, D)
```
